```python
import jax
import jax.numpy as jnp

def _softmax(x, axis=-1):
    return jax.nn.softmax(x, axis=axis)

def _gelu(x):
    return jax.nn.gelu(x, approximate=True)

def _silu(x):
    return jax.nn.silu(x)

def _sigmoid(x):
    return jax.nn.sigmoid(x)

def _layernorm(x, axis=-1, eps=1e-05):
    m = jnp.mean(x, axis=axis, keepdims=True)
    v = jnp.var(x, axis=axis, keepdims=True)
    return (x - m) / jnp.sqrt(v + eps)

def _scatter_add(tgt, idx, src, axis=0):
    return tgt.at[idx].add(src)

def _segment_sum(src, seg, n):
    return jax.ops.segment_sum(src, seg, n)

class _Rng:

    def __init__(self, key):
        self._k = key

    def _next(self):
        self._k, sub = jax.random.split(self._k)
        return sub

    def normal(self, shape):
        return jax.random.normal(self._next(), shape, dtype=jnp.bfloat16)

    def randint(self, lo, hi, shape):
        return jax.random.randint(self._next(), shape, lo, hi, dtype=jnp.int32)

    def uniform(self, shape, lo=0.0, hi=1.0):
        return jax.random.uniform(self._next(), shape, jnp.bfloat16, lo, hi)

    def permutation(self, n):
        return jax.random.permutation(self._next(), n)
kernel_name = 'concat_heads__memory_aug_recurrent_mem_tr__sliding_local_dilated__prompt'

def setup_inputs():
    _rng = _Rng(jax.random.key(int.from_bytes(__import__("os").urandom(4), "little")))
    _w = lambda a: (lambda t: t.astype(jnp.bfloat16) if jnp.issubdtype(t.dtype, jnp.floating) else t)(jnp.asarray(a))

    def _A_setup():
        B, S, Dm = (1, 2048, 1024)
        H, Dh = (32, 128)
        M, seg = (8, 32)
        seg = min(seg, S)
        S = S // seg * seg
        return {'x': _w((lambda *s: _rng.normal(s) * 0.05)(B, S, Dm)), 'mem0': _w((lambda *s: _rng.normal(s) * 0.05)(B, M, Dm)), 'Wq': _w((lambda *s: _rng.normal(s) * 0.05)(Dm, H, Dh) * Dm ** (-0.5)), 'Wk': _w((lambda *s: _rng.normal(s) * 0.05)(Dm, H, Dh) * Dm ** (-0.5)), 'Wv': _w((lambda *s: _rng.normal(s) * 0.05)(Dm, H, Dh) * Dm ** (-0.5)), 'Wo': _w((lambda *s: _rng.normal(s) * 0.05)(H, Dh, Dm) * (H * Dh) ** (-0.5)), 'seg_len': seg}
    _A_in = _A_setup()

    def _B_setup():
        B, S, D = (1, 2048, 1024)
        return {'x': _w((lambda *s: _rng.normal(s) * 0.05)(B, S, D)), 'wqkv': _w((lambda *s: _rng.normal(s) * 0.05)(D, 3 * D)), 'wo': _w((lambda *s: _rng.normal(s) * 0.05)(D, D))}
    _B_in = _B_setup()
    return {'A_x': _A_in['x'], 'A_mem0': _A_in['mem0'], 'A_Wq': _A_in['Wq'], 'A_Wk': _A_in['Wk'], 'A_Wv': _A_in['Wv'], 'A_Wo': _A_in['Wo'], 'A_seg_len': _A_in['seg_len'], 'B_x': _B_in['x'], 'B_wqkv': _B_in['wqkv'], 'B_wo': _B_in['wo']}

def reference(A_x, A_mem0, A_Wq, A_Wk, A_Wv, A_Wo, A_seg_len, B_x, B_wqkv, B_wo):

    def _A_ref(x, mem0, Wq, Wk, Wv, Wo, seg_len):
        B, S, Dm = x.shape
        H, Dh = (Wq.shape[1], Wq.shape[2])
        M = mem0.shape[1]
        scale = Dh ** (-0.5)
        n_seg = S // seg_len
        L = M + seg_len
        idx = jnp.arange(L)
        mask = (idx[:, None] < M) | (idx[:, None] >= idx[None, :])
        mem = mem0
        outs = []
        for s in range(n_seg):
            xs = x[:, s * seg_len:(s + 1) * seg_len, :].copy()
            h = jnp.concatenate([mem, xs], axis=1)
            q = jnp.einsum('btd,dhe->bhte', h, Wq)
            k = jnp.einsum('btd,dhe->bhte', h, Wk)
            v = jnp.einsum('btd,dhe->bhte', h, Wv)
            scores = jnp.einsum('bhqe,bhke->bhqk', q, k) * scale
            scores = jnp.where(mask[None, None], scores, -1000000000.0)
            p = _softmax(scores, axis=-1)
            o = jnp.einsum('bhqk,bhke->bhqe', p, v)
            o = jnp.einsum('bhte,hed->btd', o, Wo)
            mem = o[:, :M, :].copy()
            outs.append(o[:, M:, :])
        return jnp.concatenate(outs, axis=1)

    def _B_ref(x, wqkv, wo):
        B, S, D = x.shape
        H = 32
        Dh = D // H
        W, dil = (8, 2)
        qkv = (lambda x, *d: x.transpose(*d))((x @ wqkv).reshape(B, S, 3, H, Dh), 2, 0, 3, 1, 4)
        q, k, v = (qkv[0], qkv[1], qkv[2])
        scale = Dh ** (-0.5)
        pos = jnp.arange(S)
        off = jnp.arange(W) * dil
        idx = pos[:, None] - off[None, :]
        mask = idx >= 0
        idx_c = jnp.where(mask, idx, 0).reshape(-1)
        kg = k[:, :, idx_c, :].reshape(B, H, S, W, Dh)
        vg = v[:, :, idx_c, :].reshape(B, H, S, W, Dh)
        logits = jnp.einsum('bhsd,bhswd->bhsw', q, kg) * scale
        logits = jnp.where(mask[None, None, :, :], logits, -1000000000.0)
        attn = _softmax(logits, axis=-1)
        o = jnp.einsum('bhsw,bhswd->bhsd', attn, vg)
        return (lambda x, *d: x.transpose(*d))(o, 0, 2, 1, 3).reshape(B, S, D) @ wo
    a = _A_ref(A_x, A_mem0, A_Wq, A_Wk, A_Wv, A_Wo, A_seg_len)
    b = _B_ref(B_x, B_wqkv, B_wo)
    return jnp.concatenate([a, b], axis=-1)
```

```python
import functools

import jax
import jax.numpy as jnp
from jax import lax
import jax.experimental.pallas as pl
import jax.experimental.pallas.tpu as pltpu

bf16, f32, u32, i32 = jnp.bfloat16, jnp.float32, jnp.uint32, jnp.int32

S, DM = 2048, 1024
HA, DH, MEM, SEG = 32, 128, 8, 32
LA = MEM + SEG
HB, NW, DIL = 32, 8, 2
HALO = 16
NEG = -1000000000.0

SB = 128
NSTEP = S // SB
RB = 8
NRB = SB // RB
PITCH = 20
NCH = 8
GPC = 3 * (DM // 16) // NCH
WOR = HA * DH // NCH
SPLIT = 24
LAG1, LAG2 = 1, 2

_NT = (((1,), (1,)), ((), ()))


def _as_bf16(x):
    return pltpu.bitcast(x, bf16)


def _as_u32(x):
    return pltpu.bitcast(x, u32)


def _unpack2(a):
    lo = pltpu.bitcast(a << 16, f32).astype(bf16)
    hi = pltpu.bitcast(a & jnp.uint32(0xFFFF0000), f32).astype(bf16)
    return _as_u32(lo), _as_u32(hi)


def _kernel(xa_hbm, mem0_hbm, wq_hbm, wk_hbm, wv_hbm, wo_hbm, xb_hbm, wqkvb_hbm, wob_hbm,
            out_hbm,
            xa, xb, outa, outb, rawa, rawo, rawb, rawob, wa, woa, wt, wos,
            tg0, tg1, kb0, kb1, vb0, vb1, ob0, ob1,
            ha, hb, oca, ocb, part, ex, df, zero,
            sem_in, sem_ch, sem_out, *qbufs):
    zero[0] = 0
    kbuf, vbuf, obuf, tgs = (kb0, kb1), (vb0, vb1), (ob0, ob1), (tg0, tg1)

    cp_xb = pltpu.make_async_copy(xb_hbm, xb, sem_in.at[0])
    cp_wb = pltpu.make_async_copy(wqkvb_hbm, rawb, sem_in.at[1])
    cp_wob = pltpu.make_async_copy(wob_hbm, rawob, sem_in.at[2])
    cp_xa = pltpu.make_async_copy(xa_hbm, xa, sem_in.at[3])
    cp_m0 = pltpu.make_async_copy(mem0_hbm, ha.at[pl.ds(LA, MEM), :], sem_in.at[4])

    RG = 16 * HA

    def chunk_copies(c):
        cps = []
        g0, g1 = c * GPC, (c + 1) * GPC
        for t, w in enumerate((wq_hbm, wk_hbm, wv_hbm)):
            lo, hi = max(g0, t * 64), min(g1, (t + 1) * 64)
            if lo < hi:
                cps.append(pltpu.make_async_copy(
                    w.at[pl.ds((lo - t * 64) * RG, (hi - lo) * RG), :],
                    rawa.at[pl.ds(lo * RG, (hi - lo) * RG), :], sem_ch.at[0, c]))
        cps.append(pltpu.make_async_copy(
            wo_hbm.at[pl.ds(c * WOR, WOR), :], rawo.at[pl.ds(c * WOR, WOR), :], sem_ch.at[1, c]))
        return cps

    def chunk_wait(c):
        ra = rawa.at[pl.ds(pl.multiple_of(c * (GPC * RG), GPC * RG), GPC * RG), :]
        pltpu.make_async_copy(ra, ra, sem_ch.at[0, c]).wait()
        ro = rawo.at[pl.ds(pl.multiple_of(c * WOR, WOR), WOR), :]
        pltpu.make_async_copy(ro, ro, sem_ch.at[1, c]).wait()

    cp_wb.start()
    cp_xb.start()
    cp_wob.start()
    for c in range(NCH):
        for cp in chunk_copies(c):
            cp.start()
    cp_xa.start()
    cp_m0.start()

    def prep_qkv(i, carry):
        t = i // 4
        for half in range(2):
            kb_ = (i % 4) * 2 + half
            tg = tgs[half]
            k0 = pl.multiple_of(kb_ * 128, 128)
            for ch in range(8):
                col = pl.ds(pl.multiple_of(t * DM + ch * 128, 128), 128)
                at = _as_u32(rawb[pl.ds(k0, 128), col].T)
                for hh in range(4):
                    tg[pl.ds((ch * 4 + hh) * PITCH, 16), :] = at[hh * 16:(hh + 1) * 16]
            for dp in range(16):
                lo, hi = _unpack2(tg[pl.ds(dp, 32, stride=PITCH), :])
                for d, z in ((2 * dp, lo), (2 * dp + 1, hi)):
                    wt[t * 8 + d // 4, pl.ds((d % 4) * 16, 16), pl.ds(k0, 128)] = z
        return carry

    def prep_wo(j, carry):
        a = _as_u32(rawob[:, pl.ds(pl.multiple_of(j * 128, 128), 128)])
        for h in range(HB):
            tg0[pl.ds(h * PITCH, 16), :] = a[h * 16:(h + 1) * 16]
        for dp in range(16):
            lo, hi = _unpack2(tg0[pl.ds(dp, 32, stride=PITCH), :])
            wos[j, pl.ds(2 * dp * 16, 16), :] = lo
            wos[j, pl.ds((2 * dp + 1) * 16, 16), :] = hi
        return carry

    cp_wb.wait()
    lax.fori_loop(0, 12, prep_qkv, 0)
    cp_wob.wait()
    lax.fori_loop(0, 8, prep_wo, 0)
    cp_xb.wait()

    scale_b = (DM // HB) ** -0.5

    def b_qkv_dots(r0, p):
        def mk(t, c):
            def th():
                x = xb[pl.ds(r0, SB), :]
                y = lax.dot_general(x, _as_bf16(wt[t * 8 + c]), _NT, preferred_element_type=f32)
                if t == 0:
                    for rb in range(NRB):
                        qbufs[p * NRB + rb][c] = y[rb * RB:(rb + 1) * RB]
                else:
                    g = kbuf if t == 1 else vbuf
                    g[p][c, 0:HALO, :] = g[1 - p][c, SB:SB + HALO, :]
                    g[p][c, HALO:HALO + SB, :] = y
                return y[SB - 16:SB]
            return th
        return [mk(t, c) for t in (1, 2, 0) for c in range(8)]

    def b_out_dots(r0, p):
        def mk(j):
            def th():
                o = _as_bf16(obuf[p][...])
                y = jnp.dot(o, _as_bf16(wos[j]), preferred_element_type=f32)
                outb[pl.ds(r0, SB), j * 128:(j + 1) * 128] = y.astype(bf16)
                return y[SB - 16:SB]
            return th
        return [mk(j) for j in range(8)]

    def b_attn_job(p, rb, first):
        def job(token):
            z = zero[0]
            q_ref, k_ref, v_ref = qbufs[p * NRB + rb], kbuf[p], vbuf[p]
            if token is not None:
                q_ref[8] = token[0:RB]
            b0 = rb * RB
            acc = [None] * NW
            for c in range(8):
                q = q_ref[z + c]
                for w in range(NW):
                    pr = q * k_ref[c, pl.ds(HALO + b0 - DIL * w, RB), :]
                    acc[w] = pr if acc[w] is None else acc[w] + pr
            lg = []
            for w in range(NW):
                a = acc[w]
                a = a + pltpu.roll(a, 64, 1)
                a = a + pltpu.roll(a, 32, 1)
                a = a * scale_b
                if first and b0 < DIL * w:
                    row = b0 + lax.broadcasted_iota(i32, (RB, 128), 0)
                    a = jnp.where(row >= DIL * w, a, NEG)
                lg.append(a)
            m = functools.reduce(jnp.maximum, lg)
            es = [jnp.exp(a - m) for a in lg]
            inv = 1.0 / functools.reduce(lambda a, b: a + b, es)
            ps = [e * inv for e in es]
            for c in range(8):
                o = None
                for w in range(NW):
                    pr = ps[w] * v_ref[c, pl.ds(HALO + b0 - DIL * w, RB), :]
                    o = pr if o is None else o + pr
                obuf[p][pl.ds(b0 // 2, RB // 2), c * 128:(c + 1) * 128] = _as_u32(o.astype(bf16))
        return job

    def repack_job(g, slot):
        def job(token):
            if token is not None:
                rawa[pl.ds(NCH * GPC * RG, 16), :] = token.astype(bf16)
            tg = tgs[slot]
            a = _as_u32(rawa[pl.ds(pl.multiple_of(g * RG, RG), RG), :])
            for d in range(16):
                tg[pl.ds(d * PITCH, 16), :] = a[d * 16:(d + 1) * 16]
            t = g // 64
            d0 = pl.multiple_of((g % 64) * 8, 8)
            for pp in range(16):
                lo, hi = _unpack2(tg[pl.ds(pp, 16, stride=PITCH), :])
                wa[6 * pp + t, pl.ds(d0, 8), :] = lo
                wa[6 * pp + 3 + t, pl.ds(d0, 8), :] = hi
        return job

    def wocopy_job(r0, nrows):
        def job(token):
            if token is not None:
                rawo[pl.ds(HA * DH, 16), 0:128] = token.astype(bf16)
            v = _as_u32(rawo[pl.ds(pl.multiple_of(r0, nrows), nrows), :])
            h0 = pl.multiple_of(r0 // 2, nrows // 2)
            for j in range(8):
                woa[j, pl.ds(h0, nrows // 2), :] = v[:, j * 128:(j + 1) * 128]
        return job

    def chunk_jobs(c):
        jobs = []
        for i in range(GPC):
            jobs.append(repack_job(c * GPC + i, i % 2))
            if i % 3 == 2:
                jobs.append(wocopy_job(c * WOR + (i // 3) * 64, 64))
        return jobs

    def run(dots, *job_lists):
        rel = {}
        for jobs, span in job_lists:
            for i, job in enumerate(jobs):
                rel.setdefault(i * span // len(jobs) - 1, []).append(job)
        for job in rel.get(-1, []):
            job(None)
        for i, th in enumerate(dots):
            tok = th()
            for job in rel.get(i, []):
                job(tok)

    def b_out_start(r0):
        pltpu.make_async_copy(outb.at[pl.ds(r0, SB), :],
                              out_hbm.at[pl.ds(r0, SB), pl.ds(DM, DM)], sem_out.at[1]).start()

    def attn_jobs(p, first=False):
        return [b_attn_job(p, rb, first) for rb in range(NRB)]

    zeros_halo = jnp.zeros((8, HALO, 128), f32)
    kb1[:, SB:SB + HALO, :] = zeros_halo
    vb1[:, SB:SB + HALO, :] = zeros_halo
    run(b_qkv_dots(0, 0))
    vb0[:, 0:HALO, :] = jnp.broadcast_to(vb0[:, HALO:HALO + 1, :], (8, HALO, 128))
    run(b_qkv_dots(SB, 1), (attn_jobs(0, first=True), 23))

    def b_body(it, carry):
        chunk_wait(it)
        r0 = pl.multiple_of((2 * it + 2) * SB, 2 * SB)
        cj = chunk_jobs(it)
        n = len(cj) // 2
        run(b_qkv_dots(r0, 0) + b_out_dots(r0 - 2 * SB, 0), (attn_jobs(1), 31), (cj[:n], 32))
        run(b_qkv_dots(r0 + SB, 1) + b_out_dots(r0 - SB, 1), (attn_jobs(0), 30), (cj[n:], 31))
        b_out_start(r0 - 2 * SB)
        b_out_start(r0 - SB)
        return carry

    lax.fori_loop(0, NSTEP // 2 - 1, b_body, 0)
    chunk_wait(NCH - 1)
    cj = chunk_jobs(NCH - 1)
    run(b_out_dots(S - 2 * SB, 0), (attn_jobs(1), 6))
    run(b_out_dots(S - SB, 1), (cj, 7))
    b_out_start(S - 2 * SB)
    b_out_start(S - SB)

    cp_xa.wait()
    cp_m0.wait()
    scale_a = DH ** -0.5
    NP = HA // 2
    L2 = 2 * LA
    r = lax.broadcasted_iota(i32, (L2, L2), 0)
    c = lax.broadcasted_iota(i32, (L2, L2), 1)
    same = (r >= LA) == (c >= LA)
    rr = jnp.where(r >= LA, r - LA, r)
    cc = jnp.where(c >= LA, c - LA, c)
    valid = same & ((cc >= SEG) | (rr >= SEG) | (cc <= rr))
    fill = jnp.where(same, NEG, -jnp.inf).astype(f32)
    k1 = SPLIT * DH

    def segment(which, r0):
        h_ref = ha if which == 0 else hb
        oc_ref = oca if which == 0 else ocb
        nrow_o = 32 if which == 0 else 48
        h = h_ref[...]

        def proj(i):
            y = jnp.dot(h, _as_bf16(wa[i]), preferred_element_type=f32)
            if which == 0:
                ex[i] = y[32:40]
                return jnp.concatenate([y[0:32], y[40:48]], axis=0)
            return jnp.concatenate([ex[i], y[8:32], y[0:8]], axis=0)

        def wo_part1(j):
            o1 = _as_bf16(oc_ref[:, :k1])
            part[0:nrow_o, j * 128:(j + 1) * 128] = jnp.dot(
                o1, _as_bf16(woa[j, :k1 // 2, :]), preferred_element_type=f32)

        qs, ks, vs, ps, ls = {}, {}, {}, {}, {}
        nj = 0
        for t in range(NP + LAG2):
            if t < NP:
                ys = [proj(6 * t + i) for i in range(6)]
                qs[t] = jnp.concatenate([ys[0], ys[3]], axis=0).astype(bf16)
                ks[t] = jnp.concatenate([ys[1], ys[4]], axis=0).astype(bf16)
                vs[t] = jnp.concatenate([ys[2], ys[5]], axis=0).astype(bf16)
            else:
                wo_part1(nj)
                wo_part1(nj + 1)
                nj += 2
            p_ = t - LAG1
            if 0 <= p_ < NP:
                sc = lax.dot_general(qs.pop(p_), ks.pop(p_), _NT, preferred_element_type=f32) * scale_a
                sc = jnp.where(valid, sc, fill)
                m = jnp.max(sc, axis=-1, keepdims=True)
                p = jnp.exp(sc - m)
                ls[p_] = jnp.sum(p, axis=-1, keepdims=True)
                ps[p_] = p.astype(bf16)
            p_ = t - LAG2
            if 0 <= p_ < NP:
                o = jnp.dot(ps.pop(p_), vs.pop(p_), preferred_element_type=f32) * (1.0 / ls.pop(p_))
                for e in range(2):
                    hd = 2 * p_ + e
                    oh = o[LA * e:LA * e + LA]
                    if which == 0:
                        df[hd] = oh[24:32]
                        z = jnp.concatenate([oh[0:24], oh[32:40]], axis=0)
                    else:
                        z = jnp.concatenate([oh, df[hd]], axis=0)
                    oc_ref[:, hd * DH:(hd + 1) * DH] = _as_u32(z.astype(bf16))
        for j in range(nj, 8):
            wo_part1(j)
        o2 = _as_bf16(oc_ref[:, k1:])
        for j in range(8):
            cs = slice(j * 128, (j + 1) * 128)
            y = part[0:nrow_o, cs] + jnp.dot(o2, _as_bf16(woa[j, k1 // 2:, :]), preferred_element_type=f32)
            if which == 0:
                outa[pl.ds(r0, 24), cs] = y[0:24].astype(bf16)
                hb[0:8, cs] = y[24:32].astype(bf16)
            else:
                outa[pl.ds(r0 + 24, 8), cs] = y[40:48].astype(bf16)
                outa[pl.ds(r0 + 32, 32), cs] = y[0:32].astype(bf16)
                ha[40:48, cs] = y[32:40].astype(bf16)

    def a_body(it, carry):
        r0 = pl.multiple_of(it * 64, 64)
        ha[0:40, :] = xa[pl.ds(r0, 40), :]
        hb[8:32, :] = xa[pl.ds(r0 + 40, 24), :]
        segment(0, r0)
        segment(1, r0)
        pltpu.make_async_copy(outa.at[pl.ds(r0, 64), :],
                              out_hbm.at[pl.ds(r0, 64), pl.ds(0, DM)], sem_out.at[0]).start()
        return carry

    lax.fori_loop(0, S // 64, a_body, 0)

    pltpu.make_async_copy(outb, out_hbm.at[:, pl.ds(DM, DM)], sem_out.at[1]).wait()
    pltpu.make_async_copy(outa, out_hbm.at[:, pl.ds(0, DM)], sem_out.at[0]).wait()


@functools.partial(jax.jit, static_argnames=("A_seg_len",))
def pallas_concat_heads__memory_aug_recurrent_mem_tr__sliding_local_dilated__prompt_kernel(
    A_x, A_mem0, A_Wq, A_Wk, A_Wv, A_Wo, A_seg_len, B_x, B_wqkv, B_wo,
):
    assert A_seg_len == SEG and A_x.shape == (1, S, DM) and B_x.shape == (1, S, DM)
    vm = pltpu.VMEM
    scratch = [
        vm((S, DM), bf16), vm((S, DM), bf16),
        vm((S, DM), bf16), vm((S, DM), bf16),
        vm((3 * DM * HA + 16, DH), bf16),
        vm((HA * DH + 16, DM), bf16),
        vm((DM, 3 * DM), bf16), vm((DM, DM), bf16),
        vm((3 * HA, DM // 2, DH), u32),
        vm((8, HA * DH // 2, 128), u32),
        vm((24, 64, DM), u32), vm((8, DM // 2, 128), u32),
        vm((33 * PITCH, 128), u32), vm((33 * PITCH, 128), u32),
        vm((8, SB + HALO, 128), f32), vm((8, SB + HALO, 128), f32),
        vm((8, SB + HALO, 128), f32), vm((8, SB + HALO, 128), f32),
        vm((SB // 2, DM), u32), vm((SB // 2, DM), u32),
        vm((48, DM), bf16), vm((32, DM), bf16),
        vm((16, HA * DH), u32), vm((24, HA * DH), u32),
        vm((48, DM), f32),
        vm((3 * HA, 8, 128), f32), vm((HA, 8, 128), f32),
        pltpu.SMEM((1,), i32),
        pltpu.SemaphoreType.DMA((5,)),
        pltpu.SemaphoreType.DMA((2, NCH)),
        pltpu.SemaphoreType.DMA((2,)),
    ] + [vm((9, RB, 128), f32)] * (2 * NRB)
    out = pl.pallas_call(
        _kernel,
        out_shape=jax.ShapeDtypeStruct((S, 2 * DM), bf16),
        in_specs=[pl.BlockSpec(memory_space=pl.ANY)] * 9,
        out_specs=pl.BlockSpec(memory_space=pl.ANY),
        scratch_shapes=scratch,
        compiler_params=pltpu.CompilerParams(vmem_limit_bytes=120 * 1024 * 1024),
        name="concat_heads_kernel",
    )(
        A_x.reshape(S, DM), A_mem0.reshape(MEM, DM),
        A_Wq.reshape(DM * HA, DH), A_Wk.reshape(DM * HA, DH), A_Wv.reshape(DM * HA, DH),
        A_Wo.reshape(HA * DH, DM),
        B_x.reshape(S, DM), B_wqkv, B_wo,
    )
    return out.reshape(1, S, 2 * DM)
```

```python
import contextlib
import functools

import jax
import jax.numpy as jnp
from jax import lax
import jax.experimental.pallas as pl
import jax.experimental.pallas.tpu as pltpu

bf16, f32, u32, i32 = jnp.bfloat16, jnp.float32, jnp.uint32, jnp.int32

S, DM = 2048, 1024
HA, DH, MEM, SEG = 32, 128, 8, 32
LA = MEM + SEG
HB, NW, DIL = 32, 8, 2
HALO = 16
NEG = -1000000000.0

SB = 128
NSTEP = S // SB
RB = 8
NRB = SB // RB
TP = 514
TREG = HA * TP
DP = 18
BREG = HB * DP
NCH = 6
GPC = 3 * (DM // 16) // NCH
RG = 16 * HA
WOR = 640
WOREST = HA * DH - NCH * WOR
SPLIT = 24
LAG1, LAG2 = 1, 3

_NT = (((1,), (1,)), ((), ()))


def scope(name):
    return jax.named_scope(name) if 0 else contextlib.nullcontext()


def _as_bf16(x):
    return pltpu.bitcast(x, bf16)


def _as_u32(x):
    return pltpu.bitcast(x, u32)


def _interleave(a, b):
    lo = (a & jnp.uint32(0xFFFF)) | (b << 16)
    hi = (a >> 16) | (b & jnp.uint32(0xFFFF0000))
    return lo, hi


def _recip(x):
    r = pl.reciprocal(x, approx=True)
    return r * (2.0 - x * r)


def _kernel(xa_hbm, mem0_hbm, wq_hbm, wk_hbm, wv_hbm, wo_hbm, xb_hbm, wqkvb_hbm, wob_hbm,
            out_hbm,
            xa, xb, outa, outb, rawa, rawo, rawb, rawob, wa, woa, wt, wos,
            kb0, kb1, vb0, vb1, ob0, ob1, xs0, xs1,
            ha, hb, oca, ocb, part, ex, df, sv, qkvb, pb, zero,
            sem, sem_out, *qbufs):
    zero[0] = 0
    kbuf, vbuf, obuf, xsb = (kb0, kb1), (vb0, vb1), (ob0, ob1), (xs0, xs1)

    nsem = [0]

    def cp(src, dst):
        c = pltpu.make_async_copy(src, dst, sem.at[nsem[0]])
        nsem[0] += 1
        return c

    def rows(ref, r0, n):
        return ref.at[pl.ds(r0, n), :]

    cp_ch = []
    for c in range(NCH):
        w = (wq_hbm, wk_hbm, wv_hbm)[c // 2]
        cp_ch.append(cp(rows(w, (c % 2) * GPC * RG, GPC * RG), rows(rawa, c * GPC * RG, GPC * RG)))
        cp_ch.append(cp(rows(wo_hbm, c * WOR, WOR), rows(rawo, c * WOR, WOR)))
    cp_worest = cp(rows(wo_hbm, NCH * WOR, WOREST), rows(rawo, NCH * WOR, WOREST))
    cp_xb0 = cp(rows(xb_hbm, 0, 2 * SB), rows(xb, 0, 2 * SB))
    cp_xb1 = cp(rows(xb_hbm, 2 * SB, 3 * SB), rows(xb, 2 * SB, 3 * SB))
    cp_xb2 = cp(rows(xb_hbm, 5 * SB, S - 5 * SB), rows(xb, 5 * SB, S - 5 * SB))
    NPK = 4
    cp_wk = [cp(wqkvb_hbm.at[pl.ds(i * (DM // NPK), DM // NPK), pl.ds(DM, DM)],
                rawb.at[1, pl.ds(i * (DM // NPK), DM // NPK), :]) for i in range(NPK)]
    cp_wv = cp(wqkvb_hbm.at[:, pl.ds(2 * DM, DM)], rawb.at[2])
    cp_wq = cp(wqkvb_hbm.at[:, pl.ds(0, DM)], rawb.at[0])
    cp_wob = cp(wob_hbm, rawob)
    cp_xa = cp(xa_hbm, xa)
    cp_m0 = cp(mem0_hbm, rows(ha, LA, MEM))
    for c in [cp_xb0] + cp_wk + [cp_wv, cp_wq, cp_wob, cp_xb1] + cp_ch[:2] + [cp_xb2] + cp_ch[2:] + [cp_worest, cp_m0, cp_xa]:
        c.start()

    def chunk_wait(c):
        ra = rows(rawa, pl.multiple_of(c * (GPC * RG), GPC * RG), GPC * RG)
        pltpu.make_async_copy(ra, ra, sem.at[2 * c]).wait()
        ro = rows(rawo, pl.multiple_of(c * WOR, 128), WOR)
        pltpu.make_async_copy(ro, ro, sem.at[2 * c + 1]).wait()

    def prep_qkv_job(t, kb_, ch):
        def job(token):
            z = zero[0]
            if token is not None:
                rawb[3, 0:16, 0:128] = token.astype(bf16)
            at = _as_u32(rawb[z + t, kb_ * 128:(kb_ + 1) * 128, ch * 128:(ch + 1) * 128].T)
            base = (t * 8 + kb_) * BREG
            for pr in range(2):
                lo, hi = _interleave(at[pr * 32:pr * 32 + 16], at[pr * 32 + 16:pr * 32 + 32])
                wt[pl.ds(base + ch * 2 + pr, 16, stride=2 * DP), :] = lo
                wt[pl.ds(base + DP + ch * 2 + pr, 16, stride=2 * DP), :] = hi
        return job

    def prep_qkv_jobs(t, kbs):
        return [prep_qkv_job(t, kb_, ch) for kb_ in kbs for ch in range(8)]

    def prep_wo_job(hp):
        def job(token):
            a = _as_u32(rawob[hp * 64:hp * 64 + 32, :])
            b = _as_u32(rawob[hp * 64 + 32:hp * 64 + 64, :])
            lo, hi = _interleave(a, b)
            for j in range(8):
                wos[pl.ds(j * BREG + hp, 16, stride=2 * DP), :] = lo[:, j * 128:(j + 1) * 128]
                wos[pl.ds(j * BREG + DP + hp, 16, stride=2 * DP), :] = hi[:, j * 128:(j + 1) * 128]
        return job

    scale_b = (DM // HB) ** -0.5

    def b_proj_dots(p, ts):
        def mk(t, c):
            def th():
                z = zero[0]
                x = _as_bf16(xsb[p][z if 0 else 0])
                w = jnp.concatenate([
                    jnp.concatenate([wt[pl.ds((t * 8 + kb_) * BREG + (4 * c + dd) * DP, 16), :]
                                     for dd in range(4)], axis=0)
                    for kb_ in range(8)], axis=1)
                y = lax.dot_general(x, _as_bf16(w), _NT, preferred_element_type=f32)
                if t == 0:
                    for rb in range(NRB):
                        qbufs[p * NRB + rb][c] = y[rb * RB:(rb + 1) * RB]
                else:
                    g = kbuf if t == 1 else vbuf
                    g[p][c, 0:HALO, :] = g[1 - p][c, SB:SB + HALO, :]
                    g[p][(z if 0 else 0) + c, HALO:HALO + SB, :] = y
                return y
            return th
        return [mk(t, c) for t in ts for c in range(8)]

    def b_out_dots(r0, p):
        def mk(j):
            def th():
                o = _as_bf16(obuf[p][...])
                w = jnp.concatenate([wos[pl.ds(j * BREG + d * DP, 16), :] for d in range(32)], axis=0)
                y = jnp.dot(o, _as_bf16(w), preferred_element_type=f32)
                outb[pl.ds(r0, SB), j * 128:(j + 1) * 128] = y.astype(bf16)
                return y
            return th
        return [mk(j) for j in range(8)]

    def b_attn_job(p, rb, first):
        def job(token):
            z = zero[0]
            q_ref, k_ref, v_ref = qbufs[p * NRB + rb], kbuf[p], vbuf[p]
            if token is not None:
                q_ref[8] = token[0:RB]
            b0 = rb * RB
            acc = [None] * NW
            for c in range(8):
                q = q_ref[z + c]
                for w in range(NW):
                    pr = q * k_ref[c, pl.ds(HALO + b0 - DIL * w, RB), :]
                    acc[w] = pr if acc[w] is None else acc[w] + pr
            lg = []
            for w in range(NW):
                a = acc[w]
                a = a + pltpu.roll(a, 64, 1)
                a = a + pltpu.roll(a, 32, 1)
                a = a * scale_b
                if first and b0 < DIL * w:
                    row = b0 + lax.broadcasted_iota(i32, (RB, 128), 0)
                    a = jnp.where(row >= DIL * w, a, NEG)
                lg.append(a)
            m = functools.reduce(jnp.maximum, lg)
            es = [jnp.exp(a - m) for a in lg]
            inv = _recip(functools.reduce(lambda a, b: a + b, es))
            ps = [e * inv for e in es]
            for c in range(8):
                o = None
                for w in range(NW):
                    pr = ps[w] * v_ref[c, pl.ds(HALO + b0 - DIL * w, RB), :]
                    o = pr if o is None else o + pr
                obuf[p][pl.ds(b0 // 2, RB // 2), c * 128:(c + 1) * 128] = _as_u32(o.astype(bf16))
        return job

    def attn_jobs(p, first=False):
        return [b_attn_job(p, rb, first) for rb in range(NRB)]

    def xcvt_jobs(r0, p):
        def mk(i):
            def job(token):
                xsb[p][0, i * 8:(i + 1) * 8, :] = _as_u32(xb[pl.ds(pl.multiple_of(r0 + i * 16, 16), 16), :])
            return job
        return [mk(i) for i in range(SB // 16)]

    RAWA_PAD = 3 * DM * HA
    RAWO_PAD = HA * DH

    def repack_job(src0, dst0, half):
        def job(token):
            if token is not None:
                rawa[pl.ds(RAWA_PAD + RG, 16), :] = token.astype(bf16)
            src = rows(rawa, src0, RG)
            dst = rows(wa, dst0, TREG)
            for ii in range(half * 4, half * 4 + 4):
                lo, hi = _interleave(_as_u32(src[ii * 64:ii * 64 + 32, :]), _as_u32(src[ii * 64 + 32:ii * 64 + 64, :]))
                dst[pl.ds(ii, 16, stride=2 * TP), :] = lo
                dst[pl.ds(ii + TP, 16, stride=2 * TP), :] = hi
        return job

    def wocopy_job(src0, dst0):
        def job(token):
            if token is not None:
                rawo[pl.ds(RAWO_PAD + 32, 16), 0:128] = token.astype(bf16)
            v = _as_u32(rawo[pl.ds(src0, 32), :])
            for j in range(8):
                woa[j, pl.ds(dst0, 16), :] = v[:, j * 128:(j + 1) * 128]
        return job

    def chunk_jobs(it):
        c = jnp.maximum(it - 1, 0)
        real = it > 0
        ja, jo = [], []
        for i in range(GPC):
            src0 = pl.multiple_of(jnp.where(real, (c * GPC + i) * RG, RAWA_PAD), RG)
            dst0 = pl.multiple_of((c // 2) * TREG + ((c % 2) * GPC + i) * 8, 8)
            ja += [repack_job(src0, dst0, 0), repack_job(src0, dst0, 1)]
        for i in range(WOR // 32):
            src0 = pl.multiple_of(jnp.where(real, c * WOR + i * 32, RAWO_PAD), 32)
            dst0 = pl.multiple_of(c * (WOR // 2) + i * 16, 16)
            jo.append(wocopy_job(src0, dst0))
        return ja, jo

    def run(dots, *job_lists):
        rel = {}
        for jobs, lo, hi, tr in job_lists:
            for i, job in enumerate(jobs):
                rel.setdefault(lo + i * (hi - lo) // len(jobs) - 1, []).append((job, tr))
        for job, _ in rel.get(-1, []):
            job(None)
        for i, th in enumerate(dots):
            y = th()
            for job, tr in rel.get(i, []):
                job(y[tr:tr + 16])

    def b_out_start(r0, n):
        pltpu.make_async_copy(rows(outb, r0, n),
                              out_hbm.at[pl.ds(r0, n), pl.ds(DM, DM)], sem_out.at[1]).start()

    zeros_halo = jnp.zeros((8, HALO, 128), f32)
    KA = 31
    z8 = pl.multiple_of(zero[0], 8)
    keep = jnp.zeros((8, 128), u32)
    for bit, ref in ((1, qkvb), (2, pb)):
        if KA & bit:
            ref[0, 0:8, :] = jnp.zeros((8, 128), u32)
            keep = keep | ref[zero[0], 0:8, :]
    for bit, ref in ((4, oca), (4, ocb)):
        if KA & bit:
            ref[0:8, 0:128] = jnp.zeros((8, 128), u32)
            keep = keep | ref[pl.ds(z8, 8), 0:128]
    for bit, ref in ((8, ex), (8, df), (8, sv)):
        if KA & bit:
            ref[0] = jnp.zeros((8, 128), f32)
            keep = keep | _as_u32(ref[zero[0]])
    if KA & 16:
        part[0:8, 0:128] = jnp.zeros((8, 128), f32)
        keep = keep | _as_u32(part[pl.ds(z8, 8), 0:128])
    outa[0:16, 0:128] = _as_bf16(keep)
    kb1[:, SB:SB + HALO, :] = zeros_halo
    vb1[:, SB:SB + HALO, :] = zeros_halo
    rawa[pl.ds(RAWA_PAD, RG), :] = jnp.zeros((RG, DH), bf16)
    rawo[pl.ds(RAWO_PAD, 32), :] = jnp.zeros((32, DM), bf16)

    def phase_b():
        with scope('s0_wait_x'):
            cp_xb0.wait()
        with scope('s1_prepk'):
            run([], (xcvt_jobs(0, 0) + xcvt_jobs(SB, 1), 0, 0, 0))
            for i in range(NPK):
                cp_wk[i].wait()
                run([], (prep_qkv_jobs(1, range(i * 8 // NPK, (i + 1) * 8 // NPK)), 0, 0, 0))
            run(b_proj_dots(0, (1,)))
        with scope('s2_waitv'):
            cp_wv.wait()
        with scope('s3'):
            run(b_proj_dots(1, (1,)) + b_proj_dots(0, (2,))[:0], (prep_qkv_jobs(2, range(8)), 0, 6, 0))
            run(b_proj_dots(0, (2,)))
            vb0[:, 0:HALO, :] = jnp.broadcast_to(vb0[:, HALO:HALO + 1, :], (8, HALO, 128))
        with scope('s4_waitq'):
            cp_wq.wait()
        with scope('s5'):
            run(b_proj_dots(1, (2,)), (prep_qkv_jobs(0, range(8)), 0, 6, 0))
            run(b_proj_dots(0, (0,)))
        with scope('s6_waito'):
            cp_wob.wait()
            cp_xb1.wait()
        with scope('s7'):
            run(b_proj_dots(1, (0,)) + b_out_dots(0, 0), (attn_jobs(0, first=True), 0, 7, 0),
                ([prep_wo_job(hp) for hp in range(16)], 0, 0, 0), (xcvt_jobs(2 * SB, 0), 0, 0, 0))

        KVQ = (1, 2, 0)
        ASP = 22

        def b_body(it, carry):
            with scope('b_wait'):
                @pl.when(it == 1)
                def _():
                    cp_xb2.wait()

                @pl.when(it > 0)
                def _():
                    chunk_wait(it - 1)

            r0 = pl.multiple_of((2 * it + 2) * SB, 2 * SB)
            ja, jo = chunk_jobs(it)
            if 0: ja = ja[:2]
            if 0: jo = jo[:2]
            na, no = len(ja) // 2, len(jo) // 2
            run(b_proj_dots(0, KVQ) + b_out_dots(r0 - SB, 1), (attn_jobs(1), 0, ASP, 112),
                (ja[:na], 0, 32, 0), (jo[:no], 0, 32, 64), (xcvt_jobs(r0 + SB, 1), 0, 20, 0))
            run(b_proj_dots(1, KVQ) + b_out_dots(r0, 0), (attn_jobs(0), 0, ASP, 112),
                (ja[na:], 0, 32, 0), (jo[no:], 0, 31, 64),
                (xcvt_jobs(jnp.minimum(r0 + 2 * SB, S - SB), 0), 0, 20, 0))
            b_out_start(r0 - 2 * SB, 2 * SB)
            return carry

        with scope('b_loop'):
            lax.fori_loop(0, NSTEP // 2 - 1, b_body, 0)
        cp_worest.wait()
        jo = [wocopy_job(NCH * WOR + i * 32, NCH * WOR // 2 + i * 16) for i in range(WOREST // 32)]
        with scope('b_epi'):
            run(b_out_dots(S - SB, 1), (attn_jobs(1), 0, 0, 0), (jo, 0, 0, 0))
        b_out_start(S - 2 * SB, 2 * SB)

    if not 0:
        phase_b()

    cp_xa.wait()
    cp_m0.wait()
    scale_a = DH ** -0.5
    NP = HA // 2
    L2 = 2 * LA
    NVS = (2, 1)

    def masks(NV):
        QR = LA - 8 * NV
        r = lax.broadcasted_iota(i32, (2 * QR, L2), 0)
        c = lax.broadcasted_iota(i32, (2 * QR, L2), 1)
        same = (r >= QR) == (c >= LA)
        rr = jnp.where(r >= QR, r - QR, r) + 8 * NV
        cc = jnp.where(c >= LA, c - LA, c)
        valid = same & ((cc >= SEG) | (rr >= SEG) | (cc <= rr))
        fill = jnp.where(same, NEG, -jnp.inf).astype(f32)
        return valid, fill

    msk = {nv: masks(nv) for nv in set(NVS)}
    sub8 = lax.broadcasted_iota(i32, (8, 128), 0)

    qscale = scale_a * 1.4426950408889634
    tsum = lambda xs: functools.reduce(lambda a, b: a + b, xs)

    def vpu_part(q, k8, v8, causal, prev):
        ss = []
        for j in range(8):
            s_ = jnp.broadcast_to(jnp.sum(q * k8[j:j + 1], axis=-1, keepdims=True), (8, 128))
            if causal and j > 0:
                s_ = jnp.where(sub8 >= j, s_, NEG * 1.4426950408889634)
            ss.append(s_)
        m = functools.reduce(jnp.maximum, ss if prev is None else ss + [prev[0]])
        es = [jnp.exp2(s_ - m) for s_ in ss]
        l = tsum(es)
        o = tsum([e * v8[j:j + 1] for j, e in enumerate(es)])
        if prev is not None:
            al = jnp.exp2(prev[0] - m)
            l = l + prev[1] * al
            o = o + prev[2] * al
        return m, l, o

    k1 = SPLIT * DH
    TL = 2

    def segment(which, r0):
        h_ref = ha if which == 0 else hb
        oc_ref = oca if which == 0 else ocb
        nrow_o = 32 if which == 0 else 48
        NV = NVS[which]
        QR = LA - 8 * NV
        valid, fill = msk[NV]
        h = h_ref[...]
        zvec = jnp.full((8, 128), zero[0], i32).astype(u32)

        def tied(w, vals0, vals1):
            n = w.shape[0]
            parts = [w[0:n // 2], w[n // 2:n]]
            for i, vals in enumerate((vals0, vals1)):
                if vals:
                    tie = functools.reduce(lambda a, b: a | b, [_as_u32(x) for x in vals]) & zvec
                    parts[i] = jnp.concatenate([parts[i][0:n // 2 - 8], parts[i][n // 2 - 8:] | tie], axis=0)
            return jnp.concatenate(parts, axis=0)

        NH = 6 if which == 1 else 0
        KH = 4 * 128
        order = [(2 * t + e, i) for t in range(NP) for e in range(2) for i in range(3)]
        pre = {}
        for hd, t in order[:NH]:
            pre[hd, t] = jnp.dot(h[:, :KH], _as_bf16(wa[pl.ds(t * TREG + hd * TP, KH // 2), :]),
                                 preferred_element_type=f32)

        def proj(hd, t, ties):
            if (hd, t) in pre:
                y = jnp.dot(h[:, KH:], _as_bf16(wa[pl.ds(t * TREG + hd * TP + KH // 2, (DM - KH) // 2), :]),
                            preferred_element_type=f32)
                y = y + pre.pop((hd, t))
            else:
                w = tied(wa[pl.ds(t * TREG + hd * TP, DM // 2), :], *ties)
                y = jnp.dot(h, _as_bf16(w), preferred_element_type=f32)
            if which == 0:
                ex[t * HA + hd] = y[32:40]
                return jnp.concatenate([y[0:32], y[40:48]], axis=0)
            return jnp.concatenate([ex[t * HA + hd], y[8:32], y[0:8]], axis=0)

        def wo_part1(j, ties):
            o1 = _as_bf16(oc_ref[:, :k1])
            part[0:nrow_o, j * 128:(j + 1) * 128] = jnp.dot(
                o1, _as_bf16(tied(woa[j, :k1 // 2, :], *ties)), preferred_element_type=f32)

        def vpu_jobs(t, ys):
            out = []
            for e in range(2):
                hd = 2 * t + e
                q, k, v = ys[3 * e:3 * e + 3]
                jobs = []
                ov[hd] = []
                for g in range(NV):
                    q0 = q[8 * g:8 * g + 8] * qscale
                    if which == 1 and g == 0:
                        st = [sv[i * HA + hd] for i in range(3)]
                    else:
                        st = None
                        for b in range(g, -1, -1):
                            st = vpu_part(q0, k[8 * b:8 * b + 8], v[8 * b:8 * b + 8], b == g, st)
                            jobs.append(list(st[1:]))
                    _, l, o = vpu_part(q0, k[SEG:LA], v[SEG:LA], False, st)
                    ov[hd].append(o * _recip(l))
                    jobs.append([ov[hd][-1]])
                if which == 0 and NVS[1]:
                    st = vpu_part(ex[hd] * qscale, ex[HA + hd], ex[2 * HA + hd], True, None)
                    for i in range(3):
                        sv[i * HA + hd] = st[i]
                    jobs.append(list(st[1:]))
                out += jobs
            slots = [[] for _ in range(12)]
            for i, jb in enumerate(out):
                slots[(2 * i + 1) * 6 // len(out)] += jb
            return slots

        ov, pend, ps = {}, {}, {}
        nj = 0
        for t in range(NP + LAG2):
            ties = pend.pop(t - TL, [[]] * 12)
            if t < NP:
                ys = [proj(2 * t + e, i, ties[6 * e + 2 * i:6 * e + 2 * i + 2]) for e in range(2) for i in range(3)]
                qkvb[(which * NP + t) * 3, 0:QR, :] = _as_u32(
                    jnp.concatenate([ys[0][8 * NV:], ys[3][8 * NV:]], axis=0).astype(bf16))
                for i in range(1, 3):
                    qkvb[(which * NP + t) * 3 + i] = _as_u32(jnp.concatenate([ys[i], ys[3 + i]], axis=0).astype(bf16))
                pend[t] = vpu_jobs(t, ys)
            else:
                wo_part1(nj, (sum(ties[0:3], []), sum(ties[3:6], [])))
                wo_part1(nj + 1, (sum(ties[6:9], []), sum(ties[9:12], [])))
                nj += 2
            p_ = t - LAG1
            if 0 <= p_ < NP:
                sc = lax.dot_general(_as_bf16(qkvb[(which * NP + p_) * 3, 0:QR, :]), _as_bf16(qkvb[(which * NP + p_) * 3 + 1]), _NT,
                                     preferred_element_type=f32) * scale_a
                sc = jnp.where(valid, sc, fill)
                m = jnp.max(sc, axis=-1, keepdims=True)
                p = jnp.exp(sc - m)
                pn = (p * _recip(jnp.sum(p, axis=-1, keepdims=True))).astype(bf16)
                if 1:
                    pb[which * NP + p_, 0:QR, 0:L2] = _as_u32(pn)
                else:
                    ps[p_] = pn
            p_ = t - LAG2
            if 0 <= p_ < NP:
                o = jnp.dot(_as_bf16(pb[which * NP + p_, 0:QR, 0:L2]) if 1 else ps.pop(p_), _as_bf16(qkvb[(which * NP + p_) * 3 + 2]),
                            preferred_element_type=f32)
                for e in range(2):
                    hd = 2 * p_ + e
                    oh = jnp.concatenate(ov.pop(hd) + [o[QR * e:QR * e + QR]], axis=0)
                    if which == 0:
                        df[hd] = oh[24:32]
                        z = jnp.concatenate([oh[32:40], oh[0:24]], axis=0)
                    else:
                        z = jnp.concatenate([oh, df[hd]], axis=0)
                    oc_ref[:, hd * DH:(hd + 1) * DH] = _as_u32(z.astype(bf16))
        for j in range(nj, 8):
            wo_part1(j, ([], []))
        o2 = _as_bf16(oc_ref[:, k1:])
        for j in range(8):
            cs = slice(j * 128, (j + 1) * 128)
            y = part[0:nrow_o, cs] + jnp.dot(o2, _as_bf16(woa[j, k1 // 2:, :]), preferred_element_type=f32)
            if which == 0:
                hb[0:8, cs] = y[0:8].astype(bf16)
                outa[pl.ds(r0, 24), cs] = y[8:32].astype(bf16)
            else:
                outa[pl.ds(r0 + 24, 8), cs] = y[40:48].astype(bf16)
                outa[pl.ds(r0 + 32, 32), cs] = y[0:32].astype(bf16)
                ha[40:48, cs] = y[32:40].astype(bf16)

    UA = 1

    def a_body(it, carry):
        for u in range(UA):
            r0 = pl.multiple_of((it * UA + u) * 64, 64)
            ha[0:40, :] = xa[pl.ds(r0, 40), :]
            hb[8:32, :] = xa[pl.ds(r0 + 40, 24), :]
            segment(0, r0)
            segment(1, r0)
        r0 = pl.multiple_of(it * UA * 64, 64)
        pltpu.make_async_copy(rows(outa, r0, 64 * UA),
                              out_hbm.at[pl.ds(r0, 64 * UA), pl.ds(0, DM)], sem_out.at[0]).start()
        return carry

    if 0:
        outa[0:16, 0:128] = _as_bf16(wa[pl.ds(pl.multiple_of(zero[0], 8), 8), :]) + _as_bf16(woa[zero[0], 0:8, :])
        pltpu.make_async_copy(outa, out_hbm.at[:, pl.ds(0, DM)], sem_out.at[0]).start()
    else:
        with scope('a_loop'):
            lax.fori_loop(0, S // 64 // UA, a_body, 0)

    with scope('final_wait'):
        pltpu.make_async_copy(outb, out_hbm.at[:, pl.ds(DM, DM)], sem_out.at[1]).wait()
        pltpu.make_async_copy(outa, out_hbm.at[:, pl.ds(0, DM)], sem_out.at[0]).wait()


@functools.partial(jax.jit, static_argnames=("A_seg_len",))
def pallas_concat_heads__memory_aug_recurrent_mem_tr__sliding_local_dilated__prompt_kernel(
    A_x, A_mem0, A_Wq, A_Wk, A_Wv, A_Wo, A_seg_len, B_x, B_wqkv, B_wo,
):
    assert A_seg_len == SEG and A_x.shape == (1, S, DM) and B_x.shape == (1, S, DM)
    vm = pltpu.VMEM
    scratch = [
        vm((S, DM), bf16), vm((S, DM), bf16),
        vm((S, DM), bf16), vm((S, DM), bf16),
        vm((3 * DM * HA + RG + 16, DH), bf16),
        vm((HA * DH + 48, DM), bf16),
        vm((4, DM, DM), bf16), vm((DM, DM), bf16),
        vm((3 * TREG + DM // 2 + 2 * TP, DH), u32),
        vm((8, HA * DH // 2, 128), u32),
        vm((25 * BREG, 128), u32), vm((9 * BREG, 128), u32),
        vm((8, SB + HALO, 128), f32), vm((8, SB + HALO, 128), f32),
        vm((8, SB + HALO, 128), f32), vm((8, SB + HALO, 128), f32),
        vm((SB // 2, DM), u32), vm((SB // 2, DM), u32),
        vm((1, SB // 2, DM), u32), vm((1, SB // 2, DM), u32),
        vm((48, DM), bf16), vm((32, DM), bf16),
        vm((16, HA * DH), u32), vm((24, HA * DH), u32),
        vm((48, DM), f32),
        vm((3 * HA, 8, 128), f32), vm((HA, 8, 128), f32), vm((3 * HA, 8, 128), f32),
        vm((96, LA, 128), u32), vm((32, LA, 128), u32),
        pltpu.SMEM((1,), i32),
        pltpu.SemaphoreType.DMA((32,)),
        pltpu.SemaphoreType.DMA((2,)),
    ] + [vm((9, RB, 128), f32)] * (2 * NRB)
    out = pl.pallas_call(
        _kernel,
        out_shape=jax.ShapeDtypeStruct((S, 2 * DM), bf16),
        in_specs=[pl.BlockSpec(memory_space=pl.ANY)] * 9,
        out_specs=pl.BlockSpec(memory_space=pl.ANY),
        scratch_shapes=scratch,
        compiler_params=pltpu.CompilerParams(vmem_limit_bytes=120 * 1024 * 1024),
        name="concat_heads_kernel",
    )(
        A_x.reshape(S, DM), A_mem0.reshape(MEM, DM),
        A_Wq.reshape(DM * HA, DH), A_Wk.reshape(DM * HA, DH), A_Wv.reshape(DM * HA, DH),
        A_Wo.reshape(HA * DH, DM),
        B_x.reshape(S, DM), B_wqkv, B_wo,
    )
    return out.reshape(1, S, 2 * DM)
```

```python
import contextlib
import functools

import jax
import jax.numpy as jnp
from jax import lax
import jax.experimental.pallas as pl
import jax.experimental.pallas.tpu as pltpu

bf16, f32, u32, i32 = jnp.bfloat16, jnp.float32, jnp.uint32, jnp.int32

S, DM = 2048, 1024
HA, DH, MEM, SEG = 32, 128, 8, 32
LA = MEM + SEG
HB, NW, DIL = 32, 8, 2
HALO = 16
NEG = -1000000000.0
LOG2E = 1.4426950408889634

SB = 128
NSTEP = S // SB
RB = 8
NRB = SB // RB
TP = 514
TREG = HA * TP
DP = 18
BREG = HB * DP
NCH = 6
GPC = 3 * (DM // 16) // NCH
RG = 16 * HA
WOR = 640
WOREST = HA * DH - NCH * WOR
MB = 48
SPLIT = 24
LAG1, LAG2 = 1, 3

_NT = (((1,), (1,)), ((), ()))


def scope(name):
    return jax.named_scope(name) if 0 else contextlib.nullcontext()


def _as_bf16(x):
    return pltpu.bitcast(x, bf16)


def _as_u32(x):
    return pltpu.bitcast(x, u32)


def _interleave(a, b):
    lo = (a & jnp.uint32(0xFFFF)) | (b << 16)
    hi = (a >> 16) | (b & jnp.uint32(0xFFFF0000))
    return lo, hi


def _recip(x):
    r = pl.reciprocal(x, approx=True)
    return r * (2.0 - x * r)


def _kernel(xa_hbm, mem0_hbm, wq_hbm, wk_hbm, wv_hbm, wo_hbm, xb_hbm, wqkvb_hbm, wob_hbm,
            out_hbm,
            xa, xb, outa, outb, rawa, rawo, rawb, rawob, wa, woa, wt, wos,
            kb0, kb1, vb0, vb1, xs0, xs1, ob0, ob1,
            ha, hb, oca, ocb, part, ex, df, sv, qkvb, pb, oball, obs, zero,
            sem, sem_out, *qbufs):
    zero[0] = 0
    kbuf, vbuf, xsb = (kb0, kb1), (vb0, vb1), (xs0, xs1)

    nsem = [0]

    def cp(src, dst):
        c = pltpu.make_async_copy(src, dst, sem.at[nsem[0]])
        nsem[0] += 1
        return c

    def rows(ref, r0, n):
        return ref.at[pl.ds(r0, n), :]

    cp_ch = []
    for c in range(NCH):
        w = (wq_hbm, wk_hbm, wv_hbm)[c // 2]
        cp_ch.append(cp(rows(w, (c % 2) * GPC * RG, GPC * RG), rows(rawa, c * GPC * RG, GPC * RG)))
        cp_ch.append(cp(rows(wo_hbm, c * WOR, WOR), rows(rawo, c * WOR, WOR)))
    cp_worest = cp(rows(wo_hbm, NCH * WOR, WOREST), rows(rawo, NCH * WOR, WOREST))
    cp_xb0 = cp(rows(xb_hbm, 0, SB), rows(xb, 0, SB))
    cp_xb1 = cp(rows(xb_hbm, SB, SB), rows(xb, SB, SB))
    cp_xb2 = cp(rows(xb_hbm, 2 * SB, SB), rows(xb, 2 * SB, SB))
    cp_xb3 = cp(rows(xb_hbm, 3 * SB, 3 * SB), rows(xb, 3 * SB, 3 * SB))
    SEM_X = nsem[0]
    cp_xbs = [cp(rows(xb_hbm, (6 + 2 * c) * SB, 2 * SB), rows(xb, (6 + 2 * c) * SB, 2 * SB)) for c in range(5)]

    def cp_wb(t, k0, n):
        return cp(wqkvb_hbm.at[pl.ds(k0, n), pl.ds(t * DM, DM)], rawb.at[t, pl.ds(k0, n), :])

    KVQ = (1, 2, 0)
    KQV = (1, 0, 2)
    cp_w0 = [cp_wb(KQV[0], 0, DM // 4), cp_wb(KQV[0], DM // 4, DM // 4)]
    cp_wp = [None] + [cp_wb(KQV[h // 2], (h % 2) * (DM // 2), DM // 2) for h in range(1, 6)]
    cp_wob = cp(wob_hbm, rawob.at[:, pl.ds(0, DM)])
    cp_xa = cp(xa_hbm, xa)
    cp_m0 = cp(mem0_hbm, rows(ha, LA, MEM))
    order = cp_w0 + [cp_xb0, cp_xb1] + cp_wp[1:5] + [cp_xb2, cp_wp[5], cp_xb3, cp_wob]
    for c in range(NCH):
        order += cp_ch[2 * c:2 * c + 2] + cp_xbs[c:c + 1]
    for c in order + [cp_worest, cp_m0, cp_xa]:
        c.start()

    def chunk_wait(c):
        ra = rows(rawa, pl.multiple_of(c * (GPC * RG), GPC * RG), GPC * RG)
        pltpu.make_async_copy(ra, ra, sem.at[2 * c]).wait()
        ro = rows(rawo, pl.multiple_of(c * WOR, 128), WOR)
        pltpu.make_async_copy(ro, ro, sem.at[2 * c + 1]).wait()

    def prep_qkv_job(t, kb_, ch):
        def job(token):
            at = _as_u32(rawb[t, kb_ * 128:(kb_ + 1) * 128, ch * 128:(ch + 1) * 128].T)
            base = (t * 8 + kb_) * BREG
            for pr in range(2):
                lo, hi = _interleave(at[pr * 32:pr * 32 + 16], at[pr * 32 + 16:pr * 32 + 32])
                wt[pl.ds(base + ch * 2 + pr, 16, stride=2 * DP), :] = lo
                wt[pl.ds(base + DP + ch * 2 + pr, 16, stride=2 * DP), :] = hi
        return job

    def prep_qkv_jobs(t, kbs):
        return [prep_qkv_job(t, kb_, ch) for kb_ in kbs for ch in range(8)]

    def prep_wo_job(src_col, dst0, hq):
        def job(token):
            if token is not None:
                rawob[0:16, DM + 128:DM + 256] = token.astype(bf16)
            dst = rows(wos, dst0, BREG + 2 * DP)
            for hp in range(4 * hq, 4 * hq + 4):
                a = _as_u32(rawob[hp * 64:hp * 64 + 32, pl.ds(src_col, 128)])
                b = _as_u32(rawob[hp * 64 + 32:hp * 64 + 64, pl.ds(src_col, 128)])
                lo, hi = _interleave(a, b)
                dst[pl.ds(hp, 16, stride=2 * DP), :] = lo
                dst[pl.ds(DP + hp, 16, stride=2 * DP), :] = hi
        return job

    def tied(w, zvec, *vals_list):
        n = w.shape[0] // len(vals_list)
        parts = []
        for i, vals in enumerate(vals_list):
            pt = w[i * n:(i + 1) * n]
            if vals:
                tie = functools.reduce(lambda a, b: a | b, [_as_u32(x) for x in vals]) & zvec
                pt = jnp.concatenate([pt[0:n - 8], pt[n - 8:] | tie], axis=0)
            parts.append(pt)
        return jnp.concatenate(parts, axis=0)

    def zeros_vec():
        return jnp.full((8, 128), zero[0], i32).astype(u32)

    scale_b = (DM // HB) ** -0.5

    def b_proj_dots(p, ts, half=None):
        kbs = range(8) if half is None else range(4 * half, 4 * half + 4)

        def mk(t, c):
            def th(ties):
                x = _as_bf16(xsb[p][:, kbs[0] * 128:(kbs[-1] + 1) * 128])
                tiles = [jnp.concatenate([wt[pl.ds((t * 8 + kb_) * BREG + (4 * c + dd) * DP, 16), :]
                                          for dd in range(4)], axis=0) for kb_ in kbs]
                if ties:
                    tiles[-1] = tied(tiles[-1], zeros_vec(), ties)
                y = lax.dot_general(x, _as_bf16(jnp.concatenate(tiles, axis=1)), _NT, preferred_element_type=f32)
                if t == 0:
                    for rb in range(NRB):
                        yr = y[rb * RB:(rb + 1) * RB]
                        qbufs[p * NRB + rb][c] = yr + qbufs[p * NRB + rb][c] if half == 1 else yr
                else:
                    g = kbuf if t == 1 else vbuf
                    if half != 0:
                        g[p][c, 0:HALO, :] = g[1 - p][c, SB:SB + HALO, :]
                    g[p][c, HALO:HALO + SB, :] = y + g[p][c, HALO:HALO + SB, :] if half == 1 else y
                return y
            return th
        return [mk(t, c) for t in ts for c in range(8)]

    def b_out_dots(r0):
        def mk(j):
            def th(ties):
                o = _as_bf16(oball[r0 // 2:(r0 + SB) // 2, :])
                w = jnp.concatenate([wos[pl.ds(j * BREG + d * DP, 16), :] for d in range(32)], axis=0)
                y = jnp.dot(o, _as_bf16(w), preferred_element_type=f32)
                outb[pl.ds(r0, SB), j * 128:(j + 1) * 128] = y.astype(bf16)
                return y
            return th
        return [mk(j) for j in range(8)]

    def b_attn_qk(p, rb, first, token):
        q_ref, k_ref = qbufs[p * NRB + rb], kbuf[p]
        z = 0
        if token is not None:
            z = zero[0]
            q_ref[8] = token[0:RB]
        b0 = rb * RB
        acc = [None] * NW
        for c in range(8):
            q = q_ref[z + c]
            for w in range(NW):
                pr = q * k_ref[c, pl.ds(HALO + b0 - DIL * w, RB), :]
                acc[w] = pr if acc[w] is None else acc[w] + pr
        lg = []
        for w in range(NW):
            a = acc[w]
            a = a + pltpu.roll(a, 64, 1)
            a = a + pltpu.roll(a, 32, 1)
            a = a * (scale_b * LOG2E)
            if first and b0 < DIL * w:
                row = b0 + lax.broadcasted_iota(i32, (RB, 128), 0)
                a = jnp.where(row >= DIL * w, a, NEG * LOG2E)
            lg.append(a)
        m = functools.reduce(jnp.maximum, lg)
        es = [jnp.exp2(a - m) for a in lg]
        inv = _recip(functools.reduce(lambda a, b: a + b, es))
        return [e * inv for e in es]

    def b_attn_pv(p, rb, r0, ps):
        v_ref, b0 = vbuf[p], rb * RB
        dst = (ob0, ob1)[p] if r0 is None else rows(oball, pl.multiple_of(r0 // 2, SB // 2), SB // 2)
        outs = []
        for c in range(8):
            o = None
            for w in range(NW):
                pr = ps[w] * v_ref[c, pl.ds(HALO + b0 - DIL * w, RB), :]
                o = pr if o is None else o + pr
            dst[pl.ds(b0 // 2, RB // 2), c * 128:(c + 1) * 128] = _as_u32(o.astype(bf16))
            outs.append(o)
        return outs

    def attn_jobs(p, r0):
        def mk(rb):
            def job(token):
                if 1 == 3 and not isinstance(r0, int):
                    b_attn_pv(p, rb, None, b_attn_qk(p, rb, False, token))
                    if rb % 2 == 0:
                        return None
                    v = (ob0, ob1)[p][(rb // 2) * 8:(rb // 2) * 8 + 8, :]
                    oball[pl.ds(pl.multiple_of(r0 // 2 + (rb // 2) * 8, 8), 8), :] = v
                    return [v[:, c * 128:(c + 1) * 128] for c in range(8)]
                outs = b_attn_pv(p, rb, r0, b_attn_qk(p, rb, False, token if 1 else None))
                if 1 == 2:
                    return [oball[pl.ds(pl.multiple_of(zero[0], 8), 8), 0:128]]
                return outs if 1 else None
            return job
        return [mk(rb) for rb in range(NRB)]

    def xcvt_jobs(r0, p):
        def mk(i):
            def job(token):
                xsb[p][i * 8:(i + 1) * 8, :] = _as_u32(xb[pl.ds(pl.multiple_of(r0 + i * 16, 16), 16), :])
            return job
        return [mk(i) for i in range(SB // 16)]

    RAWA_PAD = 3 * DM * HA
    RAWO_PAD = HA * DH

    def repack_job(src0, dst0, half):
        def job(token):
            if token is not None:
                rawa[pl.ds(RAWA_PAD + RG, 16), :] = token.astype(bf16)
            src = rows(rawa, src0, RG)
            dst = rows(wa, dst0, TREG)
            for ii in range(half * 4, half * 4 + 4):
                lo, hi = _interleave(_as_u32(src[ii * 64:ii * 64 + 32, :]), _as_u32(src[ii * 64 + 32:ii * 64 + 64, :]))
                dst[pl.ds(ii, 16, stride=2 * TP), :] = lo
                dst[pl.ds(ii + TP, 16, stride=2 * TP), :] = hi
        return job

    def wocopy_job(src0, dst0):
        def job(token):
            if token is not None:
                rawo[pl.ds(RAWO_PAD + 32, 16), 0:128] = token.astype(bf16)
            v = _as_u32(rawo[pl.ds(src0, 32), :])
            for j in range(8):
                woa[j, pl.ds(dst0, 16), :] = v[:, j * 128:(j + 1) * 128]
        return job

    def chunk_jobs(it):
        c = jnp.maximum(it - 1, 0)
        real = it > 0
        ja, jo = [], []
        for i in range(GPC):
            src0 = pl.multiple_of(jnp.where(real, (c * GPC + i) * RG, RAWA_PAD), RG)
            dst0 = pl.multiple_of((c // 2) * TREG + ((c % 2) * GPC + i) * 8, 8)
            ja += [repack_job(src0, dst0, 0), repack_job(src0, dst0, 1)]
        for i in range(WOR // 32):
            src0 = pl.multiple_of(jnp.where(real, c * WOR + i * 32, RAWO_PAD), 32)
            dst0 = pl.multiple_of(c * (WOR // 2) + i * 16, 16)
            jo.append(wocopy_job(src0, dst0))
        jw = []
        for i in range(2):
            j = jnp.minimum(2 * c + i, 7)
            src_col = pl.multiple_of(jnp.where(real, j * 128, DM), 128)
            jw += [prep_wo_job(src_col, pl.multiple_of(j * BREG, 8), hq) for hq in range(4)]
        return ja, jo, jw

    TD = 4

    def run(dots, *job_lists, carry=None):
        rel = {}
        for jobs, lo, hi, tr in job_lists:
            for i, job in enumerate(jobs):
                rel.setdefault(lo + i * (hi - lo) // len(jobs) - 1, []).append((job, tr))
        due = {} if carry is None else carry

        def fire(i, y):
            for job, tr in rel.get(i, []):
                vals = job(None if y is None else y[tr:tr + 16])
                if vals and TD:
                    due.setdefault(min(i + TD, len(dots) - 1) if 1 else i + TD, []).extend(vals)

        fire(-1, None)
        for i, th in enumerate(dots):
            fire(i, th(due.pop(i, [])))
        return {k - len(dots): v for k, v in due.items()}

    def b_out_start(r0, n):
        pltpu.make_async_copy(rows(outb, r0, n),
                              out_hbm.at[pl.ds(r0, n), pl.ds(DM, DM)], sem_out.at[1]).start()

    zeros_halo = jnp.zeros((8, HALO, 128), f32)
    KA = 31
    z8 = pl.multiple_of(zero[0], 8)
    keep = jnp.zeros((8, 128), u32)
    for bit, ref in ((1, qkvb), (2, pb)):
        if KA & bit:
            ref[0, 0:8, :] = jnp.zeros((8, 128), u32)
            keep = keep | ref[zero[0], 0:8, :]
    for bit, ref in ((4, oca), (4, ocb), (4, obs)):
        if KA & bit:
            ref[0:8, 0:128] = jnp.zeros((8, 128), u32)
            keep = keep | ref[pl.ds(z8, 8), 0:128]
    for bit, ref in ((8, ex), (8, df), (8, sv)):
        if KA & bit:
            ref[0] = jnp.zeros((8, 128), f32)
            keep = keep | _as_u32(ref[zero[0]])
    if KA & 16:
        part[0:8, 0:128] = jnp.zeros((8, 128), f32)
        keep = keep | _as_u32(part[pl.ds(z8, 8), 0:128])
    outa[0:16, 0:128] = _as_bf16(keep)
    kb1[:, SB:SB + HALO, :] = zeros_halo
    vb1[:, SB:SB + HALO, :] = zeros_halo
    rawa[pl.ds(RAWA_PAD, RG), :] = jnp.zeros((RG, DH), bf16)
    rawo[pl.ds(RAWO_PAD, 32), :] = jnp.zeros((32, DM), bf16)
    rawob[:, DM:DM + 128] = jnp.zeros((DM, 128), bf16)

    def phase_b():
        with scope('s0'):
            for i in range(2):
                cp_w0[i].wait()
                run([], (prep_qkv_jobs(KQV[0], range(2 * i, 2 * i + 2)), 0, 0, 0))
            cp_xb0.wait()
            run([], (xcvt_jobs(0, 0), 0, 0, 0))
            run(b_proj_dots(0, KQV[0:1], 0))
            cp_xb1.wait()
            run([], (xcvt_jobs(SB, 1), 0, 0, 0))
        for h in range(1, 6):
            with scope('w%d' % h):
                cp_wp[h].wait()
                if h == 5:
                    cp_xb2.wait()
            with scope('s%d' % h):
                t0, t1 = KQV[(h - 1) // 2], KQV[h // 2]
                run([], (prep_qkv_jobs(t1, range(4 * (h % 2), 4 * (h % 2) + 4)), 0, 0, 0))
                dots = b_proj_dots(1, (t0,), (h - 1) % 2) + b_proj_dots(0, (t1,), h % 2)
                NQ4 = 8
                Q0 = 8
                if h < 4:
                    run(dots)
                elif h == 4:
                    due = {}
                    for rb in range(NQ4):
                        ps_ = b_attn_qk(0, rb, True, None)
                        for w in range(NW):
                            qbufs[rb][w] = ps_[w]
                        due.setdefault(Q0 + rb * (16 - Q0) // NQ4, []).extend(ps_)
                    run(dots, carry=due)
                else:
                    pss = [[qbufs[rb][w] for w in range(NW)] if rb < NQ4 else b_attn_qk(0, rb, True, None)
                           for rb in range(NRB)]
                    due = {}
                    for rb in range(NQ4, NRB):
                        due.setdefault(Q0 + (rb - NQ4) * (16 - Q0) // (NRB - NQ4), []).extend(pss[rb])
                    run(dots, carry=due)
                    vb0[:, 0:HALO, :] = jnp.broadcast_to(vb0[:, HALO:HALO + 1, :], (8, HALO, 128))
                    outs = [b_attn_pv(0, rb, 0, pss[rb]) for rb in range(NRB)]
                    run([], (xcvt_jobs(2 * SB, 0), 0, 0, 0))
                    P0 = 0
                    due = {}
                    for rb in range(NRB if P0 else 0):
                        due.setdefault(P0 + rb * (8 - P0) // NRB, []).extend(outs[rb])
                    run(b_proj_dots(1, (t1,), 1), carry=due)
        with scope('w6'):
            cp_xb3.wait()

        ASP = 21

        def side(ja, jo, jw, n):
            JM = 1
            if JM == 2:
                return [(ja[:1] + jo[:1] + jw[:1], 0, n, 0)]
            if JM == 0:
                return [(ja[::2], 1, n + 1, 0), (ja[1::2], 1, n + 1, 64), (jo, 1, n + 1, 32), (jw, 1, n + 1, 96)]
            allj = ja + jo + jw
            return [(allj[0::2], 1, n + 1, 0), (allj[1::2], 1, n + 1, 64)]

        def sink(n):
            def job(token):
                z = pl.multiple_of(zero[0], 8)
                vals = []
                SK = 0
                if SK & 1: vals.append(oball[pl.ds(z, 8), 0:128])
                if SK & 2: vals.append(wa[pl.ds(z, 8), :])
                if SK & 4: vals.append(woa[zero[0], 0:8, :])
                if SK & 8: vals.append(wos[pl.ds(z, 8), :])
                return vals
            return ([job], n, n, 0)

        def b_body(it, carry):
            with scope('b_wait'):
                @pl.when(it == 1)
                def _():
                    cp_wob.wait()

                @pl.when(jnp.logical_and(it > 0, it <= 5))
                def _():
                    xr = rows(xb, pl.multiple_of((4 + 2 * it) * SB, 2 * SB), 2 * SB)
                    pltpu.make_async_copy(xr, xr, sem.at[SEM_X + it - 1]).wait()

                @pl.when(it > 0)
                def _():
                    chunk_wait(it - 1)

            r0 = pl.multiple_of((2 * it + 2) * SB, 2 * SB)
            ja, jo, jw = chunk_jobs(it)
            na, no, nw = len(ja) // 2, len(jo) // 2, len(jw) // 2
            due = run(b_proj_dots(0, KVQ), (attn_jobs(1, r0 - SB), 1, ASP, 112),
                      *side(ja[:na], jo[:no], jw[:nw], 23),
                      (xcvt_jobs(r0 + SB, 1), 0, 20, 0), sink(23))
            run(b_proj_dots(1, KVQ), (attn_jobs(0, r0), 1, ASP, 112),
                *side(ja[na:], jo[no:], jw[nw:], 23),
                (xcvt_jobs(jnp.minimum(r0 + 2 * SB, S - SB), 0), 0, 20, 0), sink(23), carry=due)
            return carry

        with scope('b_loop'):
            lax.fori_loop(0, NSTEP // 2 - 1, b_body, 0)
        cp_worest.wait()
        jo = [wocopy_job(NCH * WOR + i * 32, NCH * WOR // 2 + i * 16) for i in range(WOREST // 32)]
        with scope('b_epi'):
            r1 = (S // 64) * MB
            dots = sum([b_out_dots(r) for r in range(r1, S, SB)], [])
            run(dots, (attn_jobs(1, S - SB), 0, len(dots) - 11, 112), (jo, 0, 0, 0))
        b_out_start(r1, S - r1)

    if not 0:
        phase_b()

    cp_xa.wait()
    cp_m0.wait()
    scale_a = DH ** -0.5
    NP = HA // 2
    L2 = 2 * LA
    NVS = (2, 1)

    def masks(NV):
        QR = LA - 8 * NV
        r = lax.broadcasted_iota(i32, (2 * QR, L2), 0)
        c = lax.broadcasted_iota(i32, (2 * QR, L2), 1)
        same = (r >= QR) == (c >= LA)
        rr = jnp.where(r >= QR, r - QR, r) + 8 * NV
        cc = jnp.where(c >= LA, c - LA, c)
        valid = same & ((cc >= SEG) | (rr >= SEG) | (cc <= rr))
        fill = jnp.where(same, NEG, -jnp.inf).astype(f32)
        return valid, fill

    msk = {nv: masks(nv) for nv in set(NVS)}
    sub8 = lax.broadcasted_iota(i32, (8, 128), 0)

    qscale = scale_a * LOG2E
    tsum = lambda xs: functools.reduce(lambda a, b: a + b, xs)

    def vpu_part(q, k8, v8, causal, prev):
        ss = []
        for j in range(8):
            s_ = jnp.broadcast_to(jnp.sum(q * k8[j:j + 1], axis=-1, keepdims=True), (8, 128))
            if causal and j > 0:
                s_ = jnp.where(sub8 >= j, s_, NEG * LOG2E)
            ss.append(s_)
        m = functools.reduce(jnp.maximum, ss if prev is None else ss + [prev[0]])
        es = [jnp.exp2(s_ - m) for s_ in ss]
        l = tsum(es)
        o = tsum([e * v8[j:j + 1] for j, e in enumerate(es)])
        if prev is not None:
            al = jnp.exp2(prev[0] - m)
            l = l + prev[1] * al
            o = o + prev[2] * al
        return m, l, o

    k1 = SPLIT * DH
    TL = 2

    def bout_half(rb0, i, acc):
        j, half = i // 2, i % 2
        o = _as_bf16(obs[0:MB // 2, half * 512:(half + 1) * 512])
        w = jnp.concatenate([wos[pl.ds(j * BREG + d * DP, 16), :] for d in range(half * 16, half * 16 + 16)], axis=0)
        y = jnp.dot(o, _as_bf16(w), preferred_element_type=f32)
        if half == 0:
            acc.append(y)
        else:
            outb[pl.ds(rb0, MB), j * 128:(j + 1) * 128] = (y + acc.pop()).astype(bf16)

    def segment(which, r0, rb0):
        h_ref = ha if which == 0 else hb
        oc_ref = oca if which == 0 else ocb
        nrow_o = 32 if which == 0 else 48
        NV = NVS[which]
        QR = LA - 8 * NV
        valid, fill = msk[NV]
        h = h_ref[...]
        zvec = zeros_vec()

        NH = 6 if which == 1 else 0
        KH = 4 * 128
        order = [(2 * t + e, i) for t in range(NP) for e in range(2) for i in range(3)]
        pre = {}
        for hd, t in order[:NH]:
            pre[hd, t] = jnp.dot(h[:, :KH], _as_bf16(wa[pl.ds(t * TREG + hd * TP, KH // 2), :]),
                                 preferred_element_type=f32)

        def proj(hd, t, ties):
            if (hd, t) in pre:
                y = jnp.dot(h[:, KH:], _as_bf16(wa[pl.ds(t * TREG + hd * TP + KH // 2, (DM - KH) // 2), :]),
                            preferred_element_type=f32)
                y = y + pre.pop((hd, t))
            else:
                w = tied(wa[pl.ds(t * TREG + hd * TP, DM // 2), :], zvec, *ties)
                y = jnp.dot(h, _as_bf16(w), preferred_element_type=f32)
            if which == 0:
                ex[t * HA + hd] = y[32:40]
                return jnp.concatenate([y[0:32], y[40:48]], axis=0)
            return jnp.concatenate([ex[t * HA + hd], y[8:32], y[0:8]], axis=0)

        def wo_part1(j, ties):
            o1 = _as_bf16(oc_ref[:, :k1])
            part[0:nrow_o, j * 128:(j + 1) * 128] = jnp.dot(
                o1, _as_bf16(tied(woa[j, :k1 // 2, :], zvec, *ties)), preferred_element_type=f32)

        def vpu_jobs(t, ys):
            out = []
            for e in range(2):
                hd = 2 * t + e
                q, k, v = ys[3 * e:3 * e + 3]
                jobs = []
                ov[hd] = []
                for g in range(NV):
                    q0 = q[8 * g:8 * g + 8] * qscale
                    if which == 1 and g == 0:
                        st = [sv[i * HA + hd] for i in range(3)]
                    else:
                        st = None
                        for b in range(g, -1, -1):
                            st = vpu_part(q0, k[8 * b:8 * b + 8], v[8 * b:8 * b + 8], b == g, st)
                            jobs.append(list(st[1:]))
                    _, l, o = vpu_part(q0, k[SEG:LA], v[SEG:LA], False, st)
                    ov[hd].append(o * _recip(l))
                    jobs.append([ov[hd][-1]])
                if which == 0 and NVS[1]:
                    st = vpu_part(ex[hd] * qscale, ex[HA + hd], ex[2 * HA + hd], True, None)
                    for i in range(3):
                        sv[i * HA + hd] = st[i]
                    jobs.append(list(st[1:]))
                out += jobs
            slots = [[] for _ in range(12)]
            for i, jb in enumerate(out):
                slots[(2 * i + 1) * 6 // len(out)] += jb
            return slots

        ov, pend, ps, bacc = {}, {}, {}, []
        nj = 0
        for t in range(NP + LAG2):
            ties = pend.pop(t - TL, [[]] * 12)
            if t < NP:
                ys = [proj(2 * t + e, i, ties[6 * e + 2 * i:6 * e + 2 * i + 2]) for e in range(2) for i in range(3)]
                qkvb[(which * NP + t) * 3, 0:QR, :] = _as_u32(
                    jnp.concatenate([ys[0][8 * NV:], ys[3][8 * NV:]], axis=0).astype(bf16))
                for i in range(1, 3):
                    qkvb[(which * NP + t) * 3 + i] = _as_u32(jnp.concatenate([ys[i], ys[3 + i]], axis=0).astype(bf16))
                pend[t] = vpu_jobs(t, ys)
            else:
                wo_part1(nj, (sum(ties[0:3], []), sum(ties[3:6], [])))
                wo_part1(nj + 1, (sum(ties[6:9], []), sum(ties[9:12], [])))
                nj += 2
            p_ = t - LAG1
            if 0 <= p_ < NP:
                if which == 1 and MB:
                    bout_half(rb0, p_, bacc)
                sc = lax.dot_general(_as_bf16(qkvb[(which * NP + p_) * 3, 0:QR, :]), _as_bf16(qkvb[(which * NP + p_) * 3 + 1]), _NT,
                                     preferred_element_type=f32) * scale_a
                sc = jnp.where(valid, sc, fill)
                m = jnp.max(sc, axis=-1, keepdims=True)
                p = jnp.exp(sc - m)
                pn = (p * _recip(jnp.sum(p, axis=-1, keepdims=True))).astype(bf16)
                if 1:
                    pb[which * NP + p_, 0:QR, 0:L2] = _as_u32(pn)
                else:
                    ps[p_] = pn
            p_ = t - LAG2
            if 0 <= p_ < NP:
                o = jnp.dot(_as_bf16(pb[which * NP + p_, 0:QR, 0:L2]) if 1 else ps.pop(p_), _as_bf16(qkvb[(which * NP + p_) * 3 + 2]),
                            preferred_element_type=f32)
                for e in range(2):
                    hd = 2 * p_ + e
                    oh = jnp.concatenate(ov.pop(hd) + [o[QR * e:QR * e + QR]], axis=0)
                    if which == 0:
                        df[hd] = oh[24:32]
                        z = jnp.concatenate([oh[32:40], oh[0:24]], axis=0)
                    else:
                        z = jnp.concatenate([oh, df[hd]], axis=0)
                    oc_ref[:, hd * DH:(hd + 1) * DH] = _as_u32(z.astype(bf16))
        for j in range(nj, 8):
            wo_part1(j, ([], []))
        o2 = _as_bf16(oc_ref[:, k1:])
        for j in range(8):
            cs = slice(j * 128, (j + 1) * 128)
            y = part[0:nrow_o, cs] + jnp.dot(o2, _as_bf16(woa[j, k1 // 2:, :]), preferred_element_type=f32)
            if which == 0:
                hb[0:8, cs] = y[0:8].astype(bf16)
                outa[pl.ds(r0, 24), cs] = y[8:32].astype(bf16)
            else:
                outa[pl.ds(r0 + 24, 8), cs] = y[40:48].astype(bf16)
                outa[pl.ds(r0 + 32, 32), cs] = y[0:32].astype(bf16)
                ha[40:48, cs] = y[32:40].astype(bf16)

    UA = 1

    def a_body(it, carry):
        for u in range(UA):
            r0 = pl.multiple_of((it * UA + u) * 64, 64)
            ha[0:40, :] = xa[pl.ds(r0, 40), :]
            hb[8:32, :] = xa[pl.ds(r0 + 40, 24), :]
            rb0 = pl.multiple_of((it * UA + u) * MB, 16)
            if MB:
                obs[0:MB // 2, :] = oball[pl.ds(pl.multiple_of((it * UA + u) * (MB // 2), 8), MB // 2), :]
            segment(0, r0, rb0)
            segment(1, r0, rb0)
        r0 = pl.multiple_of(it * UA * 64, 64)
        pltpu.make_async_copy(rows(outa, r0, 64 * UA),
                              out_hbm.at[pl.ds(r0, 64 * UA), pl.ds(0, DM)], sem_out.at[0]).start()
        b_out_start(pl.multiple_of(it * UA * MB, 16), UA * MB)
        return carry

    if 0:
        outa[0:16, 0:128] = _as_bf16(wa[pl.ds(pl.multiple_of(zero[0], 8), 8), :]) + _as_bf16(woa[zero[0], 0:8, :])
        pltpu.make_async_copy(outa, out_hbm.at[:, pl.ds(0, DM)], sem_out.at[0]).start()
        b_out_start(0, (S // 64) * MB)
    else:
        with scope('a_loop'):
            lax.fori_loop(0, S // 64 // UA, a_body, 0)

    with scope('final_wait'):
        pltpu.make_async_copy(outb, out_hbm.at[:, pl.ds(DM, DM)], sem_out.at[1]).wait()
        pltpu.make_async_copy(outa, out_hbm.at[:, pl.ds(0, DM)], sem_out.at[0]).wait()


@functools.partial(jax.jit, static_argnames=("A_seg_len",))
def pallas_concat_heads__memory_aug_recurrent_mem_tr__sliding_local_dilated__prompt_kernel(
    A_x, A_mem0, A_Wq, A_Wk, A_Wv, A_Wo, A_seg_len, B_x, B_wqkv, B_wo,
):
    assert A_seg_len == SEG and A_x.shape == (1, S, DM) and B_x.shape == (1, S, DM)
    vm = pltpu.VMEM
    scratch = [
        vm((S, DM), bf16), vm((S, DM), bf16),
        vm((S, DM), bf16), vm((S, DM), bf16),
        vm((3 * DM * HA + RG + 16, DH), bf16),
        vm((HA * DH + 48, DM), bf16),
        vm((3, DM, DM), bf16), vm((DM, DM + 256), bf16),
        vm((3 * TREG + DM // 2 + 2 * TP, DH), u32),
        vm((8, HA * DH // 2, 128), u32),
        vm((25 * BREG, 128), u32), vm((9 * BREG, 128), u32),
        vm((8, SB + HALO, 128), f32), vm((8, SB + HALO, 128), f32),
        vm((8, SB + HALO, 128), f32), vm((8, SB + HALO, 128), f32),
        vm((SB // 2, DM), u32), vm((SB // 2, DM), u32),
        vm((SB // 2, DM), u32), vm((SB // 2, DM), u32),
        vm((48, DM), bf16), vm((32, DM), bf16),
        vm((16, HA * DH), u32), vm((24, HA * DH), u32),
        vm((48, DM), f32),
        vm((3 * HA, 8, 128), f32), vm((HA, 8, 128), f32), vm((3 * HA, 8, 128), f32),
        vm((96, LA, 128), u32), vm((32, LA, 128), u32),
        vm((S // 2, DM), u32), vm((32, DM), u32),
        pltpu.SMEM((1,), i32),
        pltpu.SemaphoreType.DMA((32,)),
        pltpu.SemaphoreType.DMA((2,)),
    ] + [vm((9, RB, 128), f32)] * (2 * NRB)
    out = pl.pallas_call(
        _kernel,
        out_shape=jax.ShapeDtypeStruct((S, 2 * DM), bf16),
        in_specs=[pl.BlockSpec(memory_space=pl.ANY)] * 9,
        out_specs=pl.BlockSpec(memory_space=pl.ANY),
        scratch_shapes=scratch,
        compiler_params=pltpu.CompilerParams(
            vmem_limit_bytes=120 * 1024 * 1024,
            disable_bounds_checks=bool(0),
            disable_semaphore_checks=bool(0),
            shape_invariant_numerics=bool(1),
        ),
        name="concat_heads_kernel",
    )(
        A_x.reshape(S, DM), A_mem0.reshape(MEM, DM),
        A_Wq.reshape(DM * HA, DH), A_Wk.reshape(DM * HA, DH), A_Wv.reshape(DM * HA, DH),
        A_Wo.reshape(HA * DH, DM),
        B_x.reshape(S, DM), B_wqkv, B_wo,
    )
    return out.reshape(1, S, 2 * DM)
```

```python
import contextlib
import functools

import jax
import jax.numpy as jnp
from jax import lax
import jax.experimental.pallas as pl
import jax.experimental.pallas.tpu as pltpu

bf16, f32, u32, i32 = jnp.bfloat16, jnp.float32, jnp.uint32, jnp.int32

S, DM = 2048, 1024
HA, DH, MEM, SEG = 32, 128, 8, 32
LA = MEM + SEG
HB, NW, DIL = 32, 8, 2
HALO = 16
NEG = -1000000000.0
LOG2E = 1.4426950408889634

SB = 128
NSTEP = S // SB
RB = 8
NRB = SB // RB
TP = 514
TREG = HA * TP
DP = 18
BREG = HB * DP
NCH = 6
GPC = 3 * (DM // 16) // NCH
RG = 16 * HA
WOR = 640
WOREST = HA * DH - NCH * WOR
MB = 48
SPLIT = 24
LAG1, LAG2 = 1, 3

_NT = (((1,), (1,)), ((), ()))


def scope(name):
    return jax.named_scope(name) if 0 else contextlib.nullcontext()


def _as_bf16(x):
    return pltpu.bitcast(x, bf16)


def _as_u32(x):
    return pltpu.bitcast(x, u32)


def _interleave(a, b):
    lo = (a & jnp.uint32(0xFFFF)) | (b << 16)
    hi = (a >> 16) | (b & jnp.uint32(0xFFFF0000))
    return lo, hi


def _recip(x):
    r = pl.reciprocal(x, approx=True)
    return r * (2.0 - x * r)


def _kernel(xa_hbm, mem0_hbm, wq_hbm, wk_hbm, wv_hbm, wo_hbm, xb_hbm, wqkvb_hbm, wob_hbm,
            out_hbm,
            xa, xb, outa, outb, rawa, rawo, rawb, rawob, wa, woa, wt, wos,
            kb0, kb1, vb0, vb1, xs0, xs1, ob0, ob1,
            ha, hb, oca, ocb, part, ex, df, sv, qkvb, pb, oball, obs, zero,
            sem, sem_out, *qbufs):
    zero[0] = 0
    kbuf, vbuf, xsb = (kb0, kb1), (vb0, vb1), (xs0, xs1)

    nsem = [0]

    def cp(src, dst):
        c = pltpu.make_async_copy(src, dst, sem.at[nsem[0]])
        nsem[0] += 1
        return c

    def rows(ref, r0, n):
        return ref.at[pl.ds(r0, n), :]

    cp_ch = []
    for c in range(NCH):
        w = (wq_hbm, wk_hbm, wv_hbm)[c // 2]
        cp_ch.append(cp(rows(w, (c % 2) * GPC * RG, GPC * RG), rows(rawa, c * GPC * RG, GPC * RG)))
        cp_ch.append(cp(rows(wo_hbm, c * WOR, WOR), rows(rawo, c * WOR, WOR)))
    cp_worest = cp(rows(wo_hbm, NCH * WOR, WOREST), rows(rawo, NCH * WOR, WOREST))
    cp_xb0 = cp(rows(xb_hbm, 0, SB), rows(xb, 0, SB))
    cp_xb1 = cp(rows(xb_hbm, SB, SB), rows(xb, SB, SB))
    cp_xb2 = cp(rows(xb_hbm, 2 * SB, SB), rows(xb, 2 * SB, SB))
    cp_xb3 = cp(rows(xb_hbm, 3 * SB, 3 * SB), rows(xb, 3 * SB, 3 * SB))
    SEM_X = nsem[0]
    cp_xbs = [cp(rows(xb_hbm, (6 + 2 * c) * SB, 2 * SB), rows(xb, (6 + 2 * c) * SB, 2 * SB)) for c in range(5)]

    def cp_wb(t, k0, n):
        return cp(wqkvb_hbm.at[pl.ds(k0, n), pl.ds(t * DM, DM)], rawb.at[t, pl.ds(k0, n), :])

    KVQ = (1, 2, 0)
    KQV = (1, 0, 2)
    cp_w0 = [cp_wb(KQV[0], 0, DM // 4), cp_wb(KQV[0], DM // 4, DM // 4)]
    cp_wp = [None] + [cp_wb(KQV[h // 2], (h % 2) * (DM // 2), DM // 2) for h in range(1, 6)]
    cp_wob = cp(wob_hbm, rawob.at[:, pl.ds(0, DM)])
    cp_xa = cp(xa_hbm, xa)
    cp_m0 = cp(mem0_hbm, rows(ha, LA, MEM))
    order = cp_w0 + [cp_xb0, cp_xb1] + cp_wp[1:5] + [cp_xb2, cp_wp[5], cp_xb3]
    for c in range(NCH):
        order += cp_ch[2 * c:2 * c + 2] + cp_xbs[c:c + 1] + ([cp_wob] if c == 0 else [])
    for c in order + [cp_worest, cp_m0, cp_xa]:
        c.start()

    def chunk_wait(c):
        ra = rows(rawa, pl.multiple_of(c * (GPC * RG), GPC * RG), GPC * RG)
        pltpu.make_async_copy(ra, ra, sem.at[2 * c]).wait()
        ro = rows(rawo, pl.multiple_of(c * WOR, 128), WOR)
        pltpu.make_async_copy(ro, ro, sem.at[2 * c + 1]).wait()

    def prep_qkv_job(t, kb_, ch):
        def job(token):
            at = _as_u32(rawb[t, kb_ * 128:(kb_ + 1) * 128, ch * 128:(ch + 1) * 128].T)
            base = (t * 8 + kb_) * BREG
            for pr in range(2):
                lo, hi = _interleave(at[pr * 32:pr * 32 + 16], at[pr * 32 + 16:pr * 32 + 32])
                wt[pl.ds(base + ch * 2 + pr, 16, stride=2 * DP), :] = lo
                wt[pl.ds(base + DP + ch * 2 + pr, 16, stride=2 * DP), :] = hi
        return job

    def prep_qkv_jobs(t, kbs):
        return [prep_qkv_job(t, kb_, ch) for kb_ in kbs for ch in range(8)]

    def prep_wo_job(src_col, dst0, hq):
        def job(token):
            if token is not None:
                rawob[0:16, DM + 128:DM + 256] = token.astype(bf16)
            dst = rows(wos, dst0, BREG + 40)
            for hp in range(4 * hq, 4 * hq + 4):
                a = _as_u32(rawob[hp * 64:hp * 64 + 32, pl.ds(src_col, 128)])
                b = _as_u32(rawob[hp * 64 + 32:hp * 64 + 64, pl.ds(src_col, 128)])
                lo, hi = _interleave(a, b)
                dst[pl.ds(hp, 16, stride=2 * DP), :] = lo
                dst[pl.ds(DP + hp, 16, stride=2 * DP), :] = hi
        return job

    def tied(w, zvec, *vals_list):
        n = w.shape[0] // len(vals_list)
        parts = []
        for i, vals in enumerate(vals_list):
            pt = w[i * n:(i + 1) * n]
            if vals:
                tie = functools.reduce(lambda a, b: a | b, [_as_u32(x) for x in vals]) & zvec
                pt = jnp.concatenate([pt[0:n - 8], pt[n - 8:] | tie], axis=0)
            parts.append(pt)
        return jnp.concatenate(parts, axis=0)

    def zeros_vec():
        return jnp.full((8, 128), zero[0], i32).astype(u32)

    scale_b = (DM // HB) ** -0.5

    def b_proj_dots(p, ts, half=None):
        kbs = range(8) if half is None else range(4 * half, 4 * half + 4)

        def mk(t, c):
            def th(ties):
                x = _as_bf16(xsb[p][:, kbs[0] * 128:(kbs[-1] + 1) * 128])
                tiles = [jnp.concatenate([wt[pl.ds((t * 8 + kb_) * BREG + (4 * c + dd) * DP, 16), :]
                                          for dd in range(4)], axis=0) for kb_ in kbs]
                if ties:
                    tiles[-1] = tied(tiles[-1], zeros_vec(), ties)
                y = lax.dot_general(x, _as_bf16(jnp.concatenate(tiles, axis=1)), _NT, preferred_element_type=f32)
                if t == 0:
                    for rb in range(NRB):
                        yr = y[rb * RB:(rb + 1) * RB]
                        qbufs[p * NRB + rb][c] = yr + qbufs[p * NRB + rb][c] if half == 1 else yr
                else:
                    g = kbuf if t == 1 else vbuf
                    if half != 0:
                        g[p][c, 0:HALO, :] = g[1 - p][c, SB:SB + HALO, :]
                    g[p][c, HALO:HALO + SB, :] = y + g[p][c, HALO:HALO + SB, :] if half == 1 else y
                return y
            return th
        return [mk(t, c) for t in ts for c in range(8)]

    def b_out_dots(r0):
        def mk(j):
            def th(ties):
                o = _as_bf16(oball[r0 // 2:(r0 + SB) // 2, :])
                w = jnp.concatenate([wos[pl.ds(j * BREG + d * DP, 16), :] for d in range(32)], axis=0)
                y = jnp.dot(o, _as_bf16(w), preferred_element_type=f32)
                outb[pl.ds(r0, SB), j * 128:(j + 1) * 128] = y.astype(bf16)
                return y
            return th
        return [mk(j) for j in range(8)]

    def b_attn_qk(p, rb, first, token):
        q_ref, k_ref = qbufs[p * NRB + rb], kbuf[p]
        z, gate = 0, None
        if token is not None:
            token = token[8:8 + RB]
            if 1:
                gate = _as_u32(token) & zeros_vec()
            else:
                z = zero[0]
                q_ref[8] = token
        b0 = rb * RB
        acc = [None] * NW
        for c in range(8):
            q = q_ref[z + c]
            if gate is not None:
                q = pltpu.bitcast(_as_u32(q) | gate, f32)
            for w in range(NW):
                pr = q * k_ref[c, pl.ds(HALO + b0 - DIL * w, RB), :]
                acc[w] = pr if acc[w] is None else acc[w] + pr
        lg = []
        for w in range(NW):
            a = acc[w]
            a = a + pltpu.roll(a, 64, 1)
            a = a + pltpu.roll(a, 32, 1)
            a = a * (scale_b * LOG2E)
            if first and b0 < DIL * w:
                row = b0 + lax.broadcasted_iota(i32, (RB, 128), 0)
                a = jnp.where(row >= DIL * w, a, NEG * LOG2E)
            lg.append(a)
        m = functools.reduce(jnp.maximum, lg)
        es = [jnp.exp2(a - m) for a in lg]
        inv = _recip(functools.reduce(lambda a, b: a + b, es))
        return [e * inv for e in es]

    def b_attn_pv(p, rb, r0, ps):
        v_ref, b0 = vbuf[p], rb * RB
        dst = (ob0, ob1)[p] if r0 is None else rows(oball, pl.multiple_of(r0 // 2, SB // 2), SB // 2)
        outs = []
        for c in range(8):
            o = None
            for w in range(NW):
                pr = ps[w] * v_ref[c, pl.ds(HALO + b0 - DIL * w, RB), :]
                o = pr if o is None else o + pr
            dst[pl.ds(b0 // 2, RB // 2), c * 128:(c + 1) * 128] = _as_u32(o.astype(bf16))
            outs.append(o)
        return outs

    def attn_jobs(p, r0):
        def mk(rb):
            def job(token):
                if 1 == 3 and not isinstance(r0, int):
                    b_attn_pv(p, rb, None, b_attn_qk(p, rb, False, token))
                    if rb % 2 == 0:
                        return None
                    v = (ob0, ob1)[p][(rb // 2) * 8:(rb // 2) * 8 + 8, :]
                    oball[pl.ds(pl.multiple_of(r0 // 2 + (rb // 2) * 8, 8), 8), :] = v
                    return [v[:, c * 128:(c + 1) * 128] for c in range(8)]
                outs = b_attn_pv(p, rb, r0, b_attn_qk(p, rb, False, token if 1 else None))
                if 1 == 2:
                    return [oball[pl.ds(pl.multiple_of(zero[0], 8), 8), 0:128]]
                return outs if 1 else None
            return job
        return [mk(rb) for rb in range(NRB)]

    def xcvt_jobs(r0, p):
        def mk(i):
            def job(token):
                xsb[p][i * 8:(i + 1) * 8, :] = _as_u32(xb[pl.ds(pl.multiple_of(r0 + i * 16, 16), 16), :])
            return job
        return [mk(i) for i in range(SB // 16)]

    RAWA_PAD = 3 * DM * HA
    RAWO_PAD = HA * DH

    def repack_job(src0, dst0, half):
        def job(token):
            if token is not None:
                rawa[pl.ds(RAWA_PAD + RG, 16), :] = token.astype(bf16)
            src = rows(rawa, src0, RG)
            dst = rows(wa, dst0, TREG + 1032)
            for ii in range(half * 4, half * 4 + 4):
                lo, hi = _interleave(_as_u32(src[ii * 64:ii * 64 + 32, :]), _as_u32(src[ii * 64 + 32:ii * 64 + 64, :]))
                dst[pl.ds(ii, 16, stride=2 * TP), :] = lo
                dst[pl.ds(ii + TP, 16, stride=2 * TP), :] = hi
        return job

    def wocopy_job(src0, dst0):
        def job(token):
            if token is not None:
                rawo[pl.ds(RAWO_PAD + 32, 16), 0:128] = token.astype(bf16)
            v = _as_u32(rawo[pl.ds(src0, 32), :])
            for j in range(8):
                woa[j, pl.ds(dst0, 16), :] = v[:, j * 128:(j + 1) * 128]
        return job

    def chunk_jobs(it):
        c = jnp.maximum(it - 1, 0)
        real = it > 0
        ja, jo = [], []
        for i in range(GPC):
            src0 = pl.multiple_of(jnp.where(real, (c * GPC + i) * RG, RAWA_PAD), RG)
            dst0 = pl.multiple_of((c // 2) * TREG + ((c % 2) * GPC + i) * 8, 8)
            ja += [repack_job(src0, dst0, 0), repack_job(src0, dst0, 1)]
        for i in range(WOR // 32):
            src0 = pl.multiple_of(jnp.where(real, c * WOR + i * 32, RAWO_PAD), 32)
            dst0 = pl.multiple_of(c * (WOR // 2) + i * 16, 16)
            jo.append(wocopy_job(src0, dst0))
        jw = []
        for i in range(2):
            j = jnp.clip(2 * (it - 2) + i, 0, 7)
            src_col = pl.multiple_of(jnp.where(it > 1, j * 128, DM), 128)
            jw += [prep_wo_job(src_col, pl.multiple_of(j * BREG, 8), hq) for hq in range(4)]
        return ja, jo, jw

    TD = 5

    def run(dots, *job_lists, carry=None):
        rel = {}
        for jobs, lo, hi, tr in job_lists:
            for i, job in enumerate(jobs):
                rel.setdefault(lo + i * (hi - lo) // len(jobs) - 1, []).append((job, tr))
        due = {} if carry is None else carry

        def fire(i, y):
            for job, tr in rel.get(i, []):
                vals = job(None if y is None else y[tr:tr + 16])
                if vals and TD:
                    due.setdefault(min(i + TD, len(dots) - 1) if 1 else i + TD, []).extend(vals)

        fire(-1, None)
        for i, th in enumerate(dots):
            fire(i, th(due.pop(i, [])))
        return {k - len(dots): v for k, v in due.items()}

    def b_out_start(r0, n):
        pltpu.make_async_copy(rows(outb, r0, n),
                              out_hbm.at[pl.ds(r0, n), pl.ds(DM, DM)], sem_out.at[1]).start()

    zeros_halo = jnp.zeros((8, HALO, 128), f32)
    KA = 31
    z8 = pl.multiple_of(zero[0], 8)
    keep = jnp.zeros((8, 128), u32)
    for bit, ref in ((1, qkvb), (2, pb)):
        if KA & bit:
            ref[0, 0:8, :] = jnp.zeros((8, 128), u32)
            keep = keep | ref[zero[0], 0:8, :]
    for bit, ref in ((4, oca), (4, ocb), (4, obs)):
        if KA & bit:
            ref[0:8, 0:128] = jnp.zeros((8, 128), u32)
            keep = keep | ref[pl.ds(z8, 8), 0:128]
    for bit, ref in ((8, ex), (8, df), (8, sv)):
        if KA & bit:
            ref[0] = jnp.zeros((8, 128), f32)
            keep = keep | _as_u32(ref[zero[0]])
    if KA & 16:
        part[0:8, 0:128] = jnp.zeros((8, 128), f32)
        keep = keep | _as_u32(part[pl.ds(z8, 8), 0:128])
    outa[0:16, 0:128] = _as_bf16(keep)
    kb1[:, SB:SB + HALO, :] = zeros_halo
    vb1[:, SB:SB + HALO, :] = zeros_halo
    rawa[pl.ds(RAWA_PAD, RG), :] = jnp.zeros((RG, DH), bf16)
    rawo[pl.ds(RAWO_PAD, 32), :] = jnp.zeros((32, DM), bf16)
    rawob[:, DM:DM + 128] = jnp.zeros((DM, 128), bf16)

    def phase_b():
        with scope('s0'):
            for i in range(2):
                cp_w0[i].wait()
                run([], (prep_qkv_jobs(KQV[0], range(2 * i, 2 * i + 2)), 0, 0, 0))
            cp_xb0.wait()
            run([], (xcvt_jobs(0, 0), 0, 0, 0))
            run(b_proj_dots(0, KQV[0:1], 0))
            cp_xb1.wait()
            run([], (xcvt_jobs(SB, 1), 0, 0, 0))
        for h in range(1, 6):
            with scope('w%d' % h):
                cp_wp[h].wait()
                if h == 5:
                    cp_xb2.wait()
            with scope('s%d' % h):
                t0, t1 = KQV[(h - 1) // 2], KQV[h // 2]
                run([], (prep_qkv_jobs(t1, range(4 * (h % 2), 4 * (h % 2) + 4)), 0, 0, 0))
                dots = b_proj_dots(1, (t0,), (h - 1) % 2) + b_proj_dots(0, (t1,), h % 2)
                NQ4 = 8
                Q0 = 8
                if h < 4:
                    run(dots)
                elif h == 4:
                    due = {}
                    for rb in range(NQ4):
                        ps_ = b_attn_qk(0, rb, True, None)
                        for w in range(NW):
                            qbufs[rb][w] = ps_[w]
                        due.setdefault(Q0 + rb * (16 - Q0) // NQ4, []).extend(ps_)
                    run(dots, carry=due)
                else:
                    pss = [[qbufs[rb][w] for w in range(NW)] if rb < NQ4 else b_attn_qk(0, rb, True, None)
                           for rb in range(NRB)]
                    due = {}
                    for rb in range(NQ4, NRB):
                        due.setdefault(Q0 + (rb - NQ4) * (16 - Q0) // (NRB - NQ4), []).extend(pss[rb])
                    run(dots, carry=due)
                    vb0[:, 0:HALO, :] = jnp.broadcast_to(vb0[:, HALO:HALO + 1, :], (8, HALO, 128))
                    outs = [b_attn_pv(0, rb, 0, pss[rb]) for rb in range(NRB)]
                    run([], (xcvt_jobs(2 * SB, 0), 0, 0, 0))
                    P0 = 0
                    due = {}
                    for rb in range(NRB if P0 else 0):
                        due.setdefault(P0 + rb * (8 - P0) // NRB, []).extend(outs[rb])
                    run(b_proj_dots(1, (t1,), 1), carry=due)
        with scope('w6'):
            cp_xb3.wait()

        ASP = 20

        def side(ja, jo, jw, n):
            JM = 1
            if JM == 2:
                return [(ja[:1] + jo[:1] + jw[:1], 0, n, 0)]
            if JM == 0:
                return [(ja[::2], 1, n + 1, 0), (ja[1::2], 1, n + 1, 64), (jo, 1, n + 1, 32), (jw, 1, n + 1, 96)]
            allj = ja + jo + jw
            return [(allj[0::2], 1, n + 1, 0), (allj[1::2], 1, n + 1, 48)]

        def sink(n):
            def job(token):
                z = pl.multiple_of(zero[0], 8)
                vals = []
                SK = 0
                if SK & 1: vals.append(oball[pl.ds(z, 8), 0:128])
                if SK & 2: vals.append(wa[pl.ds(z, 8), :])
                if SK & 4: vals.append(woa[zero[0], 0:8, :])
                if SK & 8: vals.append(wos[pl.ds(z, 8), :])
                return vals
            return ([job], n, n, 0)

        def b_body(it, carry):
            with scope('b_wait'):
                @pl.when(it == 2)
                def _():
                    cp_wob.wait()

                @pl.when(jnp.logical_and(it > 0, it <= 5))
                def _():
                    xr = rows(xb, pl.multiple_of((4 + 2 * it) * SB, 2 * SB), 2 * SB)
                    pltpu.make_async_copy(xr, xr, sem.at[SEM_X + it - 1]).wait()

                @pl.when(it > 0)
                def _():
                    chunk_wait(it - 1)

            r0 = pl.multiple_of((2 * it + 2) * SB, 2 * SB)
            ja, jo, jw = chunk_jobs(it)
            na, no, nw = len(ja) // 2, len(jo) // 2, len(jw) // 2
            due = run(b_proj_dots(0, KVQ), (attn_jobs(1, r0 - SB), 1, ASP, 112),
                      *side(ja[:na], jo[:no], jw[:nw], 23),
                      (xcvt_jobs(r0 + SB, 1), 0, 20, 0), sink(23))
            run(b_proj_dots(1, KVQ), (attn_jobs(0, r0), 1, ASP, 112),
                *side(ja[na:], jo[no:], jw[nw:], 23),
                (xcvt_jobs(jnp.minimum(r0 + 2 * SB, S - SB), 0), 0, 20, 0), sink(23), carry=due)
            return carry

        with scope('b_loop'):
            lax.fori_loop(0, NSTEP // 2 - 1, b_body, 0)
        cp_worest.wait()
        jo = [wocopy_job(NCH * WOR + i * 32, NCH * WOR // 2 + i * 16) for i in range(WOREST // 32)]
        with scope('b_epi'):
            r1 = (S // 64) * MB
            dots = sum([b_out_dots(r) for r in range(r1, S, SB)], [])
            run(dots, (attn_jobs(1, S - SB), 0, len(dots) - 11, 112), (jo, 0, 0, 0))
        b_out_start(r1, S - r1)

    if not 0:
        phase_b()
    else:
        for c in order + [cp_worest]:
            c.wait()
        b_out_start((S // 64) * MB, S - (S // 64) * MB)

    cp_xa.wait()
    cp_m0.wait()
    scale_a = DH ** -0.5
    NP = HA // 2
    L2 = 2 * LA
    NVS = (2, 1)

    def masks(NV):
        QR = LA - 8 * NV
        r = lax.broadcasted_iota(i32, (2 * QR, L2), 0)
        c = lax.broadcasted_iota(i32, (2 * QR, L2), 1)
        same = (r >= QR) == (c >= LA)
        rr = jnp.where(r >= QR, r - QR, r) + 8 * NV
        cc = jnp.where(c >= LA, c - LA, c)
        valid = same & ((cc >= SEG) | (rr >= SEG) | (cc <= rr))
        fill = jnp.where(same, NEG * LOG2E if 0 else NEG, -jnp.inf).astype(f32)
        return valid, fill

    msk = {nv: masks(nv) for nv in set(NVS)}
    sub8 = lax.broadcasted_iota(i32, (8, 128), 0)

    qscale = scale_a * LOG2E
    tsum = lambda xs: functools.reduce(lambda a, b: a + b, xs)

    def vpu_part(q, k8, v8, causal, prev):
        ss = []
        for j in range(8):
            s_ = jnp.broadcast_to(jnp.sum(q * k8[j:j + 1], axis=-1, keepdims=True), (8, 128))
            if causal and j > 0:
                s_ = jnp.where(sub8 >= j, s_, NEG * LOG2E)
            ss.append(s_)
        m = functools.reduce(jnp.maximum, ss if prev is None else ss + [prev[0]])
        es = [jnp.exp2(s_ - m) for s_ in ss]
        l = tsum(es)
        o = tsum([e * v8[j:j + 1] for j, e in enumerate(es)])
        if prev is not None:
            al = jnp.exp2(prev[0] - m)
            l = l + prev[1] * al
            o = o + prev[2] * al
        return m, l, o

    k1 = SPLIT * DH
    TL = 2

    def bout_half(rb0, i, acc):
        j, half = i // 2, i % 2
        o = _as_bf16(obs[0:MB // 2, half * 512:(half + 1) * 512])
        w = jnp.concatenate([wos[pl.ds(j * BREG + d * DP, 16), :] for d in range(half * 16, half * 16 + 16)], axis=0)
        y = jnp.dot(o, _as_bf16(w), preferred_element_type=f32)
        if half == 0:
            acc.append(y)
        else:
            outb[pl.ds(rb0, MB), j * 128:(j + 1) * 128] = (y + acc.pop()).astype(bf16)

    OG = 4

    def segment(which, r0, rb0, it):
        h_ref = ha if which == 0 else hb
        oc_ref = oca if which == 0 else ocb
        nrow_o = 32 if which == 0 else 48
        NV = NVS[which]
        QR = LA - 8 * NV
        valid, fill = msk[NV]
        h = h_ref[...]
        zvec = zeros_vec()

        NH = 6 if which == 1 else 0
        KH = 4 * 128
        pord = {0: [(0, 0), (0, 1), (0, 2), (1, 0), (1, 1), (1, 2)],
                1: [(0, 1), (0, 0), (1, 1), (1, 0), (0, 2), (1, 2)],
                2: [(0, 2), (0, 1), (0, 0), (1, 2), (1, 1), (1, 0)],
                3: [(0, 2), (1, 2), (0, 1), (0, 0), (1, 1), (1, 0)]}[(0, 0)[which]]
        order = [(2 * t + e, i) for t in range(NP) for e, i in pord]
        pre = {}
        for hd, t in order[:NH]:
            pre[hd, t] = jnp.dot(h[:, :KH], _as_bf16(wa[pl.ds(t * TREG + hd * TP, KH // 2), :]),
                                 preferred_element_type=f32)

        def proj(hd, t, ties):
            if (hd, t) in pre:
                y = jnp.dot(h[:, KH:], _as_bf16(wa[pl.ds(t * TREG + hd * TP + KH // 2, (DM - KH) // 2), :]),
                            preferred_element_type=f32)
                y = y + pre.pop((hd, t))
            else:
                w = tied(wa[pl.ds(t * TREG + hd * TP, DM // 2), :], zvec, *ties)
                y = jnp.dot(h, _as_bf16(w), preferred_element_type=f32)
            if which == 0:
                ex[t * HA + hd] = y[32:40]
                return jnp.concatenate([y[0:32], y[40:48]], axis=0)
            return jnp.concatenate([ex[t * HA + hd], y[8:32], y[0:8]], axis=0)

        def wo_part1(j, ties):
            o1 = _as_bf16(oc_ref[:, :k1])
            part[0:nrow_o, j * 128:(j + 1) * 128] = jnp.dot(
                o1, _as_bf16(tied(woa[j, :k1 // 2, :], zvec, *ties)), preferred_element_type=f32)

        def vpu_jobs(t, ys):
            out = []
            for e in range(2):
                hd = 2 * t + e
                q, k, v = ys[3 * e:3 * e + 3]
                jobs = []
                ov[hd] = []
                for g in range(NV):
                    q0 = q[8 * g:8 * g + 8] * qscale
                    if which == 1 and g == 0:
                        st = [sv[i * HA + hd] for i in range(3)]
                    else:
                        st = None
                        for b in range(g, -1, -1):
                            st = vpu_part(q0, k[8 * b:8 * b + 8], v[8 * b:8 * b + 8], b == g, st)
                            jobs.append(list(st[1:]))
                    _, l, o = vpu_part(q0, k[SEG:LA], v[SEG:LA], False, st)
                    ov[hd].append(o * _recip(l))
                    jobs.append([ov[hd][-1]])
                if which == 0 and NVS[1]:
                    st = vpu_part(ex[hd] * qscale, ex[HA + hd], ex[2 * HA + hd], True, None)
                    for i in range(3):
                        sv[i * HA + hd] = st[i]
                    jobs.append(list(st[1:]))
                out += jobs
            for i, jb in enumerate(out):
                slots.setdefault(12 * t + SO + (2 * i + 1) * 6 // len(out), []).extend(jb)

        def scores(p_):
            if not 0 <= p_ < NP:
                return
            if which == 1 and MB:
                bout_half(rb0, p_, bacc)
            sc = lax.dot_general(_as_bf16(qkvb[(which * NP + p_) * 3, 0:QR, :]), _as_bf16(qkvb[(which * NP + p_) * 3 + 1]), _NT,
                                 preferred_element_type=f32)
            if 0:
                sc = jnp.where(valid, sc * qscale, fill)
                p = jnp.exp2(sc - jnp.max(sc, axis=-1, keepdims=True))
            else:
                sc = jnp.where(valid, sc * scale_a, fill)
                p = jnp.exp(sc - jnp.max(sc, axis=-1, keepdims=True))
            ps[p_] = (p * _recip(jnp.sum(p, axis=-1, keepdims=True))).astype(bf16)

        def pv(p_):
            if not 0 <= p_ < NP:
                return
            o = jnp.dot(ps.pop(p_), _as_bf16(qkvb[(which * NP + p_) * 3 + 2]), preferred_element_type=f32)
            for e in range(2):
                hd = 2 * p_ + e
                oh = jnp.concatenate(ov.pop(hd) + [o[QR * e:QR * e + QR]], axis=0)
                if which == 0:
                    df[hd] = oh[24:32]
                    z = jnp.concatenate([oh[32:40], oh[0:24]], axis=0)
                else:
                    z = jnp.concatenate([oh, df[hd]], axis=0)
                oc_ref[:, hd * DH:(hd + 1) * DH] = _as_u32(z.astype(bf16))

        SO = (21, 20)[which]
        SCP = (10, 13)[which]
        PVP = (21, 24)[which]
        ov, slots, ps, bacc = {}, {}, {}, []
        nj = 0

        def after(n):
            if 1 and (n - PVP) % 6 == 0:
                pv((n - PVP) // 6)
            if (n - SCP) % 6 == 0:
                scores((n - SCP) // 6)
            if not 1 and (n - PVP) % 6 == 0:
                pv((n - PVP) // 6)

        for t in range(NP):
            ys = [None] * 6
            for m, (e, i) in enumerate(pord):
                n = 6 * t + m
                ys[3 * e + i] = proj(2 * t + e, i, (slots.pop(2 * n, []), slots.pop(2 * n + 1, [])))
                if m == 5:
                    qkvb[(which * NP + t) * 3, 0:QR, :] = _as_u32(
                        jnp.concatenate([ys[0][8 * NV:], ys[3][8 * NV:]], axis=0).astype(bf16))
                    for i in range(1, 3):
                        qkvb[(which * NP + t) * 3 + i] = _as_u32(jnp.concatenate([ys[i], ys[3 + i]], axis=0).astype(bf16))
                    vpu_jobs(t, ys)
                after(n + 1)
        n = 6 * NP
        while nj < 8:
            wo_part1(nj, (sum([slots.pop(2 * n + i, []) for i in range(3)], []),
                          sum([slots.pop(2 * n + i, []) for i in range(3, 6)], [])))
            nj += 1
            for i in range(3):
                n += 1
                after(n)
        assert not ps and not ov and not slots
        if which == 1:
            @pl.when(it % OG == OG - 1)
            def _():
                b_out_start(pl.multiple_of(rb0 - (OG - 1) * MB, 16), OG * MB)
        o2 = _as_bf16(oc_ref[:, k1:])
        for j in range(8):
            cs = slice(j * 128, (j + 1) * 128)
            y = part[0:nrow_o, cs] + jnp.dot(o2, _as_bf16(woa[j, k1 // 2:, :]), preferred_element_type=f32)
            if which == 0:
                hb[0:8, cs] = y[0:8].astype(bf16)
                outa[pl.ds(r0, 24), cs] = y[8:32].astype(bf16)
            else:
                outa[pl.ds(r0 + 32, 32), cs] = y[0:32].astype(bf16)
                ha[40:48, cs] = y[32:40].astype(bf16)
                outa[pl.ds(r0 + 24, 8), cs] = y[40:48].astype(bf16)

    UA = 1

    def a_out_start(r0, n):
        r0 = pl.multiple_of(r0, 8)
        pltpu.make_async_copy(rows(outa, r0, n), out_hbm.at[pl.ds(r0, n), pl.ds(0, DM)], sem_out.at[0]).start()

    def a_body(it, carry):
        for u in range(UA):
            r0 = pl.multiple_of((it * UA + u) * 64, 64)
            ha[0:40, :] = xa[pl.ds(r0, 40), :]
            hb[8:32, :] = xa[pl.ds(r0 + 40, 24), :]
            rb0 = pl.multiple_of((it * UA + u) * MB, 16)
            if MB:
                obs[0:MB // 2, :] = oball[pl.ds(pl.multiple_of((it * UA + u) * (MB // 2), 8), MB // 2), :]
            segment(0, r0, rb0, it)
            @pl.when(it == OG - 1)
            def _():
                a_out_start(0, 64 * OG - 40)

            @pl.when(jnp.logical_and(it % OG == OG - 1, it >= OG))
            def _():
                a_out_start(r0 + 24 - 64 * OG, 64 * OG)

            segment(1, r0, rb0, it)
        return carry

    if 0:
        outa[0:16, 0:128] = _as_bf16(wa[pl.ds(pl.multiple_of(zero[0], 8), 8), :]) + _as_bf16(woa[zero[0], 0:8, :])
        pltpu.make_async_copy(outa, out_hbm.at[:, pl.ds(0, DM)], sem_out.at[0]).start()
        b_out_start(0, (S // 64) * MB)
    else:
        with scope('a_loop'):
            lax.fori_loop(0, S // 64 // UA, a_body, 0)
        a_out_start(S - 40, 40)

    with scope('final_wait'):
        pltpu.make_async_copy(outb, out_hbm.at[:, pl.ds(DM, DM)], sem_out.at[1]).wait()
        pltpu.make_async_copy(outa, out_hbm.at[:, pl.ds(0, DM)], sem_out.at[0]).wait()


@jax.jit
def pallas_concat_heads__memory_aug_recurrent_mem_tr__sliding_local_dilated__prompt_kernel(
    A_x, A_mem0, A_Wq, A_Wk, A_Wv, A_Wo, A_seg_len, B_x, B_wqkv, B_wo,
):
    del A_seg_len
    assert A_x.shape == (1, S, DM) and B_x.shape == (1, S, DM)
    vm = pltpu.VMEM
    scratch = [
        vm((S, DM), bf16), vm((S, DM), bf16),
        vm((S, DM), bf16), vm((S, DM), bf16),
        vm((3 * DM * HA + RG + 16, DH), bf16),
        vm((HA * DH + 48, DM), bf16),
        vm((3, DM, DM), bf16), vm((DM, DM + 256), bf16),
        vm((3 * TREG + DM // 2 + 1032, DH), u32),
        vm((8, HA * DH // 2, 128), u32),
        vm((25 * BREG, 128), u32), vm((9 * BREG, 128), u32),
        vm((8, SB + HALO, 128), f32), vm((8, SB + HALO, 128), f32),
        vm((8, SB + HALO, 128), f32), vm((8, SB + HALO, 128), f32),
        vm((SB // 2, DM), u32), vm((SB // 2, DM), u32),
        vm((SB // 2, DM), u32), vm((SB // 2, DM), u32),
        vm((48, DM), bf16), vm((32, DM), bf16),
        vm((16, HA * DH), u32), vm((24, HA * DH), u32),
        vm((48, DM), f32),
        vm((3 * HA, 8, 128), f32), vm((HA, 8, 128), f32), vm((3 * HA, 8, 128), f32),
        vm((96, LA, 128), u32), vm((32, LA, 128), u32),
        vm((S // 2, DM), u32), vm((32, DM), u32),
        pltpu.SMEM((1,), i32),
        pltpu.SemaphoreType.DMA((32,)),
        pltpu.SemaphoreType.DMA((2,)),
    ] + [vm((9, RB, 128), f32)] * (2 * NRB)
    out = pl.pallas_call(
        _kernel,
        out_shape=jax.ShapeDtypeStruct((S, 2 * DM), bf16),
        in_specs=[pl.BlockSpec(memory_space=pl.ANY)] * 9,
        out_specs=pl.BlockSpec(memory_space=pl.ANY),
        scratch_shapes=scratch,
        compiler_params=pltpu.CompilerParams(
            vmem_limit_bytes=120 * 1024 * 1024,
            disable_bounds_checks=bool(1),
            disable_semaphore_checks=bool(1),
        ),
        name="concat_heads_kernel",
    )(
        A_x.reshape(S, DM), A_mem0.reshape(MEM, DM),
        A_Wq.reshape(DM * HA, DH), A_Wk.reshape(DM * HA, DH), A_Wv.reshape(DM * HA, DH),
        A_Wo.reshape(HA * DH, DM),
        B_x.reshape(S, DM), B_wqkv, B_wo,
    )
    return out.reshape(1, S, 2 * DM)
```

```python
import functools

import jax
import jax.numpy as jnp
from jax import lax
import jax.experimental.pallas as pl
import jax.experimental.pallas.tpu as pltpu

bf16, f32, u32, i32 = jnp.bfloat16, jnp.float32, jnp.uint32, jnp.int32

S, DM = 2048, 1024
HA, DH, MEM, SEG = 32, 128, 8, 32
LA = MEM + SEG
HB, NW, DIL = 32, 8, 2
HALO = 16
NEG = -1000000000.0
LOG2E = 1.4426950408889634

SB = 128
NSTEP = S // SB
RB = 8
NRB = SB // RB
TP = 514
TREG = HA * TP
TPAD = 1032
DP = 18
BREG = HB * DP
NCH = 6
GPC = 3 * (DM // 16) // NCH
RG = 16 * HA
WOR = 640
WOREST = HA * DH - NCH * WOR
RAWA_PAD = 3 * DM * HA
RAWO_PAD = HA * DH
NIT = S // (2 * SEG)
MB = 48
OG = 4
NP = HA // 2
SPLIT = 24
NVS = (2, 1)
NSEM = 32

_NT = (((1,), (1,)), ((), ()))


def _as_bf16(x):
    return pltpu.bitcast(x, bf16)


def _as_u32(x):
    return pltpu.bitcast(x, u32)


def _sum(xs):
    return functools.reduce(lambda a, b: a + b, xs)


def _interleave(a, b):
    lo = (a & jnp.uint32(0xFFFF)) | (b << 16)
    hi = (a >> 16) | (b & jnp.uint32(0xFFFF0000))
    return lo, hi


def _recip(x):
    r = pl.reciprocal(x, approx=True)
    return r * (2.0 - x * r)


def _rows(ref, r0, n):
    return ref.at[pl.ds(r0, n), :]


def _kernel(xa_hbm, mem0_hbm, wq_hbm, wk_hbm, wv_hbm, wo_hbm, xb_hbm, wqkvb_hbm, wob_hbm,
            out_hbm,
            xa, xb, outa, outb, rawa, rawo, rawb, rawob, wa, woa, wt, wos,
            qb0, qb1, kb0, kb1, vb0, vb1, xs0, xs1, oball, obs,
            ha, hb, oca, ocb, part, ex, df, sv, qkvb, zero,
            sem, sem_out):
    zero[0] = 0
    qbuf, kbuf, vbuf, xsb = (qb0, qb1), (kb0, kb1), (vb0, vb1), (xs0, xs1)

    nsem = [0]

    def cp(src, dst):
        c = pltpu.make_async_copy(src, dst, sem.at[nsem[0]])
        nsem[0] += 1
        return c

    def cp_xb(b0, nb):
        return cp(_rows(xb_hbm, b0 * SB, nb * SB), _rows(xb, b0 * SB, nb * SB))

    def cp_wb(t, k0, n):
        return cp(wqkvb_hbm.at[pl.ds(k0, n), pl.ds(t * DM, DM)], rawb.at[t, pl.ds(k0, n), :])

    cp_ch = []
    for c in range(NCH):
        w = (wq_hbm, wk_hbm, wv_hbm)[c // 2]
        cp_ch.append(cp(_rows(w, (c % 2) * GPC * RG, GPC * RG), _rows(rawa, c * GPC * RG, GPC * RG)))
        cp_ch.append(cp(_rows(wo_hbm, c * WOR, WOR), _rows(rawo, c * WOR, WOR)))
    sem_x = nsem[0]
    cp_xbs = [cp_xb(6 + 2 * c, 2) for c in range(5)]
    cp_worest = cp(_rows(wo_hbm, NCH * WOR, WOREST), _rows(rawo, NCH * WOR, WOREST))
    cp_xb0, cp_xb1, cp_xb2, cp_xb3 = cp_xb(0, 1), cp_xb(1, 1), cp_xb(2, 1), cp_xb(3, 3)
    KVQ, KQV = (1, 2, 0), (1, 0, 2)
    cp_w0 = [cp_wb(KQV[0], 0, DM // 4), cp_wb(KQV[0], DM // 4, DM // 4)]
    cp_wp = [None] + [cp_wb(KQV[h // 2], (h % 2) * (DM // 2), DM // 2) for h in range(1, 6)]
    cp_wob = cp(wob_hbm, rawob.at[:, pl.ds(0, DM)])
    cp_xa = cp(xa_hbm, xa)
    cp_m0 = cp(mem0_hbm, _rows(ha, LA, MEM))
    assert nsem[0] == NSEM
    order = cp_w0 + [cp_xb0, cp_xb1] + cp_wp[1:5] + [cp_xb2, cp_wp[5], cp_xb3]
    for c in range(NCH):
        order += cp_ch[2 * c:2 * c + 2] + cp_xbs[c:c + 1] + ([cp_wob] if c == 0 else [])
    order += [cp_worest, cp_m0, cp_xa]
    for c in order:
        c.start()

    def wait_like(dst, s):
        pltpu.make_async_copy(dst, dst, sem.at[s]).wait()

    def a_out_start(r0, n):
        r0 = pl.multiple_of(r0, 8)
        pltpu.make_async_copy(_rows(outa, r0, n), out_hbm.at[pl.ds(r0, n), pl.ds(0, DM)],
                              sem_out.at[0]).start()

    def b_out_start(r0, n):
        pltpu.make_async_copy(_rows(outb, r0, n), out_hbm.at[pl.ds(r0, n), pl.ds(DM, DM)],
                              sem_out.at[1]).start()

    def zeros_vec():
        return jnp.full((8, 128), zero[0], i32).astype(u32)

    def tied(w, zvec, *vals_list):
        n = w.shape[0] // len(vals_list)
        parts = []
        for i, vals in enumerate(vals_list):
            pt = w[i * n:(i + 1) * n]
            if vals:
                tie = functools.reduce(lambda a, b: a | b, [_as_u32(x) for x in vals]) & zvec
                pt = jnp.concatenate([pt[0:n - 8], pt[n - 8:] | tie], axis=0)
            parts.append(pt)
        return jnp.concatenate(parts, axis=0)

    def run(dots, *job_lists, due=None):
        rel = {}
        for jobs, lo, hi, tr in job_lists:
            for i, job in enumerate(jobs):
                rel.setdefault(lo + i * (hi - lo) // len(jobs) - 1, []).append((job, tr))
        due = {} if due is None else due

        def fire(i, y):
            for job, tr in rel.get(i, []):
                vals = job(None if y is None else y[tr:tr + 16])
                if vals:
                    due.setdefault(min(i + 5, len(dots) - 1), []).extend(vals)

        fire(-1, None)
        for i, th in enumerate(dots):
            fire(i, th(due.pop(i, [])))

    def prep_qkv(t, kbs):
        for kb_ in kbs:
            base = (t * 8 + kb_) * BREG
            for ch in range(8):
                at = _as_u32(rawb[t, kb_ * 128:(kb_ + 1) * 128, ch * 128:(ch + 1) * 128].T)
                for pr in range(2):
                    lo, hi = _interleave(at[pr * 32:pr * 32 + 16], at[pr * 32 + 16:pr * 32 + 32])
                    wt[pl.ds(base + ch * 2 + pr, 16, stride=2 * DP), :] = lo
                    wt[pl.ds(base + DP + ch * 2 + pr, 16, stride=2 * DP), :] = hi

    def prep_wo_job(src_col, dst0, hq):
        def job(token):
            rawob[0:16, DM + 128:DM + 256] = token.astype(bf16)
            dst = _rows(wos, dst0, BREG + 40)
            for hp in range(4 * hq, 4 * hq + 4):
                a = _as_u32(rawob[hp * 64:hp * 64 + 32, pl.ds(src_col, 128)])
                b = _as_u32(rawob[hp * 64 + 32:hp * 64 + 64, pl.ds(src_col, 128)])
                lo, hi = _interleave(a, b)
                dst[pl.ds(hp, 16, stride=2 * DP), :] = lo
                dst[pl.ds(DP + hp, 16, stride=2 * DP), :] = hi
        return job

    def repack_job(src0, dst0, half):
        def job(token):
            rawa[pl.ds(RAWA_PAD + RG, 16), :] = token.astype(bf16)
            src = _rows(rawa, src0, RG)
            dst = _rows(wa, dst0, TREG + TPAD)
            for ii in range(half * 4, half * 4 + 4):
                lo, hi = _interleave(_as_u32(src[ii * 64:ii * 64 + 32, :]),
                                     _as_u32(src[ii * 64 + 32:ii * 64 + 64, :]))
                dst[pl.ds(ii, 16, stride=2 * TP), :] = lo
                dst[pl.ds(ii + TP, 16, stride=2 * TP), :] = hi
        return job

    def wocopy_job(src0, dst0):
        def job(token):
            if token is not None:
                rawo[pl.ds(RAWO_PAD + 32, 16), 0:128] = token.astype(bf16)
            v = _as_u32(rawo[pl.ds(src0, 32), :])
            for j in range(8):
                woa[j, pl.ds(dst0, 16), :] = v[:, j * 128:(j + 1) * 128]
        return job

    def chunk_jobs(it):
        c = jnp.maximum(it - 1, 0)
        ja, jo, jw = [], [], []
        for i in range(GPC):
            src0 = pl.multiple_of(jnp.where(it > 0, (c * GPC + i) * RG, RAWA_PAD), RG)
            dst0 = pl.multiple_of((c // 2) * TREG + ((c % 2) * GPC + i) * 8, 8)
            ja += [repack_job(src0, dst0, 0), repack_job(src0, dst0, 1)]
        for i in range(WOR // 32):
            src0 = pl.multiple_of(jnp.where(it > 0, c * WOR + i * 32, RAWO_PAD), 32)
            jo.append(wocopy_job(src0, pl.multiple_of(c * (WOR // 2) + i * 16, 16)))
        for i in range(2):
            j = jnp.clip(2 * (it - 2) + i, 0, 7)
            src_col = pl.multiple_of(jnp.where(it > 1, j * 128, DM), 128)
            jw += [prep_wo_job(src_col, pl.multiple_of(j * BREG, 8), hq) for hq in range(4)]
        half = lambda js, h: js[h * len(js) // 2:(h + 1) * len(js) // 2]
        return [half(ja, h) + half(jo, h) + half(jw, h) for h in range(2)]

    def xcvt(r0, p):
        for i in range(SB // 16):
            xsb[p][i * 8:(i + 1) * 8, :] = _as_u32(xb[pl.ds(pl.multiple_of(r0 + i * 16, 16), 16), :])

    def xcvt_jobs(r0, p):
        def mk(i):
            def job(token):
                xsb[p][i * 8:(i + 1) * 8, :] = _as_u32(xb[pl.ds(pl.multiple_of(r0 + i * 16, 16), 16), :])
            return job
        return [mk(i) for i in range(SB // 16)]

    scale_b = (DM // HB) ** -0.5

    def b_proj_dots(p, ts, half=None):
        kbs = range(8) if half is None else range(4 * half, 4 * half + 4)

        def mk(t, c):
            def th(ties):
                x = _as_bf16(xsb[p][:, kbs[0] * 128:(kbs[-1] + 1) * 128])
                tiles = [jnp.concatenate([wt[pl.ds((t * 8 + kb_) * BREG + (4 * c + dd) * DP, 16), :]
                                          for dd in range(4)], axis=0) for kb_ in kbs]
                if ties:
                    tiles[-1] = tied(tiles[-1], zeros_vec(), ties)
                y = lax.dot_general(x, _as_bf16(jnp.concatenate(tiles, axis=1)), _NT,
                                    preferred_element_type=f32)
                if t == 0:
                    qbuf[p][c] = y + qbuf[p][c] if half == 1 else y
                else:
                    g = kbuf if t == 1 else vbuf
                    if half != 0:
                        g[p][c, 0:HALO, :] = g[1 - p][c, SB:SB + HALO, :]
                    g[p][c, HALO:HALO + SB, :] = y + g[p][c, HALO:HALO + SB, :] if half == 1 else y
                return y
            return th
        return [mk(t, c) for t in ts for c in range(8)]

    def wos_tile(j, d0, d1):
        return _as_bf16(jnp.concatenate([wos[pl.ds(j * BREG + d * DP, 16), :] for d in range(d0, d1)], axis=0))

    def b_out_dots(r0):
        def mk(j):
            def th(ties):
                o = _as_bf16(oball[r0 // 2:(r0 + SB) // 2, :])
                y = jnp.dot(o, wos_tile(j, 0, HB), preferred_element_type=f32)
                outb[pl.ds(r0, SB), j * 128:(j + 1) * 128] = y.astype(bf16)
                return y
            return th
        return [mk(j) for j in range(8)]

    def b_attn_qk(p, rb, first, token):
        gate = None if token is None else _as_u32(token[8:16]) & zeros_vec()
        b0 = rb * RB
        acc = [None] * NW
        for c in range(8):
            q = qbuf[p][c, b0:b0 + RB, :]
            if gate is not None:
                q = pltpu.bitcast(_as_u32(q) | gate, f32)
            for w in range(NW):
                pr = q * kbuf[p][c, pl.ds(HALO + b0 - DIL * w, RB), :]
                acc[w] = pr if acc[w] is None else acc[w] + pr
        lg = []
        for w in range(NW):
            a = acc[w]
            a = a + pltpu.roll(a, 64, 1)
            a = a + pltpu.roll(a, 32, 1)
            a = a * (scale_b * LOG2E)
            if first and b0 < DIL * w:
                row = b0 + lax.broadcasted_iota(i32, (RB, 128), 0)
                a = jnp.where(row >= DIL * w, a, NEG * LOG2E)
            lg.append(a)
        m = functools.reduce(jnp.maximum, lg)
        es = [jnp.exp2(a - m) for a in lg]
        inv = _recip(_sum(es))
        return [e * inv for e in es]

    def b_attn_pv(p, rb, r0, ps):
        b0 = rb * RB
        dst = _rows(oball, pl.multiple_of(r0 // 2, SB // 2), SB // 2)
        outs = []
        for c in range(8):
            o = _sum([ps[w] * vbuf[p][c, pl.ds(HALO + b0 - DIL * w, RB), :] for w in range(NW)])
            dst[pl.ds(b0 // 2, RB // 2), c * 128:(c + 1) * 128] = _as_u32(o.astype(bf16))
            outs.append(o)
        return outs

    def attn_jobs(p, r0):
        def mk(rb):
            return lambda token: b_attn_pv(p, rb, r0, b_attn_qk(p, rb, False, token))
        return [mk(rb) for rb in range(NRB)]

    z8 = pl.multiple_of(zero[0], 8)
    keep = jnp.zeros((8, 128), u32)
    qkvb[0, 0:8, :] = keep
    keep = keep | qkvb[zero[0], 0:8, :]
    for ref in (oca, ocb, obs):
        ref[0:8, 0:128] = jnp.zeros((8, 128), u32)
        keep = keep | ref[pl.ds(z8, 8), 0:128]
    for ref in (ex, df, sv):
        ref[0] = jnp.zeros((8, 128), f32)
        keep = keep | _as_u32(ref[zero[0]])
    part[0:8, 0:128] = jnp.zeros((8, 128), f32)
    keep = keep | _as_u32(part[pl.ds(z8, 8), 0:128])
    outa[0:16, 0:128] = _as_bf16(keep)
    rawa[pl.ds(RAWA_PAD, RG), :] = jnp.zeros((RG, DH), bf16)
    rawo[pl.ds(RAWO_PAD, 32), :] = jnp.zeros((32, DM), bf16)
    rawob[:, DM:DM + 128] = jnp.zeros((DM, 128), bf16)

    def phase_b():
        for i in range(2):
            cp_w0[i].wait()
            prep_qkv(KQV[0], range(2 * i, 2 * i + 2))
        cp_xb0.wait()
        xcvt(0, 0)
        run(b_proj_dots(0, KQV[0:1], 0))
        cp_xb1.wait()
        xcvt(SB, 1)
        NQ4, Q0 = 8, 8
        for h in range(1, 6):
            cp_wp[h].wait()
            if h == 5:
                cp_xb2.wait()
            t0, t1 = KQV[(h - 1) // 2], KQV[h // 2]
            prep_qkv(t1, range(4 * (h % 2), 4 * (h % 2) + 4))
            dots = b_proj_dots(1, (t0,), (h - 1) % 2) + b_proj_dots(0, (t1,), h % 2)
            due = {}
            if h == 4:
                for rb in range(NQ4):
                    ps_ = b_attn_qk(0, rb, True, None)
                    for w in range(NW):
                        qb0[w, rb * RB:(rb + 1) * RB, :] = ps_[w]
                    due.setdefault(Q0 + rb * (16 - Q0) // NQ4, []).extend(ps_)
            if h == 5:
                pss = [[qb0[w, rb * RB:(rb + 1) * RB, :] for w in range(NW)] if rb < NQ4
                       else b_attn_qk(0, rb, True, None) for rb in range(NRB)]
                for rb in range(NQ4, NRB):
                    due.setdefault(Q0 + (rb - NQ4) * (16 - Q0) // (NRB - NQ4), []).extend(pss[rb])
            run(dots, due=due)
            if h == 5:
                vb0[:, 0:HALO, :] = jnp.broadcast_to(vb0[:, HALO:HALO + 1, :], (8, HALO, 128))
                for rb in range(NRB):
                    b_attn_pv(0, rb, 0, pss[rb])
                xcvt(2 * SB, 0)
                run(b_proj_dots(1, (t1,), 1))
        cp_xb3.wait()

        def b_step(p, r_attn, r_next, side):
            run(b_proj_dots(p, KVQ),
                (attn_jobs(1 - p, r_attn), 1, 20, 112),
                (side[0::2], 1, 24, 0), (side[1::2], 1, 24, 48),
                (xcvt_jobs(r_next, 1 - p), 0, 20, 0))

        def b_body(it, carry):
            @pl.when(it == 2)
            def _():
                cp_wob.wait()

            @pl.when(jnp.logical_and(it > 0, it <= 5))
            def _():
                wait_like(_rows(xb, pl.multiple_of((4 + 2 * it) * SB, 2 * SB), 2 * SB), sem_x + it - 1)

            @pl.when(it > 0)
            def _():
                c = it - 1
                wait_like(_rows(rawa, pl.multiple_of(c * (GPC * RG), GPC * RG), GPC * RG), 2 * c)
                wait_like(_rows(rawo, pl.multiple_of(c * WOR, 128), WOR), 2 * c + 1)

            r0 = pl.multiple_of((2 * it + 2) * SB, 2 * SB)
            side = chunk_jobs(it)
            b_step(0, r0 - SB, r0 + SB, side[0])
            b_step(1, r0, jnp.minimum(r0 + 2 * SB, S - SB), side[1])
            return carry

        lax.fori_loop(0, NSTEP // 2 - 1, b_body, 0)
        cp_worest.wait()
        cp_m0.wait()
        cp_xa.wait()
        jo = [wocopy_job(NCH * WOR + i * 32, NCH * WOR // 2 + i * 16) for i in range(WOREST // 32)]
        dots = sum([b_out_dots(r) for r in range(NIT * MB, S, SB)], [])
        run(dots, (attn_jobs(1, S - SB), 0, len(dots) - 11, 112), (jo, 0, 0, 0))

    phase_b()
    b_out_start(NIT * MB, S - NIT * MB)

    scale_a = DH ** -0.5
    qscale = scale_a * LOG2E
    k1 = SPLIT * DH
    sub8 = lax.broadcasted_iota(i32, (8, 128), 0)

    def masks(nv):
        qr = LA - 8 * nv
        r = lax.broadcasted_iota(i32, (2 * qr, 2 * LA), 0)
        c = lax.broadcasted_iota(i32, (2 * qr, 2 * LA), 1)
        same = (r >= qr) == (c >= LA)
        rr = jnp.where(r >= qr, r - qr, r) + 8 * nv
        cc = jnp.where(c >= LA, c - LA, c)
        valid = same & ((cc >= SEG) | (rr >= SEG) | (cc <= rr))
        return valid, jnp.where(same, NEG, -jnp.inf).astype(f32)

    msk = [masks(nv) for nv in NVS]

    def vpu_part(q, k8, v8, causal, prev):
        ss = []
        for j in range(8):
            s_ = jnp.broadcast_to(jnp.sum(q * k8[j:j + 1], axis=-1, keepdims=True), (8, 128))
            if causal and j > 0:
                s_ = jnp.where(sub8 >= j, s_, NEG * LOG2E)
            ss.append(s_)
        m = functools.reduce(jnp.maximum, ss if prev is None else ss + [prev[0]])
        es = [jnp.exp2(s_ - m) for s_ in ss]
        l = _sum(es)
        o = _sum([e * v8[j:j + 1] for j, e in enumerate(es)])
        if prev is not None:
            al = jnp.exp2(prev[0] - m)
            l = l + prev[1] * al
            o = o + prev[2] * al
        return m, l, o

    def segment(which, it, r0, rb0):
        h_ref, oc_ref = (ha, oca) if which == 0 else (hb, ocb)
        nrow_o = 32 if which == 0 else 48
        nv = NVS[which]
        qr = LA - 8 * nv
        valid, fill = msk[which]
        h = h_ref[...]
        zvec = zeros_vec()
        so = (21, 20)[which]
        scp = (10, 13)[which]
        pvp = (21, 24)[which]
        assert pvp + 6 * (SPLIT // 2 - 1) <= 6 * NP
        ov, slots, ps, bacc, pre = {}, {}, {}, [], {}

        def wa_tile(hd, t, k0, kn):
            return wa[pl.ds(t * TREG + hd * TP + k0 // 2, kn // 2), :]

        KH = DM // 2
        if which == 1:
            for hd in range(2):
                for t in range(3):
                    pre[hd, t] = jnp.dot(h[:, :KH], _as_bf16(wa_tile(hd, t, 0, KH)), preferred_element_type=f32)

        def proj(hd, t, ties):
            if (hd, t) in pre:
                y = jnp.dot(h[:, KH:], _as_bf16(wa_tile(hd, t, KH, KH)), preferred_element_type=f32)
                y = y + pre.pop((hd, t))
            else:
                y = jnp.dot(h, _as_bf16(tied(wa_tile(hd, t, 0, DM), zvec, *ties)), preferred_element_type=f32)
            if which == 0:
                ex[t * HA + hd] = y[32:40]
                return jnp.concatenate([y[0:32], y[40:48]], axis=0)
            return jnp.concatenate([ex[t * HA + hd], y[8:32], y[0:8]], axis=0)

        def vpu_jobs(t, ys):
            out = []
            for e in range(2):
                hd = 2 * t + e
                q, k, v = ys[3 * e:3 * e + 3]
                ov[hd] = []
                for g in range(nv):
                    q0 = q[8 * g:8 * g + 8] * qscale
                    if which == 1 and g == 0:
                        st = [sv[i * HA + hd] for i in range(3)]
                    else:
                        st = None
                        for b in range(g, -1, -1):
                            st = vpu_part(q0, k[8 * b:8 * b + 8], v[8 * b:8 * b + 8], b == g, st)
                            out.append(list(st[1:]))
                    _, l, o = vpu_part(q0, k[SEG:LA], v[SEG:LA], False, st)
                    ov[hd].append(o * _recip(l))
                    out.append([ov[hd][-1]])
                if which == 0:
                    st = vpu_part(ex[hd] * qscale, ex[HA + hd], ex[2 * HA + hd], True, None)
                    for i in range(3):
                        sv[i * HA + hd] = st[i]
                    out.append(list(st[1:]))
            for i, jb in enumerate(out):
                slots.setdefault(12 * t + so + (2 * i + 1) * 6 // len(out), []).extend(jb)

        def bout_half(i):
            j, half = i // 2, i % 2
            o = _as_bf16(obs[:, half * KH:(half + 1) * KH])
            y = jnp.dot(o, wos_tile(j, half * 16, half * 16 + 16), preferred_element_type=f32)
            if half == 0:
                bacc.append(y)
            else:
                outb[pl.ds(rb0, MB), j * 128:(j + 1) * 128] = (y + bacc.pop()).astype(bf16)

        def scores(p_):
            if which == 1:
                bout_half(p_)
            q3 = (which * NP + p_) * 3
            sc = lax.dot_general(_as_bf16(qkvb[q3, 0:qr, :]), _as_bf16(qkvb[q3 + 1]), _NT,
                                 preferred_element_type=f32)
            sc = jnp.where(valid, sc * scale_a, fill)
            p = jnp.exp(sc - jnp.max(sc, axis=-1, keepdims=True))
            ps[p_] = (p * _recip(jnp.sum(p, axis=-1, keepdims=True))).astype(bf16)

        def pv(p_):
            o = jnp.dot(ps.pop(p_), _as_bf16(qkvb[(which * NP + p_) * 3 + 2]), preferred_element_type=f32)
            for e in range(2):
                hd = 2 * p_ + e
                oh = jnp.concatenate(ov.pop(hd) + [o[qr * e:qr * e + qr]], axis=0)
                if which == 0:
                    df[hd] = oh[24:32]
                    z = jnp.concatenate([oh[32:40], oh[0:24]], axis=0)
                else:
                    z = jnp.concatenate([oh, df[hd]], axis=0)
                oc_ref[:, hd * DH:(hd + 1) * DH] = _as_u32(z.astype(bf16))

        def after(n):
            for pos, fn in ((pvp, pv), (scp, scores)):
                if (n - pos) % 6 == 0 and 0 <= (n - pos) // 6 < NP:
                    fn((n - pos) // 6)

        for t in range(NP):
            ys = []
            for m in range(6):
                n = 6 * t + m
                ys.append(proj(2 * t + m // 3, m % 3, (slots.pop(2 * n, []), slots.pop(2 * n + 1, []))))
                if m == 5:
                    q3 = (which * NP + t) * 3
                    qkvb[q3, 0:qr, :] = _as_u32(
                        jnp.concatenate([ys[0][8 * nv:], ys[3][8 * nv:]], axis=0).astype(bf16))
                    for i in range(1, 3):
                        qkvb[q3 + i] = _as_u32(jnp.concatenate([ys[i], ys[3 + i]], axis=0).astype(bf16))
                    vpu_jobs(t, ys)
                after(n + 1)
        n = 6 * NP
        for j in range(8):
            ties = [sum([slots.pop(2 * n + i, []) for i in range(lo, lo + 3)], []) for lo in (0, 3)]
            part[0:nrow_o, j * 128:(j + 1) * 128] = jnp.dot(
                _as_bf16(oc_ref[:, :k1]), _as_bf16(tied(woa[j, :k1 // 2, :], zvec, *ties)),
                preferred_element_type=f32)
            for i in range(3):
                n += 1
                after(n)
        assert not (ps or ov or slots or bacc or pre)
        if which == 1:
            @pl.when(it % OG == OG - 1)
            def _():
                b_out_start(pl.multiple_of(rb0 - (OG - 1) * MB, 16), OG * MB)
        o2 = _as_bf16(oc_ref[:, k1:])
        for j in range(8):
            cs = slice(j * 128, (j + 1) * 128)
            y = part[0:nrow_o, cs] + jnp.dot(o2, _as_bf16(woa[j, k1 // 2:, :]), preferred_element_type=f32)
            if which == 0:
                hb[0:8, cs] = y[0:8].astype(bf16)
                outa[pl.ds(r0, 24), cs] = y[8:32].astype(bf16)
            else:
                outa[pl.ds(r0 + 32, 32), cs] = y[0:32].astype(bf16)
                ha[40:48, cs] = y[32:40].astype(bf16)
                outa[pl.ds(r0 + 24, 8), cs] = y[40:48].astype(bf16)

    def a_body(it, carry):
        r0 = pl.multiple_of(it * 64, 64)
        rb0 = pl.multiple_of(it * MB, 16)
        ha[0:40, :] = xa[pl.ds(r0, 40), :]
        hb[8:32, :] = xa[pl.ds(r0 + 40, 24), :]
        obs[...] = oball[pl.ds(pl.multiple_of(it * (MB // 2), 8), MB // 2), :]
        segment(0, it, r0, rb0)

        @pl.when(it == OG - 1)
        def _():
            a_out_start(0, 64 * OG - 40)

        @pl.when(jnp.logical_and(it % OG == OG - 1, it >= OG))
        def _():
            a_out_start(r0 + 24 - 64 * OG, 64 * OG)

        segment(1, it, r0, rb0)
        return carry

    lax.fori_loop(0, NIT, a_body, 0)
    a_out_start(S - 40, 40)

    pltpu.make_async_copy(outb, out_hbm.at[:, pl.ds(DM, DM)], sem_out.at[1]).wait()
    pltpu.make_async_copy(outa, out_hbm.at[:, pl.ds(0, DM)], sem_out.at[0]).wait()


@jax.jit
def pallas_concat_heads__memory_aug_recurrent_mem_tr__sliding_local_dilated__prompt_kernel(
    A_x, A_mem0, A_Wq, A_Wk, A_Wv, A_Wo, A_seg_len, B_x, B_wqkv, B_wo,
):
    del A_seg_len
    assert A_x.shape == (1, S, DM) and B_x.shape == (1, S, DM)
    vm = pltpu.VMEM
    scratch = [
        vm((S, DM), bf16), vm((S, DM), bf16),
        vm((S, DM), bf16), vm((S, DM), bf16),
        vm((RAWA_PAD + RG + 16, DH), bf16),
        vm((RAWO_PAD + 48, DM), bf16),
        vm((3, DM, DM), bf16), vm((DM, DM + 256), bf16),
        vm((3 * TREG + DM // 2 + TPAD, DH), u32),
        vm((8, HA * DH // 2, 128), u32),
        vm((25 * BREG, 128), u32), vm((9 * BREG, 128), u32),
        vm((8, SB, 128), f32), vm((8, SB, 128), f32),
        vm((8, SB + HALO, 128), f32), vm((8, SB + HALO, 128), f32),
        vm((8, SB + HALO, 128), f32), vm((8, SB + HALO, 128), f32),
        vm((SB // 2, DM), u32), vm((SB // 2, DM), u32),
        vm((S // 2, DM), u32), vm((MB // 2, DM), u32),
        vm((48, DM), bf16), vm((32, DM), bf16),
        vm((16, HA * DH), u32), vm((24, HA * DH), u32),
        vm((48, DM), f32),
        vm((3 * HA, 8, 128), f32), vm((HA, 8, 128), f32),
        vm((3 * HA, 8, 128), f32),
        vm((6 * NP, LA, 128), u32),
        pltpu.SMEM((1,), i32),
        pltpu.SemaphoreType.DMA((NSEM,)),
        pltpu.SemaphoreType.DMA((2,)),
    ]
    out = pl.pallas_call(
        _kernel,
        out_shape=jax.ShapeDtypeStruct((S, 2 * DM), bf16),
        in_specs=[pl.BlockSpec(memory_space=pl.ANY)] * 9,
        out_specs=pl.BlockSpec(memory_space=pl.ANY),
        scratch_shapes=scratch,
        compiler_params=pltpu.CompilerParams(
            vmem_limit_bytes=120 * 1024 * 1024,
            disable_bounds_checks=True,
            disable_semaphore_checks=True,
        ),
        name="concat_heads_kernel",
    )(
        A_x.reshape(S, DM), A_mem0.reshape(MEM, DM),
        A_Wq.reshape(DM * HA, DH), A_Wk.reshape(DM * HA, DH), A_Wv.reshape(DM * HA, DH),
        A_Wo.reshape(HA * DH, DM),
        B_x.reshape(S, DM), B_wqkv, B_wo,
    )
    return out.reshape(1, S, 2 * DM)
```

```python
import functools

import jax
import jax.numpy as jnp
from jax import lax
import jax.experimental.pallas as pl
import jax.experimental.pallas.tpu as pltpu

bf16, f32, u32, i32 = jnp.bfloat16, jnp.float32, jnp.uint32, jnp.int32

S, DM = 2048, 1024
HA, DH, MEM, SEG = 32, 128, 8, 32
LA = MEM + SEG
HB, NW, DIL = 32, 8, 2
HALO = 16
NEG = -1000000000.0
LOG2E = 1.4426950408889634

SB = 128
NSTEP = S // SB
RB = 8
NRB = SB // RB
TP = 514
TREG = HA * TP
TPAD = 1032
DP = 18
BREG = HB * DP
NCH = 6
GPC = 3 * (DM // 16) // NCH
RG = 16 * HA
WOR = 640
WOREST = HA * DH - NCH * WOR
RAWA_PAD = 3 * DM * HA
RAWO_PAD = HA * DH
NIT = S // (2 * SEG)
MB = 48
OG = 4
NP = HA // 2
SPLIT = 24
NVS = (2, 1)
NSEM = 32

_NT = (((1,), (1,)), ((), ()))


def _as_bf16(x):
    return pltpu.bitcast(x, bf16)


def _as_u32(x):
    return pltpu.bitcast(x, u32)


def _sum(xs):
    return functools.reduce(lambda a, b: a + b, xs)


def _interleave(a, b):
    lo = (a & jnp.uint32(0xFFFF)) | (b << 16)
    hi = (a >> 16) | (b & jnp.uint32(0xFFFF0000))
    return lo, hi


def _recip(x):
    r = pl.reciprocal(x, approx=True)
    return r * (2.0 - x * r)


def _rows(ref, r0, n):
    return ref.at[pl.ds(r0, n), :]


def _kernel(xa_hbm, mem0_hbm, wq_hbm, wk_hbm, wv_hbm, wo_hbm, xb_hbm, wqkvb_hbm, wob_hbm,
            out_hbm,
            xa, xb, outa, outb, rawa, rawo, rawb, rawob, wa, woa, wt, wos,
            qb0, qb1, kb0, kb1, vb0, vb1, xs0, xs1, oball, obs,
            ha, hb, oca, ocb, part, ex, df, sv, qkvb, zero,
            sem, sem_out):
    zero[0] = 0
    qbuf, kbuf, vbuf, xsb = (qb0, qb1), (kb0, kb1), (vb0, vb1), (xs0, xs1)

    nsem = [0]

    def cp(src, dst):
        c = pltpu.make_async_copy(src, dst, sem.at[nsem[0]])
        nsem[0] += 1
        return c

    def cp_xb(b0, nb):
        return cp(_rows(xb_hbm, b0 * SB, nb * SB), _rows(xb, b0 * SB, nb * SB))

    def cp_wb(t, k0, n):
        return cp(wqkvb_hbm.at[pl.ds(k0, n), pl.ds(t * DM, DM)], rawb.at[t, pl.ds(k0, n), :])

    cp_ch = []
    for c in range(NCH):
        w = (wq_hbm, wk_hbm, wv_hbm)[c // 2]
        cp_ch.append(cp(_rows(w, (c % 2) * GPC * RG, GPC * RG), _rows(rawa, c * GPC * RG, GPC * RG)))
        cp_ch.append(cp(_rows(wo_hbm, c * WOR, WOR), _rows(rawo, c * WOR, WOR)))
    sem_x = nsem[0]
    cp_xbs = [cp_xb(6 + 2 * c, 2) for c in range(5)]
    cp_worest = cp(_rows(wo_hbm, NCH * WOR, WOREST), _rows(rawo, NCH * WOR, WOREST))
    cp_xb0, cp_xb1, cp_xb2, cp_xb3 = cp_xb(0, 1), cp_xb(1, 1), cp_xb(2, 1), cp_xb(3, 3)
    KVQ, KQV = (1, 2, 0), (1, 0, 2)
    cp_w0 = [cp_wb(KQV[0], 0, DM // 4), cp_wb(KQV[0], DM // 4, DM // 4)]
    cp_wp = [None] + [cp_wb(KQV[h // 2], (h % 2) * (DM // 2), DM // 2) for h in range(1, 6)]
    cp_wob = cp(wob_hbm, rawob.at[:, pl.ds(0, DM)])
    cp_xa = cp(xa_hbm, xa)
    cp_m0 = cp(mem0_hbm, _rows(ha, LA, MEM))
    assert nsem[0] == NSEM
    order = cp_w0 + [cp_xb0, cp_xb1] + cp_wp[1:5] + [cp_xb2, cp_wp[5], cp_xb3]
    for c in range(NCH):
        order += cp_ch[2 * c:2 * c + 2] + cp_xbs[c:c + 1] + ([cp_wob] if c == 0 else [])
    order += [cp_worest, cp_m0, cp_xa]
    for c in order:
        c.start()

    def wait_like(dst, s):
        pltpu.make_async_copy(dst, dst, sem.at[s]).wait()

    def a_out_start(r0, n):
        r0 = pl.multiple_of(r0, 8)
        pltpu.make_async_copy(_rows(outa, r0, n), out_hbm.at[pl.ds(r0, n), pl.ds(0, DM)],
                              sem_out.at[0]).start()

    def b_out_start(r0, n):
        pltpu.make_async_copy(_rows(outb, r0, n), out_hbm.at[pl.ds(r0, n), pl.ds(DM, DM)],
                              sem_out.at[1]).start()

    def zeros_vec():
        return jnp.full((8, 128), zero[0], i32).astype(u32)

    def tied(w, zvec, *vals_list):
        n = w.shape[0] // len(vals_list)
        parts = []
        for i, vals in enumerate(vals_list):
            pt = w[i * n:(i + 1) * n]
            if vals:
                tie = functools.reduce(lambda a, b: a | b, [_as_u32(x) for x in vals]) & zvec
                pt = jnp.concatenate([pt[0:n - 8], pt[n - 8:] | tie], axis=0)
            parts.append(pt)
        return jnp.concatenate(parts, axis=0)

    def run(dots, *job_lists, due=None, td=6):
        rel = {}
        for jobs, lo, hi, tr in job_lists:
            for i, job in enumerate(jobs):
                rel.setdefault(lo + i * (hi - lo) // len(jobs) - 1, []).append((job, tr))
        due = {} if due is None else due

        def fire(i, y):
            for job, tr in rel.get(i, []):
                vals = job(None if y is None else y[tr:tr + 16])
                if vals:
                    due.setdefault(min(i + td, len(dots) - 1), []).extend(vals)

        fire(-1, None)
        for i, th in enumerate(dots):
            fire(i, th(due.pop(i, [])))

    def prep_qkv(t, kbs):
        for kb_ in kbs:
            base = (t * 8 + kb_) * BREG
            for ch in range(8):
                at = _as_u32(rawb[t, kb_ * 128:(kb_ + 1) * 128, ch * 128:(ch + 1) * 128].T)
                for pr in range(2):
                    lo, hi = _interleave(at[pr * 32:pr * 32 + 16], at[pr * 32 + 16:pr * 32 + 32])
                    wt[pl.ds(base + ch * 2 + pr, 16, stride=2 * DP), :] = lo
                    wt[pl.ds(base + DP + ch * 2 + pr, 16, stride=2 * DP), :] = hi

    def prep_wo_job(src_col, dst0, hq):
        def job(token):
            rawob[0:16, DM + 128:DM + 256] = token.astype(bf16)
            dst = _rows(wos, dst0, BREG + 40)
            for hp in range(4 * hq, 4 * hq + 4):
                a = _as_u32(rawob[hp * 64:hp * 64 + 32, pl.ds(src_col, 128)])
                b = _as_u32(rawob[hp * 64 + 32:hp * 64 + 64, pl.ds(src_col, 128)])
                lo, hi = _interleave(a, b)
                dst[pl.ds(hp, 16, stride=2 * DP), :] = lo
                dst[pl.ds(DP + hp, 16, stride=2 * DP), :] = hi
        return job

    def repack_job(src0, dst0, half):
        def job(token):
            rawa[pl.ds(RAWA_PAD + RG, 16), :] = token.astype(bf16)
            src = _rows(rawa, src0, RG)
            dst = _rows(wa, dst0, TREG + TPAD)
            for ii in range(half * 4, half * 4 + 4):
                lo, hi = _interleave(_as_u32(src[ii * 64:ii * 64 + 32, :]),
                                     _as_u32(src[ii * 64 + 32:ii * 64 + 64, :]))
                dst[pl.ds(ii, 16, stride=2 * TP), :] = lo
                dst[pl.ds(ii + TP, 16, stride=2 * TP), :] = hi
        return job

    def wocopy_job(src0, dst0):
        def job(token):
            if token is not None:
                rawo[pl.ds(RAWO_PAD + 32, 16), 0:128] = token.astype(bf16)
            v = _as_u32(rawo[pl.ds(src0, 32), :])
            for j in range(8):
                woa[j, pl.ds(dst0, 16), :] = v[:, j * 128:(j + 1) * 128]
        return job

    def chunk_jobs(it):
        c = jnp.maximum(it - 1, 0)
        ja, jo, jw = [], [], []
        for i in range(GPC):
            src0 = pl.multiple_of(jnp.where(it > 0, (c * GPC + i) * RG, RAWA_PAD), RG)
            dst0 = pl.multiple_of((c // 2) * TREG + ((c % 2) * GPC + i) * 8, 8)
            ja += [repack_job(src0, dst0, 0), repack_job(src0, dst0, 1)]
        for i in range(WOR // 32):
            src0 = pl.multiple_of(jnp.where(it > 0, c * WOR + i * 32, RAWO_PAD), 32)
            jo.append(wocopy_job(src0, pl.multiple_of(c * (WOR // 2) + i * 16, 16)))
        for i in range(2):
            j = jnp.clip(2 * (it - 2) + i, 0, 7)
            src_col = pl.multiple_of(jnp.where(it > 1, j * 128, DM), 128)
            jw += [prep_wo_job(src_col, pl.multiple_of(j * BREG, 8), hq) for hq in range(4)]
        half = lambda js, h: js[h * len(js) // 2:(h + 1) * len(js) // 2]
        return [half(ja, h) + half(jo, h) + half(jw, h) for h in range(2)]

    def xcvt(r0, p):
        for i in range(SB // 16):
            xsb[p][i * 8:(i + 1) * 8, :] = _as_u32(xb[pl.ds(pl.multiple_of(r0 + i * 16, 16), 16), :])

    def xcvt_jobs(r0, p):
        def mk(i):
            def job(token):
                xsb[p][i * 8:(i + 1) * 8, :] = _as_u32(xb[pl.ds(pl.multiple_of(r0 + i * 16, 16), 16), :])
            return job
        return [mk(i) for i in range(SB // 16)]

    scale_b = (DM // HB) ** -0.5

    def b_proj_dots(p, ts, half=None):
        kbs = range(8) if half is None else range(4 * half, 4 * half + 4)

        def mk(t, c):
            def th(ties):
                x = _as_bf16(xsb[p][:, kbs[0] * 128:(kbs[-1] + 1) * 128])
                tiles = [jnp.concatenate([wt[pl.ds((t * 8 + kb_) * BREG + (4 * c + dd) * DP, 16), :]
                                          for dd in range(4)], axis=0) for kb_ in kbs]
                if ties:
                    tiles[-1] = tied(tiles[-1], zeros_vec(), ties)
                y = lax.dot_general(x, _as_bf16(jnp.concatenate(tiles, axis=1)), _NT,
                                    preferred_element_type=f32)
                if t == 0:
                    qbuf[p][c] = y + qbuf[p][c] if half == 1 else y
                else:
                    g = kbuf if t == 1 else vbuf
                    if half != 0:
                        g[p][c, 0:HALO, :] = g[1 - p][c, SB:SB + HALO, :]
                    g[p][c, HALO:HALO + SB, :] = y + g[p][c, HALO:HALO + SB, :] if half == 1 else y
                return y
            return th
        return [mk(t, c) for t in ts for c in range(8)]

    def wos_tile(j, d0, d1):
        return _as_bf16(jnp.concatenate([wos[pl.ds(j * BREG + d * DP, 16), :] for d in range(d0, d1)], axis=0))

    def b_out_dots(r0):
        def mk(j):
            def th(ties):
                o = _as_bf16(oball[r0 // 2:(r0 + SB) // 2, :])
                y = jnp.dot(o, wos_tile(j, 0, HB), preferred_element_type=f32)
                outb[pl.ds(r0, SB), j * 128:(j + 1) * 128] = y.astype(bf16)
                return y
            return th
        return [mk(j) for j in range(8)]

    def b_attn_qk(p, rb, first, token):
        gate = None if token is None else _as_u32(token[8:16]) & zeros_vec()
        b0 = rb * RB
        if 1 & 1:
            q = qbuf[p][:, b0:b0 + RB, :]
            if gate is not None:
                q = pltpu.bitcast(pltpu.bitcast(q, u32) | gate[None], f32)
            acc = [jnp.sum(q * kbuf[p][:, pl.ds(HALO + b0 - DIL * w, RB), :], axis=0) for w in range(NW)]
        else:
            acc = [None] * NW
            for c in range(8):
                q = qbuf[p][c, b0:b0 + RB, :]
                if gate is not None:
                    q = pltpu.bitcast(_as_u32(q) | gate, f32)
                for w in range(NW):
                    pr = q * kbuf[p][c, pl.ds(HALO + b0 - DIL * w, RB), :]
                    acc[w] = pr if acc[w] is None else acc[w] + pr
        lg = []
        for w in range(NW):
            a = acc[w]
            a = a + pltpu.roll(a, 64, 1)
            a = a + pltpu.roll(a, 32, 1)
            a = a * (scale_b * LOG2E)
            if first and b0 < DIL * w:
                row = b0 + lax.broadcasted_iota(i32, (RB, 128), 0)
                a = jnp.where(row >= DIL * w, a, NEG * LOG2E)
            lg.append(a)
        m = functools.reduce(jnp.maximum, lg)
        es = [jnp.exp2(a - m) for a in lg]
        inv = _recip(_sum(es))
        return [e * inv for e in es]

    def b_attn_pv(p, rb, r0, ps):
        b0 = rb * RB
        dst = _rows(oball, pl.multiple_of(r0 // 2, SB // 2), SB // 2)
        if 1 & 2:
            o = _sum([ps[w][None] * vbuf[p][:, pl.ds(HALO + b0 - DIL * w, RB), :] for w in range(NW)])
            outs = [o[c] for c in range(8)]
            dst[pl.ds(b0 // 2, RB // 2), :] = _as_u32(jnp.concatenate(outs, axis=1).astype(bf16))
            return outs
        outs = []
        for c in range(8):
            o = _sum([ps[w] * vbuf[p][c, pl.ds(HALO + b0 - DIL * w, RB), :] for w in range(NW)])
            dst[pl.ds(b0 // 2, RB // 2), c * 128:(c + 1) * 128] = _as_u32(o.astype(bf16))
            outs.append(o)
        return outs

    def attn_jobs(p, r0):
        def mk(rb):
            return lambda token: b_attn_pv(p, rb, r0, b_attn_qk(p, rb, False, token))
        return [mk(rb) for rb in range(NRB)]

    z8 = pl.multiple_of(zero[0], 8)
    keep = jnp.zeros((8, 128), u32)
    qkvb[0, 0:8, :] = keep
    keep = keep | qkvb[zero[0], 0:8, :]
    for ref in (oca, ocb, obs):
        ref[0:8, 0:128] = jnp.zeros((8, 128), u32)
        keep = keep | ref[pl.ds(z8, 8), 0:128]
    for ref in (ex, df, sv):
        ref[0] = jnp.zeros((8, 128), f32)
        keep = keep | _as_u32(ref[zero[0]])
    part[0:8, 0:128] = jnp.zeros((8, 128), f32)
    keep = keep | _as_u32(part[pl.ds(z8, 8), 0:128])
    outa[0:16, 0:128] = _as_bf16(keep)
    rawa[pl.ds(RAWA_PAD, RG), :] = jnp.zeros((RG, DH), bf16)
    rawo[pl.ds(RAWO_PAD, 32), :] = jnp.zeros((32, DM), bf16)
    rawob[:, DM:DM + 128] = jnp.zeros((DM, 128), bf16)

    def phase_b():
        for i in range(2):
            cp_w0[i].wait()
            prep_qkv(KQV[0], range(2 * i, 2 * i + 2))
        cp_xb0.wait()
        xcvt(0, 0)
        run(b_proj_dots(0, KQV[0:1], 0))
        cp_xb1.wait()
        xcvt(SB, 1)
        NQ4 = 8
        for h in range(1, 6):
            cp_wp[h].wait()
            if h == 5:
                cp_xb2.wait()
            t0, t1 = KQV[(h - 1) // 2], KQV[h // 2]
            prep_qkv(t1, range(4 * (h % 2), 4 * (h % 2) + 4))
            dots = b_proj_dots(1, (t0,), (h - 1) % 2) + b_proj_dots(0, (t1,), h % 2)
            if h >= 4:
                def qk_job(rb):
                    def job(token):
                        ps_ = b_attn_qk(0, rb, True, token)
                        for w in range(NW):
                            qb0[w, rb * RB:(rb + 1) * RB, :] = ps_[w]
                        return ps_
                    return job
                rbs = range(NQ4) if h == 4 else range(NQ4, NRB)
                run(dots, ([qk_job(rb) for rb in rbs], 4, 12, 112), td=6)
            else:
                run(dots)
            if h == 5:
                vb0[:, 0:HALO, :] = jnp.broadcast_to(vb0[:, HALO:HALO + 1, :], (8, HALO, 128))

                def pv_job(rb):
                    def job(token):
                        ps_ = qb0[:, rb * RB:(rb + 1) * RB, :]
                        if token is not None:
                            gate = _as_u32(token[8:16]) & zeros_vec()
                            ps_ = pltpu.bitcast(pltpu.bitcast(ps_, u32) | gate[None], f32)
                        outs = b_attn_pv(0, rb, 0, [ps_[w] for w in range(NW)])
                        return outs if 0 else None
                    return job
                xcvt(2 * SB, 0)
                pj = [pv_job(rb) for rb in range(NRB)]
                run(b_proj_dots(1, (t1,), 1), (pj[0::2], 0, 7, 48),
                    (pj[1::2], 0, 7, 112), td=3)
        cp_xb3.wait()

        def b_step(p, r_attn, r_next, side):
            run(b_proj_dots(p, KVQ),
                (attn_jobs(1 - p, r_attn), 1, 21, 112),
                (side[0::2], 1, 24, 0), (side[1::2], 1, 24, 48),
                (xcvt_jobs(r_next, 1 - p), 0, 20, 0))

        def b_body(it, carry):
            @pl.when(it == 2)
            def _():
                cp_wob.wait()

            @pl.when(jnp.logical_and(it > 0, it <= 5))
            def _():
                wait_like(_rows(xb, pl.multiple_of((4 + 2 * it) * SB, 2 * SB), 2 * SB), sem_x + it - 1)

            @pl.when(it > 0)
            def _():
                c = it - 1
                wait_like(_rows(rawa, pl.multiple_of(c * (GPC * RG), GPC * RG), GPC * RG), 2 * c)
                wait_like(_rows(rawo, pl.multiple_of(c * WOR, 128), WOR), 2 * c + 1)

            r0 = pl.multiple_of((2 * it + 2) * SB, 2 * SB)
            side = chunk_jobs(it)
            b_step(0, r0 - SB, r0 + SB, side[0])
            b_step(1, r0, jnp.minimum(r0 + 2 * SB, S - SB), side[1])
            return carry

        lax.fori_loop(0, NSTEP // 2 - 1, b_body, 0)
        cp_worest.wait()
        cp_m0.wait()
        cp_xa.wait()
        jo = [wocopy_job(NCH * WOR + i * 32, NCH * WOR // 2 + i * 16) for i in range(WOREST // 32)]
        dots = sum([b_out_dots(r) for r in range(NIT * MB, S, SB)], [])
        run(dots, (attn_jobs(1, S - SB), 0, len(dots) - 11, 112), (jo, 0, 0, 0))

    phase_b()
    b_out_start(NIT * MB, S - NIT * MB)

    scale_a = DH ** -0.5
    qscale = scale_a * LOG2E
    k1 = SPLIT * DH
    sub8 = lax.broadcasted_iota(i32, (8, 128), 0)
    tri = lax.broadcasted_iota(i32, (8, 8, 128), 1) >= lax.broadcasted_iota(i32, (8, 8, 128), 0)

    def masks(nv):
        qr = LA - 8 * nv
        r = lax.broadcasted_iota(i32, (2 * qr, 2 * LA), 0)
        c = lax.broadcasted_iota(i32, (2 * qr, 2 * LA), 1)
        same = (r >= qr) == (c >= LA)
        rr = jnp.where(r >= qr, r - qr, r) + 8 * nv
        cc = jnp.where(c >= LA, c - LA, c)
        valid = same & ((cc >= SEG) | (rr >= SEG) | (cc <= rr))
        return valid, jnp.where(same, NEG, -jnp.inf).astype(f32)

    msk = [masks(nv) for nv in NVS]

    def bc8(a):
        if 2 == 1:
            return a[:, None, :]
        if 2 == 2:
            return jnp.concatenate([jnp.broadcast_to(a[j:j + 1], (8, 128)) for j in range(8)], axis=0).reshape(8, 8, 128)
        return lax.broadcast_in_dim(a, (8, 8, 128), (0, 2))

    def vpu_part(q, k8, v8, causal, prev):
        if 2:
            s_ = jnp.sum(q[None] * bc8(k8), axis=-1, keepdims=True)
            s_ = jnp.broadcast_to(s_, (8, 8, 128))
            if causal:
                s_ = jnp.where(tri, s_, NEG * LOG2E)
            m = jnp.max(s_, axis=0)
            if prev is not None:
                m = jnp.maximum(m, prev[0])
            e = jnp.exp2(s_ - m[None])
            l = jnp.sum(e, axis=0)
            o = jnp.sum(e * bc8(v8), axis=0)
        else:
            ss = []
            for j in range(8):
                s_ = jnp.broadcast_to(jnp.sum(q * k8[j:j + 1], axis=-1, keepdims=True), (8, 128))
                if causal and j > 0:
                    s_ = jnp.where(sub8 >= j, s_, NEG * LOG2E)
                ss.append(s_)
            m = functools.reduce(jnp.maximum, ss if prev is None else ss + [prev[0]])
            es = [jnp.exp2(s_ - m) for s_ in ss]
            l = _sum(es)
            o = _sum([e * v8[j:j + 1] for j, e in enumerate(es)])
        if prev is not None:
            al = jnp.exp2(prev[0] - m)
            l = l + prev[1] * al
            o = o + prev[2] * al
        return m, l, o

    def segment(which, it, r0, rb0):
        h_ref, oc_ref = (ha, oca) if which == 0 else (hb, ocb)
        nrow_o = 32 if which == 0 else 48
        nv = NVS[which]
        qr = LA - 8 * nv
        valid, fill = msk[which]
        h = h_ref[...]
        zvec = zeros_vec()
        so = (19, 18)[which]
        scp = (10, 13)[which]
        pvp = (20, 25)[which]
        assert pvp + 6 * (SPLIT // 2 - 1) <= 6 * NP
        ov, slots, ps, bacc, pre = {}, {}, {}, [], {}

        def wa_tile(hd, t, k0, kn):
            return wa[pl.ds(t * TREG + hd * TP + k0 // 2, kn // 2), :]

        KH = DM // 2
        if which == 1:
            for hd in range(2):
                for t in range(3):
                    pre[hd, t] = jnp.dot(h[:, :KH], _as_bf16(wa_tile(hd, t, 0, KH)), preferred_element_type=f32)

        def proj(hd, t, ties):
            if (hd, t) in pre:
                y = jnp.dot(h[:, KH:], _as_bf16(wa_tile(hd, t, KH, KH)), preferred_element_type=f32)
                y = y + pre.pop((hd, t))
            else:
                y = jnp.dot(h, _as_bf16(tied(wa_tile(hd, t, 0, DM), zvec, *ties)), preferred_element_type=f32)
            if which == 0:
                ex[t * HA + hd] = y[32:40]
                return jnp.concatenate([y[0:32], y[40:48]], axis=0)
            return jnp.concatenate([ex[t * HA + hd], y[8:32], y[0:8]], axis=0)

        def vpu_jobs(t, ys):
            out = []
            for e in range(2):
                hd = 2 * t + e
                q, k, v = ys[3 * e:3 * e + 3]
                ov[hd] = []
                for g in range(nv):
                    q0 = q[8 * g:8 * g + 8] * qscale
                    if which == 1 and g == 0:
                        st = [sv[i * HA + hd] for i in range(3)]
                    else:
                        st = None
                        for b in range(g, -1, -1):
                            st = vpu_part(q0, k[8 * b:8 * b + 8], v[8 * b:8 * b + 8], b == g, st)
                            out.append(list(st[1:]))
                    _, l, o = vpu_part(q0, k[SEG:LA], v[SEG:LA], False, st)
                    ov[hd].append(o * _recip(l))
                    out.append([ov[hd][-1]])
                if which == 0:
                    st = vpu_part(ex[hd] * qscale, ex[HA + hd], ex[2 * HA + hd], True, None)
                    for i in range(3):
                        sv[i * HA + hd] = st[i]
                    out.append(list(st[1:]))
            for i, jb in enumerate(out):
                slots.setdefault(12 * t + so + (2 * i + 1) * 6 // len(out), []).extend(jb)

        def bout_half(i):
            j, half = i // 2, i % 2
            o = _as_bf16(obs[:, half * KH:(half + 1) * KH])
            y = jnp.dot(o, wos_tile(j, half * 16, half * 16 + 16), preferred_element_type=f32)
            if half == 0:
                bacc.append(y)
            else:
                outb[pl.ds(rb0, MB), j * 128:(j + 1) * 128] = (y + bacc.pop()).astype(bf16)

        def scores(p_):
            if which == 1:
                bout_half(p_)
            q3 = (which * NP + p_) * 3
            sc = lax.dot_general(_as_bf16(qkvb[q3, 0:qr, :]), _as_bf16(qkvb[q3 + 1]), _NT,
                                 preferred_element_type=f32)
            sc = jnp.where(valid, sc * scale_a, fill)
            p = jnp.exp(sc - jnp.max(sc, axis=-1, keepdims=True))
            ps[p_] = (p * _recip(jnp.sum(p, axis=-1, keepdims=True))).astype(bf16)

        def pv(p_):
            o = jnp.dot(ps.pop(p_), _as_bf16(qkvb[(which * NP + p_) * 3 + 2]), preferred_element_type=f32)
            for e in range(2):
                hd = 2 * p_ + e
                oh = jnp.concatenate(ov.pop(hd) + [o[qr * e:qr * e + qr]], axis=0)
                if which == 0:
                    df[hd] = oh[24:32]
                    z = jnp.concatenate([oh[32:40], oh[0:24]], axis=0)
                else:
                    z = jnp.concatenate([oh, df[hd]], axis=0)
                oc_ref[:, hd * DH:(hd + 1) * DH] = _as_u32(z.astype(bf16))

        def after(n):
            for pos, fn in ((pvp, pv), (scp, scores)):
                if (n - pos) % 6 == 0 and 0 <= (n - pos) // 6 < NP:
                    fn((n - pos) // 6)

        for t in range(NP):
            ys = []
            for m in range(6):
                n = 6 * t + m
                ys.append(proj(2 * t + m // 3, m % 3, (slots.pop(2 * n, []), slots.pop(2 * n + 1, []))))
                if m == 5:
                    q3 = (which * NP + t) * 3
                    qkvb[q3, 0:qr, :] = _as_u32(
                        jnp.concatenate([ys[0][8 * nv:], ys[3][8 * nv:]], axis=0).astype(bf16))
                    for i in range(1, 3):
                        qkvb[q3 + i] = _as_u32(jnp.concatenate([ys[i], ys[3 + i]], axis=0).astype(bf16))
                    vpu_jobs(t, ys)
                after(n + 1)
        n = 6 * NP
        for j in range(8):
            ties = [sum([slots.pop(2 * n + i, []) for i in range(lo, lo + 3)], []) for lo in (0, 3)]
            part[0:nrow_o, j * 128:(j + 1) * 128] = jnp.dot(
                _as_bf16(oc_ref[:, :k1]), _as_bf16(tied(woa[j, :k1 // 2, :], zvec, *ties)),
                preferred_element_type=f32)
            for i in range(3):
                n += 1
                after(n)
        assert not (ps or ov or slots or bacc or pre)
        if which == 1:
            @pl.when(it % OG == OG - 1)
            def _():
                b_out_start(pl.multiple_of(rb0 - (OG - 1) * MB, 16), OG * MB)
        o2 = _as_bf16(oc_ref[:, k1:])
        for j in range(8):
            cs = slice(j * 128, (j + 1) * 128)
            y = part[0:nrow_o, cs] + jnp.dot(o2, _as_bf16(woa[j, k1 // 2:, :]), preferred_element_type=f32)
            if which == 0:
                hb[0:8, cs] = y[0:8].astype(bf16)
                outa[pl.ds(r0, 24), cs] = y[8:32].astype(bf16)
            else:
                outa[pl.ds(r0 + 32, 32), cs] = y[0:32].astype(bf16)
                ha[40:48, cs] = y[32:40].astype(bf16)
                outa[pl.ds(r0 + 24, 8), cs] = y[40:48].astype(bf16)

    def a_body(it, carry):
        r0 = pl.multiple_of(it * 64, 64)
        rb0 = pl.multiple_of(it * MB, 16)
        ha[0:40, :] = xa[pl.ds(r0, 40), :]
        hb[8:32, :] = xa[pl.ds(r0 + 40, 24), :]
        obs[...] = oball[pl.ds(pl.multiple_of(it * (MB // 2), 8), MB // 2), :]
        segment(0, it, r0, rb0)

        @pl.when(it == OG - 1)
        def _():
            a_out_start(0, 64 * OG - 40)

        @pl.when(jnp.logical_and(it % OG == OG - 1, it >= OG))
        def _():
            a_out_start(r0 + 24 - 64 * OG, 64 * OG)

        segment(1, it, r0, rb0)
        return carry

    lax.fori_loop(0, NIT, a_body, 0)
    a_out_start(S - 40, 40)

    pltpu.make_async_copy(outb, out_hbm.at[:, pl.ds(DM, DM)], sem_out.at[1]).wait()
    pltpu.make_async_copy(outa, out_hbm.at[:, pl.ds(0, DM)], sem_out.at[0]).wait()


@jax.jit
def pallas_concat_heads__memory_aug_recurrent_mem_tr__sliding_local_dilated__prompt_kernel(
    A_x, A_mem0, A_Wq, A_Wk, A_Wv, A_Wo, A_seg_len, B_x, B_wqkv, B_wo,
):
    del A_seg_len
    assert A_x.shape == (1, S, DM) and B_x.shape == (1, S, DM)
    vm = pltpu.VMEM
    scratch = [
        vm((S, DM), bf16), vm((S, DM), bf16),
        vm((S, DM), bf16), vm((S, DM), bf16),
        vm((RAWA_PAD + RG + 16, DH), bf16),
        vm((RAWO_PAD + 48, DM), bf16),
        vm((3, DM, DM), bf16), vm((DM, DM + 256), bf16),
        vm((3 * TREG + DM // 2 + TPAD, DH), u32),
        vm((8, HA * DH // 2, 128), u32),
        vm((25 * BREG, 128), u32), vm((9 * BREG, 128), u32),
        vm((8, SB, 128), f32), vm((8, SB, 128), f32),
        vm((8, SB + HALO, 128), f32), vm((8, SB + HALO, 128), f32),
        vm((8, SB + HALO, 128), f32), vm((8, SB + HALO, 128), f32),
        vm((SB // 2, DM), u32), vm((SB // 2, DM), u32),
        vm((S // 2, DM), u32), vm((MB // 2, DM), u32),
        vm((48, DM), bf16), vm((32, DM), bf16),
        vm((16, HA * DH), u32), vm((24, HA * DH), u32),
        vm((48, DM), f32),
        vm((3 * HA, 8, 128), f32), vm((HA, 8, 128), f32),
        vm((3 * HA, 8, 128), f32),
        vm((6 * NP, LA, 128), u32),
        pltpu.SMEM((1,), i32),
        pltpu.SemaphoreType.DMA((NSEM,)),
        pltpu.SemaphoreType.DMA((2,)),
    ]
    out = pl.pallas_call(
        _kernel,
        out_shape=jax.ShapeDtypeStruct((S, 2 * DM), bf16),
        in_specs=[pl.BlockSpec(memory_space=pl.ANY)] * 9,
        out_specs=pl.BlockSpec(memory_space=pl.ANY),
        scratch_shapes=scratch,
        compiler_params=pltpu.CompilerParams(
            vmem_limit_bytes=120 * 1024 * 1024,
            disable_bounds_checks=True,
            disable_semaphore_checks=True,
        ),
        name="concat_heads_kernel",
    )(
        A_x.reshape(S, DM), A_mem0.reshape(MEM, DM),
        A_Wq.reshape(DM * HA, DH), A_Wk.reshape(DM * HA, DH), A_Wv.reshape(DM * HA, DH),
        A_Wo.reshape(HA * DH, DM),
        B_x.reshape(S, DM), B_wqkv, B_wo,
    )
    return out.reshape(1, S, 2 * DM)
```

```python
import functools

import jax
import jax.numpy as jnp
from jax import lax
import jax.experimental.pallas as pl
import jax.experimental.pallas.tpu as pltpu

bf16, f32, u32, i32 = jnp.bfloat16, jnp.float32, jnp.uint32, jnp.int32

S, DM = 2048, 1024
HA, DH, MEM, SEG = 32, 128, 8, 32
LA = MEM + SEG
HB, NW, DIL = 32, 8, 2
HALO = 16
NEG = -1000000000.0
LOG2E = 1.4426950408889634

SB = 128
NSTEP = S // SB
RB = 8
NRB = SB // RB
TP = 514
TREG = HA * TP
TPAD = 1032
DP = 18
BREG = HB * DP
NCH = 6
GPC = 3 * (DM // 16) // NCH
RG = 16 * HA
WOR = 640
WOREST = HA * DH - NCH * WOR
RAWA_PAD = 3 * DM * HA
RAWO_PAD = HA * DH
NIT = S // (2 * SEG)
MB = 48
OG = 4
NP = HA // 2
SPLIT = 24
NVS = (2, 1)
NSEM = 32

_NT = (((1,), (1,)), ((), ()))


def _as_bf16(x):
    return pltpu.bitcast(x, bf16)


def _as_u32(x):
    return pltpu.bitcast(x, u32)


def _sum(xs):
    return functools.reduce(lambda a, b: a + b, xs)


def _interleave(a, b):
    lo = (a & jnp.uint32(0xFFFF)) | (b << 16)
    hi = (a >> 16) | (b & jnp.uint32(0xFFFF0000))
    return lo, hi


def _recip(x):
    r = pl.reciprocal(x, approx=True)
    return r * (2.0 - x * r)


def _rows(ref, r0, n):
    return ref.at[pl.ds(r0, n), :]


def _kernel(xa_hbm, mem0_hbm, wq_hbm, wk_hbm, wv_hbm, wo_hbm, xb_hbm, wqkvb_hbm, wob_hbm,
            out_hbm,
            xa, xb, outa, outb, rawa, rawo, rawb, rawob, wa, woa, wt, wos,
            qb0, qb1, kb0, kb1, vb0, vb1, xs0, xs1, oball, obs,
            ha, hb, oca, ocb, part, ex, df, sv, qkvb, zero,
            sem, sem_out):
    zero[0] = 0
    qbuf, kbuf, vbuf, xsb = (qb0, qb1), (kb0, kb1), (vb0, vb1), (xs0, xs1)

    nsem = [0]

    def cp(src, dst):
        c = pltpu.make_async_copy(src, dst, sem.at[nsem[0]])
        nsem[0] += 1
        return c

    def cp_xb(b0, nb):
        return cp(_rows(xb_hbm, b0 * SB, nb * SB), _rows(xb, b0 * SB, nb * SB))

    def cp_wb(t, k0, n):
        return cp(wqkvb_hbm.at[pl.ds(k0, n), pl.ds(t * DM, DM)], rawb.at[t, pl.ds(k0, n), :])

    cp_ch = []
    for c in range(NCH):
        w = (wq_hbm, wk_hbm, wv_hbm)[c // 2]
        cp_ch.append(cp(_rows(w, (c % 2) * GPC * RG, GPC * RG), _rows(rawa, c * GPC * RG, GPC * RG)))
        cp_ch.append(cp(_rows(wo_hbm, c * WOR, WOR), _rows(rawo, c * WOR, WOR)))
    sem_x = nsem[0]
    cp_xbs = [cp_xb(6 + 2 * c, 2) for c in range(5)]
    cp_worest = cp(_rows(wo_hbm, NCH * WOR, WOREST), _rows(rawo, NCH * WOR, WOREST))
    cp_xb0, cp_xb1, cp_xb2, cp_xb3 = cp_xb(0, 1), cp_xb(1, 1), cp_xb(2, 1), cp_xb(3, 3)
    KVQ, KQV = (1, 2, 0), (1, 0, 2)
    cp_w0 = [cp_wb(KQV[0], 0, DM // 4), cp_wb(KQV[0], DM // 4, DM // 4)]
    cp_wp = [None] + [cp_wb(KQV[h // 2], (h % 2) * (DM // 2), DM // 2) for h in range(1, 6)]
    cp_wob = cp(wob_hbm, rawob.at[:, pl.ds(0, DM)])
    cp_xa = cp(xa_hbm, _rows(xa, 0, S))
    cp_m0 = cp(mem0_hbm, _rows(ha, LA, MEM))
    assert nsem[0] == NSEM
    order = cp_w0 + [cp_xb0, cp_xb1] + cp_wp[1:5] + [cp_xb2, cp_wp[5], cp_xb3]
    for c in range(NCH):
        order += cp_ch[2 * c:2 * c + 2] + cp_xbs[c:c + 1] + ([cp_wob] if c == 0 else [])
    order += [cp_worest, cp_m0, cp_xa]
    for c in order:
        c.start()

    def wait_like(dst, s):
        pltpu.make_async_copy(dst, dst, sem.at[s]).wait()

    def a_out_start(r0, n):
        r0 = pl.multiple_of(r0, 8)
        pltpu.make_async_copy(_rows(outa, r0, n), out_hbm.at[pl.ds(r0, n), pl.ds(0, DM)],
                              sem_out.at[0]).start()

    def b_out_start(r0, n):
        pltpu.make_async_copy(_rows(outb, r0, n), out_hbm.at[pl.ds(r0, n), pl.ds(DM, DM)],
                              sem_out.at[1]).start()

    def zeros_vec():
        return jnp.full((8, 128), zero[0], i32).astype(u32)

    def tied(w, zvec, *vals_list):
        n = w.shape[0] // len(vals_list)
        parts = []
        for i, vals in enumerate(vals_list):
            pt = w[i * n:(i + 1) * n]
            if vals:
                tie = functools.reduce(lambda a, b: a | b, [_as_u32(x) for x in vals]) & zvec
                pt = jnp.concatenate([pt[0:n - 8], pt[n - 8:] | tie], axis=0)
            parts.append(pt)
        return jnp.concatenate(parts, axis=0)

    def gated(x, token):
        gate = _as_u32(token[8:16]) & zeros_vec()
        return pltpu.bitcast(_as_u32(x) | gate[None], f32)

    def run(dots, *job_lists, td=6):
        rel = {}
        for jobs, lo, hi, tr in job_lists:
            for i, job in enumerate(jobs):
                rel.setdefault(lo + i * (hi - lo) // len(jobs) - 1, []).append((job, tr))
        due = {}

        def fire(i, y):
            for job, tr in rel.get(i, []):
                vals = job(None if y is None else y[tr:tr + 16])
                if vals:
                    due.setdefault(min(i + td, len(dots) - 1), []).extend(vals)

        fire(-1, None)
        for i, th in enumerate(dots):
            fire(i, th(due.pop(i, [])))

    def prep_qkv(t, kbs):
        for kb_ in kbs:
            base = (t * 8 + kb_) * BREG
            for ch in range(8):
                at = _as_u32(rawb[t, kb_ * 128:(kb_ + 1) * 128, ch * 128:(ch + 1) * 128].T)
                for pr in range(2):
                    lo, hi = _interleave(at[pr * 32:pr * 32 + 16], at[pr * 32 + 16:pr * 32 + 32])
                    wt[pl.ds(base + ch * 2 + pr, 16, stride=2 * DP), :] = lo
                    wt[pl.ds(base + DP + ch * 2 + pr, 16, stride=2 * DP), :] = hi

    def prep_wo_job(src_col, dst0, hq):
        def job(token):
            rawob[0:16, DM + 128:DM + 256] = token.astype(bf16)
            dst = _rows(wos, dst0, BREG + 40)
            for hp in range(4 * hq, 4 * hq + 4):
                a = _as_u32(rawob[hp * 64:hp * 64 + 32, pl.ds(src_col, 128)])
                b = _as_u32(rawob[hp * 64 + 32:hp * 64 + 64, pl.ds(src_col, 128)])
                lo, hi = _interleave(a, b)
                dst[pl.ds(hp, 16, stride=2 * DP), :] = lo
                dst[pl.ds(DP + hp, 16, stride=2 * DP), :] = hi
        return job

    def repack_job(src0, dst0, half):
        def job(token):
            rawa[pl.ds(RAWA_PAD + RG, 16), :] = token.astype(bf16)
            src = _rows(rawa, src0, RG)
            dst = _rows(wa, dst0, TREG + TPAD)
            for ii in range(half * 4, half * 4 + 4):
                lo, hi = _interleave(_as_u32(src[ii * 64:ii * 64 + 32, :]),
                                     _as_u32(src[ii * 64 + 32:ii * 64 + 64, :]))
                dst[pl.ds(ii, 16, stride=2 * TP), :] = lo
                dst[pl.ds(ii + TP, 16, stride=2 * TP), :] = hi
        return job

    def wocopy_job(src0, dst0):
        def job(token):
            if token is not None:
                rawo[pl.ds(RAWO_PAD + 32, 16), 0:128] = token.astype(bf16)
            v = _as_u32(rawo[pl.ds(src0, 32), :])
            for j in range(8):
                woa[j, pl.ds(dst0, 16), :] = v[:, j * 128:(j + 1) * 128]
        return job

    def chunk_jobs(it):
        c = jnp.maximum(it - 1, 0)
        ja, jo, jw = [], [], []
        for i in range(GPC):
            src0 = pl.multiple_of(jnp.where(it > 0, (c * GPC + i) * RG, RAWA_PAD), RG)
            dst0 = pl.multiple_of((c // 2) * TREG + ((c % 2) * GPC + i) * 8, 8)
            ja += [repack_job(src0, dst0, 0), repack_job(src0, dst0, 1)]
        for i in range(WOR // 32):
            src0 = pl.multiple_of(jnp.where(it > 0, c * WOR + i * 32, RAWO_PAD), 32)
            jo.append(wocopy_job(src0, pl.multiple_of(c * (WOR // 2) + i * 16, 16)))
        for i in range(2):
            j = jnp.clip(2 * (it - 2) + i, 0, 7)
            src_col = pl.multiple_of(jnp.where(it > 1, j * 128, DM), 128)
            jw += [prep_wo_job(src_col, pl.multiple_of(j * BREG, 8), hq) for hq in range(4)]
        half = lambda js, h: js[h * len(js) // 2:(h + 1) * len(js) // 2]
        return [half(ja, h) + half(jo, h) + half(jw, h) for h in range(2)]

    def xcvt_jobs(r0, p):
        def mk(i):
            def job(token):
                xsb[p][i * 8:(i + 1) * 8, :] = _as_u32(xb[pl.ds(pl.multiple_of(r0 + i * 16, 16), 16), :])
            return job
        return [mk(i) for i in range(SB // 16)]

    def xcvt(r0, p):
        for job in xcvt_jobs(r0, p):
            job(None)

    scale_b = (DM // HB) ** -0.5

    def b_proj_dots(p, ts, half=None):
        kbs = range(8) if half is None else range(4 * half, 4 * half + 4)

        def mk(t, c):
            def th(ties):
                x = _as_bf16(xsb[p][:, kbs[0] * 128:(kbs[-1] + 1) * 128])
                tiles = [jnp.concatenate([wt[pl.ds((t * 8 + kb_) * BREG + (4 * c + dd) * DP, 16), :]
                                          for dd in range(4)], axis=0) for kb_ in kbs]
                if ties:
                    tiles[-1] = tied(tiles[-1], zeros_vec(), ties)
                y = lax.dot_general(x, _as_bf16(jnp.concatenate(tiles, axis=1)), _NT,
                                    preferred_element_type=f32)
                if t == 0:
                    qbuf[p][c] = y + qbuf[p][c] if half == 1 else y
                else:
                    g = kbuf if t == 1 else vbuf
                    if half != 0:
                        g[p][c, 0:HALO, :] = g[1 - p][c, SB:SB + HALO, :]
                    g[p][c, HALO:HALO + SB, :] = y + g[p][c, HALO:HALO + SB, :] if half == 1 else y
                return y
            return th
        return [mk(t, c) for t in ts for c in range(8)]

    def wos_tile(j, d0, d1):
        return _as_bf16(jnp.concatenate([wos[pl.ds(j * BREG + d * DP, 16), :] for d in range(d0, d1)], axis=0))

    def b_out_dots(r0):
        def mk(j):
            def th(ties):
                o = _as_bf16(oball[r0 // 2:(r0 + SB) // 2, :])
                y = jnp.dot(o, wos_tile(j, 0, HB), preferred_element_type=f32)
                outb[pl.ds(r0, SB), j * 128:(j + 1) * 128] = y.astype(bf16)
                return y
            return th
        return [mk(j) for j in range(8)]

    def b_attn_qk(p, rb, first, token):
        b0 = rb * RB
        q = qbuf[p][:, b0:b0 + RB, :]
        if token is not None:
            q = gated(q, token)
        acc = [jnp.sum(q * kbuf[p][:, pl.ds(HALO + b0 - DIL * w, RB), :], axis=0) for w in range(NW)]
        lg = []
        for w in range(NW):
            a = acc[w]
            a = a + pltpu.roll(a, 64, 1)
            a = a + pltpu.roll(a, 32, 1)
            a = a * (scale_b * LOG2E)
            if first and b0 < DIL * w:
                row = b0 + lax.broadcasted_iota(i32, (RB, 128), 0)
                a = jnp.where(row >= DIL * w, a, NEG * LOG2E)
            lg.append(a)
        m = functools.reduce(jnp.maximum, lg)
        es = [jnp.exp2(a - m) for a in lg]
        inv = _recip(_sum(es))
        return [e * inv for e in es]

    def b_attn_pv(p, rb, r0, ps):
        b0 = rb * RB
        dst = _rows(oball, pl.multiple_of(r0 // 2, SB // 2), SB // 2)
        outs = []
        for c in range(8):
            o = _sum([ps[w] * vbuf[p][c, pl.ds(HALO + b0 - DIL * w, RB), :] for w in range(NW)])
            dst[pl.ds(b0 // 2, RB // 2), c * 128:(c + 1) * 128] = _as_u32(o.astype(bf16))
            outs.append(o)
        return outs

    def attn_jobs(p, r0):
        def mk(rb):
            return lambda token: b_attn_pv(p, rb, r0, b_attn_qk(p, rb, False, token))
        return [mk(rb) for rb in range(NRB)]

    z8 = pl.multiple_of(zero[0], 8)
    keep = jnp.zeros((8, 128), u32)
    qkvb[0, 0:8, :] = keep
    keep = keep | qkvb[zero[0], 0:8, :]
    for ref in (oca, ocb, obs):
        ref[0:8, 0:128] = jnp.zeros((8, 128), u32)
        keep = keep | ref[pl.ds(z8, 8), 0:128]
    for ref in (ex, df, sv):
        ref[0] = jnp.zeros((8, 128), f32)
        keep = keep | _as_u32(ref[zero[0]])
    part[0:8, 0:128] = jnp.zeros((8, 128), f32)
    keep = keep | _as_u32(part[pl.ds(z8, 8), 0:128])
    outa[0:16, 0:128] = _as_bf16(keep)
    rawa[pl.ds(RAWA_PAD, RG), :] = jnp.zeros((RG, DH), bf16)
    rawo[pl.ds(RAWO_PAD, 32), :] = jnp.zeros((32, DM), bf16)
    rawob[:, DM:DM + 128] = jnp.zeros((DM, 128), bf16)

    def phase_b():
        for i in range(2):
            cp_w0[i].wait()
            prep_qkv(KQV[0], range(2 * i, 2 * i + 2))
        cp_xb0.wait()
        xcvt(0, 0)
        run(b_proj_dots(0, KQV[0:1], 0))
        cp_xb1.wait()
        xcvt(SB, 1)
        NQ4 = 8
        for h in range(1, 6):
            cp_wp[h].wait()
            if h == 5:
                cp_xb2.wait()
            t0, t1 = KQV[(h - 1) // 2], KQV[h // 2]
            prep_qkv(t1, range(4 * (h % 2), 4 * (h % 2) + 4))
            dots = b_proj_dots(1, (t0,), (h - 1) % 2) + b_proj_dots(0, (t1,), h % 2)
            if h >= 4:
                def qk_job(rb):
                    def job(token):
                        ps_ = b_attn_qk(0, rb, True, token)
                        for w in range(NW):
                            qb0[w, rb * RB:(rb + 1) * RB, :] = ps_[w]
                        return ps_
                    return job
                rbs = range(NQ4) if h == 4 else range(NQ4, NRB)
                run(dots, ([qk_job(rb) for rb in rbs], 4, 12, 112), td=6)
            else:
                run(dots)
            if h == 5:
                vb0[:, 0:HALO, :] = jnp.broadcast_to(vb0[:, HALO:HALO + 1, :], (8, HALO, 128))

                def pv_job(rb):
                    def job(token):
                        ps_ = qb0[:, rb * RB:(rb + 1) * RB, :]
                        if token is not None:
                            ps_ = gated(ps_, token)
                        b_attn_pv(0, rb, 0, [ps_[w] for w in range(NW)])
                    return job
                xcvt(2 * SB, 0)
                pj = [pv_job(rb) for rb in range(NRB)]
                run(b_proj_dots(1, (t1,), 1), (pj[0::2], 0, 7, 48),
                    (pj[1::2], 0, 7, 112))
        cp_xb3.wait()

        def b_step(p, r_attn, r_next, side):
            run(b_proj_dots(p, KVQ),
                (attn_jobs(1 - p, r_attn), 1, 21, 112),
                (side[0::2], 1, 24, 0), (side[1::2], 1, 24, 48),
                (xcvt_jobs(r_next, 1 - p), 0, 20, 0))

        def b_body(it, carry):
            @pl.when(it == 2)
            def _():
                cp_wob.wait()

            @pl.when(jnp.logical_and(it > 0, it <= 5))
            def _():
                wait_like(_rows(xb, pl.multiple_of((4 + 2 * it) * SB, 2 * SB), 2 * SB), sem_x + it - 1)

            @pl.when(it > 0)
            def _():
                c = it - 1
                wait_like(_rows(rawa, pl.multiple_of(c * (GPC * RG), GPC * RG), GPC * RG), 2 * c)
                wait_like(_rows(rawo, pl.multiple_of(c * WOR, 128), WOR), 2 * c + 1)

            r0 = pl.multiple_of((2 * it + 2) * SB, 2 * SB)
            side = chunk_jobs(it)
            b_step(0, r0 - SB, r0 + SB, side[0])
            b_step(1, r0, jnp.minimum(r0 + 2 * SB, S - SB), side[1])
            return carry

        lax.fori_loop(0, NSTEP // 2 - 1, b_body, 0)
        cp_worest.wait()
        cp_m0.wait()
        cp_xa.wait()
        jo = [wocopy_job(NCH * WOR + i * 32, NCH * WOR // 2 + i * 16) for i in range(WOREST // 32)]
        dots = sum([b_out_dots(r) for r in range(NIT * MB, S, SB)], [])
        run(dots, (attn_jobs(1, S - SB), 0, len(dots) - 11, 112), (jo, 0, 0, 0))

    phase_b()
    b_out_start(NIT * MB, S - NIT * MB)

    scale_a = DH ** -0.5
    qscale = scale_a * LOG2E
    k1 = SPLIT * DH
    tri = lax.broadcasted_iota(i32, (8, 8, 128), 1) >= lax.broadcasted_iota(i32, (8, 8, 128), 0)

    def masks(nv):
        qr = LA - 8 * nv
        r = lax.broadcasted_iota(i32, (2 * qr, 2 * LA), 0)
        c = lax.broadcasted_iota(i32, (2 * qr, 2 * LA), 1)
        same = (r >= qr) == (c >= LA)
        rr = jnp.where(r >= qr, r - qr, r) + 8 * nv
        cc = jnp.where(c >= LA, c - LA, c)
        valid = same & ((cc >= SEG) | (rr >= SEG) | (cc <= rr))
        return valid, jnp.where(same, NEG, -jnp.inf).astype(f32)

    msk = [masks(nv) for nv in NVS]

    def bc8(a):
        return jnp.concatenate([jnp.broadcast_to(a[j:j + 1], (8, 128)) for j in range(8)],
                               axis=0).reshape(8, 8, 128)

    def vpu_part(q, k8, v8, causal, prev):
        s_ = jnp.broadcast_to(jnp.sum(q[None] * bc8(k8), axis=-1, keepdims=True), (8, 8, 128))
        if causal:
            s_ = jnp.where(tri, s_, NEG * LOG2E)
        m = jnp.max(s_, axis=0)
        if prev is not None:
            m = jnp.maximum(m, prev[0])
        e = jnp.exp2(s_ - m[None])
        l = jnp.sum(e, axis=0)
        o = jnp.sum(e * bc8(v8), axis=0)
        if prev is not None:
            al = jnp.exp2(prev[0] - m)
            l = l + prev[1] * al
            o = o + prev[2] * al
        return m, l, o

    def stage(it):
        r0 = pl.multiple_of(it * 64, 64)
        ha[0:40, :] = xa[pl.ds(r0, 40), :]
        hb[8:32, :] = xa[pl.ds(r0 + 40, 24), :]
        obs[...] = oball[pl.ds(pl.multiple_of(it * (MB // 2), 8), MB // 2), :]

    def segment(which, it, r0, rb0):
        h_ref, oc_ref = (ha, oca) if which == 0 else (hb, ocb)
        nrow_o = 32 if which == 0 else 48
        nv = NVS[which]
        qr = LA - 8 * nv
        valid, fill = msk[which]
        h = h_ref[...]
        zvec = zeros_vec()
        so = (19, 18)[which]
        scp = (10, 13)[which]
        pvp = (20, 25)[which]
        assert pvp + 6 * (SPLIT // 2 - 1) <= 6 * NP
        ov, slots, ps, bacc, pre = {}, {}, {}, [], {}

        def wa_tile(hd, t, k0, kn):
            return wa[pl.ds(t * TREG + hd * TP + k0 // 2, kn // 2), :]

        KH = DM // 2
        if which == 1:
            for hd in range(2):
                for t in range(3):
                    pre[hd, t] = jnp.dot(h[:, :KH], _as_bf16(wa_tile(hd, t, 0, KH)), preferred_element_type=f32)

        def proj(hd, t, ties):
            if (hd, t) in pre:
                y = jnp.dot(h[:, KH:], _as_bf16(wa_tile(hd, t, KH, KH)), preferred_element_type=f32)
                y = y + pre.pop((hd, t))
            else:
                y = jnp.dot(h, _as_bf16(tied(wa_tile(hd, t, 0, DM), zvec, *ties)), preferred_element_type=f32)
            if which == 0:
                ex[t * HA + hd] = y[32:40]
                return jnp.concatenate([y[0:32], y[40:48]], axis=0)
            return jnp.concatenate([ex[t * HA + hd], y[8:32], y[0:8]], axis=0)

        def vpu_jobs(t, ys):
            out = []
            for e in range(2):
                hd = 2 * t + e
                q, k, v = ys[3 * e:3 * e + 3]
                ov[hd] = []
                for g in range(nv):
                    q0 = q[8 * g:8 * g + 8] * qscale
                    if which == 1 and g == 0:
                        st = [sv[i * HA + hd] for i in range(3)]
                    else:
                        st = None
                        for b in range(g, -1, -1):
                            st = vpu_part(q0, k[8 * b:8 * b + 8], v[8 * b:8 * b + 8], b == g, st)
                            out.append(list(st[1:]))
                    _, l, o = vpu_part(q0, k[SEG:LA], v[SEG:LA], False, st)
                    ov[hd].append(o * _recip(l))
                    out.append([ov[hd][-1]])
                if which == 0:
                    st = vpu_part(ex[hd] * qscale, ex[HA + hd], ex[2 * HA + hd], True, None)
                    for i in range(3):
                        sv[i * HA + hd] = st[i]
                    out.append(list(st[1:]))
            for i, jb in enumerate(out):
                slots.setdefault(12 * t + so + (2 * i + 1) * 6 // len(out), []).extend(jb)

        def bout_half(i):
            j, half = i // 2, i % 2
            o = _as_bf16(obs[:, half * KH:(half + 1) * KH])
            y = jnp.dot(o, wos_tile(j, half * 16, half * 16 + 16), preferred_element_type=f32)
            if half == 0:
                bacc.append(y)
            else:
                outb[pl.ds(rb0, MB), j * 128:(j + 1) * 128] = (y + bacc.pop()).astype(bf16)

        def scores(p_):
            if which == 1:
                bout_half(p_)
            q3 = (which * NP + p_) * 3
            sc = lax.dot_general(_as_bf16(qkvb[q3, 0:qr, :]), _as_bf16(qkvb[q3 + 1]), _NT,
                                 preferred_element_type=f32)
            sc = jnp.where(valid, sc * scale_a, fill)
            p = jnp.exp(sc - jnp.max(sc, axis=-1, keepdims=True))
            ps[p_] = (p * _recip(jnp.sum(p, axis=-1, keepdims=True))).astype(bf16)

        def pv(p_):
            o = jnp.dot(ps.pop(p_), _as_bf16(qkvb[(which * NP + p_) * 3 + 2]), preferred_element_type=f32)
            for e in range(2):
                hd = 2 * p_ + e
                oh = jnp.concatenate(ov.pop(hd) + [o[qr * e:qr * e + qr]], axis=0)
                if which == 0:
                    df[hd] = oh[24:32]
                    z = jnp.concatenate([oh[32:40], oh[0:24]], axis=0)
                else:
                    z = jnp.concatenate([oh, df[hd]], axis=0)
                oc_ref[:, hd * DH:(hd + 1) * DH] = _as_u32(z.astype(bf16))

        def after(n):
            for pos, fn in ((pvp, pv), (scp, scores)):
                if (n - pos) % 6 == 0 and 0 <= (n - pos) // 6 < NP:
                    fn((n - pos) // 6)

        for t in range(NP):
            ys = []
            for m in range(6):
                n = 6 * t + m
                ys.append(proj(2 * t + m // 3, m % 3, (slots.pop(2 * n, []), slots.pop(2 * n + 1, []))))
                if m == 5:
                    q3 = (which * NP + t) * 3
                    qkvb[q3, 0:qr, :] = _as_u32(
                        jnp.concatenate([ys[0][8 * nv:], ys[3][8 * nv:]], axis=0).astype(bf16))
                    for i in range(1, 3):
                        qkvb[q3 + i] = _as_u32(jnp.concatenate([ys[i], ys[3 + i]], axis=0).astype(bf16))
                    vpu_jobs(t, ys)
                after(n + 1)
        n = 6 * NP
        for j in range(8):
            ties = [sum([slots.pop(2 * n + i, []) for i in range(lo, lo + 3)], []) for lo in (0, 3)]
            part[0:nrow_o, j * 128:(j + 1) * 128] = jnp.dot(
                _as_bf16(oc_ref[:, :k1]), _as_bf16(tied(woa[j, :k1 // 2, :], zvec, *ties)),
                preferred_element_type=f32)
            for i in range(3):
                n += 1
                after(n)
        assert not (ps or ov or slots or bacc or pre)
        if which == 1:
            @pl.when(it % OG == OG - 1)
            def _():
                b_out_start(pl.multiple_of(rb0 - (OG - 1) * MB, 16), OG * MB)
        o2 = _as_bf16(oc_ref[:, k1:])
        for j in range(8):
            cs = slice(j * 128, (j + 1) * 128)
            y = part[0:nrow_o, cs] + jnp.dot(o2, _as_bf16(woa[j, k1 // 2:, :]), preferred_element_type=f32)
            if which == 0:
                hb[0:8, cs] = y[0:8].astype(bf16)
                outa[pl.ds(r0, 24), cs] = y[8:32].astype(bf16)
            else:
                outa[pl.ds(r0 + 32, 32), cs] = y[0:32].astype(bf16)
                ha[40:48, cs] = y[32:40].astype(bf16)
                outa[pl.ds(r0 + 24, 8), cs] = y[40:48].astype(bf16)
                if j == 6:
                    xa[S:S + 16, 0:128] = y[0:16].astype(bf16)
                    oball[S // 2:S // 2 + 8, 0:128] = _as_u32(y[0:8])
                    stage(jnp.minimum(it + 1, NIT - 1))

    def a_body(it, carry):
        r0 = pl.multiple_of(it * 64, 64)
        rb0 = pl.multiple_of(it * MB, 16)
        segment(0, it, r0, rb0)

        @pl.when(it == OG - 1)
        def _():
            a_out_start(0, 64 * OG - 40)

        @pl.when(jnp.logical_and(it % OG == OG - 1, it >= OG))
        def _():
            a_out_start(r0 + 24 - 64 * OG, 64 * OG)

        segment(1, it, r0, rb0)
        return carry

    stage(0)
    lax.fori_loop(0, NIT, a_body, 0)
    a_out_start(S - 40, 40)

    pltpu.make_async_copy(outb, out_hbm.at[:, pl.ds(DM, DM)], sem_out.at[1]).wait()
    pltpu.make_async_copy(outa, out_hbm.at[:, pl.ds(0, DM)], sem_out.at[0]).wait()


@jax.jit
def pallas_concat_heads__memory_aug_recurrent_mem_tr__sliding_local_dilated__prompt_kernel(
    A_x, A_mem0, A_Wq, A_Wk, A_Wv, A_Wo, A_seg_len, B_x, B_wqkv, B_wo,
):
    del A_seg_len
    assert A_x.shape == (1, S, DM) and B_x.shape == (1, S, DM)
    vm = pltpu.VMEM
    scratch = [
        vm((S + 16, DM), bf16), vm((S, DM), bf16),
        vm((S, DM), bf16), vm((S, DM), bf16),
        vm((RAWA_PAD + RG + 16, DH), bf16),
        vm((RAWO_PAD + 48, DM), bf16),
        vm((3, DM, DM), bf16), vm((DM, DM + 256), bf16),
        vm((3 * TREG + DM // 2 + TPAD, DH), u32),
        vm((8, HA * DH // 2, 128), u32),
        vm((25 * BREG, 128), u32), vm((9 * BREG, 128), u32),
        vm((8, SB, 128), f32), vm((8, SB, 128), f32),
        vm((8, SB + HALO, 128), f32), vm((8, SB + HALO, 128), f32),
        vm((8, SB + HALO, 128), f32), vm((8, SB + HALO, 128), f32),
        vm((SB // 2, DM), u32), vm((SB // 2, DM), u32),
        vm((S // 2 + 8, DM), u32), vm((MB // 2, DM), u32),
        vm((48, DM), bf16), vm((32, DM), bf16),
        vm((16, HA * DH), u32), vm((24, HA * DH), u32),
        vm((48, DM), f32),
        vm((3 * HA, 8, 128), f32), vm((HA, 8, 128), f32),
        vm((3 * HA, 8, 128), f32),
        vm((6 * NP, LA, 128), u32),
        pltpu.SMEM((1,), i32),
        pltpu.SemaphoreType.DMA((NSEM,)),
        pltpu.SemaphoreType.DMA((2,)),
    ]
    out = pl.pallas_call(
        _kernel,
        out_shape=jax.ShapeDtypeStruct((S, 2 * DM), bf16),
        in_specs=[pl.BlockSpec(memory_space=pl.ANY)] * 9,
        out_specs=pl.BlockSpec(memory_space=pl.ANY),
        scratch_shapes=scratch,
        compiler_params=pltpu.CompilerParams(
            vmem_limit_bytes=120 * 1024 * 1024,
            disable_bounds_checks=True,
            disable_semaphore_checks=True,
        ),
        name="concat_heads_kernel",
    )(
        A_x.reshape(S, DM), A_mem0.reshape(MEM, DM),
        A_Wq.reshape(DM * HA, DH), A_Wk.reshape(DM * HA, DH), A_Wv.reshape(DM * HA, DH),
        A_Wo.reshape(HA * DH, DM),
        B_x.reshape(S, DM), B_wqkv, B_wo,
    )
    return out.reshape(1, S, 2 * DM)
```

```python
import functools

import jax
import jax.numpy as jnp
from jax import lax
import jax.experimental.pallas as pl
import jax.experimental.pallas.tpu as pltpu

bf16, f32, u32, i32 = jnp.bfloat16, jnp.float32, jnp.uint32, jnp.int32

S, DM = 2048, 1024
HA, DH, MEM, SEG = 32, 128, 8, 32
LA = MEM + SEG
HB, NW, DIL = 32, 8, 2
HALO = 16
NEG = -1000000000.0
LOG2E = 1.4426950408889634

SB = 128
NSTEP = S // SB
RB = 8
NRB = SB // RB
TP = 514
TREG = HA * TP
TPAD = 1032
DP = 18
BREG = HB * DP
NCH = 6
GPC = 3 * (DM // 16) // NCH
RG = 16 * HA
WOR = 640
WOREST = HA * DH - NCH * WOR
RAWA_PAD = 3 * DM * HA
RAWO_PAD = HA * DH
NIT = S // (2 * SEG)
MB = 48
OG = 4
NP = HA // 2
SPLIT = 24
NVS = (2, 1)
NSEM = 32

_NT = (((1,), (1,)), ((), ()))


def _as_bf16(x):
    return pltpu.bitcast(x, bf16)


def _as_u32(x):
    return pltpu.bitcast(x, u32)


def _sum(xs):
    return functools.reduce(lambda a, b: a + b, xs)


def _interleave(a, b):
    lo = (a & jnp.uint32(0xFFFF)) | (b << 16)
    hi = (a >> 16) | (b & jnp.uint32(0xFFFF0000))
    return lo, hi


def _recip(x):
    r = pl.reciprocal(x, approx=True)
    return r * (2.0 - x * r)


def _rows(ref, r0, n):
    return ref.at[pl.ds(r0, n), :]


def _kernel(xa_hbm, mem0_hbm, wq_hbm, wk_hbm, wv_hbm, wo_hbm, xb_hbm, wqkvb_hbm, wob_hbm,
            out_hbm,
            xa, xb, outa, outb, rawa, rawo, rawb, rawob, wa, woa, wt, wos,
            qb0, qb1, kb0, kb1, vb0, vb1, xs0, xs1, oball, obs,
            ha, hb, oca, ocb, part, ex, df, sv, qkvb, zero,
            sem, sem_out):
    zero[0] = 0
    qbuf, kbuf, vbuf, xsb = (qb0, qb1), (kb0, kb1), (vb0, vb1), (xs0, xs1)

    nsem = [0]

    def cp(src, dst):
        c = pltpu.make_async_copy(src, dst, sem.at[nsem[0]])
        nsem[0] += 1
        return c

    def cp_xb(b0, nb):
        return cp(_rows(xb_hbm, b0 * SB, nb * SB), _rows(xb, b0 * SB, nb * SB))

    def cp_wb(t, k0, n):
        return cp(wqkvb_hbm.at[pl.ds(k0, n), pl.ds(t * DM, DM)], rawb.at[t, pl.ds(k0, n), :])

    cp_ch = []
    for c in range(NCH):
        w = (wq_hbm, wk_hbm, wv_hbm)[c // 2]
        cp_ch.append(cp(_rows(w, (c % 2) * GPC * RG, GPC * RG), _rows(rawa, c * GPC * RG, GPC * RG)))
        cp_ch.append(cp(_rows(wo_hbm, c * WOR, WOR), _rows(rawo, c * WOR, WOR)))
    sem_x = nsem[0]
    cp_xbs = [cp_xb(6 + 2 * c, 2) for c in range(5)]
    cp_worest = cp(_rows(wo_hbm, NCH * WOR, WOREST), _rows(rawo, NCH * WOR, WOREST))
    cp_xb0, cp_xb1, cp_xb2, cp_xb3 = cp_xb(0, 1), cp_xb(1, 1), cp_xb(2, 1), cp_xb(3, 3)
    KVQ, KQV = (1, 2, 0), (1, 0, 2)
    cp_w0 = [cp_wb(KQV[0], 0, DM // 4), cp_wb(KQV[0], DM // 4, DM // 4)]
    cp_wp = [None] + [cp_wb(KQV[h // 2], (h % 2) * (DM // 2), DM // 2) for h in range(1, 6)]
    cp_wob = cp(wob_hbm, rawob.at[:, pl.ds(0, DM)])
    cp_xa = cp(xa_hbm, _rows(xa, 0, S))
    cp_m0 = cp(mem0_hbm, _rows(ha, LA, MEM))
    assert nsem[0] == NSEM
    order = cp_w0 + [cp_xb0, cp_xb1] + cp_wp[1:5] + [cp_xb2, cp_wp[5], cp_xb3]
    for c in range(NCH):
        order += cp_ch[2 * c:2 * c + 2] + cp_xbs[c:c + 1] + ([cp_wob] if c == 0 else [])
    order += [cp_worest, cp_m0, cp_xa]
    for c in order:
        c.start()

    def wait_like(dst, s):
        pltpu.make_async_copy(dst, dst, sem.at[s]).wait()

    def a_out_start(r0, n):
        r0 = pl.multiple_of(r0, 8)
        pltpu.make_async_copy(_rows(outa, r0, n), out_hbm.at[pl.ds(r0, n), pl.ds(0, DM)],
                              sem_out.at[0]).start()

    def b_out_start(r0, n):
        pltpu.make_async_copy(_rows(outb, r0, n), out_hbm.at[pl.ds(r0, n), pl.ds(DM, DM)],
                              sem_out.at[1]).start()

    def zeros_vec():
        return jnp.full((8, 128), zero[0], i32).astype(u32)

    def tied(w, zvec, *vals_list):
        n = w.shape[0] // len(vals_list)
        parts = []
        for i, vals in enumerate(vals_list):
            pt = w[i * n:(i + 1) * n]
            if vals:
                tie = functools.reduce(lambda a, b: a | b, [_as_u32(x) for x in vals]) & zvec
                pt = jnp.concatenate([pt[0:n - 8], pt[n - 8:] | tie], axis=0)
            parts.append(pt)
        return jnp.concatenate(parts, axis=0)

    def gated(x, token):
        gate = _as_u32(token[8:16]) & zeros_vec()
        return pltpu.bitcast(_as_u32(x) | gate[None], f32)

    def run(dots, *job_lists, td=6):
        rel = {}
        for jobs, lo, hi, tr in job_lists:
            for i, job in enumerate(jobs):
                rel.setdefault(lo + i * (hi - lo) // len(jobs) - 1, []).append((job, tr))
        due = {}

        def fire(i, y):
            for job, tr in rel.get(i, []):
                vals = job(None if y is None else y[tr:tr + 16])
                if vals:
                    due.setdefault(min(i + td, len(dots) - 1), []).extend(vals)

        fire(-1, None)
        for i, th in enumerate(dots):
            fire(i, th(due.pop(i, [])))

    def prep_qkv(t, kbs):
        for kb_ in kbs:
            for ch in range(8):
                at = _as_u32(rawb[t, kb_ * 128:(kb_ + 1) * 128, ch * 128:(ch + 1) * 128].T)
                for pr in range(2):
                    lo, hi = _interleave(at[pr * 32:pr * 32 + 16], at[pr * 32 + 16:pr * 32 + 32])
                    wt[t * 8 + kb_, pl.ds(ch * 2 + pr, 16, stride=2 * DP), :] = lo
                    wt[t * 8 + kb_, pl.ds(DP + ch * 2 + pr, 16, stride=2 * DP), :] = hi

    def prep_wo_job(src_col, j, hq):
        def job(token):
            rawob[0:16, DM + 128:DM + 256] = token.astype(bf16)
            dst = wos.at[j]
            for hp in range(4 * hq, 4 * hq + 4):
                src = _as_u32(rawob[hp * 64:(hp + 1) * 64, pl.ds(src_col, 128)])
                lo, hi = _interleave(src[0:16], src[16:32])
                dst[pl.ds(hp, 16, stride=2 * DP), :] = lo
                dst[pl.ds(DP + hp, 16, stride=2 * DP), :] = hi
        return job

    def repack_job(src0, dst0, half):
        def job(token):
            rawa[pl.ds(RAWA_PAD + RG, 16), :] = token.astype(bf16)
            dst = _rows(wa, dst0, TREG + TPAD)
            for ii in range(half * 4, half * 4 + 4):
                src = _as_u32(_rows(rawa, src0, RG)[ii * 64:(ii + 1) * 64, :])
                lo, hi = _interleave(src[0:16], src[16:32])
                dst[pl.ds(ii, 16, stride=2 * TP), :] = lo
                dst[pl.ds(ii + TP, 16, stride=2 * TP), :] = hi
        return job

    def wocopy_job(src0, dst0):
        def job(token):
            if token is not None:
                rawo[pl.ds(RAWO_PAD + 32, 16), 0:128] = token.astype(bf16)
            v = _as_u32(rawo[pl.ds(src0, 32), :])
            woa[:, pl.ds(dst0, 16), :] = jnp.stack([v[:, j * 128:(j + 1) * 128] for j in range(8)])
        return job

    def chunk_jobs(it):
        c = jnp.maximum(it - 1, 0)
        ja, jo, jw = [], [], []
        for i in range(GPC):
            src0 = pl.multiple_of(jnp.where(it > 0, (c * GPC + i) * RG, RAWA_PAD), RG)
            dst0 = pl.multiple_of((c // 2) * TREG + ((c % 2) * GPC + i) * 8, 8)
            ja += [repack_job(src0, dst0, 0), repack_job(src0, dst0, 1)]
        for i in range(WOR // 32):
            src0 = pl.multiple_of(jnp.where(it > 0, c * WOR + i * 32, RAWO_PAD), 32)
            jo.append(wocopy_job(src0, pl.multiple_of(c * (WOR // 2) + i * 16, 16)))
        for i in range(2):
            j = jnp.clip(2 * (it - 2) + i, 0, 7)
            src_col = pl.multiple_of(jnp.where(it > 1, j * 128, DM), 128)
            jw += [prep_wo_job(src_col, j, hq) for hq in range(4)]
        half = lambda js, h: js[h * len(js) // 2:(h + 1) * len(js) // 2]
        return [half(ja, h) + half(jo, h) + half(jw, h) for h in range(2)]

    def xcvt_jobs(r0, p):
        def mk(i):
            def job(token):
                xsb[p][i * 8:(i + 1) * 8, :] = _as_u32(xb[pl.ds(pl.multiple_of(r0 + i * 16, 16), 16), :])
            return job
        return [mk(i) for i in range(SB // 16)]

    def xcvt(r0, p):
        for job in xcvt_jobs(r0, p):
            job(None)

    scale_b = (DM // HB) ** -0.5

    def b_proj_dots(p, ts, half=None):
        kbs = range(8) if half is None else range(4 * half, 4 * half + 4)

        def mk(t, c):
            def th(ties):
                x = _as_bf16(xsb[p][:, kbs[0] * 128:(kbs[-1] + 1) * 128])
                wv = jnp.concatenate([wt[t * 8 + kbs[0]:t * 8 + kbs[-1] + 1, pl.ds((4 * c + dd) * DP, 16), :]
                                      for dd in range(4)], axis=1)
                tiles = [wv[i] for i in range(len(kbs))]
                if ties:
                    tiles[-1] = tied(tiles[-1], zeros_vec(), ties)
                y = lax.dot_general(x, _as_bf16(jnp.concatenate(tiles, axis=1)), _NT,
                                    preferred_element_type=f32)
                if t == 0:
                    qbuf[p][c] = y + qbuf[p][c] if half == 1 else y
                else:
                    g = kbuf if t == 1 else vbuf
                    if half != 0:
                        g[p][c, 0:HALO, :] = g[1 - p][c, SB:SB + HALO, :]
                    g[p][c, HALO:HALO + SB, :] = y + g[p][c, HALO:HALO + SB, :] if half == 1 else y
                return y
            return th
        return [mk(t, c) for t in ts for c in range(8)]

    def wos_all():
        return jnp.concatenate([wos[:, pl.ds(d * DP, 16), :] for d in range(HB)], axis=1)

    def b_out_dots(r0):
        w = []

        def mk(j):
            def th(ties):
                if not w:
                    w.append(wos_all())
                o = _as_bf16(oball[r0 // 2:(r0 + SB) // 2, :])
                y = jnp.dot(o, _as_bf16(w[0][j]), preferred_element_type=f32)
                outb[pl.ds(r0, SB), j * 128:(j + 1) * 128] = y.astype(bf16)
                return y
            return th
        return [mk(j) for j in range(8)]

    def b_attn_qk(p, rb, first, token):
        b0 = rb * RB
        q = qbuf[p][:, b0:b0 + RB, :]
        if token is not None:
            q = gated(q, token)
        acc = [jnp.sum(q * kbuf[p][:, pl.ds(HALO + b0 - DIL * w, RB), :], axis=0) for w in range(NW)]
        a = jnp.stack(acc)
        a = a + pltpu.roll(a, 64, 2)
        a = a + pltpu.roll(a, 32, 2)
        a = a * (scale_b * LOG2E)
        if first and b0 < DIL * (NW - 1):
            row = b0 + lax.broadcasted_iota(i32, (NW, RB, 128), 1)
            a = jnp.where(row >= DIL * lax.broadcasted_iota(i32, (NW, RB, 128), 0), a, NEG * LOG2E)
        e = jnp.exp2(a - jnp.max(a, axis=0)[None])
        e = e * _recip(jnp.sum(e, axis=0))[None]
        return [e[w] for w in range(NW)]

    def b_attn_pv(p, rb, r0, ps):
        b0 = rb * RB
        dst = _rows(oball, pl.multiple_of(r0 // 2, SB // 2), SB // 2)
        g = 4
        outs = []
        for c0 in range(0, 8, g):
            o = _sum([ps[w][None] * vbuf[p][c0:c0 + g, pl.ds(HALO + b0 - DIL * w, RB), :] for w in range(NW)])
            outs += [o[c] for c in range(g)]
        dst[pl.ds(b0 // 2, RB // 2), :] = _as_u32(jnp.concatenate(outs, axis=1).astype(bf16))
        return outs

    def attn_jobs(p, r0):
        def mk(rb):
            return lambda token: b_attn_pv(p, rb, r0, b_attn_qk(p, rb, False, token))
        return [mk(rb) for rb in range(NRB)]

    z8 = pl.multiple_of(zero[0], 8)
    keep = jnp.zeros((8, 128), u32)
    qkvb[0, 0:8, :] = keep
    keep = keep | qkvb[zero[0], 0:8, :]
    for ref in (oca, ocb, obs):
        ref[0:8, 0:128] = jnp.zeros((8, 128), u32)
        keep = keep | ref[pl.ds(z8, 8), 0:128]
    for ref in (ex, df, sv):
        ref[0] = jnp.zeros((8, 128), f32)
        keep = keep | _as_u32(ref[zero[0]])
    part[0:8, 0:128] = jnp.zeros((8, 128), f32)
    keep = keep | _as_u32(part[pl.ds(z8, 8), 0:128])
    outa[0:16, 0:128] = _as_bf16(keep)
    rawa[pl.ds(RAWA_PAD, RG), :] = jnp.zeros((RG, DH), bf16)
    rawo[pl.ds(RAWO_PAD, 32), :] = jnp.zeros((32, DM), bf16)
    rawob[:, DM:DM + 128] = jnp.zeros((DM, 128), bf16)

    def phase_b():
        for i in range(2):
            cp_w0[i].wait()
            prep_qkv(KQV[0], range(2 * i, 2 * i + 2))
        cp_xb0.wait()
        xcvt(0, 0)
        run(b_proj_dots(0, KQV[0:1], 0))
        cp_xb1.wait()
        xcvt(SB, 1)
        NQ4 = 8
        for h in range(1, 6):
            cp_wp[h].wait()
            if h == 5:
                cp_xb2.wait()
            t0, t1 = KQV[(h - 1) // 2], KQV[h // 2]
            prep_qkv(t1, range(4 * (h % 2), 4 * (h % 2) + 4))
            dots = b_proj_dots(1, (t0,), (h - 1) % 2) + b_proj_dots(0, (t1,), h % 2)
            if h >= 4:
                def qk_job(rb):
                    def job(token):
                        ps_ = b_attn_qk(0, rb, True, token)
                        qb0[:, rb * RB:(rb + 1) * RB, :] = jnp.stack(ps_)
                        return ps_
                    return job
                rbs = range(NQ4) if h == 4 else range(NQ4, NRB)
                run(dots, ([qk_job(rb) for rb in rbs], 4, 12, 112), td=6)
            else:
                run(dots)
            if h == 5:
                vb0[:, 0:HALO, :] = jnp.broadcast_to(vb0[:, HALO:HALO + 1, :], (8, HALO, 128))

                def pv_job(rb):
                    def job(token):
                        ps_ = qb0[:, rb * RB:(rb + 1) * RB, :]
                        if token is not None:
                            ps_ = gated(ps_, token)
                        b_attn_pv(0, rb, 0, [ps_[w] for w in range(NW)])
                    return job
                xcvt(2 * SB, 0)
                pj = [pv_job(rb) for rb in range(NRB)]
                run(b_proj_dots(1, (t1,), 1), (pj[0::2], 0, 7, 48),
                    (pj[1::2], 0, 7, 112))
        cp_xb3.wait()

        def b_step(p, r_attn, r_next, side):
            run(b_proj_dots(p, KVQ),
                (attn_jobs(1 - p, r_attn), 1, 21, 112),
                (side[0::2], 1, 24, 0), (side[1::2], 1, 24, 48),
                (xcvt_jobs(r_next, 1 - p), 0, 20, 0))

        def b_body(it, carry):
            @pl.when(it == 2)
            def _():
                cp_wob.wait()

            @pl.when(jnp.logical_and(it > 0, it <= 5))
            def _():
                wait_like(_rows(xb, pl.multiple_of((4 + 2 * it) * SB, 2 * SB), 2 * SB), sem_x + it - 1)

            @pl.when(it > 0)
            def _():
                c = it - 1
                wait_like(_rows(rawa, pl.multiple_of(c * (GPC * RG), GPC * RG), GPC * RG), 2 * c)
                wait_like(_rows(rawo, pl.multiple_of(c * WOR, 128), WOR), 2 * c + 1)

            r0 = pl.multiple_of((2 * it + 2) * SB, 2 * SB)
            side = chunk_jobs(it)
            b_step(0, r0 - SB, r0 + SB, side[0])
            b_step(1, r0, jnp.minimum(r0 + 2 * SB, S - SB), side[1])
            return carry

        lax.fori_loop(0, NSTEP // 2 - 1, b_body, 0)
        cp_worest.wait()
        cp_m0.wait()
        cp_xa.wait()
        jo = [wocopy_job(NCH * WOR + i * 32, NCH * WOR // 2 + i * 16) for i in range(WOREST // 32)]
        dots = sum([b_out_dots(r) for r in range(NIT * MB, S, SB)], [])
        run(dots, (attn_jobs(1, S - SB), 0, len(dots) - 11, 112), (jo, 0, 0, 0))

    phase_b()
    b_out_start(NIT * MB, S - NIT * MB)

    scale_a = DH ** -0.5
    qscale = scale_a * LOG2E
    k1 = SPLIT * DH
    tri = lax.broadcasted_iota(i32, (8, 8, 128), 1) >= lax.broadcasted_iota(i32, (8, 8, 128), 0)

    def masks(nv):
        qr = LA - 8 * nv
        r = lax.broadcasted_iota(i32, (2 * qr, 2 * LA), 0)
        c = lax.broadcasted_iota(i32, (2 * qr, 2 * LA), 1)
        same = (r >= qr) == (c >= LA)
        rr = jnp.where(r >= qr, r - qr, r) + 8 * nv
        cc = jnp.where(c >= LA, c - LA, c)
        valid = same & ((cc >= SEG) | (rr >= SEG) | (cc <= rr))
        return valid, jnp.where(same, NEG, -jnp.inf).astype(f32)

    msk = [masks(nv) for nv in NVS]

    def bc8(a):
        return jnp.concatenate([jnp.broadcast_to(a[j:j + 1], (8, 128)) for j in range(8)],
                               axis=0).reshape(8, 8, 128)

    def vpu_part(q, k8, v8, causal, prev):
        s_ = jnp.broadcast_to(jnp.sum(q[None] * k8, axis=-1, keepdims=True), (8, 8, 128))
        if causal:
            s_ = jnp.where(tri, s_, NEG * LOG2E)
        m = jnp.max(s_, axis=0)
        if prev is not None:
            m = jnp.maximum(m, prev[0])
        e = jnp.exp2(s_ - m[None])
        l = jnp.sum(e, axis=0)
        o = jnp.sum(e * v8, axis=0)
        if prev is not None:
            al = jnp.exp2(prev[0] - m)
            l = l + prev[1] * al
            o = o + prev[2] * al
        return m, l, o

    def stage(it):
        r0 = pl.multiple_of(it * 64, 64)
        ha[0:40, :] = xa[pl.ds(r0, 40), :]
        hb[8:32, :] = xa[pl.ds(r0 + 40, 24), :]
        obs[...] = oball[pl.ds(pl.multiple_of(it * (MB // 2), 8), MB // 2), :]

    def segment(which, it, r0, rb0):
        h_ref, oc_ref = (ha, oca) if which == 0 else (hb, ocb)
        nrow_o = 32 if which == 0 else 48
        nv = NVS[which]
        qr = LA - 8 * nv
        valid, fill = msk[which]
        h = h_ref[...]
        zvec = zeros_vec()
        so = (19, 18)[which]
        scp = (10, 13)[which]
        pvp = (20, 25)[which]
        assert pvp + 6 * (SPLIT // 2 - 1) <= 6 * NP
        ov, slots, ps, bacc, pre = {}, {}, {}, [], {}

        def wa_tile(hd, t, k0, kn):
            return wa[pl.ds(t * TREG + hd * TP + k0 // 2, kn // 2), :]

        KH = DM // 2
        if which == 1:
            wb = wos_all()
            for hd in range(2):
                for t in range(3):
                    pre[hd, t] = jnp.dot(h[:, :KH], _as_bf16(wa_tile(hd, t, 0, KH)), preferred_element_type=f32)

        def proj(hd, t, ties):
            if (hd, t) in pre:
                y = jnp.dot(h[:, KH:], _as_bf16(wa_tile(hd, t, KH, KH)), preferred_element_type=f32)
                y = y + pre.pop((hd, t))
            else:
                y = jnp.dot(h, _as_bf16(tied(wa_tile(hd, t, 0, DM), zvec, *ties)), preferred_element_type=f32)
            if which == 0:
                ex[t * HA + hd] = y[32:40]
                return jnp.concatenate([y[0:32], y[40:48]], axis=0)
            return jnp.concatenate([ex[t * HA + hd], y[8:32], y[0:8]], axis=0)

        def vpu_jobs(t, ys):
            out = []
            for e in range(2):
                hd = 2 * t + e
                q, k, v = ys[3 * e:3 * e + 3]
                ov[hd] = []
                cache = {}

                def blk(b0):
                    if b0 not in cache:
                        cache[b0] = bc8(k[b0:b0 + 8]), bc8(v[b0:b0 + 8])
                    return cache[b0]

                for g in range(nv):
                    q0 = q[8 * g:8 * g + 8] * qscale
                    if which == 1 and g == 0:
                        st = [sv[i * HA + hd] for i in range(3)]
                    else:
                        st = None
                        for b in range(g, -1, -1):
                            st = vpu_part(q0, *blk(8 * b), b == g, st)
                            out.append(list(st[1:]))
                    _, l, o = vpu_part(q0, *blk(SEG), False, st)
                    ov[hd].append(o * _recip(l))
                    out.append([ov[hd][-1]])
                if which == 0:
                    st = vpu_part(ex[hd] * qscale, bc8(ex[HA + hd]), bc8(ex[2 * HA + hd]), True, None)
                    for i in range(3):
                        sv[i * HA + hd] = st[i]
                    out.append(list(st[1:]))
            for i, jb in enumerate(out):
                slots.setdefault(12 * t + so + (2 * i + 1) * 6 // len(out), []).extend(jb)

        def bout_half(i):
            j, half = i // 2, i % 2
            o = _as_bf16(obs[:, half * KH:(half + 1) * KH])
            y = jnp.dot(o, _as_bf16(wb[j, half * 256:(half + 1) * 256]), preferred_element_type=f32)
            if half == 0:
                bacc.append(y)
            else:
                outb[pl.ds(rb0, MB), j * 128:(j + 1) * 128] = (y + bacc.pop()).astype(bf16)

        def scores(p_):
            if which == 1:
                bout_half(p_)
            q3 = (which * NP + p_) * 3
            sc = lax.dot_general(_as_bf16(qkvb[q3, 0:qr, :]), _as_bf16(qkvb[q3 + 1]), _NT,
                                 preferred_element_type=f32)
            sc = jnp.where(valid, sc * scale_a, fill)
            p = jnp.exp(sc - jnp.max(sc, axis=-1, keepdims=True))
            ps[p_] = (p * _recip(jnp.sum(p, axis=-1, keepdims=True))).astype(bf16)

        def pv(p_):
            o = jnp.dot(ps.pop(p_), _as_bf16(qkvb[(which * NP + p_) * 3 + 2]), preferred_element_type=f32)
            for e in range(2):
                hd = 2 * p_ + e
                oh = jnp.concatenate(ov.pop(hd) + [o[qr * e:qr * e + qr]], axis=0)
                if which == 0:
                    df[hd] = oh[24:32]
                    z = jnp.concatenate([oh[32:40], oh[0:24]], axis=0)
                else:
                    z = jnp.concatenate([oh, df[hd]], axis=0)
                oc_ref[:, hd * DH:(hd + 1) * DH] = _as_u32(z.astype(bf16))

        def after(n):
            for pos, fn in ((pvp, pv), (scp, scores)):
                if (n - pos) % 6 == 0 and 0 <= (n - pos) // 6 < NP:
                    fn((n - pos) // 6)

        for t in range(NP):
            ys = []
            for m in range(6):
                n = 6 * t + m
                ys.append(proj(2 * t + m // 3, m % 3, (slots.pop(2 * n, []), slots.pop(2 * n + 1, []))))
                if m == 5:
                    q3 = (which * NP + t) * 3
                    qkvb[q3, 0:qr, :] = _as_u32(
                        jnp.concatenate([ys[0][8 * nv:], ys[3][8 * nv:]], axis=0).astype(bf16))
                    for i in range(1, 3):
                        qkvb[q3 + i] = _as_u32(jnp.concatenate([ys[i], ys[3 + i]], axis=0).astype(bf16))
                    vpu_jobs(t, ys)
                after(n + 1)
        n = 6 * NP
        for j in range(8):
            ties = [sum([slots.pop(2 * n + i, []) for i in range(lo, lo + 3)], []) for lo in (0, 3)]
            part[0:nrow_o, j * 128:(j + 1) * 128] = jnp.dot(
                _as_bf16(oc_ref[:, :k1]), _as_bf16(tied(woa[j, :k1 // 2, :], zvec, *ties)),
                preferred_element_type=f32)
            for i in range(3):
                n += 1
                after(n)
        assert not (ps or ov or slots or bacc or pre)
        if which == 1:
            @pl.when(it % OG == OG - 1)
            def _():
                b_out_start(pl.multiple_of(rb0 - (OG - 1) * MB, 16), OG * MB)
        o2 = _as_bf16(oc_ref[:, k1:])
        for j in range(8):
            cs = slice(j * 128, (j + 1) * 128)
            y = part[0:nrow_o, cs] + jnp.dot(o2, _as_bf16(woa[j, k1 // 2:, :]), preferred_element_type=f32)
            if which == 0:
                hb[0:8, cs] = y[0:8].astype(bf16)
                outa[pl.ds(r0, 24), cs] = y[8:32].astype(bf16)
            else:
                outa[pl.ds(r0 + 32, 32), cs] = y[0:32].astype(bf16)
                ha[40:48, cs] = y[32:40].astype(bf16)
                outa[pl.ds(r0 + 24, 8), cs] = y[40:48].astype(bf16)
                if j == 6:
                    xa[S:S + 16, 0:128] = y[0:16].astype(bf16)
                    oball[S // 2:S // 2 + 8, 0:128] = _as_u32(y[0:8])
                    stage(jnp.minimum(it + 1, NIT - 1))

    def a_body(it, carry):
        r0 = pl.multiple_of(it * 64, 64)
        rb0 = pl.multiple_of(it * MB, 16)
        segment(0, it, r0, rb0)

        @pl.when(it == OG - 1)
        def _():
            a_out_start(0, 64 * OG - 40)

        @pl.when(jnp.logical_and(it % OG == OG - 1, it >= OG))
        def _():
            a_out_start(r0 + 24 - 64 * OG, 64 * OG)

        segment(1, it, r0, rb0)
        return carry

    stage(0)
    lax.fori_loop(0, NIT, a_body, 0)
    a_out_start(S - 40, 40)

    pltpu.make_async_copy(outb, out_hbm.at[:, pl.ds(DM, DM)], sem_out.at[1]).wait()
    pltpu.make_async_copy(outa, out_hbm.at[:, pl.ds(0, DM)], sem_out.at[0]).wait()


@jax.jit
def pallas_concat_heads__memory_aug_recurrent_mem_tr__sliding_local_dilated__prompt_kernel(
    A_x, A_mem0, A_Wq, A_Wk, A_Wv, A_Wo, A_seg_len, B_x, B_wqkv, B_wo,
):
    del A_seg_len
    assert A_x.shape == (1, S, DM) and B_x.shape == (1, S, DM)
    vm = pltpu.VMEM
    scratch = [
        vm((S + 16, DM), bf16), vm((S, DM), bf16),
        vm((S, DM), bf16), vm((S, DM), bf16),
        vm((RAWA_PAD + RG + 16, DH), bf16),
        vm((RAWO_PAD + 48, DM), bf16),
        vm((3, DM, DM), bf16), vm((DM, DM + 256), bf16),
        vm((3 * TREG + DM // 2 + TPAD, DH), u32),
        vm((8, HA * DH // 2, 128), u32),
        vm((24, BREG + 40, 128), u32), vm((8, BREG + 40, 128), u32),
        vm((8, SB, 128), f32), vm((8, SB, 128), f32),
        vm((8, SB + HALO, 128), f32), vm((8, SB + HALO, 128), f32),
        vm((8, SB + HALO, 128), f32), vm((8, SB + HALO, 128), f32),
        vm((SB // 2, DM), u32), vm((SB // 2, DM), u32),
        vm((S // 2 + 8, DM), u32), vm((MB // 2, DM), u32),
        vm((48, DM), bf16), vm((32, DM), bf16),
        vm((16, HA * DH), u32), vm((24, HA * DH), u32),
        vm((48, DM), f32),
        vm((3 * HA, 8, 128), f32), vm((HA, 8, 128), f32),
        vm((3 * HA, 8, 128), f32),
        vm((6 * NP, LA, 128), u32),
        pltpu.SMEM((1,), i32),
        pltpu.SemaphoreType.DMA((NSEM,)),
        pltpu.SemaphoreType.DMA((2,)),
    ]
    out = pl.pallas_call(
        _kernel,
        out_shape=jax.ShapeDtypeStruct((S, 2 * DM), bf16),
        in_specs=[pl.BlockSpec(memory_space=pl.ANY)] * 9,
        out_specs=pl.BlockSpec(memory_space=pl.ANY),
        scratch_shapes=scratch,
        compiler_params=pltpu.CompilerParams(
            vmem_limit_bytes=120 * 1024 * 1024,
            disable_bounds_checks=True,
            disable_semaphore_checks=True,
        ),
        name="concat_heads_kernel",
    )(
        A_x.reshape(S, DM), A_mem0.reshape(MEM, DM),
        A_Wq.reshape(DM * HA, DH), A_Wk.reshape(DM * HA, DH), A_Wv.reshape(DM * HA, DH),
        A_Wo.reshape(HA * DH, DM),
        B_x.reshape(S, DM), B_wqkv, B_wo,
    )
    return out.reshape(1, S, 2 * DM)
```

```python
import functools

import jax
import jax.numpy as jnp
from jax import lax
import jax.experimental.pallas as pl
import jax.experimental.pallas.tpu as pltpu

bf16, f32, u32, i32 = jnp.bfloat16, jnp.float32, jnp.uint32, jnp.int32

S, DM = 2048, 1024
HA, DH, MEM, SEG = 32, 128, 8, 32
LA = MEM + SEG
HB, NW, DIL = 32, 8, 2
HALO = 16
NEG = -1000000000.0
LOG2E = 1.4426950408889634

SB = 128
NSTEP = S // SB
RB = 8
NRB = SB // RB
TP = 514
TREG = HA * TP
TPAD = 1032
DP = 18
BREG = HB * DP
NCH = 6
GPC = 3 * (DM // 16) // NCH
RG = 16 * HA
WOR = 640
WOREST = HA * DH - NCH * WOR
RAWA_PAD = 3 * DM * HA
RAWO_PAD = HA * DH
NIT = S // (2 * SEG)
MB = 48
OG = 4
NP = HA // 2
SPLIT = 24
NVS = (2, 1)
NSEM = 32

_NT = (((1,), (1,)), ((), ()))


def _as_bf16(x):
    return pltpu.bitcast(x, bf16)


def _as_u32(x):
    return pltpu.bitcast(x, u32)


def _sum(xs):
    return functools.reduce(lambda a, b: a + b, xs)


def _interleave(a, b):
    lo = (a & jnp.uint32(0xFFFF)) | (b << 16)
    hi = (a >> 16) | (b & jnp.uint32(0xFFFF0000))
    return lo, hi


def _recip(x):
    r = pl.reciprocal(x, approx=True)
    return r * (2.0 - x * r)


def _rows(ref, r0, n):
    return ref.at[pl.ds(r0, n), :]


def _kernel(xa_hbm, mem0_hbm, wq_hbm, wk_hbm, wv_hbm, wo_hbm, xb_hbm, wqkvb_hbm, wob_hbm,
            out_hbm,
            xa, xb, outa, outb, rawa, rawo, rawb, rawob, wa, woa, wt, wos,
            qb0, qb1, kb0, kb1, vb0, vb1, xs0, xs1, oball, obs,
            ha, hb, oca, ocb, part, ex, df, sv, qkvb, zero,
            sem, sem_out):
    zero[0] = 0
    qbuf, kbuf, vbuf, xsb = (qb0, qb1), (kb0, kb1), (vb0, vb1), (xs0, xs1)

    nsem = [0]

    def cp(src, dst):
        c = pltpu.make_async_copy(src, dst, sem.at[nsem[0]])
        nsem[0] += 1
        return c

    def cp_xb(b0, nb):
        return cp(_rows(xb_hbm, b0 * SB, nb * SB), _rows(xb, b0 * SB, nb * SB))

    def cp_wb(t, k0, n):
        return cp(wqkvb_hbm.at[pl.ds(k0, n), pl.ds(t * DM, DM)], rawb.at[t, pl.ds(k0, n), :])

    cp_ch = []
    for c in range(NCH):
        w = (wq_hbm, wk_hbm, wv_hbm)[c // 2]
        cp_ch.append(cp(_rows(w, (c % 2) * GPC * RG, GPC * RG), _rows(rawa, c * GPC * RG, GPC * RG)))
        cp_ch.append(cp(_rows(wo_hbm, c * WOR, WOR), _rows(rawo, c * WOR, WOR)))
    sem_x = nsem[0]
    cp_xbs = [cp_xb(6 + 2 * c, 2) for c in range(5)]
    cp_worest = cp(_rows(wo_hbm, NCH * WOR, WOREST), _rows(rawo, NCH * WOR, WOREST))
    cp_xb0, cp_xb1, cp_xb2, cp_xb3 = cp_xb(0, 1), cp_xb(1, 1), cp_xb(2, 1), cp_xb(3, 3)
    KVQ, KQV = (1, 2, 0), (1, 0, 2)
    cp_w0 = [cp_wb(KQV[0], 0, DM // 4), cp_wb(KQV[0], DM // 4, DM // 4)]
    cp_wp = [None] + [cp_wb(KQV[h // 2], (h % 2) * (DM // 2), DM // 2) for h in range(1, 6)]
    cp_wob = cp(wob_hbm, rawob.at[:, pl.ds(0, DM)])
    cp_xa = cp(xa_hbm, _rows(xa, 0, S))
    cp_m0 = cp(mem0_hbm, _rows(ha, LA, MEM))
    assert nsem[0] == NSEM
    order = cp_w0 + [cp_xb0, cp_xb1] + cp_wp[1:5] + [cp_xb2, cp_wp[5], cp_xb3]
    for c in range(NCH):
        order += cp_ch[2 * c:2 * c + 2] + cp_xbs[c:c + 1] + ([cp_wob] if c == 0 else [])
    order += [cp_worest, cp_m0, cp_xa]
    for c in order:
        c.start()

    def wait_like(dst, s):
        pltpu.make_async_copy(dst, dst, sem.at[s]).wait()

    def a_out_start(r0, n):
        r0 = pl.multiple_of(r0, 8)
        pltpu.make_async_copy(_rows(outa, r0, n), out_hbm.at[pl.ds(r0, n), pl.ds(0, DM)],
                              sem_out.at[0]).start()

    def b_out_start(r0, n):
        pltpu.make_async_copy(_rows(outb, r0, n), out_hbm.at[pl.ds(r0, n), pl.ds(DM, DM)],
                              sem_out.at[1]).start()

    def zeros_vec():
        return jnp.full((8, 128), zero[0], i32).astype(u32)

    def tied(w, zvec, *vals_list):
        n = w.shape[0] // len(vals_list)
        parts = []
        for i, vals in enumerate(vals_list):
            pt = w[i * n:(i + 1) * n]
            if vals:
                tie = functools.reduce(lambda a, b: a | b, [_as_u32(x) for x in vals]) & zvec
                pt = jnp.concatenate([pt[0:n - 8], pt[n - 8:] | tie], axis=0)
            parts.append(pt)
        return jnp.concatenate(parts, axis=0)

    def gated(x, token):
        gate = _as_u32(token[8:16]) & zeros_vec()
        return pltpu.bitcast(_as_u32(x) | gate[None], f32)

    def run(dots, *job_lists, td=6):
        rel = {}
        for jobs, lo, hi, tr in job_lists:
            for i, job in enumerate(jobs):
                rel.setdefault(lo + i * (hi - lo) // len(jobs) - 1, []).append((job, tr))
        due = {}

        def fire(i, y):
            for job, tr in rel.get(i, []):
                vals = job(None if y is None else y[tr:tr + 16])
                if vals:
                    due.setdefault(min(i + td, len(dots) - 1), []).extend(vals)

        fire(-1, None)
        for i, th in enumerate(dots):
            fire(i, th(due.pop(i, [])))

    def prep_qkv(t, kbs):
        for kb_ in kbs:
            for ch in range(8):
                at = _as_u32(rawb[t, kb_ * 128:(kb_ + 1) * 128, ch * 128:(ch + 1) * 128].T)
                for pr in range(2):
                    lo, hi = _interleave(at[pr * 32:pr * 32 + 16], at[pr * 32 + 16:pr * 32 + 32])
                    wt[t * 8 + kb_, pl.ds(ch * 2 + pr, 16, stride=2 * DP), :] = lo
                    wt[t * 8 + kb_, pl.ds(DP + ch * 2 + pr, 16, stride=2 * DP), :] = hi

    def prep_wo_job(src_col, j, hq):
        def job(token):
            rawob[0:16, DM + 128:DM + 256] = token.astype(bf16)
            dst = wos.at[j]
            for hp in range(4 * hq, 4 * hq + 4):
                src = _as_u32(rawob[hp * 64:(hp + 1) * 64, pl.ds(src_col, 128)])
                lo, hi = _interleave(src[0:16], src[16:32])
                dst[pl.ds(hp, 16, stride=2 * DP), :] = lo
                dst[pl.ds(DP + hp, 16, stride=2 * DP), :] = hi
        return job

    def repack_job(src0, dst0, half):
        def job(token):
            rawa[pl.ds(RAWA_PAD + RG, 16), :] = token.astype(bf16)
            dst = _rows(wa, dst0, TREG + TPAD)
            for ii in range(half * 4, half * 4 + 4):
                src = _as_u32(_rows(rawa, src0, RG)[ii * 64:(ii + 1) * 64, :])
                lo, hi = _interleave(src[0:16], src[16:32])
                dst[pl.ds(ii, 16, stride=2 * TP), :] = lo
                dst[pl.ds(ii + TP, 16, stride=2 * TP), :] = hi
        return job

    def wocopy_job(src0, dst0):
        def job(token):
            if token is not None:
                rawo[pl.ds(RAWO_PAD + 32, 16), 0:128] = token.astype(bf16)
            v = _as_u32(rawo[pl.ds(src0, 32), :])
            woa[:, pl.ds(dst0, 16), :] = jnp.stack([v[:, j * 128:(j + 1) * 128] for j in range(8)])
        return job

    def chunk_jobs(it):
        c = jnp.maximum(it - 1, 0)
        ja, jo, jw = [], [], []
        for i in range(GPC):
            src0 = pl.multiple_of(jnp.where(it > 0, (c * GPC + i) * RG, RAWA_PAD), RG)
            dst0 = pl.multiple_of((c // 2) * TREG + ((c % 2) * GPC + i) * 8, 8)
            ja += [repack_job(src0, dst0, 0), repack_job(src0, dst0, 1)]
        for i in range(WOR // 32):
            src0 = pl.multiple_of(jnp.where(it > 0, c * WOR + i * 32, RAWO_PAD), 32)
            jo.append(wocopy_job(src0, pl.multiple_of(c * (WOR // 2) + i * 16, 16)))
        for i in range(2):
            j = jnp.clip(2 * (it - 2) + i, 0, 7)
            src_col = pl.multiple_of(jnp.where(it > 1, j * 128, DM), 128)
            jw += [prep_wo_job(src_col, j, hq) for hq in range(4)]
        half = lambda js, h: js[h * len(js) // 2:(h + 1) * len(js) // 2]
        return [half(ja, h) + half(jo, h) + half(jw, h) for h in range(2)]

    def xcvt_jobs(r0, p):
        def mk(i):
            def job(token):
                xsb[p][i * 8:(i + 1) * 8, :] = _as_u32(xb[pl.ds(pl.multiple_of(r0 + i * 16, 16), 16), :])
            return job
        return [mk(i) for i in range(SB // 16)]

    def xcvt(r0, p):
        for job in xcvt_jobs(r0, p):
            job(None)

    scale_b = (DM // HB) ** -0.5

    def b_proj_dots(p, ts, half=None):
        kbs = range(8) if half is None else range(4 * half, 4 * half + 4)

        def mk(t, c):
            def th(ties):
                x = _as_bf16(xsb[p][:, kbs[0] * 128:(kbs[-1] + 1) * 128])
                wv = jnp.concatenate([wt[t * 8 + kbs[0]:t * 8 + kbs[-1] + 1, pl.ds((4 * c + dd) * DP, 16), :]
                                      for dd in range(4)], axis=1)
                tiles = [wv[i] for i in range(len(kbs))]
                if ties:
                    tiles[-1] = tied(tiles[-1], zeros_vec(), ties)
                y = lax.dot_general(x, _as_bf16(jnp.concatenate(tiles, axis=1)), _NT,
                                    preferred_element_type=f32)
                if t == 0:
                    qbuf[p][c] = y + qbuf[p][c] if half == 1 else y
                else:
                    g = kbuf if t == 1 else vbuf
                    if half != 0:
                        g[p][c, 0:HALO, :] = g[1 - p][c, SB:SB + HALO, :]
                    g[p][c, HALO:HALO + SB, :] = y + g[p][c, HALO:HALO + SB, :] if half == 1 else y
                return y
            return th
        return [mk(t, c) for t in ts for c in range(8)]

    def wos_all():
        return jnp.concatenate([wos[:, pl.ds(d * DP, 16), :] for d in range(HB)], axis=1)

    def b_out_dots(r0):
        w = []

        def mk(j):
            def th(ties):
                if not w:
                    w.append(wos_all())
                o = _as_bf16(oball[r0 // 2:(r0 + SB) // 2, :])
                y = jnp.dot(o, _as_bf16(w[0][j]), preferred_element_type=f32)
                outb[pl.ds(r0, SB), j * 128:(j + 1) * 128] = y.astype(bf16)
                return y
            return th
        return [mk(j) for j in range(8)]

    def b_attn_qk(p, rb, first, token):
        b0 = rb * RB
        q = qbuf[p][:, b0:b0 + RB, :]
        if token is not None:
            q = gated(q, token)
        acc = [jnp.sum(q * kbuf[p][:, pl.ds(HALO + b0 - DIL * w, RB), :], axis=0) for w in range(NW)]
        a = jnp.stack(acc)
        a = a + pltpu.roll(a, 64, 2)
        a = a + pltpu.roll(a, 32, 2)
        a = a * (scale_b * LOG2E)
        if first and b0 < DIL * (NW - 1):
            row = b0 + lax.broadcasted_iota(i32, (NW, RB, 128), 1)
            a = jnp.where(row >= DIL * lax.broadcasted_iota(i32, (NW, RB, 128), 0), a, NEG * LOG2E)
        e = jnp.exp2(a - jnp.max(a, axis=0)[None])
        e = e * _recip(jnp.sum(e, axis=0))[None]
        return [e[w] for w in range(NW)]

    def b_attn_pv(p, rb, r0, ps):
        b0 = rb * RB
        dst = _rows(oball, pl.multiple_of(r0 // 2, SB // 2), SB // 2)
        g = 4
        outs = []
        for c0 in range(0, 8, g):
            o = _sum([ps[w][None] * vbuf[p][c0:c0 + g, pl.ds(HALO + b0 - DIL * w, RB), :] for w in range(NW)])
            outs += [o[c] for c in range(g)]
        dst[pl.ds(b0 // 2, RB // 2), :] = _as_u32(jnp.concatenate(outs, axis=1).astype(bf16))
        return outs

    def attn_jobs(p, r0):
        def mk(rb):
            return lambda token: b_attn_pv(p, rb, r0, b_attn_qk(p, rb, False, token))
        return [mk(rb) for rb in range(NRB)]

    z8 = pl.multiple_of(zero[0], 8)
    keep = jnp.zeros((8, 128), u32)
    qkvb[0, 0:8, :] = keep
    keep = keep | qkvb[zero[0], 0:8, :]
    for ref in (oca, ocb, obs):
        ref[0:8, 0:128] = jnp.zeros((8, 128), u32)
        keep = keep | ref[pl.ds(z8, 8), 0:128]
    for ref in (ex, df, sv):
        ref[0] = jnp.zeros((8, 128), f32)
        keep = keep | _as_u32(ref[zero[0]])
    part[0:8, 0:128] = jnp.zeros((8, 128), f32)
    keep = keep | _as_u32(part[pl.ds(z8, 8), 0:128])
    outa[0:16, 0:128] = _as_bf16(keep)
    rawa[pl.ds(RAWA_PAD, RG), :] = jnp.zeros((RG, DH), bf16)
    rawo[pl.ds(RAWO_PAD, 32), :] = jnp.zeros((32, DM), bf16)
    rawob[:, DM:DM + 128] = jnp.zeros((DM, 128), bf16)

    def phase_b():
        for i in range(2):
            cp_w0[i].wait()
            prep_qkv(KQV[0], range(2 * i, 2 * i + 2))
        cp_xb0.wait()
        xcvt(0, 0)
        run(b_proj_dots(0, KQV[0:1], 0))
        cp_xb1.wait()
        xcvt(SB, 1)
        NQ4 = 8
        for h in range(1, 6):
            cp_wp[h].wait()
            if h == 5:
                cp_xb2.wait()
            t0, t1 = KQV[(h - 1) // 2], KQV[h // 2]
            prep_qkv(t1, range(4 * (h % 2), 4 * (h % 2) + 4))
            dots = b_proj_dots(1, (t0,), (h - 1) % 2) + b_proj_dots(0, (t1,), h % 2)
            if h >= 4:
                def qk_job(rb):
                    def job(token):
                        ps_ = b_attn_qk(0, rb, True, token)
                        qb0[:, rb * RB:(rb + 1) * RB, :] = jnp.stack(ps_)
                        return ps_
                    return job
                rbs = range(NQ4) if h == 4 else range(NQ4, NRB)
                run(dots, ([qk_job(rb) for rb in rbs], 4, 12, 112), td=6)
            else:
                run(dots)
            if h == 5:
                vb0[:, 0:HALO, :] = jnp.broadcast_to(vb0[:, HALO:HALO + 1, :], (8, HALO, 128))

                def pv_job(rb):
                    def job(token):
                        ps_ = qb0[:, rb * RB:(rb + 1) * RB, :]
                        if token is not None:
                            ps_ = gated(ps_, token)
                        b_attn_pv(0, rb, 0, [ps_[w] for w in range(NW)])
                    return job
                xcvt(2 * SB, 0)
                pj = [pv_job(rb) for rb in range(NRB)]
                run(b_proj_dots(1, (t1,), 1), (pj[0::2], 0, 7, 48),
                    (pj[1::2], 0, 7, 112))
        cp_xb3.wait()

        def b_step(p, r_attn, r_next, side):
            run(b_proj_dots(p, KVQ),
                (attn_jobs(1 - p, r_attn), 1, 21, 112),
                (side[0::2], 1, 24, 0), (side[1::2], 1, 24, 48),
                (xcvt_jobs(r_next, 1 - p), 0, 20, 0))

        def b_body(it, carry):
            @pl.when(it == 2)
            def _():
                cp_wob.wait()

            @pl.when(jnp.logical_and(it > 0, it <= 5))
            def _():
                wait_like(_rows(xb, pl.multiple_of((4 + 2 * it) * SB, 2 * SB), 2 * SB), sem_x + it - 1)

            @pl.when(it > 0)
            def _():
                c = it - 1
                wait_like(_rows(rawa, pl.multiple_of(c * (GPC * RG), GPC * RG), GPC * RG), 2 * c)
                wait_like(_rows(rawo, pl.multiple_of(c * WOR, 128), WOR), 2 * c + 1)

            r0 = pl.multiple_of((2 * it + 2) * SB, 2 * SB)
            side = chunk_jobs(it)
            b_step(0, r0 - SB, r0 + SB, side[0])
            b_step(1, r0, jnp.minimum(r0 + 2 * SB, S - SB), side[1])
            return carry

        lax.fori_loop(0, NSTEP // 2 - 1, b_body, 0)
        cp_worest.wait()
        cp_m0.wait()
        cp_xa.wait()
        jo = [wocopy_job(NCH * WOR + i * 32, NCH * WOR // 2 + i * 16) for i in range(WOREST // 32)]
        dots = sum([b_out_dots(r) for r in range(NIT * MB, S, SB)], [])
        run(dots, (attn_jobs(1, S - SB), 0, len(dots) - 11, 112), (jo, 0, 0, 0))

    phase_b()
    b_out_start(NIT * MB, S - NIT * MB)

    scale_a = DH ** -0.5
    qscale = scale_a * LOG2E
    k1 = SPLIT * DH
    tri = lax.broadcasted_iota(i32, (8, 8, 128), 1) >= lax.broadcasted_iota(i32, (8, 8, 128), 0)

    def masks(nv):
        qr = LA - 8 * nv
        r = lax.broadcasted_iota(i32, (2 * qr, 2 * LA), 0)
        c = lax.broadcasted_iota(i32, (2 * qr, 2 * LA), 1)
        same = (r >= qr) == (c >= LA)
        rr = jnp.where(r >= qr, r - qr, r) + 8 * nv
        cc = jnp.where(c >= LA, c - LA, c)
        valid = same & ((cc >= SEG) | (rr >= SEG) | (cc <= rr))
        return valid, jnp.where(same, NEG, -jnp.inf).astype(f32)

    NVL, LT0 = 2, 10
    nvof = lambda which, t: (NVL if t >= LT0 else NVS[1]) if which == 1 else (NVS[0] if t < 16 else 1)
    nearly = lambda which, t: (0 if t >= 16 else NVS[1]) if which == 1 else nvof(0, t)
    msk = {nv: masks(nv) for nv in {nvof(w_, t_) for w_ in range(2) for t_ in range(NP)}}

    def bc8(a):
        return jnp.concatenate([jnp.broadcast_to(a[j:j + 1], (8, 128)) for j in range(8)],
                               axis=0).reshape(8, 8, 128)

    def vpu_part(q, k8, v8, causal, prev):
        s_ = jnp.broadcast_to(jnp.sum(q[None] * k8, axis=-1, keepdims=True), (8, 8, 128))
        if causal:
            s_ = jnp.where(tri, s_, NEG * LOG2E)
        m = jnp.max(s_, axis=0)
        if prev is not None:
            m = jnp.maximum(m, prev[0])
        e = jnp.exp2(s_ - m[None])
        l = jnp.sum(e, axis=0)
        o = jnp.sum(e * v8, axis=0)
        if prev is not None:
            al = jnp.exp2(prev[0] - m)
            l = l + prev[1] * al
            o = o + prev[2] * al
        return m, l, o

    def stage(it):
        r0 = pl.multiple_of(it * 64, 64)
        ha[0:40, :] = xa[pl.ds(r0, 40), :]
        hb[8:32, :] = xa[pl.ds(r0 + 40, 24), :]
        obs[...] = oball[pl.ds(pl.multiple_of(it * (MB // 2), 8), MB // 2), :]

    def segment(which, it, r0, rb0):
        h_ref, oc_ref = (ha, oca) if which == 0 else (hb, ocb)
        nrow_o = 32 if which == 0 else 48
        h = h_ref[...]
        zvec = zeros_vec()
        so = (19, 15)[which]
        scp = (10, 13)[which]
        pvp = (20, 25)[which]
        assert pvp + 6 * (SPLIT // 2 - 1) <= 6 * NP
        ov, slots, ps, bacc, pre, late, merges = {}, {}, {}, [], {}, [], []

        LS, LU, LD = -4, 23, 7
        nlate = sum(2 * (g + 2 if g else 1) for t in range(NP) for g in range(nearly(which, t), nvof(which, t)))
        lrel = {}

        def fire(n, y):
            for i, job in enumerate(lrel.pop(n, [])):
                r_ = (0, y.shape[0] - 8, 16)[i % 3]
                vals = job(_as_u32(y[r_:r_ + 8]) & zvec)
                if n + LD < 6 * NP + SPLIT:
                    slots.setdefault(2 * (n + LD) + i % 2, []).extend(vals)

        def wa_tile(hd, t, k0, kn):
            return wa[pl.ds(t * TREG + hd * TP + k0 // 2, kn // 2), :]

        KH = DM // 2
        if which == 1:
            wb = wos_all()
            for hd in range(2):
                for t in range(3):
                    pre[hd, t] = jnp.dot(h[:, :KH], _as_bf16(wa_tile(hd, t, 0, KH)), preferred_element_type=f32)

        def proj(hd, t, ties):
            if (hd, t) in pre:
                y = jnp.dot(h[:, KH:], _as_bf16(wa_tile(hd, t, KH, KH)), preferred_element_type=f32)
                y = y + pre.pop((hd, t))
            else:
                y = jnp.dot(h, _as_bf16(tied(wa_tile(hd, t, 0, DM), zvec, *ties)), preferred_element_type=f32)
            if which == 0:
                ex[t * HA + hd] = y[32:40]
                return jnp.concatenate([y[0:32], y[40:48]], axis=0)
            return jnp.concatenate([ex[t * HA + hd], y[8:32], y[0:8]], axis=0)

        def vpu_jobs(t, ys):
            out = []
            for e in range(2):
                hd = 2 * t + e
                q, k, v = ys[3 * e:3 * e + 3]
                ov[hd] = []
                cache = {}

                def blk(b0):
                    if b0 not in cache:
                        cache[b0] = bc8(k[b0:b0 + 8]), bc8(v[b0:b0 + 8])
                    return cache[b0]

                for g in range(nearly(which, t)):
                    q0 = q[8 * g:8 * g + 8] * qscale
                    if which == 1 and g == 0:
                        st = [sv[i * HA + hd] for i in range(3)]
                    else:
                        st = None
                        for b in range(g, -1, -1):
                            st = vpu_part(q0, *blk(8 * b), b == g, st)
                            out.append(list(st[1:]))
                    _, l, o = vpu_part(q0, *blk(SEG), False, st)
                    ov[hd].append(o * _recip(l))
                    out.append([ov[hd][-1]])
                for g in range(nearly(which, t), nvof(which, t)):
                    st = [None]
                    for b0 in ([8 * b for b in range(g, -1, -1)] if g else []) + [SEG]:
                        def job(tok, hd=hd, g=g, b0=b0, st=st, q=q, k=k, v=v):
                            if g == 0:
                                st[0] = [sv[i * HA + hd] for i in range(3)]
                            gate = lambda x: pltpu.bitcast(_as_u32(x) | tok, f32)
                            st[0] = vpu_part(gate(q[8 * g:8 * g + 8]) * qscale, bc8(gate(k[b0:b0 + 8])),
                                             bc8(gate(v[b0:b0 + 8])), b0 == 8 * g, st[0])
                            if b0 != SEG:
                                return list(st[0][1:])
                            ov[hd].append(st[0][2] * _recip(st[0][1]))
                            return [ov[hd][-1]]
                        lrel.setdefault(6 * NP + LS + len(late) * LU // nlate, []).append(job)
                        late.append(job)
                if which == 0:
                    st = vpu_part(ex[hd] * qscale, bc8(ex[HA + hd]), bc8(ex[2 * HA + hd]), True, None)
                    for i in range(3):
                        sv[i * HA + hd] = st[i]
                    out.append(list(st[1:]))
            for i, jb in enumerate(out):
                slots.setdefault(12 * t + so + (2 * i + 1) * 6 // len(out), []).extend(jb)

        def bout_half(i):
            j, half = i // 2, i % 2
            o = _as_bf16(obs[:, half * KH:(half + 1) * KH])
            y = jnp.dot(o, _as_bf16(wb[j, half * 256:(half + 1) * 256]), preferred_element_type=f32)
            if half == 0:
                bacc.append(y)
            else:
                outb[pl.ds(rb0, MB), j * 128:(j + 1) * 128] = (y + bacc.pop()).astype(bf16)

        def scores(p_):
            if which == 1:
                bout_half(p_)
            q3 = (which * NP + p_) * 3
            qr = LA - 8 * nvof(which, p_)
            valid, fill = msk[nvof(which, p_)]
            sc = lax.dot_general(_as_bf16(qkvb[q3, 0:qr, :]), _as_bf16(qkvb[q3 + 1]), _NT,
                                 preferred_element_type=f32)
            sc = jnp.where(valid, sc * scale_a, fill)
            p = jnp.exp(sc - jnp.max(sc, axis=-1, keepdims=True))
            ps[p_] = (p * _recip(jnp.sum(p, axis=-1, keepdims=True))).astype(bf16)

        def pv(p_):
            o = jnp.dot(ps.pop(p_), _as_bf16(qkvb[(which * NP + p_) * 3 + 2]), preferred_element_type=f32)
            qr = LA - 8 * nvof(which, p_)

            def merge():
                for e in range(2):
                    hd = 2 * p_ + e
                    oh = jnp.concatenate(ov.pop(hd) + [o[qr * e:qr * e + qr]], axis=0)
                    if which == 0:
                        df[hd] = oh[24:32]
                        z = jnp.concatenate([oh[32:40], oh[0:24]], axis=0)
                    else:
                        z = jnp.concatenate([oh, df[hd]], axis=0)
                    oc_ref[:, hd * DH:(hd + 1) * DH] = _as_u32(z.astype(bf16))
            if nvof(which, p_) > nearly(which, p_):
                merges.append(merge)
            else:
                merge()

        def after(n):
            for pos, fn in ((pvp, pv), (scp, scores)):
                if (n - pos) % 6 == 0 and 0 <= (n - pos) // 6 < NP:
                    fn((n - pos) // 6)

        for t in range(NP):
            ys = []
            for m in range(6):
                n = 6 * t + m
                ys.append(proj(2 * t + m // 3, m % 3, (slots.pop(2 * n, []), slots.pop(2 * n + 1, []))))
                if m == 5:
                    q3 = (which * NP + t) * 3
                    nv = nvof(which, t)
                    qr = LA - 8 * nv
                    qkvb[q3, 0:qr, :] = _as_u32(
                        jnp.concatenate([ys[0][8 * nv:], ys[3][8 * nv:]], axis=0).astype(bf16))
                    for i in range(1, 3):
                        qkvb[q3 + i] = _as_u32(jnp.concatenate([ys[i], ys[3 + i]], axis=0).astype(bf16))
                    vpu_jobs(t, ys)
                fire(n, ys[-1][8:32])
                after(n + 1)
        n = 6 * NP
        if not late:
            for j in range(8):
                ties = [sum([slots.pop(2 * n + i, []) for i in range(lo, lo + 3)], []) for lo in (0, 3)]
                part[0:nrow_o, j * 128:(j + 1) * 128] = jnp.dot(
                    _as_bf16(oc_ref[:, :k1]), _as_bf16(tied(woa[j, :k1 // 2, :], zvec, *ties)),
                    preferred_element_type=f32)
                for i in range(3):
                    n += 1
                    after(n)
        else:
            kc0 = LT0 // 4
            units = [(j, kc) for j in range(8) for kc in range(kc0)]
            units += [(j, kc) for kc in range(kc0, SPLIT // 8) for j in range(8)]
            for u, (j, kc) in enumerate(units):
                k0 = kc * DM
                cs = slice(j * 128, (j + 1) * 128)
                if kc >= kc0 and j == 0:
                    for p_ in range(4 * kc, 4 * kc + 4):
                        if p_ >= LT0:
                            merges.pop(0)()
                y = jnp.dot(_as_bf16(oc_ref[:, k0:k0 + DM]),
                            _as_bf16(tied(woa[j, k0 // 2:(k0 + DM) // 2, :], zvec,
                                          slots.pop(2 * n, []), slots.pop(2 * n + 1, []))),
                            preferred_element_type=f32)
                fire(n, y)
                acc = y if kc == 0 else (acc + y if kc < kc0 else part[0:nrow_o, cs] + y)
                if kc >= kc0 - 1:
                    part[0:nrow_o, cs] = acc
                n += 1
                after(n)
            for merge in merges:
                merge()
        assert not (ps or ov or slots or bacc or pre or lrel)
        if which == 1:
            @pl.when(it % OG == OG - 1)
            def _():
                b_out_start(pl.multiple_of(rb0 - (OG - 1) * MB, 16), OG * MB)
        o2 = _as_bf16(oc_ref[:, k1:])
        for j in range(8):
            cs = slice(j * 128, (j + 1) * 128)
            y = part[0:nrow_o, cs] + jnp.dot(o2, _as_bf16(woa[j, k1 // 2:, :]), preferred_element_type=f32)
            if which == 0:
                hb[0:8, cs] = y[0:8].astype(bf16)
                outa[pl.ds(r0, 24), cs] = y[8:32].astype(bf16)
            else:
                outa[pl.ds(r0 + 32, 32), cs] = y[0:32].astype(bf16)
                ha[40:48, cs] = y[32:40].astype(bf16)
                outa[pl.ds(r0 + 24, 8), cs] = y[40:48].astype(bf16)
                if j == 6:
                    xa[S:S + 16, 0:128] = y[0:16].astype(bf16)
                    oball[S // 2:S // 2 + 8, 0:128] = _as_u32(y[0:8])
                    stage(jnp.minimum(it + 1, NIT - 1))

    def a_body(it, carry):
        r0 = pl.multiple_of(it * 64, 64)
        rb0 = pl.multiple_of(it * MB, 16)
        segment(0, it, r0, rb0)

        @pl.when(it == OG - 1)
        def _():
            a_out_start(0, 64 * OG - 40)

        @pl.when(jnp.logical_and(it % OG == OG - 1, it >= OG))
        def _():
            a_out_start(r0 + 24 - 64 * OG, 64 * OG)

        segment(1, it, r0, rb0)
        return carry

    stage(0)
    lax.fori_loop(0, NIT, a_body, 0)
    a_out_start(S - 40, 40)

    pltpu.make_async_copy(outb, out_hbm.at[:, pl.ds(DM, DM)], sem_out.at[1]).wait()
    pltpu.make_async_copy(outa, out_hbm.at[:, pl.ds(0, DM)], sem_out.at[0]).wait()


@jax.jit
def pallas_concat_heads__memory_aug_recurrent_mem_tr__sliding_local_dilated__prompt_kernel(
    A_x, A_mem0, A_Wq, A_Wk, A_Wv, A_Wo, A_seg_len, B_x, B_wqkv, B_wo,
):
    del A_seg_len
    assert A_x.shape == (1, S, DM) and B_x.shape == (1, S, DM)
    vm = pltpu.VMEM
    scratch = [
        vm((S + 16, DM), bf16), vm((S, DM), bf16),
        vm((S, DM), bf16), vm((S, DM), bf16),
        vm((RAWA_PAD + RG + 16, DH), bf16),
        vm((RAWO_PAD + 48, DM), bf16),
        vm((3, DM, DM), bf16), vm((DM, DM + 256), bf16),
        vm((3 * TREG + DM // 2 + TPAD, DH), u32),
        vm((8, HA * DH // 2, 128), u32),
        vm((24, BREG + 40, 128), u32), vm((8, BREG + 40, 128), u32),
        vm((8, SB, 128), f32), vm((8, SB, 128), f32),
        vm((8, SB + HALO, 128), f32), vm((8, SB + HALO, 128), f32),
        vm((8, SB + HALO, 128), f32), vm((8, SB + HALO, 128), f32),
        vm((SB // 2, DM), u32), vm((SB // 2, DM), u32),
        vm((S // 2 + 8, DM), u32), vm((MB // 2, DM), u32),
        vm((48, DM), bf16), vm((32, DM), bf16),
        vm((16, HA * DH), u32), vm((24, HA * DH), u32),
        vm((48, DM), f32),
        vm((3 * HA, 8, 128), f32), vm((HA, 8, 128), f32),
        vm((3 * HA, 8, 128), f32),
        vm((6 * NP, LA, 128), u32),
        pltpu.SMEM((1,), i32),
        pltpu.SemaphoreType.DMA((NSEM,)),
        pltpu.SemaphoreType.DMA((2,)),
    ]
    out = pl.pallas_call(
        _kernel,
        out_shape=jax.ShapeDtypeStruct((S, 2 * DM), bf16),
        in_specs=[pl.BlockSpec(memory_space=pl.ANY)] * 9,
        out_specs=pl.BlockSpec(memory_space=pl.ANY),
        scratch_shapes=scratch,
        compiler_params=pltpu.CompilerParams(
            vmem_limit_bytes=120 * 1024 * 1024,
            disable_bounds_checks=True,
            disable_semaphore_checks=True,
        ),
        name="concat_heads_kernel",
    )(
        A_x.reshape(S, DM), A_mem0.reshape(MEM, DM),
        A_Wq.reshape(DM * HA, DH), A_Wk.reshape(DM * HA, DH), A_Wv.reshape(DM * HA, DH),
        A_Wo.reshape(HA * DH, DM),
        B_x.reshape(S, DM), B_wqkv, B_wo,
    )
    return out.reshape(1, S, 2 * DM)
```

```python
import functools

import jax
import jax.numpy as jnp
from jax import lax
import jax.experimental.pallas as pl
import jax.experimental.pallas.tpu as pltpu

bf16, f32, u32, i32 = jnp.bfloat16, jnp.float32, jnp.uint32, jnp.int32

S, DM = 2048, 1024
HA, DH, MEM, SEG = 32, 128, 8, 32
LA = MEM + SEG
HB, NW, DIL = 32, 8, 2
HALO = 16
NEG = -1000000000.0
LOG2E = 1.4426950408889634

SB = 128
NSTEP = S // SB
RB = 8
NRB = SB // RB
TP = 514
TREG = HA * TP
TPAD = 1032
DP = 18
BREG = HB * DP
NCH = 6
GPC = 3 * (DM // 16) // NCH
RG = 16 * HA
WOR = 640
WOREST = HA * DH - NCH * WOR
RAWA_PAD = 3 * DM * HA
RAWO_PAD = HA * DH
NIT = S // (2 * SEG)
MB = 48
OG = 4
NP = HA // 2
SPLIT = 24
NVS = (2, 1)
LT0 = 10
NSEM = 32

_NT = (((1,), (1,)), ((), ()))


def _as_bf16(x):
    return pltpu.bitcast(x, bf16)


def _as_u32(x):
    return pltpu.bitcast(x, u32)


def _sum(xs):
    return functools.reduce(lambda a, b: a + b, xs)


def _interleave(a, b):
    lo = (a & jnp.uint32(0xFFFF)) | (b << 16)
    hi = (a >> 16) | (b & jnp.uint32(0xFFFF0000))
    return lo, hi


def _recip(x):
    r = pl.reciprocal(x, approx=True)
    return r * (2.0 - x * r)


def _rows(ref, r0, n):
    return ref.at[pl.ds(r0, n), :]


def _kernel(xa_hbm, mem0_hbm, wq_hbm, wk_hbm, wv_hbm, wo_hbm, xb_hbm, wqkvb_hbm, wob_hbm,
            out_hbm,
            xa, xb, outa, outb, rawa, rawo, rawb, rawob, wa, woa, wt, wos,
            qb0, qb1, kb0, kb1, vb0, vb1, xs0, xs1, oball, obs,
            ha, hb, oca, ocb, part, ex, df, sv, qkvb, zero,
            sem, sem_out):
    zero[0] = 0
    qbuf, kbuf, vbuf, xsb = (qb0, qb1), (kb0, kb1), (vb0, vb1), (xs0, xs1)

    nsem = [0]

    def cp(src, dst):
        c = pltpu.make_async_copy(src, dst, sem.at[nsem[0]])
        nsem[0] += 1
        return c

    def cp_xb(b0, nb):
        return cp(_rows(xb_hbm, b0 * SB, nb * SB), _rows(xb, b0 * SB, nb * SB))

    def cp_wb(t, k0, n):
        return cp(wqkvb_hbm.at[pl.ds(k0, n), pl.ds(t * DM, DM)], rawb.at[t, pl.ds(k0, n), :])

    cp_ch = []
    for c in range(NCH):
        w = (wq_hbm, wk_hbm, wv_hbm)[c // 2]
        cp_ch.append(cp(_rows(w, (c % 2) * GPC * RG, GPC * RG), _rows(rawa, c * GPC * RG, GPC * RG)))
        cp_ch.append(cp(_rows(wo_hbm, c * WOR, WOR), _rows(rawo, c * WOR, WOR)))
    sem_x = nsem[0]
    cp_xbs = [cp_xb(6 + 2 * c, 2) for c in range(5)]
    cp_worest = cp(_rows(wo_hbm, NCH * WOR, WOREST), _rows(rawo, NCH * WOR, WOREST))
    cp_xb0, cp_xb1, cp_xb2, cp_xb3 = cp_xb(0, 1), cp_xb(1, 1), cp_xb(2, 1), cp_xb(3, 3)
    KVQ, KQV = (1, 2, 0), (1, 0, 2)
    cp_w0 = [cp_wb(KQV[0], 0, DM // 4), cp_wb(KQV[0], DM // 4, DM // 4)]
    cp_wp = [None] + [cp_wb(KQV[h // 2], (h % 2) * (DM // 2), DM // 2) for h in range(1, 6)]
    cp_wob = cp(wob_hbm, rawob.at[:, pl.ds(0, DM)])
    cp_xa = cp(xa_hbm, _rows(xa, 0, S))
    cp_m0 = cp(mem0_hbm, _rows(ha, LA, MEM))
    assert nsem[0] == NSEM
    order = cp_w0 + [cp_xb0, cp_xb1] + cp_wp[1:5] + [cp_xb2, cp_wp[5], cp_xb3]
    for c in range(NCH):
        order += cp_ch[2 * c:2 * c + 2] + cp_xbs[c:c + 1] + ([cp_wob] if c == 0 else [])
    order += [cp_worest, cp_m0, cp_xa]
    for c in order:
        c.start()

    def wait_like(dst, s):
        pltpu.make_async_copy(dst, dst, sem.at[s]).wait()

    def a_out_start(r0, n):
        r0 = pl.multiple_of(r0, 8)
        pltpu.make_async_copy(_rows(outa, r0, n), out_hbm.at[pl.ds(r0, n), pl.ds(0, DM)],
                              sem_out.at[0]).start()

    def b_out_start(r0, n):
        pltpu.make_async_copy(_rows(outb, r0, n), out_hbm.at[pl.ds(r0, n), pl.ds(DM, DM)],
                              sem_out.at[1]).start()

    def zeros_vec():
        return jnp.full((8, 128), zero[0], i32).astype(u32)

    def tied(w, zvec, *vals_list):
        n = w.shape[0] // len(vals_list)
        parts = []
        for i, vals in enumerate(vals_list):
            pt = w[i * n:(i + 1) * n]
            if vals:
                tie = functools.reduce(lambda a, b: a | b, [_as_u32(x) for x in vals]) & zvec
                pt = jnp.concatenate([pt[0:n - 8], pt[n - 8:] | tie], axis=0)
            parts.append(pt)
        return jnp.concatenate(parts, axis=0)

    def gated(x, token):
        gate = _as_u32(token[8:16]) & zeros_vec()
        return pltpu.bitcast(_as_u32(x) | gate[None], f32)

    def run(dots, *job_lists, td=6):
        rel = {}
        for jobs, lo, hi, tr in job_lists:
            for i, job in enumerate(jobs):
                rel.setdefault(lo + i * (hi - lo) // len(jobs) - 1, []).append((job, tr))
        due = {}

        def fire(i, y):
            for job, tr in rel.get(i, []):
                vals = job(None if y is None else y[tr:tr + 16])
                if vals:
                    due.setdefault(min(i + td, len(dots) - 1), []).extend(vals)

        fire(-1, None)
        for i, th in enumerate(dots):
            fire(i, th(due.pop(i, [])))

    def prep_qkv(t, kbs):
        for kb_ in kbs:
            for ch in range(8):
                at = _as_u32(rawb[t, kb_ * 128:(kb_ + 1) * 128, ch * 128:(ch + 1) * 128].T)
                for pr in range(2):
                    lo, hi = _interleave(at[pr * 32:pr * 32 + 16], at[pr * 32 + 16:pr * 32 + 32])
                    wt[t * 8 + kb_, pl.ds(ch * 2 + pr, 16, stride=2 * DP), :] = lo
                    wt[t * 8 + kb_, pl.ds(DP + ch * 2 + pr, 16, stride=2 * DP), :] = hi

    def prep_wo_job(src_col, j, hq):
        def job(token):
            rawob[0:16, DM + 128:DM + 256] = token.astype(bf16)
            dst = wos.at[j]
            for hp in range(4 * hq, 4 * hq + 4):
                src = _as_u32(rawob[hp * 64:(hp + 1) * 64, pl.ds(src_col, 128)])
                lo, hi = _interleave(src[0:16], src[16:32])
                dst[pl.ds(hp, 16, stride=2 * DP), :] = lo
                dst[pl.ds(DP + hp, 16, stride=2 * DP), :] = hi
        return job

    def repack_job(src0, dst0, half):
        def job(token):
            rawa[pl.ds(RAWA_PAD + RG, 16), :] = token.astype(bf16)
            dst = _rows(wa, dst0, TREG + TPAD)
            for ii in range(half * 4, half * 4 + 4):
                src = _as_u32(_rows(rawa, src0, RG)[ii * 64:(ii + 1) * 64, :])
                lo, hi = _interleave(src[0:16], src[16:32])
                dst[pl.ds(ii, 16, stride=2 * TP), :] = lo
                dst[pl.ds(ii + TP, 16, stride=2 * TP), :] = hi
        return job

    def wocopy_job(src0, dst0):
        def job(token):
            if token is not None:
                rawo[pl.ds(RAWO_PAD + 32, 16), 0:128] = token.astype(bf16)
            v = _as_u32(rawo[pl.ds(src0, 32), :])
            woa[:, pl.ds(dst0, 16), :] = jnp.stack([v[:, j * 128:(j + 1) * 128] for j in range(8)])
        return job

    def chunk_jobs(it):
        c = jnp.maximum(it - 1, 0)
        ja, jo, jw = [], [], []
        for i in range(GPC):
            src0 = pl.multiple_of(jnp.where(it > 0, (c * GPC + i) * RG, RAWA_PAD), RG)
            dst0 = pl.multiple_of((c // 2) * TREG + ((c % 2) * GPC + i) * 8, 8)
            ja += [repack_job(src0, dst0, 0), repack_job(src0, dst0, 1)]
        for i in range(WOR // 32):
            src0 = pl.multiple_of(jnp.where(it > 0, c * WOR + i * 32, RAWO_PAD), 32)
            jo.append(wocopy_job(src0, pl.multiple_of(c * (WOR // 2) + i * 16, 16)))
        for i in range(2):
            j = jnp.clip(2 * (it - 2) + i, 0, 7)
            src_col = pl.multiple_of(jnp.where(it > 1, j * 128, DM), 128)
            jw += [prep_wo_job(src_col, j, hq) for hq in range(4)]
        half = lambda js, h: js[h * len(js) // 2:(h + 1) * len(js) // 2]
        return [half(ja, h) + half(jo, h) + half(jw, h) for h in range(2)]

    def xcvt_jobs(r0, p):
        def mk(i):
            def job(token):
                xsb[p][i * 8:(i + 1) * 8, :] = _as_u32(xb[pl.ds(pl.multiple_of(r0 + i * 16, 16), 16), :])
            return job
        return [mk(i) for i in range(SB // 16)]

    def xcvt(r0, p):
        for job in xcvt_jobs(r0, p):
            job(None)

    scale_b = (DM // HB) ** -0.5

    def b_proj_dots(p, ts, half=None):
        kbs = range(8) if half is None else range(4 * half, 4 * half + 4)

        def mk(t, c):
            def th(ties):
                x = _as_bf16(xsb[p][:, kbs[0] * 128:(kbs[-1] + 1) * 128])
                wv = jnp.concatenate([wt[t * 8 + kbs[0]:t * 8 + kbs[-1] + 1, pl.ds((4 * c + dd) * DP, 16), :]
                                      for dd in range(4)], axis=1)
                tiles = [wv[i] for i in range(len(kbs))]
                if ties:
                    tiles[-1] = tied(tiles[-1], zeros_vec(), ties)
                y = lax.dot_general(x, _as_bf16(jnp.concatenate(tiles, axis=1)), _NT,
                                    preferred_element_type=f32)
                if t == 0:
                    qbuf[p][c] = y + qbuf[p][c] if half == 1 else y
                else:
                    g = kbuf if t == 1 else vbuf
                    if half != 0:
                        g[p][c, 0:HALO, :] = g[1 - p][c, SB:SB + HALO, :]
                    g[p][c, HALO:HALO + SB, :] = y + g[p][c, HALO:HALO + SB, :] if half == 1 else y
                return y
            return th
        return [mk(t, c) for t in ts for c in range(8)]

    def wos_all():
        return jnp.concatenate([wos[:, pl.ds(d * DP, 16), :] for d in range(HB)], axis=1)

    def b_out_dots(r0):
        w = []

        def mk(j):
            def th(ties):
                if not w:
                    w.append(wos_all())
                o = _as_bf16(oball[r0 // 2:(r0 + SB) // 2, :])
                y = jnp.dot(o, _as_bf16(w[0][j]), preferred_element_type=f32)
                outb[pl.ds(r0, SB), j * 128:(j + 1) * 128] = y.astype(bf16)
                return y
            return th
        return [mk(j) for j in range(8)]

    def b_attn_qk(p, rb, first, token):
        b0 = rb * RB
        q = qbuf[p][:, b0:b0 + RB, :]
        if token is not None:
            q = gated(q, token)
        acc = [jnp.sum(q * kbuf[p][:, pl.ds(HALO + b0 - DIL * w, RB), :], axis=0) for w in range(NW)]
        a = jnp.stack(acc)
        a = a + pltpu.roll(a, 64, 2)
        a = a + pltpu.roll(a, 32, 2)
        a = a * (scale_b * LOG2E)
        if first and b0 < DIL * (NW - 1):
            row = b0 + lax.broadcasted_iota(i32, (NW, RB, 128), 1)
            a = jnp.where(row >= DIL * lax.broadcasted_iota(i32, (NW, RB, 128), 0), a, NEG * LOG2E)
        e = jnp.exp2(a - jnp.max(a, axis=0)[None])
        e = e * _recip(jnp.sum(e, axis=0))[None]
        return [e[w] for w in range(NW)]

    def b_attn_pv(p, rb, r0, ps):
        b0 = rb * RB
        dst = _rows(oball, pl.multiple_of(r0 // 2, SB // 2), SB // 2)
        g = 4
        outs = []
        for c0 in range(0, 8, g):
            o = _sum([ps[w][None] * vbuf[p][c0:c0 + g, pl.ds(HALO + b0 - DIL * w, RB), :] for w in range(NW)])
            outs += [o[c] for c in range(g)]
        dst[pl.ds(b0 // 2, RB // 2), :] = _as_u32(jnp.concatenate(outs, axis=1).astype(bf16))
        return outs

    def attn_jobs(p, r0):
        def mk(rb):
            return lambda token: b_attn_pv(p, rb, r0, b_attn_qk(p, rb, False, token))
        return [mk(rb) for rb in range(NRB)]

    z8 = pl.multiple_of(zero[0], 8)
    keep = jnp.zeros((8, 128), u32)
    qkvb[0, 0:8, :] = keep
    keep = keep | qkvb[zero[0], 0:8, :]
    for ref in (oca, ocb, obs):
        ref[0:8, 0:128] = jnp.zeros((8, 128), u32)
        keep = keep | ref[pl.ds(z8, 8), 0:128]
    for ref in (ex, df, sv):
        ref[0] = jnp.zeros((8, 128), f32)
        keep = keep | _as_u32(ref[zero[0]])
    part[0:8, 0:128] = jnp.zeros((8, 128), f32)
    keep = keep | _as_u32(part[pl.ds(z8, 8), 0:128])
    outa[0:16, 0:128] = _as_bf16(keep)
    rawa[pl.ds(RAWA_PAD, RG), :] = jnp.zeros((RG, DH), bf16)
    rawo[pl.ds(RAWO_PAD, 32), :] = jnp.zeros((32, DM), bf16)
    rawob[:, DM:DM + 128] = jnp.zeros((DM, 128), bf16)

    def phase_b():
        for i in range(2):
            cp_w0[i].wait()
            prep_qkv(KQV[0], range(2 * i, 2 * i + 2))
        cp_xb0.wait()
        xcvt(0, 0)
        run(b_proj_dots(0, KQV[0:1], 0))
        cp_xb1.wait()
        xcvt(SB, 1)
        NQ4 = 8
        for h in range(1, 6):
            cp_wp[h].wait()
            if h == 5:
                cp_xb2.wait()
            t0, t1 = KQV[(h - 1) // 2], KQV[h // 2]
            prep_qkv(t1, range(4 * (h % 2), 4 * (h % 2) + 4))
            dots = b_proj_dots(1, (t0,), (h - 1) % 2) + b_proj_dots(0, (t1,), h % 2)
            if h >= 4:
                def qk_job(rb):
                    def job(token):
                        ps_ = b_attn_qk(0, rb, True, token)
                        qb0[:, rb * RB:(rb + 1) * RB, :] = jnp.stack(ps_)
                        return ps_
                    return job
                rbs = range(NQ4) if h == 4 else range(NQ4, NRB)
                run(dots, ([qk_job(rb) for rb in rbs], 4, 12, 112), td=6)
            else:
                run(dots)
            if h == 5:
                vb0[:, 0:HALO, :] = jnp.broadcast_to(vb0[:, HALO:HALO + 1, :], (8, HALO, 128))

                def pv_job(rb):
                    def job(token):
                        ps_ = qb0[:, rb * RB:(rb + 1) * RB, :]
                        if token is not None:
                            ps_ = gated(ps_, token)
                        b_attn_pv(0, rb, 0, [ps_[w] for w in range(NW)])
                    return job
                xcvt(2 * SB, 0)
                pj = [pv_job(rb) for rb in range(NRB)]
                run(b_proj_dots(1, (t1,), 1), (pj[0::2], 0, 7, 48),
                    (pj[1::2], 0, 7, 112))
        cp_xb3.wait()

        def b_step(p, r_attn, r_next, side):
            run(b_proj_dots(p, KVQ),
                (attn_jobs(1 - p, r_attn), 1, 21, 112),
                (side[0::2], 1, 24, 0), (side[1::2], 1, 24, 48),
                (xcvt_jobs(r_next, 1 - p), 0, 20, 0))

        def b_body(it, carry):
            @pl.when(it == 2)
            def _():
                cp_wob.wait()

            @pl.when(jnp.logical_and(it > 0, it <= 5))
            def _():
                wait_like(_rows(xb, pl.multiple_of((4 + 2 * it) * SB, 2 * SB), 2 * SB), sem_x + it - 1)

            @pl.when(it > 0)
            def _():
                c = it - 1
                wait_like(_rows(rawa, pl.multiple_of(c * (GPC * RG), GPC * RG), GPC * RG), 2 * c)
                wait_like(_rows(rawo, pl.multiple_of(c * WOR, 128), WOR), 2 * c + 1)

            r0 = pl.multiple_of((2 * it + 2) * SB, 2 * SB)
            side = chunk_jobs(it)
            b_step(0, r0 - SB, r0 + SB, side[0])
            b_step(1, r0, jnp.minimum(r0 + 2 * SB, S - SB), side[1])
            return carry

        lax.fori_loop(0, NSTEP // 2 - 1, b_body, 0)
        cp_worest.wait()
        cp_m0.wait()
        cp_xa.wait()
        jo = [wocopy_job(NCH * WOR + i * 32, NCH * WOR // 2 + i * 16) for i in range(WOREST // 32)]
        dots = sum([b_out_dots(r) for r in range(NIT * MB, S, SB)], [])
        run(dots, (attn_jobs(1, S - SB), 0, len(dots) - 11, 112), (jo, 0, 0, 0))

    phase_b()
    b_out_start(NIT * MB, S - NIT * MB)

    scale_a = DH ** -0.5
    qscale = scale_a * LOG2E
    k1 = SPLIT * DH
    tri = lax.broadcasted_iota(i32, (8, 8, 128), 1) >= lax.broadcasted_iota(i32, (8, 8, 128), 0)

    def masks(nv):
        qr = LA - 8 * nv
        r = lax.broadcasted_iota(i32, (2 * qr, 2 * LA), 0)
        c = lax.broadcasted_iota(i32, (2 * qr, 2 * LA), 1)
        same = (r >= qr) == (c >= LA)
        rr = jnp.where(r >= qr, r - qr, r) + 8 * nv
        cc = jnp.where(c >= LA, c - LA, c)
        valid = same & ((cc >= SEG) | (rr >= SEG) | (cc <= rr))
        return valid, jnp.where(same, NEG, -jnp.inf).astype(f32)

    def nvof(which, t):
        return NVS[which] + (1 if which == 1 and t >= LT0 else 0)

    msk = {nv: masks(nv) for nv in NVS}

    def bc8(a):
        return jnp.concatenate([jnp.broadcast_to(a[j:j + 1], (8, 128)) for j in range(8)],
                               axis=0).reshape(8, 8, 128)

    def vpu_part(q, k8, v8, causal, prev):
        s_ = jnp.broadcast_to(jnp.sum(q[None] * k8, axis=-1, keepdims=True), (8, 8, 128))
        if causal:
            s_ = jnp.where(tri, s_, NEG * LOG2E)
        m = jnp.max(s_, axis=0)
        if prev is not None:
            m = jnp.maximum(m, prev[0])
        e = jnp.exp2(s_ - m[None])
        l = jnp.sum(e, axis=0)
        o = jnp.sum(e * v8, axis=0)
        if prev is not None:
            al = jnp.exp2(prev[0] - m)
            l = l + prev[1] * al
            o = o + prev[2] * al
        return m, l, o

    def stage(it):
        r0 = pl.multiple_of(it * 64, 64)
        ha[0:40, :] = xa[pl.ds(r0, 40), :]
        hb[8:32, :] = xa[pl.ds(r0 + 40, 24), :]
        obs[...] = oball[pl.ds(pl.multiple_of(it * (MB // 2), 8), MB // 2), :]

    def segment(which, it, r0, rb0):
        h_ref, oc_ref = (ha, oca) if which == 0 else (hb, ocb)
        nrow_o = 32 if which == 0 else 48
        h = h_ref[...]
        zvec = zeros_vec()
        so = (18, 15)[which]
        scp = (10, 13)[which]
        pvp = (20, 25)[which]
        assert pvp + 6 * (SPLIT // 2 - 1) <= 6 * NP
        ov, slots, ps, bacc, pre, late, merges = {}, {}, {}, [], {}, [], []

        LS, LU, LD = -4, 23, 7
        nlate = sum(2 * (g + 2) for t in range(NP) for g in range(NVS[which], nvof(which, t)))
        lrel = {}

        def fire(n, y):
            for i, job in enumerate(lrel.pop(n, [])):
                r_ = (0, y.shape[0] - 8, 16)[i % 3]
                vals = job(_as_u32(y[r_:r_ + 8]) & zvec)
                if n + LD < 6 * NP + SPLIT:
                    slots.setdefault(2 * (n + LD) + i % 2, []).extend(vals)

        def wa_tile(hd, t, k0, kn):
            return wa[pl.ds(t * TREG + hd * TP + k0 // 2, kn // 2), :]

        KH = DM // 2
        if which == 1:
            wb = wos_all()
            for hd in range(2):
                for t in range(3):
                    pre[hd, t] = jnp.dot(h[:, :KH], _as_bf16(wa_tile(hd, t, 0, KH)), preferred_element_type=f32)

        def proj(hd, t, ties):
            if (hd, t) in pre:
                y = jnp.dot(h[:, KH:], _as_bf16(wa_tile(hd, t, KH, KH)), preferred_element_type=f32)
                y = y + pre.pop((hd, t))
            else:
                y = jnp.dot(h, _as_bf16(tied(wa_tile(hd, t, 0, DM), zvec, *ties)), preferred_element_type=f32)
            if which == 0:
                ex[t * HA + hd] = y[32:40]
                return jnp.concatenate([y[0:32], y[40:48]], axis=0)
            return jnp.concatenate([ex[t * HA + hd], y[8:32], y[0:8]], axis=0)

        def vpu_jobs(t, ys):
            out = []
            for e in range(2):
                hd = 2 * t + e
                q, k, v = ys[3 * e:3 * e + 3]
                ov[hd] = []
                cache = {}

                def blk(b0):
                    if b0 not in cache:
                        cache[b0] = bc8(k[b0:b0 + 8]), bc8(v[b0:b0 + 8])
                    return cache[b0]

                for g in range(NVS[which]):
                    q0 = q[8 * g:8 * g + 8] * qscale
                    if which == 1 and g == 0:
                        st = [sv[i * HA + hd] for i in range(3)]
                    else:
                        st = None
                        for b in range(g, -1, -1):
                            st = vpu_part(q0, *blk(8 * b), b == g, st)
                            out.append(list(st[1:]))
                    _, l, o = vpu_part(q0, *blk(SEG), False, st)
                    ov[hd].append(o * _recip(l))
                    out.append([ov[hd][-1]])
                for g in range(NVS[which], nvof(which, t)):
                    st = [None]
                    for b0 in [8 * b for b in range(g, -1, -1)] + [SEG]:
                        def job(tok, hd=hd, g=g, b0=b0, st=st, q=q, k=k, v=v):
                            gate = lambda x: pltpu.bitcast(_as_u32(x) | tok, f32)
                            st[0] = vpu_part(gate(q[8 * g:8 * g + 8]) * qscale, bc8(gate(k[b0:b0 + 8])),
                                             bc8(gate(v[b0:b0 + 8])), b0 == 8 * g, st[0])
                            if b0 != SEG:
                                return list(st[0][1:])
                            ov[hd].append(st[0][2] * _recip(st[0][1]))
                            return [ov[hd][-1]]
                        lrel.setdefault(6 * NP + LS + len(late) * LU // nlate, []).append(job)
                        late.append(job)
                if which == 0:
                    st = vpu_part(ex[hd] * qscale, bc8(ex[HA + hd]), bc8(ex[2 * HA + hd]), True, None)
                    for i in range(3):
                        sv[i * HA + hd] = st[i]
                    out.append(list(st[1:]))
            for i, jb in enumerate(out):
                slots.setdefault(12 * t + so + (2 * i + 1) * 6 // len(out), []).extend(jb)

        def bout_half(i):
            j, half = i // 2, i % 2
            o = _as_bf16(obs[:, half * KH:(half + 1) * KH])
            y = jnp.dot(o, _as_bf16(wb[j, half * 256:(half + 1) * 256]), preferred_element_type=f32)
            if half == 0:
                bacc.append(y)
            else:
                outb[pl.ds(rb0, MB), j * 128:(j + 1) * 128] = (y + bacc.pop()).astype(bf16)

        def scores(p_):
            if which == 1:
                bout_half(p_)
            q3 = (which * NP + p_) * 3
            qr = LA - 8 * nvof(which, p_)
            valid, fill = msk[nvof(which, p_)]
            sc = lax.dot_general(_as_bf16(qkvb[q3, 0:qr, :]), _as_bf16(qkvb[q3 + 1]), _NT,
                                 preferred_element_type=f32)
            sc = jnp.where(valid, sc * scale_a, fill)
            p = jnp.exp(sc - jnp.max(sc, axis=-1, keepdims=True))
            ps[p_] = (p * _recip(jnp.sum(p, axis=-1, keepdims=True))).astype(bf16)

        def pv(p_):
            o = jnp.dot(ps.pop(p_), _as_bf16(qkvb[(which * NP + p_) * 3 + 2]), preferred_element_type=f32)
            qr = LA - 8 * nvof(which, p_)

            def merge():
                for e in range(2):
                    hd = 2 * p_ + e
                    oh = jnp.concatenate(ov.pop(hd) + [o[qr * e:qr * e + qr]], axis=0)
                    if which == 0:
                        df[hd] = oh[24:32]
                        z = jnp.concatenate([oh[32:40], oh[0:24]], axis=0)
                    else:
                        z = jnp.concatenate([oh, df[hd]], axis=0)
                    oc_ref[:, hd * DH:(hd + 1) * DH] = _as_u32(z.astype(bf16))
            if nvof(which, p_) > NVS[which]:
                merges.append(merge)
            else:
                merge()

        def after(n):
            for pos, fn in ((pvp, pv), (scp, scores)):
                if (n - pos) % 6 == 0 and 0 <= (n - pos) // 6 < NP:
                    fn((n - pos) // 6)

        for t in range(NP):
            ys = []
            for m in range(6):
                n = 6 * t + m
                ys.append(proj(2 * t + m // 3, m % 3, (slots.pop(2 * n, []), slots.pop(2 * n + 1, []))))
                if m == 5:
                    q3 = (which * NP + t) * 3
                    nv = nvof(which, t)
                    qr = LA - 8 * nv
                    qkvb[q3, 0:qr, :] = _as_u32(
                        jnp.concatenate([ys[0][8 * nv:], ys[3][8 * nv:]], axis=0).astype(bf16))
                    for i in range(1, 3):
                        qkvb[q3 + i] = _as_u32(jnp.concatenate([ys[i], ys[3 + i]], axis=0).astype(bf16))
                    vpu_jobs(t, ys)
                fire(n, ys[-1][8:32])
                after(n + 1)
        n = 6 * NP
        if not late:
            for j in range(8):
                ties = [sum([slots.pop(2 * n + i, []) for i in range(lo, lo + 3)], []) for lo in (0, 3)]
                part[0:nrow_o, j * 128:(j + 1) * 128] = jnp.dot(
                    _as_bf16(oc_ref[:, :k1]), _as_bf16(tied(woa[j, :k1 // 2, :], zvec, *ties)),
                    preferred_element_type=f32)
                for i in range(3):
                    n += 1
                    after(n)
        else:
            kc0 = LT0 // 4
            units = [(j, kc) for j in range(8) for kc in range(kc0)]
            units += [(j, kc) for kc in range(kc0, SPLIT // 8) for j in range(8)]
            for u, (j, kc) in enumerate(units):
                k0 = kc * DM
                cs = slice(j * 128, (j + 1) * 128)
                if kc >= kc0 and j == 0:
                    for p_ in range(4 * kc, 4 * kc + 4):
                        if p_ >= LT0:
                            merges.pop(0)()
                y = jnp.dot(_as_bf16(oc_ref[:, k0:k0 + DM]),
                            _as_bf16(tied(woa[j, k0 // 2:(k0 + DM) // 2, :], zvec,
                                          slots.pop(2 * n, []), slots.pop(2 * n + 1, []))),
                            preferred_element_type=f32)
                fire(n, y)
                acc = y if kc == 0 else (acc + y if kc < kc0 else part[0:nrow_o, cs] + y)
                if kc >= kc0 - 1:
                    part[0:nrow_o, cs] = acc
                n += 1
                after(n)
            for merge in merges:
                merge()
        assert not (ps or ov or slots or bacc or pre or lrel)
        if which == 1:
            @pl.when(it % OG == OG - 1)
            def _():
                b_out_start(pl.multiple_of(rb0 - (OG - 1) * MB, 16), OG * MB)
        o2 = _as_bf16(oc_ref[:, k1:])
        for j in range(8):
            cs = slice(j * 128, (j + 1) * 128)
            y = part[0:nrow_o, cs] + jnp.dot(o2, _as_bf16(woa[j, k1 // 2:, :]), preferred_element_type=f32)
            if which == 0:
                hb[0:8, cs] = y[0:8].astype(bf16)
                outa[pl.ds(r0, 24), cs] = y[8:32].astype(bf16)
            else:
                outa[pl.ds(r0 + 32, 32), cs] = y[0:32].astype(bf16)
                ha[40:48, cs] = y[32:40].astype(bf16)
                outa[pl.ds(r0 + 24, 8), cs] = y[40:48].astype(bf16)
                if j == 6:
                    xa[S:S + 16, 0:128] = y[0:16].astype(bf16)
                    oball[S // 2:S // 2 + 8, 0:128] = _as_u32(y[0:8])
                    stage(jnp.minimum(it + 1, NIT - 1))

    def a_body(it, carry):
        r0 = pl.multiple_of(it * 64, 64)
        rb0 = pl.multiple_of(it * MB, 16)
        segment(0, it, r0, rb0)

        @pl.when(it == OG - 1)
        def _():
            a_out_start(0, 64 * OG - 40)

        @pl.when(jnp.logical_and(it % OG == OG - 1, it >= OG))
        def _():
            a_out_start(r0 + 24 - 64 * OG, 64 * OG)

        segment(1, it, r0, rb0)
        return carry

    stage(0)
    lax.fori_loop(0, NIT, a_body, 0)
    a_out_start(S - 40, 40)

    pltpu.make_async_copy(outb, out_hbm.at[:, pl.ds(DM, DM)], sem_out.at[1]).wait()
    pltpu.make_async_copy(outa, out_hbm.at[:, pl.ds(0, DM)], sem_out.at[0]).wait()


@jax.jit
def pallas_concat_heads__memory_aug_recurrent_mem_tr__sliding_local_dilated__prompt_kernel(
    A_x, A_mem0, A_Wq, A_Wk, A_Wv, A_Wo, A_seg_len, B_x, B_wqkv, B_wo,
):
    del A_seg_len
    assert A_x.shape == (1, S, DM) and B_x.shape == (1, S, DM)
    vm = pltpu.VMEM
    scratch = [
        vm((S + 16, DM), bf16), vm((S, DM), bf16),
        vm((S, DM), bf16), vm((S, DM), bf16),
        vm((RAWA_PAD + RG + 16, DH), bf16),
        vm((RAWO_PAD + 48, DM), bf16),
        vm((3, DM, DM), bf16), vm((DM, DM + 256), bf16),
        vm((3 * TREG + DM // 2 + TPAD, DH), u32),
        vm((8, HA * DH // 2, 128), u32),
        vm((24, BREG + 40, 128), u32), vm((8, BREG + 40, 128), u32),
        vm((8, SB, 128), f32), vm((8, SB, 128), f32),
        vm((8, SB + HALO, 128), f32), vm((8, SB + HALO, 128), f32),
        vm((8, SB + HALO, 128), f32), vm((8, SB + HALO, 128), f32),
        vm((SB // 2, DM), u32), vm((SB // 2, DM), u32),
        vm((S // 2 + 8, DM), u32), vm((MB // 2, DM), u32),
        vm((48, DM), bf16), vm((32, DM), bf16),
        vm((16, HA * DH), u32), vm((24, HA * DH), u32),
        vm((48, DM), f32),
        vm((3 * HA, 8, 128), f32), vm((HA, 8, 128), f32),
        vm((3 * HA, 8, 128), f32),
        vm((6 * NP, LA, 128), u32),
        pltpu.SMEM((1,), i32),
        pltpu.SemaphoreType.DMA((NSEM,)),
        pltpu.SemaphoreType.DMA((2,)),
    ]
    out = pl.pallas_call(
        _kernel,
        out_shape=jax.ShapeDtypeStruct((S, 2 * DM), bf16),
        in_specs=[pl.BlockSpec(memory_space=pl.ANY)] * 9,
        out_specs=pl.BlockSpec(memory_space=pl.ANY),
        scratch_shapes=scratch,
        compiler_params=pltpu.CompilerParams(
            vmem_limit_bytes=120 * 1024 * 1024,
            disable_bounds_checks=True,
            disable_semaphore_checks=True,
        ),
        name="concat_heads_kernel",
    )(
        A_x.reshape(S, DM), A_mem0.reshape(MEM, DM),
        A_Wq.reshape(DM * HA, DH), A_Wk.reshape(DM * HA, DH), A_Wv.reshape(DM * HA, DH),
        A_Wo.reshape(HA * DH, DM),
        B_x.reshape(S, DM), B_wqkv, B_wo,
    )
    return out.reshape(1, S, 2 * DM)
```

```python
import functools

import jax
import jax.numpy as jnp
from jax import lax
import jax.experimental.pallas as pl
import jax.experimental.pallas.tpu as pltpu

bf16, f32, u32, i32 = jnp.bfloat16, jnp.float32, jnp.uint32, jnp.int32

S, DM = 2048, 1024
HA, DH, MEM, SEG = 32, 128, 8, 32
LA = MEM + SEG
HB, NW, DIL = 32, 8, 2
HALO = 16
NEG = -1000000000.0
LOG2E = 1.4426950408889634

SB = 128
NSTEP = S // SB
RB = 8
NRB = SB // RB
TP = 514
TREG = HA * TP
TPAD = 1032
DP = 18
BREG = HB * DP
NCH = 6
GPC = 3 * (DM // 16) // NCH
RG = 16 * HA
WOR = 640
WOREST = HA * DH - NCH * WOR
RAWA_PAD = 3 * DM * HA
RAWO_PAD = HA * DH
NIT = S // (2 * SEG)
MB = 48
OG = 4
NP = HA // 2
SPLIT = 24
LATE = 14
NI = 2
NSEM = 32

_NT = (((1,), (1,)), ((), ()))


def _as_bf16(x):
    return pltpu.bitcast(x, bf16)


def _as_u32(x):
    return pltpu.bitcast(x, u32)


def _sum(xs):
    return functools.reduce(lambda a, b: a + b, xs)


def _interleave(a, b):
    lo = (a & jnp.uint32(0xFFFF)) | (b << 16)
    hi = (a >> 16) | (b & jnp.uint32(0xFFFF0000))
    return lo, hi


def _recip(x):
    r = pl.reciprocal(x, approx=True)
    return r * (2.0 - x * r)


def _rows(ref, r0, n):
    return ref.at[pl.ds(r0, n), :]


def _kernel(xa_hbm, mem0_hbm, wq_hbm, wk_hbm, wv_hbm, wo_hbm, xb_hbm, wqkvb_hbm, wob_hbm,
            out_hbm,
            xa, xb, outa, outb, rawa, rawo, rawb, rawob, wa, woa, wt, wos,
            qb0, qb1, kb0, kb1, vb0, vb1, xs0, xs1, oball, obs,
            ha, hb, oca, ocb, part, ex, df, sv, qkvb, zero,
            sem, sem_out):
    zero[0] = 0
    qbuf, kbuf, vbuf, xsb = (qb0, qb1), (kb0, kb1), (vb0, vb1), (xs0, xs1)

    nsem = [0]

    def cp(src, dst):
        c = pltpu.make_async_copy(src, dst, sem.at[nsem[0]])
        nsem[0] += 1
        return c

    def cp_xb(b0, nb):
        return cp(_rows(xb_hbm, b0 * SB, nb * SB), _rows(xb, b0 * SB, nb * SB))

    def cp_wb(t, k0, n):
        return cp(wqkvb_hbm.at[pl.ds(k0, n), pl.ds(t * DM, DM)], rawb.at[t, pl.ds(k0, n), :])

    cp_ch = []
    for c in range(NCH):
        w = (wq_hbm, wk_hbm, wv_hbm)[c // 2]
        cp_ch.append(cp(_rows(w, (c % 2) * GPC * RG, GPC * RG), _rows(rawa, c * GPC * RG, GPC * RG)))
        cp_ch.append(cp(_rows(wo_hbm, c * WOR, WOR), _rows(rawo, c * WOR, WOR)))
    sem_x = nsem[0]
    cp_xbs = [cp_xb(6 + 2 * c, 2) for c in range(5)]
    cp_worest = cp(_rows(wo_hbm, NCH * WOR, WOREST), _rows(rawo, NCH * WOR, WOREST))
    cp_xb0, cp_xb1, cp_xb2, cp_xb3 = cp_xb(0, 1), cp_xb(1, 1), cp_xb(2, 1), cp_xb(3, 3)
    KVQ, KQV = (1, 2, 0), (1, 0, 2)
    cp_w0 = [cp_wb(KQV[0], 0, DM // 4), cp_wb(KQV[0], DM // 4, DM // 4)]
    cp_wp = [None] + [cp_wb(KQV[h // 2], (h % 2) * (DM // 2), DM // 2) for h in range(1, 6)]
    cp_wob = cp(wob_hbm, rawob.at[:, pl.ds(0, DM)])
    cp_xa = cp(xa_hbm, _rows(xa, 0, S))
    cp_m0 = cp(mem0_hbm, _rows(ha, LA, MEM))
    assert nsem[0] == NSEM
    order = cp_w0 + [cp_xb0, cp_xb1] + cp_wp[1:5] + [cp_xb2, cp_wp[5], cp_xb3]
    for c in range(NCH):
        order += cp_ch[2 * c:2 * c + 2] + cp_xbs[c:c + 1] + ([cp_wob] if c == 0 else [])
    order += [cp_worest, cp_m0, cp_xa]
    for c in order:
        c.start()

    def wait_like(dst, s):
        pltpu.make_async_copy(dst, dst, sem.at[s]).wait()

    def a_out_start(r0, n):
        r0 = pl.multiple_of(r0, 8)
        pltpu.make_async_copy(_rows(outa, r0, n), out_hbm.at[pl.ds(r0, n), pl.ds(0, DM)],
                              sem_out.at[0]).start()

    def b_out_start(r0, n):
        pltpu.make_async_copy(_rows(outb, r0, n), out_hbm.at[pl.ds(r0, n), pl.ds(DM, DM)],
                              sem_out.at[1]).start()

    def zeros_vec():
        return jnp.full((8, 128), zero[0], i32).astype(u32)

    def tied(w, zvec, *vals_list):
        n = w.shape[0] // len(vals_list)
        parts = []
        for i, vals in enumerate(vals_list):
            pt = w[i * n:(i + 1) * n]
            if vals:
                tie = functools.reduce(lambda a, b: a | b, [_as_u32(x) for x in vals]) & zvec
                pt = jnp.concatenate([pt[0:n - 8], pt[n - 8:] | tie], axis=0)
            parts.append(pt)
        return jnp.concatenate(parts, axis=0)

    def gated(x, token):
        gate = _as_u32(token[8:16]) & zeros_vec()
        return pltpu.bitcast(_as_u32(x) | gate[None], f32)

    def run(dots, *job_lists, td=6):
        rel = {}
        for jobs, lo, hi, tr in job_lists:
            for i, job in enumerate(jobs):
                rel.setdefault(lo + i * (hi - lo) // len(jobs) - 1, []).append((job, tr))
        due = {}

        def fire(i, y):
            for job, tr in rel.get(i, []):
                vals = job(None if y is None else y[tr:tr + 16])
                if vals:
                    due.setdefault(min(i + td, len(dots) - 1), []).extend(vals)

        fire(-1, None)
        for i, th in enumerate(dots):
            fire(i, th(due.pop(i, [])))

    def prep_qkv(t, kbs):
        for kb_ in kbs:
            for ch in range(8):
                at = _as_u32(rawb[t, kb_ * 128:(kb_ + 1) * 128, ch * 128:(ch + 1) * 128].T)
                for pr in range(2):
                    lo, hi = _interleave(at[pr * 32:pr * 32 + 16], at[pr * 32 + 16:pr * 32 + 32])
                    wt[t * 8 + kb_, pl.ds(ch * 2 + pr, 16, stride=2 * DP), :] = lo
                    wt[t * 8 + kb_, pl.ds(DP + ch * 2 + pr, 16, stride=2 * DP), :] = hi

    def prep_wo_job(src_col, j, hq):
        def job(token):
            rawob[0:16, DM + 128:DM + 256] = token.astype(bf16)
            dst = wos.at[j]
            for hp in range(4 * hq, 4 * hq + 4):
                src = _as_u32(rawob[hp * 64:(hp + 1) * 64, pl.ds(src_col, 128)])
                lo, hi = _interleave(src[0:16], src[16:32])
                dst[pl.ds(hp, 16, stride=2 * DP), :] = lo
                dst[pl.ds(DP + hp, 16, stride=2 * DP), :] = hi
        return job

    def repack_job(src0, dst0, half):
        def job(token):
            rawa[pl.ds(RAWA_PAD + RG, 16), :] = token.astype(bf16)
            dst = _rows(wa, dst0, TREG + TPAD)
            for ii in range(half * 4, half * 4 + 4):
                src = _as_u32(_rows(rawa, src0, RG)[ii * 64:(ii + 1) * 64, :])
                lo, hi = _interleave(src[0:16], src[16:32])
                dst[pl.ds(ii, 16, stride=2 * TP), :] = lo
                dst[pl.ds(ii + TP, 16, stride=2 * TP), :] = hi
        return job

    def wocopy_job(src0, dst0):
        def job(token):
            if token is not None:
                rawo[pl.ds(RAWO_PAD + 32, 16), 0:128] = token.astype(bf16)
            v = _as_u32(rawo[pl.ds(src0, 32), :])
            woa[:, pl.ds(dst0, 16), :] = jnp.stack([v[:, j * 128:(j + 1) * 128] for j in range(8)])
        return job

    def chunk_jobs(it):
        c = jnp.maximum(it - 1, 0)
        ja, jo, jw = [], [], []
        for i in range(GPC):
            src0 = pl.multiple_of(jnp.where(it > 0, (c * GPC + i) * RG, RAWA_PAD), RG)
            dst0 = pl.multiple_of((c // 2) * TREG + ((c % 2) * GPC + i) * 8, 8)
            ja += [repack_job(src0, dst0, 0), repack_job(src0, dst0, 1)]
        for i in range(WOR // 32):
            src0 = pl.multiple_of(jnp.where(it > 0, c * WOR + i * 32, RAWO_PAD), 32)
            jo.append(wocopy_job(src0, pl.multiple_of(c * (WOR // 2) + i * 16, 16)))
        for i in range(2):
            j = jnp.clip(2 * (it - 2) + i, 0, 7)
            src_col = pl.multiple_of(jnp.where(it > 1, j * 128, DM), 128)
            jw += [prep_wo_job(src_col, j, hq) for hq in range(4)]
        half = lambda js, h: js[h * len(js) // 2:(h + 1) * len(js) // 2]
        return [half(ja, h) + half(jo, h) + half(jw, h) for h in range(2)]

    def xcvt_jobs(r0, p):
        def mk(i):
            def job(token):
                xsb[p][i * 8:(i + 1) * 8, :] = _as_u32(xb[pl.ds(pl.multiple_of(r0 + i * 16, 16), 16), :])
            return job
        return [mk(i) for i in range(SB // 16)]

    def xcvt(r0, p):
        for job in xcvt_jobs(r0, p):
            job(None)

    scale_b = (DM // HB) ** -0.5

    def b_proj_dots(p, ts, half=None):
        kbs = range(8) if half is None else range(4 * half, 4 * half + 4)

        def mk(t, c):
            def th(ties):
                x = _as_bf16(xsb[p][:, kbs[0] * 128:(kbs[-1] + 1) * 128])
                wv = jnp.concatenate([wt[t * 8 + kbs[0]:t * 8 + kbs[-1] + 1, pl.ds((4 * c + dd) * DP, 16), :]
                                      for dd in range(4)], axis=1)
                tiles = [wv[i] for i in range(len(kbs))]
                if ties:
                    tiles[-1] = tied(tiles[-1], zeros_vec(), ties)
                y = lax.dot_general(x, _as_bf16(jnp.concatenate(tiles, axis=1)), _NT,
                                    preferred_element_type=f32)
                if t == 0:
                    qbuf[p][c] = y + qbuf[p][c] if half == 1 else y
                else:
                    g = kbuf if t == 1 else vbuf
                    if half != 0:
                        g[p][c, 0:HALO, :] = g[1 - p][c, SB:SB + HALO, :]
                    g[p][c, HALO:HALO + SB, :] = y + g[p][c, HALO:HALO + SB, :] if half == 1 else y
                return y
            return th
        return [mk(t, c) for t in ts for c in range(8)]

    def wos_all():
        return jnp.concatenate([wos[:, pl.ds(d * DP, 16), :] for d in range(HB)], axis=1)

    def b_out_dots(r0):
        w = []

        def mk(j):
            def th(ties):
                if not w:
                    w.append(wos_all())
                o = _as_bf16(oball[r0 // 2:(r0 + SB) // 2, :])
                y = jnp.dot(o, _as_bf16(w[0][j]), preferred_element_type=f32)
                outb[pl.ds(r0, SB), j * 128:(j + 1) * 128] = y.astype(bf16)
                return y
            return th
        return [mk(j) for j in range(8)]

    def b_attn_qk(p, rb, first, token):
        b0 = rb * RB
        q = qbuf[p][:, b0:b0 + RB, :]
        if token is not None:
            q = gated(q, token)
        acc = [jnp.sum(q * kbuf[p][:, pl.ds(HALO + b0 - DIL * w, RB), :], axis=0) for w in range(NW)]
        a = jnp.stack(acc)
        a = a + pltpu.roll(a, 64, 2)
        a = a + pltpu.roll(a, 32, 2)
        a = a * (scale_b * LOG2E)
        if first and b0 < DIL * (NW - 1):
            row = b0 + lax.broadcasted_iota(i32, (NW, RB, 128), 1)
            a = jnp.where(row >= DIL * lax.broadcasted_iota(i32, (NW, RB, 128), 0), a, NEG * LOG2E)
        e = jnp.exp2(a - jnp.max(a, axis=0)[None])
        e = e * _recip(jnp.sum(e, axis=0))[None]
        return [e[w] for w in range(NW)]

    def b_attn_pv(p, rb, r0, ps):
        b0 = rb * RB
        dst = _rows(oball, pl.multiple_of(r0 // 2, SB // 2), SB // 2)
        g = 4
        outs = []
        for c0 in range(0, 8, g):
            o = _sum([ps[w][None] * vbuf[p][c0:c0 + g, pl.ds(HALO + b0 - DIL * w, RB), :] for w in range(NW)])
            outs += [o[c] for c in range(g)]
        dst[pl.ds(b0 // 2, RB // 2), :] = _as_u32(jnp.concatenate(outs, axis=1).astype(bf16))
        return outs

    def attn_jobs(p, r0):
        def mk(rb):
            return lambda token: b_attn_pv(p, rb, r0, b_attn_qk(p, rb, False, token))
        return [mk(rb) for rb in range(NRB)]

    z8 = pl.multiple_of(zero[0], 8)
    keep = jnp.zeros((8, 128), u32)
    qkvb[0, 0:8, :] = keep
    keep = keep | qkvb[zero[0], 0:8, :]
    for ref in (oca, ocb, obs):
        ref[0:8, 0:128] = jnp.zeros((8, 128), u32)
        keep = keep | ref[pl.ds(z8, 8), 0:128]
    for ref in (ex, df, sv):
        ref[0] = jnp.zeros((8, 128), f32)
        keep = keep | _as_u32(ref[zero[0]])
    part[0:8, 0:128] = jnp.zeros((8, 128), f32)
    keep = keep | _as_u32(part[pl.ds(z8, 8), 0:128])
    outa[0:16, 0:128] = _as_bf16(keep)
    rawa[pl.ds(RAWA_PAD, RG), :] = jnp.zeros((RG, DH), bf16)
    rawo[pl.ds(RAWO_PAD, 32), :] = jnp.zeros((32, DM), bf16)
    rawob[:, DM:DM + 128] = jnp.zeros((DM, 128), bf16)

    def phase_b():
        for i in range(2):
            cp_w0[i].wait()
            prep_qkv(KQV[0], range(2 * i, 2 * i + 2))
        cp_xb0.wait()
        xcvt(0, 0)
        run(b_proj_dots(0, KQV[0:1], 0))
        cp_xb1.wait()
        xcvt(SB, 1)
        NQ4 = 8
        for h in range(1, 6):
            cp_wp[h].wait()
            if h == 5:
                cp_xb2.wait()
            t0, t1 = KQV[(h - 1) // 2], KQV[h // 2]
            prep_qkv(t1, range(4 * (h % 2), 4 * (h % 2) + 4))
            dots = b_proj_dots(1, (t0,), (h - 1) % 2) + b_proj_dots(0, (t1,), h % 2)
            if h >= 4:
                def qk_job(rb):
                    def job(token):
                        ps_ = b_attn_qk(0, rb, True, token)
                        qb0[:, rb * RB:(rb + 1) * RB, :] = jnp.stack(ps_)
                        return ps_
                    return job
                rbs = range(NQ4) if h == 4 else range(NQ4, NRB)
                run(dots, ([qk_job(rb) for rb in rbs], 4, 12, 112), td=6)
            else:
                run(dots)
            if h == 5:
                vb0[:, 0:HALO, :] = jnp.broadcast_to(vb0[:, HALO:HALO + 1, :], (8, HALO, 128))

                def pv_job(rb):
                    def job(token):
                        ps_ = qb0[:, rb * RB:(rb + 1) * RB, :]
                        if token is not None:
                            ps_ = gated(ps_, token)
                        b_attn_pv(0, rb, 0, [ps_[w] for w in range(NW)])
                    return job
                xcvt(2 * SB, 0)
                pj = [pv_job(rb) for rb in range(NRB)]
                run(b_proj_dots(1, (t1,), 1), (pj[0::2], 0, 7, 48),
                    (pj[1::2], 0, 7, 112))
        cp_xb3.wait()

        def b_step(p, r_attn, r_next, side):
            run(b_proj_dots(p, KVQ),
                (attn_jobs(1 - p, r_attn), 1, 21, 112),
                (side[0::2], 1, 24, 0), (side[1::2], 1, 24, 48),
                (xcvt_jobs(r_next, 1 - p), 0, 20, 0))

        def b_body(it, carry):
            @pl.when(it == 2)
            def _():
                cp_wob.wait()

            @pl.when(jnp.logical_and(it > 0, it <= 5))
            def _():
                wait_like(_rows(xb, pl.multiple_of((4 + 2 * it) * SB, 2 * SB), 2 * SB), sem_x + it - 1)

            @pl.when(it > 0)
            def _():
                c = it - 1
                wait_like(_rows(rawa, pl.multiple_of(c * (GPC * RG), GPC * RG), GPC * RG), 2 * c)
                wait_like(_rows(rawo, pl.multiple_of(c * WOR, 128), WOR), 2 * c + 1)

            r0 = pl.multiple_of((2 * it + 2) * SB, 2 * SB)
            side = chunk_jobs(it)
            b_step(0, r0 - SB, r0 + SB, side[0])
            b_step(1, r0, jnp.minimum(r0 + 2 * SB, S - SB), side[1])
            return carry

        lax.fori_loop(0, NSTEP // 2 - 1, b_body, 0)
        cp_worest.wait()
        cp_m0.wait()
        cp_xa.wait()
        jo = [wocopy_job(NCH * WOR + i * 32, NCH * WOR // 2 + i * 16) for i in range(WOREST // 32)]
        dots = sum([b_out_dots(r) for r in range(NIT * MB, S, SB)], [])
        run(dots, (attn_jobs(1, S - SB), 0, len(dots) - 11, 112), (jo, 0, 0, 0))

    phase_b()
    b_out_start(NIT * MB, S - NIT * MB)

    scale_a = DH ** -0.5
    qscale = scale_a * LOG2E
    k1 = SPLIT * DH
    tri = lax.broadcasted_iota(i32, (8, 8, 128), 1) >= lax.broadcasted_iota(i32, (8, 8, 128), 0)

    def masks(nv):
        qr = LA - 8 * nv
        r = lax.broadcasted_iota(i32, (2 * qr, 2 * LA), 0)
        c = lax.broadcasted_iota(i32, (2 * qr, 2 * LA), 1)
        same = (r >= qr) == (c >= LA)
        rr = jnp.where(r >= qr, r - qr, r) + 8 * nv
        cc = jnp.where(c >= LA, c - LA, c)
        valid = same & ((cc >= SEG) | (rr >= SEG) | (cc <= rr))
        return valid, jnp.where(same, NEG, -jnp.inf).astype(f32)

    def nvof(which, t):
        return 3 if which == 1 and t >= LATE else 2

    def nearly(which, t):
        return 1 if which == 1 and t >= LATE else 2

    msk = {nv: masks(nv) for nv in (2, 3)}

    def bc8(a):
        return jnp.concatenate([jnp.broadcast_to(a[j:j + 1], (8, 128)) for j in range(8)],
                               axis=0).reshape(8, 8, 128)

    def vpu_part(q, k8, v8, causal, prev):
        s_ = jnp.broadcast_to(jnp.sum(q[None] * k8, axis=-1, keepdims=True), (8, 8, 128))
        if causal:
            s_ = jnp.where(tri, s_, NEG * LOG2E)
        m = jnp.max(s_, axis=0)
        if prev is not None:
            m = jnp.maximum(m, prev[0])
        e = jnp.exp2(s_ - m[None])
        l = jnp.sum(e, axis=0)
        o = jnp.sum(e * v8, axis=0)
        if prev is not None:
            al = jnp.exp2(prev[0] - m)
            l = l + prev[1] * al
            o = o + prev[2] * al
        return m, l, o

    def stage(it):
        r0 = pl.multiple_of(it * 64, 64)
        ha[0:40, :] = xa[pl.ds(r0, 40), :]
        hb[8:32, :] = xa[pl.ds(r0 + 40, 24), :]
        obs[...] = oball[pl.ds(pl.multiple_of(it * (MB // 2), 8), MB // 2), :]

    def segment(which, it, r0, rb0):
        h_ref, oc_ref = (ha, oca) if which == 0 else (hb, ocb)
        nrow_o = 32 if which == 0 else 48
        h = h_ref[...]
        zvec = zeros_vec()
        so = (18, 19)[which]
        scp = (10, 9)[which]
        pvp = (20, 20)[which]
        c0 = NI * which
        nend = 6 * NP + SPLIT - 4 * c0
        assert 2 * LATE >= SPLIT
        ov, slots, ps, bacc, pre, late, merges = {}, {}, {}, [], {}, [], {}

        LS, LU, LD = -4, 16, 6
        nlate = sum(2 * (g + 2) for t in range(NP) for g in range(nearly(which, t), nvof(which, t)))
        lrel, done = {}, set()

        def fire(n, y):
            for i, job in enumerate(lrel.pop(n, [])):
                r_ = (0, y.shape[0] - 8, 16)[i % 3]
                vals = job(_as_u32(y[r_:r_ + 8]) & zvec)
                if n + LD < nend:
                    slots.setdefault(2 * (n + LD) + i % 2, []).extend(vals)

        def wa_tile(hd, t, k0, kn):
            return wa[pl.ds(t * TREG + hd * TP + k0 // 2, kn // 2), :]

        KH = DM // 2
        if which == 1:
            wb = wos_all()
            for hd in range(2):
                for t in range(3):
                    pre[hd, t] = jnp.dot(h[:, :KH], _as_bf16(wa_tile(hd, t, 0, KH)), preferred_element_type=f32)

        def proj(hd, t, ties):
            if (hd, t) in pre:
                y = jnp.dot(h[:, KH:], _as_bf16(wa_tile(hd, t, KH, KH)), preferred_element_type=f32)
                y = y + pre.pop((hd, t))
            else:
                y = jnp.dot(h, _as_bf16(tied(wa_tile(hd, t, 0, DM), zvec, *ties)), preferred_element_type=f32)
            if which == 0:
                ex[t * HA + hd] = y[32:40]
                return jnp.concatenate([y[0:32], y[40:48]], axis=0)
            return jnp.concatenate([ex[t * HA + hd], y[8:32], y[0:8]], axis=0)

        def vpu_jobs(t, ys):
            out = []
            for e in range(2):
                hd = 2 * t + e
                q, k, v = ys[3 * e:3 * e + 3]
                ov[hd] = []
                cache = {}

                def blk(b0):
                    if b0 not in cache:
                        cache[b0] = bc8(k[b0:b0 + 8]), bc8(v[b0:b0 + 8])
                    return cache[b0]

                for g in range(nearly(which, t)):
                    q0 = q[8 * g:8 * g + 8] * qscale
                    if which == 1 and g == 0:
                        st = [sv[i * HA + hd] for i in range(3)]
                    else:
                        st = None
                        for b in range(g, -1, -1):
                            st = vpu_part(q0, *blk(8 * b), b == g, st)
                            out.append(list(st[1:]))
                    _, l, o = vpu_part(q0, *blk(SEG), False, st)
                    ov[hd].append(o * _recip(l))
                    out.append([ov[hd][-1]])
                for g in range(nearly(which, t), nvof(which, t)):
                    st = [None]
                    for b0 in [8 * b for b in range(g, -1, -1)] + [SEG]:
                        def job(tok, hd=hd, g=g, b0=b0, st=st, q=q, k=k, v=v):
                            gate = lambda x: pltpu.bitcast(_as_u32(x) | tok, f32)
                            st[0] = vpu_part(gate(q[8 * g:8 * g + 8]) * qscale, bc8(gate(k[b0:b0 + 8])),
                                             bc8(gate(v[b0:b0 + 8])), b0 == 8 * g, st[0])
                            if b0 != SEG:
                                return list(st[0][1:])
                            ov[hd].append(st[0][2] * _recip(st[0][1]))
                            return [ov[hd][-1]]
                        lrel.setdefault(6 * NP + LS + len(late) * LU // nlate, []).append(job)
                        late.append(job)
                if which == 0:
                    st = vpu_part(ex[hd] * qscale, bc8(ex[HA + hd]), bc8(ex[2 * HA + hd]), True, None)
                    for i in range(3):
                        sv[i * HA + hd] = st[i]
                    out.append(list(st[1:]))
            for i, jb in enumerate(out):
                slots.setdefault(12 * t + so + (2 * i + 1) * 6 // len(out), []).extend(jb)

        def bout_half(i):
            j, half = i // 2, i % 2
            o = _as_bf16(obs[:, half * KH:(half + 1) * KH])
            y = jnp.dot(o, _as_bf16(wb[j, half * 256:(half + 1) * 256]), preferred_element_type=f32)
            if half == 0:
                bacc.append(y)
            else:
                outb[pl.ds(rb0, MB), j * 128:(j + 1) * 128] = (y + bacc.pop()).astype(bf16)

        def wo_early(hc, j):
            assert all(hd in done for hd in range(4 * hc, 4 * hc + 4))
            cs = slice(j * 128, (j + 1) * 128)
            y = jnp.dot(_as_bf16(oc_ref[:, hc * KH:(hc + 1) * KH]),
                        _as_bf16(woa[j, hc * 256:(hc + 1) * 256, :]), preferred_element_type=f32)
            part[0:nrow_o, cs] = y if hc == 0 else part[0:nrow_o, cs] + y

        providers, ppos = [], []
        if which == 1:
            providers = [functools.partial(bout_half, i) for i in range(16)]
            providers += [functools.partial(wo_early, hc, j) for hc in range(NI) for j in range(8)]
            ppos = sorted([scp + 6 * i - d for i in range(NP) for d in (0, 2)])

        def scores(p_):
            q3 = (which * NP + p_) * 3
            qr = LA - 8 * nvof(which, p_)
            valid, fill = msk[nvof(which, p_)]
            sc = lax.dot_general(_as_bf16(qkvb[q3, 0:qr, :]), _as_bf16(qkvb[q3 + 1]), _NT,
                                 preferred_element_type=f32)
            sc = jnp.where(valid, sc * scale_a, fill)
            p = jnp.exp(sc - jnp.max(sc, axis=-1, keepdims=True))
            ps[p_] = (p * _recip(jnp.sum(p, axis=-1, keepdims=True))).astype(bf16)

        def pv(p_):
            o = jnp.dot(ps.pop(p_), _as_bf16(qkvb[(which * NP + p_) * 3 + 2]), preferred_element_type=f32)
            qr = LA - 8 * nvof(which, p_)

            def merge():
                for e in range(2):
                    hd = 2 * p_ + e
                    oh = jnp.concatenate(ov.pop(hd) + [o[qr * e:qr * e + qr]], axis=0)
                    if which == 0:
                        df[hd] = oh[24:32]
                        z = jnp.concatenate([oh[32:40], oh[0:24]], axis=0)
                    else:
                        z = jnp.concatenate([oh, df[hd]], axis=0)
                    oc_ref[:, hd * DH:(hd + 1) * DH] = _as_u32(z.astype(bf16))
                    done.add(hd)
            if nvof(which, p_) > nearly(which, p_):
                merges[p_] = merge
            else:
                merge()

        def after(n):
            for pos, fn in ((pvp, pv), (scp, scores)):
                if fn is scores:
                    while ppos and ppos[0] <= n:
                        ppos.pop(0)
                        providers.pop(0)()
                if (n - pos) % 6 == 0 and 0 <= (n - pos) // 6 < NP:
                    fn((n - pos) // 6)

        for t in range(NP):
            ys = []
            for m in range(6):
                n = 6 * t + m
                ys.append(proj(2 * t + m // 3, m % 3, (slots.pop(2 * n, []), slots.pop(2 * n + 1, []))))
                if m == 5:
                    q3 = (which * NP + t) * 3
                    nv = nvof(which, t)
                    qr = LA - 8 * nv
                    qkvb[q3, 0:qr, :] = _as_u32(
                        jnp.concatenate([ys[0][8 * nv:], ys[3][8 * nv:]], axis=0).astype(bf16))
                    for i in range(1, 3):
                        qkvb[q3 + i] = _as_u32(jnp.concatenate([ys[i], ys[3 + i]], axis=0).astype(bf16))
                    vpu_jobs(t, ys)
                fire(n, ys[-1][8:32])
                after(n + 1)
        n = 6 * NP
        step = 2 if which == 1 else SPLIT // 4
        for j in range(8):
            cs = slice(j * 128, (j + 1) * 128)
            assert len(providers) <= 7 - j and all(hd in done for hd in range(SPLIT))
            acc = None if c0 == 0 else part[0:nrow_o, cs]
            for c in range(c0, SPLIT // 4, step):
                nun = step // 2
                ties = [sum([slots.pop(2 * n + i, []) for i in range(lo, lo + nun)], []) for lo in (0, nun)]
                y = jnp.dot(_as_bf16(oc_ref[:, c * KH:(c + step) * KH]),
                            _as_bf16(tied(woa[j, c * 256:(c + step) * 256, :], zvec, *ties)),
                            preferred_element_type=f32)
                fire(n, y)
                acc = y if acc is None else acc + y
                for _ in range(nun):
                    n += 1
                    after(n)
            part[0:nrow_o, cs] = acc
        for merge in merges.values():
            merge()
        assert n == nend
        assert not (ps or ov or slots or bacc or pre or lrel or providers)
        if which == 1:
            @pl.when(it % OG == OG - 1)
            def _():
                b_out_start(pl.multiple_of(rb0 - (OG - 1) * MB, 16), OG * MB)
        o2 = _as_bf16(oc_ref[:, k1:])
        for j in range(8):
            cs = slice(j * 128, (j + 1) * 128)
            y = part[0:nrow_o, cs] + jnp.dot(o2, _as_bf16(woa[j, k1 // 2:, :]), preferred_element_type=f32)
            if which == 0:
                hb[0:8, cs] = y[0:8].astype(bf16)
                outa[pl.ds(r0, 24), cs] = y[8:32].astype(bf16)
            else:
                outa[pl.ds(r0 + 32, 32), cs] = y[0:32].astype(bf16)
                ha[40:48, cs] = y[32:40].astype(bf16)
                outa[pl.ds(r0 + 24, 8), cs] = y[40:48].astype(bf16)
                if j == 6:
                    xa[S:S + 16, 0:128] = y[0:16].astype(bf16)
                    oball[S // 2:S // 2 + 8, 0:128] = _as_u32(y[0:8])
                    stage(jnp.minimum(it + 1, NIT - 1))

    def a_body(it, carry):
        r0 = pl.multiple_of(it * 64, 64)
        rb0 = pl.multiple_of(it * MB, 16)
        segment(0, it, r0, rb0)

        @pl.when(it == OG - 1)
        def _():
            a_out_start(0, 64 * OG - 40)

        @pl.when(jnp.logical_and(it % OG == OG - 1, it >= OG))
        def _():
            a_out_start(r0 + 24 - 64 * OG, 64 * OG)

        segment(1, it, r0, rb0)
        return carry

    stage(0)
    lax.fori_loop(0, NIT, a_body, 0)
    a_out_start(S - 40, 40)

    pltpu.make_async_copy(outb, out_hbm.at[:, pl.ds(DM, DM)], sem_out.at[1]).wait()
    pltpu.make_async_copy(outa, out_hbm.at[:, pl.ds(0, DM)], sem_out.at[0]).wait()


@jax.jit
def pallas_concat_heads__memory_aug_recurrent_mem_tr__sliding_local_dilated__prompt_kernel(
    A_x, A_mem0, A_Wq, A_Wk, A_Wv, A_Wo, A_seg_len, B_x, B_wqkv, B_wo,
):
    del A_seg_len
    assert A_x.shape == (1, S, DM) and B_x.shape == (1, S, DM)
    vm = pltpu.VMEM
    scratch = [
        vm((S + 16, DM), bf16), vm((S, DM), bf16),
        vm((S, DM), bf16), vm((S, DM), bf16),
        vm((RAWA_PAD + RG + 16, DH), bf16),
        vm((RAWO_PAD + 48, DM), bf16),
        vm((3, DM, DM), bf16), vm((DM, DM + 256), bf16),
        vm((3 * TREG + DM // 2 + TPAD, DH), u32),
        vm((8, HA * DH // 2, 128), u32),
        vm((24, BREG + 40, 128), u32), vm((8, BREG + 40, 128), u32),
        vm((8, SB, 128), f32), vm((8, SB, 128), f32),
        vm((8, SB + HALO, 128), f32), vm((8, SB + HALO, 128), f32),
        vm((8, SB + HALO, 128), f32), vm((8, SB + HALO, 128), f32),
        vm((SB // 2, DM), u32), vm((SB // 2, DM), u32),
        vm((S // 2 + 8, DM), u32), vm((MB // 2, DM), u32),
        vm((48, DM), bf16), vm((32, DM), bf16),
        vm((16, HA * DH), u32), vm((24, HA * DH), u32),
        vm((48, DM), f32),
        vm((3 * HA, 8, 128), f32), vm((HA, 8, 128), f32),
        vm((3 * HA, 8, 128), f32),
        vm((6 * NP, LA, 128), u32),
        pltpu.SMEM((1,), i32),
        pltpu.SemaphoreType.DMA((NSEM,)),
        pltpu.SemaphoreType.DMA((2,)),
    ]
    out = pl.pallas_call(
        _kernel,
        out_shape=jax.ShapeDtypeStruct((S, 2 * DM), bf16),
        in_specs=[pl.BlockSpec(memory_space=pl.ANY)] * 9,
        out_specs=pl.BlockSpec(memory_space=pl.ANY),
        scratch_shapes=scratch,
        compiler_params=pltpu.CompilerParams(
            vmem_limit_bytes=120 * 1024 * 1024,
            disable_bounds_checks=True,
            disable_semaphore_checks=True,
        ),
        name="concat_heads_kernel",
    )(
        A_x.reshape(S, DM), A_mem0.reshape(MEM, DM),
        A_Wq.reshape(DM * HA, DH), A_Wk.reshape(DM * HA, DH), A_Wv.reshape(DM * HA, DH),
        A_Wo.reshape(HA * DH, DM),
        B_x.reshape(S, DM), B_wqkv, B_wo,
    )
    return out.reshape(1, S, 2 * DM)
```

```python
import functools

import jax
import jax.numpy as jnp
from jax import lax
import jax.experimental.pallas as pl
import jax.experimental.pallas.tpu as pltpu

bf16, f32, u32, i32 = jnp.bfloat16, jnp.float32, jnp.uint32, jnp.int32

S, DM = 2048, 1024
HA, DH, MEM, SEG = 32, 128, 8, 32
LA = MEM + SEG
HB, NW, DIL = 32, 8, 2
HALO = 16
NEG = -1000000000.0
LOG2E = 1.4426950408889634

SB = 128
NSTEP = S // SB
RB = 8
NRB = SB // RB
TP = 514
TREG = HA * TP
TPAD = 1032
DP = 18
BREG = HB * DP
NCH = 6
GPC = 3 * (DM // 16) // NCH
RG = 16 * HA
WOR = 640
WOREST = HA * DH - NCH * WOR
RAWA_PAD = 3 * DM * HA
RAWO_PAD = HA * DH
NIT = S // (2 * SEG)
MB = (48, 64)
NJ0 = 4
OG = 4
NP = HA // 2
SPLIT = 24
LATE = 14
NI = 2
JORD = (0, 4, 1, 5, 2, 6, 3, 7)
NSEM = 32

_NT = (((1,), (1,)), ((), ()))


def _as_bf16(x):
    return pltpu.bitcast(x, bf16)


def _as_u32(x):
    return pltpu.bitcast(x, u32)


def _sum(xs):
    return functools.reduce(lambda a, b: a + b, xs)


def _interleave(a, b, gate=None):
    mlo, mhi = jnp.uint32(0xFFFF), jnp.uint32(0xFFFF0000)
    if gate is not None:
        mlo, mhi = gate | mlo, gate | mhi
    lo = (a & mlo) | (b << 16)
    hi = (a >> 16) | (b & mhi)
    return lo, hi


def _recip(x):
    r = pl.reciprocal(x, approx=True)
    return r * (2.0 - x * r)


def _rows(ref, r0, n):
    return ref.at[pl.ds(r0, n), :]


def _kernel(xa_hbm, mem0_hbm, wq_hbm, wk_hbm, wv_hbm, wo_hbm, xb_hbm, wqkvb_hbm, wob_hbm,
            out_hbm,
            xa, xb, outa, outb, rawa, rawo, rawb, rawob, wa, woa, wt, wos,
            qb0, qb1, kb0, kb1, vb0, vb1, xs0, xs1, oball, obs0, obs1,
            ha, hb, oca, ocb, part, ex, df, sv, qkvb, wk0, zero,
            sem, sem_out):
    zero[0] = 0
    qbuf, kbuf, vbuf, xsb = (qb0, qb1), (kb0, kb1), (vb0, vb1), (xs0, xs1)

    nsem = [0]

    def cp(src, dst):
        c = pltpu.make_async_copy(src, dst, sem.at[nsem[0]])
        nsem[0] += 1
        return c

    def cp_xb(b0, nb):
        return cp(_rows(xb_hbm, b0 * SB, nb * SB), _rows(xb, b0 * SB, nb * SB))

    def cp_wb(t, k0, n):
        return cp(wqkvb_hbm.at[pl.ds(k0, n), pl.ds(t * DM, DM)], rawb.at[t, pl.ds(k0, n), :])

    cp_ch = []
    for c in range(NCH):
        w = (wq_hbm, wk_hbm, wv_hbm)[c // 2]
        cp_ch.append(cp(_rows(w, (c % 2) * GPC * RG, GPC * RG), _rows(rawa, c * GPC * RG, GPC * RG)))
        cp_ch.append(cp(_rows(wo_hbm, c * WOR, WOR), _rows(rawo, c * WOR, WOR)))
    sem_x = nsem[0]
    cp_xbs = [cp_xb(6 + 2 * c, 2) for c in range(5)]
    cp_worest = cp(_rows(wo_hbm, NCH * WOR, WOREST), _rows(rawo, NCH * WOR, WOREST))
    cp_xb0, cp_xb1, cp_xb2, cp_xb3 = cp_xb(0, 1), cp_xb(1, 1), cp_xb(2, 1), cp_xb(3, 3)
    KVQ, KQV = (1, 2, 0), (1, 0, 2)
    cp_w0 = [cp_wb(KQV[0], 0, DM // 4), cp_wb(KQV[0], DM // 4, DM // 4)]
    cp_wp = [None] + [cp_wb(KQV[h // 2], (h % 2) * (DM // 2), DM // 2) for h in range(1, 6)]
    cp_wob = cp(wob_hbm, rawob.at[:, pl.ds(0, DM)])
    cp_xa = cp(xa_hbm, _rows(xa, 0, S))
    cp_m0 = cp(mem0_hbm, _rows(ha, LA, MEM))
    assert nsem[0] == NSEM
    order = cp_w0 + [cp_xb0, cp_xb1] + cp_wp[1:5] + [cp_xb2, cp_wp[5], cp_xb3]
    for c in range(NCH):
        order += cp_ch[2 * c:2 * c + 2] + cp_xbs[c:c + 1] + ([cp_wob] if c == 1 else [])
    order += [cp_worest, cp_m0, cp_xa]
    for c in order:
        c.start()

    def wait_like(dst, s):
        pltpu.make_async_copy(dst, dst, sem.at[s]).wait()

    def a_out_start(r0, n):
        r0 = pl.multiple_of(r0, 8)
        pltpu.make_async_copy(_rows(outa, r0, n), out_hbm.at[pl.ds(r0, n), pl.ds(0, DM)],
                              sem_out.at[0]).start()

    def b_out_start(r0, n, part_):
        c0, nc = (0, NJ0 * 128) if part_ == 0 else (NJ0 * 128, DM - NJ0 * 128)
        pltpu.make_async_copy(outb.at[pl.ds(r0, n), pl.ds(c0, nc)],
                              out_hbm.at[pl.ds(r0, n), pl.ds(DM + c0, nc)], sem_out.at[1]).start()

    def zeros_vec():
        return jnp.full((8, 128), zero[0], i32).astype(u32)

    def tied(w, zvec, *vals_list):
        n = w.shape[0] // len(vals_list)
        parts = []
        for i, vals in enumerate(vals_list):
            pt = w[i * n:(i + 1) * n]
            if vals:
                tie = functools.reduce(lambda a, b: a | b, [_as_u32(x) for x in vals]) & zvec
                pt = jnp.concatenate([pt[0:n - 8], pt[n - 8:] | tie], axis=0)
            parts.append(pt)
        return jnp.concatenate(parts, axis=0)

    def gate16(token):
        g = _as_u32(token[8:16]) & zeros_vec()
        return jnp.concatenate([g, g], axis=0)

    def gated(x, token):
        gate = _as_u32(token[8:16]) & zeros_vec()
        return pltpu.bitcast(_as_u32(x) | gate[None], f32)

    def run(dots, *job_lists, td=6):
        rel = {}
        for jobs, lo, hi, tr in job_lists:
            for i, job in enumerate(jobs):
                rel.setdefault(lo + i * (hi - lo) // len(jobs) - 1, []).append((job, tr))
        due = {}

        def fire(i, y):
            for job, tr in rel.get(i, []):
                vals = job(None if y is None else y[tr:tr + 16])
                if vals:
                    due.setdefault(min(i + td, len(dots) - 1), []).extend(vals)

        fire(-1, None)
        for i, th in enumerate(dots):
            fire(i, th(due.pop(i, [])))

    def prep_qkv(t, kbs):
        for kb_ in kbs:
            for ch in range(8):
                at = _as_u32(rawb[t, kb_ * 128:(kb_ + 1) * 128, ch * 128:(ch + 1) * 128].T)
                for pr in range(2):
                    lo, hi = _interleave(at[pr * 32:pr * 32 + 16], at[pr * 32 + 16:pr * 32 + 32])
                    wt[t * 8 + kb_, pl.ds(ch * 2 + pr, 16, stride=2 * DP), :] = lo
                    wt[t * 8 + kb_, pl.ds(DP + ch * 2 + pr, 16, stride=2 * DP), :] = hi

    def prep_wo_job(src_col, j, hq):
        def job(token):
            gate = gate16(token)
            dst = wos.at[j]
            for hp in range(4 * hq, 4 * hq + 4):
                src = _as_u32(rawob[hp * 64:(hp + 1) * 64, pl.ds(src_col, 128)])
                lo, hi = _interleave(src[0:16], src[16:32], gate)
                dst[pl.ds(hp, 16, stride=2 * DP), :] = lo
                dst[pl.ds(DP + hp, 16, stride=2 * DP), :] = hi
        return job

    def repack_job(src0, dst0, half):
        def job(token):
            gate = gate16(token)
            dst = _rows(wa, dst0, TREG + TPAD)
            for ii in range(half * 4, half * 4 + 4):
                src = _as_u32(_rows(rawa, src0, RG)[ii * 64:(ii + 1) * 64, :])
                lo, hi = _interleave(src[0:16], src[16:32], gate)
                dst[pl.ds(ii, 16, stride=2 * TP), :] = lo
                dst[pl.ds(ii + TP, 16, stride=2 * TP), :] = hi
        return job

    def wocopy_job(src0, dst0):
        def job(token):
            v = _as_u32(rawo[pl.ds(src0, 32), :])
            v = jnp.stack([v[:, j * 128:(j + 1) * 128] for j in range(8)])
            if token is not None:
                v = v | gate16(token)[None]
            woa[:, pl.ds(dst0, 16), :] = v
        return job

    def chunk_jobs(it):
        c = jnp.maximum(it - 1, 0)
        ja, jo, jw = [], [], []
        for i in range(GPC):
            src0 = pl.multiple_of(jnp.where(it > 0, (c * GPC + i) * RG, RAWA_PAD), RG)
            dst0 = pl.multiple_of((c // 2) * TREG + ((c % 2) * GPC + i) * 8, 8)
            ja += [repack_job(src0, dst0, 0), repack_job(src0, dst0, 1)]
        for i in range(WOR // 32):
            src0 = pl.multiple_of(jnp.where(it > 0, c * WOR + i * 32, RAWO_PAD), 32)
            jo.append(wocopy_job(src0, pl.multiple_of(c * (WOR // 2) + i * 16, 16)))
        for i in range(2):
            j = jnp.maximum(2 * (it - 3) + i, 0)
            src_col = pl.multiple_of(jnp.where(it > 2, j * 128, DM), 128)
            jw += [prep_wo_job(src_col, j, hq) for hq in range(4)]
        half = lambda js, h: js[h * len(js) // 2:(h + 1) * len(js) // 2]
        return [half(ja, h) + half(jo, h) + half(jw, h) for h in range(2)]

    def xcvt_jobs(r0, p):
        def mk(i):
            def job(token):
                xsb[p][i * 8:(i + 1) * 8, :] = _as_u32(xb[pl.ds(pl.multiple_of(r0 + i * 16, 16), 16), :])
            return job
        return [mk(i) for i in range(SB // 16)]

    def xcvt(r0, p):
        for job in xcvt_jobs(r0, p):
            job(None)

    scale_b = (DM // HB) ** -0.5

    def wt_tiles(t, c, kbs):
        wv = jnp.concatenate([wt[t * 8 + kbs[0]:t * 8 + kbs[-1] + 1, pl.ds((4 * c + dd) * DP, 16), :]
                              for dd in range(4)], axis=1)
        return [wv[i] for i in range(len(kbs))]

    def untranspose(h):
        for i, w_ in enumerate(wt_tiles(KQV[h // 2], 0, range(4 * (h % 2), 4 * (h % 2) + 4))):
            wk0[h, i * 64:(i + 1) * 64, :] = _as_u32(_as_bf16(w_).T)

    def b_proj_dots(p, ts, half=None):
        kbs = range(8) if half is None else range(4 * half, 4 * half + 4)

        def mk(t, c):
            def th(ties):
                x = _as_bf16(xsb[p][:, kbs[0] * 128:(kbs[-1] + 1) * 128])
                tiles = wt_tiles(t, c, kbs)
                if ties:
                    tiles[-1] = tied(tiles[-1], zeros_vec(), ties)
                if half is None and (p, t, c) == (0, KVQ[0], 0):
                    y = jnp.dot(x[:, :DM // 2], _as_bf16(wk0[0]), preferred_element_type=f32)
                    y = lax.dot_general(x[:, DM // 2:], _as_bf16(jnp.concatenate(tiles[4:], axis=1)), _NT,
                                        preferred_element_type=f32) + y
                elif half is not None and (p, c) == (1, 0) and 2 * KQV.index(t) + half < 5:
                    y = jnp.dot(x, _as_bf16(wk0[2 * KQV.index(t) + half]), preferred_element_type=f32)
                else:
                    y = lax.dot_general(x, _as_bf16(jnp.concatenate(tiles, axis=1)), _NT,
                                        preferred_element_type=f32)
                if t == 0:
                    qbuf[p][c] = y + qbuf[p][c] if half == 1 else y
                else:
                    g = kbuf if t == 1 else vbuf
                    if half != 0:
                        g[p][c, 0:HALO, :] = g[1 - p][c, SB:SB + HALO, :]
                    g[p][c, HALO:HALO + SB, :] = y + g[p][c, HALO:HALO + SB, :] if half == 1 else y
                return y
            return th
        return [mk(t, c) for t in ts for c in range(8)]

    def wos_all():
        return jnp.concatenate([wos[:, pl.ds(d * DP, 16), :] for d in range(HB)], axis=1)

    def b_out_dots(r0):
        w = []

        def mk(j):
            def th(ties):
                if not w:
                    w.append(wos_all())
                o = _as_bf16(oball[r0 // 2:(r0 + SB) // 2, :])
                y = jnp.dot(o, _as_bf16(w[0][j]), preferred_element_type=f32)
                outb[pl.ds(r0, SB), j * 128:(j + 1) * 128] = y.astype(bf16)
                return y
            return th
        return [mk(j) for j in range(NJ0)]

    def b_attn_qk(p, rb, first, token):
        b0 = rb * RB
        q = qbuf[p][:, b0:b0 + RB, :]
        if token is not None:
            q = gated(q, token)
        acc = [jnp.sum(q * kbuf[p][:, pl.ds(HALO + b0 - DIL * w, RB), :], axis=0) for w in range(NW)]
        a = jnp.stack(acc)
        a = a + pltpu.roll(a, 64, 2)
        a = a + pltpu.roll(a, 32, 2)
        a = a * (scale_b * LOG2E)
        if first and b0 < DIL * (NW - 1):
            row = b0 + lax.broadcasted_iota(i32, (NW, RB, 128), 1)
            a = jnp.where(row >= DIL * lax.broadcasted_iota(i32, (NW, RB, 128), 0), a, NEG * LOG2E)
        e = jnp.exp2(a - jnp.max(a, axis=0)[None])
        e = e * _recip(jnp.sum(e, axis=0))[None]
        return [e[w] for w in range(NW)]

    def b_attn_pv(p, rb, r0, ps):
        b0 = rb * RB
        dst = _rows(oball, pl.multiple_of(r0 // 2, SB // 2), SB // 2)
        g = 4
        outs = []
        for c0 in range(0, 8, g):
            o = _sum([ps[w][None] * vbuf[p][c0:c0 + g, pl.ds(HALO + b0 - DIL * w, RB), :] for w in range(NW)])
            outs += [o[c] for c in range(g)]
        dst[pl.ds(b0 // 2, RB // 2), :] = _as_u32(jnp.concatenate(outs, axis=1).astype(bf16))
        return outs

    def attn_jobs(p, r0):
        def mk(rb):
            return lambda token: b_attn_pv(p, rb, r0, b_attn_qk(p, rb, False, token))
        return [mk(rb) for rb in range(NRB)]

    z8 = pl.multiple_of(zero[0], 8)
    keep = jnp.zeros((8, 128), u32)
    qkvb[0, 0:8, :] = keep
    keep = keep | qkvb[zero[0], 0:8, :]
    for ref in (oca, ocb, obs0, obs1):
        ref[0:8, 0:128] = jnp.zeros((8, 128), u32)
        keep = keep | ref[pl.ds(z8, 8), 0:128]
    for ref in (ex, df, sv):
        ref[0] = jnp.zeros((8, 128), f32)
        keep = keep | _as_u32(ref[zero[0]])
    part[0:8, 0:128] = jnp.zeros((8, 128), f32)
    keep = keep | _as_u32(part[pl.ds(z8, 8), 0:128])
    outa[0:16, 0:128] = _as_bf16(keep)
    rawa[pl.ds(RAWA_PAD, RG), :] = jnp.zeros((RG, DH), bf16)
    rawo[pl.ds(RAWO_PAD, 32), :] = jnp.zeros((32, DM), bf16)
    rawob[:, DM:DM + 128] = jnp.zeros((DM, 128), bf16)

    def phase_b():
        for i in range(2):
            cp_w0[i].wait()
            prep_qkv(KQV[0], range(2 * i, 2 * i + 2))
        cp_xb0.wait()
        xcvt(0, 0)
        run(b_proj_dots(0, KQV[0:1], 0))
        cp_xb1.wait()
        xcvt(SB, 1)
        untranspose(0)
        NQ4 = 8
        for h in range(1, 6):
            cp_wp[h].wait()
            if h == 5:
                cp_xb2.wait()
            t0, t1 = KQV[(h - 1) // 2], KQV[h // 2]
            prep_qkv(t1, range(4 * (h % 2), 4 * (h % 2) + 4))
            if h < 5:
                untranspose(h)
            dots = b_proj_dots(1, (t0,), (h - 1) % 2) + b_proj_dots(0, (t1,), h % 2)
            if h >= 4:
                def qk_job(rb):
                    def job(token):
                        ps_ = b_attn_qk(0, rb, True, token)
                        qb0[:, rb * RB:(rb + 1) * RB, :] = jnp.stack(ps_)
                        return ps_
                    return job
                rbs = range(NQ4) if h == 4 else range(NQ4, NRB)
                run(dots, ([qk_job(rb) for rb in rbs], 4, 12, 112), td=6)
            else:
                run(dots)
            if h == 5:
                vb0[:, 0:HALO, :] = jnp.broadcast_to(vb0[:, HALO:HALO + 1, :], (8, HALO, 128))

                def pv_job(rb):
                    def job(token):
                        ps_ = qb0[:, rb * RB:(rb + 1) * RB, :]
                        if token is not None:
                            ps_ = gated(ps_, token)
                        b_attn_pv(0, rb, 0, [ps_[w] for w in range(NW)])
                    return job
                xcvt(2 * SB, 0)
                pj = [pv_job(rb) for rb in range(NRB)]
                run(b_proj_dots(1, (t1,), 1), (pj[0::2], 0, 7, 48),
                    (pj[1::2], 0, 7, 112))
        cp_xb3.wait()

        def b_step(p, r_attn, r_next, side):
            run(b_proj_dots(p, KVQ),
                (attn_jobs(1 - p, r_attn), 1, 21, 112),
                (side[0::2], 1, 24, 16), (side[1::2], 1, 24, 40),
                (xcvt_jobs(r_next, 1 - p), 0, 20, 0))

        def b_body(it, carry):
            @pl.when(it == 3)
            def _():
                cp_wob.wait()

            @pl.when(jnp.logical_and(it > 0, it <= 5))
            def _():
                wait_like(_rows(xb, pl.multiple_of((4 + 2 * it) * SB, 2 * SB), 2 * SB), sem_x + it - 1)

            @pl.when(it > 0)
            def _():
                c = it - 1
                wait_like(_rows(rawa, pl.multiple_of(c * (GPC * RG), GPC * RG), GPC * RG), 2 * c)
                wait_like(_rows(rawo, pl.multiple_of(c * WOR, 128), WOR), 2 * c + 1)

            r0 = pl.multiple_of((2 * it + 2) * SB, 2 * SB)
            side = chunk_jobs(it)
            b_step(0, r0 - SB, r0 + SB, side[0])
            b_step(1, r0, jnp.minimum(r0 + 2 * SB, S - SB), side[1])
            return carry

        lax.fori_loop(0, NSTEP // 2 - 1, b_body, 0)
        cp_worest.wait()
        cp_m0.wait()
        cp_xa.wait()
        jo = [wocopy_job(NCH * WOR + i * 32, NCH * WOR // 2 + i * 16) for i in range(WOREST // 32)]
        dots = sum([b_out_dots(r) for r in range(NIT * MB[0], S, SB)], [])
        aj = attn_jobs(1, S - SB)
        nd = len(dots) - NJ0 - 1
        run(dots, (aj[0::2], 0, nd, 48), (aj[1::2], 0, nd, 112), (jo, 0, 0, 0))

    phase_b()
    b_out_start(NIT * MB[0], S - NIT * MB[0], 0)

    scale_a = DH ** -0.5
    qscale = scale_a * LOG2E
    k1 = SPLIT * DH
    tri = lax.broadcasted_iota(i32, (8, 8, 128), 1) >= lax.broadcasted_iota(i32, (8, 8, 128), 0)

    def masks(nv):
        qr = LA - 8 * nv
        r = lax.broadcasted_iota(i32, (2 * qr, 2 * LA), 0)
        c = lax.broadcasted_iota(i32, (2 * qr, 2 * LA), 1)
        same = (r >= qr) == (c >= LA)
        rr = jnp.where(r >= qr, r - qr, r) + 8 * nv
        cc = jnp.where(c >= LA, c - LA, c)
        valid = same & ((cc >= SEG) | (rr >= SEG) | (cc <= rr))
        return valid, jnp.where(same, NEG, -jnp.inf).astype(f32)

    def nvof(which, t):
        return 3 if which == 1 and t >= LATE else 2

    def nearly(which, t):
        return 1 if which == 1 and t >= LATE else 2

    msk = {nv: masks(nv) for nv in (2, 3)}

    def bc8(a):
        return jnp.concatenate([jnp.broadcast_to(a[j:j + 1], (8, 128)) for j in range(8)],
                               axis=0).reshape(8, 8, 128)

    def vpu_part(q, k8, v8, causal, prev):
        s_ = jnp.broadcast_to(jnp.sum(q[None] * k8, axis=-1, keepdims=True), (8, 8, 128))
        if causal:
            s_ = jnp.where(tri, s_, NEG * LOG2E)
        m = jnp.max(s_, axis=0)
        if prev is not None:
            m = jnp.maximum(m, prev[0])
        e = jnp.exp2(s_ - m[None])
        l = jnp.sum(e, axis=0)
        o = jnp.sum(e * v8, axis=0)
        if prev is not None:
            al = jnp.exp2(prev[0] - m)
            l = l + prev[1] * al
            o = o + prev[2] * al
        return m, l, o

    def stage_x(it):
        r0 = pl.multiple_of(it * 64, 64)
        ha[0:40, :] = xa[pl.ds(r0, 40), :]
        hb[8:32, :] = xa[pl.ds(r0 + 40, 24), :]

    def stage_o(it):
        for obs, mb in zip((obs0, obs1), MB):
            obs[...] = oball[pl.ds(pl.multiple_of(it * (mb // 2), 8), mb // 2), :]

    def segment(which, it, r0):
        h_ref, oc_ref = (ha, oca) if which == 0 else (hb, ocb)
        nrow_o = 32 if which == 0 else 48
        h = h_ref[...]
        zvec = zeros_vec()
        so = (18, 19)[which]
        scp = (10, 9)[which]
        pvp = (20, 20)[which]
        c0 = NI * which
        nend = 6 * NP + SPLIT - 4 * c0
        assert 2 * LATE >= SPLIT
        ov, slots, ps, bacc, pre, late, merges = {}, {}, {}, [], {}, [], {}

        LS, LU, LD = -4, 16, 6
        nlate = sum(2 * (g + 2) for t in range(NP) for g in range(nearly(which, t), nvof(which, t)))
        lrel, done = {}, set()

        def fire(n, y):
            for i, job in enumerate(lrel.pop(n, [])):
                r_ = (0, y.shape[0] - 8, 16)[i % 3]
                vals = job(_as_u32(y[r_:r_ + 8]) & zvec)
                if n + LD < nend:
                    slots.setdefault(2 * (n + LD) + i % 2, []).extend(vals)

        def wa_tile(hd, t, k0, kn):
            return wa[pl.ds(t * TREG + hd * TP + k0 // 2, kn // 2), :]

        KH = DM // 2
        if which == 1:
            wb = wos_all()
            for hd in range(2):
                for t in range(3):
                    pre[hd, t] = jnp.dot(h[:, :KH], _as_bf16(wa_tile(hd, t, 0, KH)), preferred_element_type=f32)

        def proj(hd, t, ties):
            if (hd, t) in pre:
                y = jnp.dot(h[:, KH:], _as_bf16(wa_tile(hd, t, KH, KH)), preferred_element_type=f32)
                y = y + pre.pop((hd, t))
            else:
                y = jnp.dot(h, _as_bf16(tied(wa_tile(hd, t, 0, DM), zvec, *ties)), preferred_element_type=f32)
            if which == 0:
                ex[t * HA + hd] = y[32:40]
                return jnp.concatenate([y[0:32], y[40:48]], axis=0)
            return jnp.concatenate([ex[t * HA + hd], y[8:32], y[0:8]], axis=0)

        def vpu_jobs(t, ys):
            out = []
            for e in range(2):
                hd = 2 * t + e
                q, k, v = ys[3 * e:3 * e + 3]
                ov[hd] = []
                cache = {}

                def blk(b0):
                    if b0 not in cache:
                        cache[b0] = bc8(k[b0:b0 + 8]), bc8(v[b0:b0 + 8])
                    return cache[b0]

                for g in range(nearly(which, t)):
                    q0 = q[8 * g:8 * g + 8] * qscale
                    if which == 1 and g == 0:
                        st = [sv[i * HA + hd] for i in range(3)]
                    else:
                        st = None
                        for b in range(g, -1, -1):
                            st = vpu_part(q0, *blk(8 * b), b == g, st)
                            out.append(list(st[1:]))
                    _, l, o = vpu_part(q0, *blk(SEG), False, st)
                    ov[hd].append(o * _recip(l))
                    out.append([ov[hd][-1]])
                for g in range(nearly(which, t), nvof(which, t)):
                    st = [None]
                    for b0 in [8 * b for b in range(g, -1, -1)] + [SEG]:
                        def job(tok, hd=hd, g=g, b0=b0, st=st, q=q, k=k, v=v):
                            gate = lambda x: pltpu.bitcast(_as_u32(x) | tok, f32)
                            st[0] = vpu_part(gate(q[8 * g:8 * g + 8]) * qscale, bc8(gate(k[b0:b0 + 8])),
                                             bc8(gate(v[b0:b0 + 8])), b0 == 8 * g, st[0])
                            if b0 != SEG:
                                return list(st[0][1:])
                            ov[hd].append(st[0][2] * _recip(st[0][1]))
                            return [ov[hd][-1]]
                        lrel.setdefault(6 * NP + LS + len(late) * LU // nlate, []).append(job)
                        late.append(job)
                if which == 0:
                    st = vpu_part(ex[hd] * qscale, bc8(ex[HA + hd]), bc8(ex[2 * HA + hd]), True, None)
                    for i in range(3):
                        sv[i * HA + hd] = st[i]
                    out.append(list(st[1:]))
            for i, jb in enumerate(out):
                slots.setdefault(12 * t + so + (2 * i + 1) * 6 // len(out), []).extend(jb)

        def bout_half(i):
            j, half = JORD[i // 2], i % 2
            obs, mb = (obs0, MB[0]) if j < NJ0 else (obs1, MB[1])
            o = _as_bf16(obs[:, half * KH:(half + 1) * KH])
            y = jnp.dot(o, _as_bf16(wb[j, half * 256:(half + 1) * 256]), preferred_element_type=f32)
            if half == 0:
                bacc.append(y)
            else:
                outb[pl.ds(pl.multiple_of(it * mb, 16), mb), j * 128:(j + 1) * 128] = (y + bacc.pop()).astype(bf16)

        def wo_early(hc, j):
            assert all(hd in done for hd in range(4 * hc, 4 * hc + 4))
            cs = slice(j * 128, (j + 1) * 128)
            y = jnp.dot(_as_bf16(oc_ref[:, hc * KH:(hc + 1) * KH]),
                        _as_bf16(woa[j, hc * 256:(hc + 1) * 256, :]), preferred_element_type=f32)
            part[0:nrow_o, cs] = y if hc == 0 else part[0:nrow_o, cs] + y

        providers, ppos = [], []
        if which == 1:
            providers = [functools.partial(bout_half, i) for i in range(16)]
            providers += [functools.partial(wo_early, hc, j) for hc in range(NI) for j in range(8)]
            ppos = sorted([scp + 6 * i - d for i in range(NP) for d in (0, 2)])

        def scores(p_):
            q3 = (which * NP + p_) * 3
            qr = LA - 8 * nvof(which, p_)
            valid, fill = msk[nvof(which, p_)]
            sc = lax.dot_general(_as_bf16(qkvb[q3, 0:qr, :]), _as_bf16(qkvb[q3 + 1]), _NT,
                                 preferred_element_type=f32)
            sc = jnp.where(valid, sc * scale_a, fill)
            p = jnp.exp(sc - jnp.max(sc, axis=-1, keepdims=True))
            ps[p_] = (p * _recip(jnp.sum(p, axis=-1, keepdims=True))).astype(bf16)

        def pv(p_):
            o = jnp.dot(ps.pop(p_), _as_bf16(qkvb[(which * NP + p_) * 3 + 2]), preferred_element_type=f32)
            qr = LA - 8 * nvof(which, p_)

            def merge():
                for e in range(2):
                    hd = 2 * p_ + e
                    oh = jnp.concatenate(ov.pop(hd) + [o[qr * e:qr * e + qr]], axis=0)
                    if which == 0:
                        df[hd] = oh[24:32]
                        z = jnp.concatenate([oh[32:40], oh[0:24]], axis=0)
                    else:
                        z = jnp.concatenate([oh, df[hd]], axis=0)
                    oc_ref[:, hd * DH:(hd + 1) * DH] = _as_u32(z.astype(bf16))
                    done.add(hd)
            if nvof(which, p_) > nearly(which, p_):
                merges[p_] = merge
            else:
                merge()

        def after(n):
            for pos, fn in ((pvp, pv), (scp, scores)):
                if fn is scores:
                    while ppos and ppos[0] <= n:
                        ppos.pop(0)
                        providers.pop(0)()
                if (n - pos) % 6 == 0 and 0 <= (n - pos) // 6 < NP:
                    fn((n - pos) // 6)

        for t in range(NP):
            ys = []
            for m in range(6):
                n = 6 * t + m
                ys.append(proj(2 * t + m // 3, m % 3, (slots.pop(2 * n, []), slots.pop(2 * n + 1, []))))
                if m == 5:
                    q3 = (which * NP + t) * 3
                    nv = nvof(which, t)
                    qr = LA - 8 * nv
                    qkvb[q3, 0:qr, :] = _as_u32(
                        jnp.concatenate([ys[0][8 * nv:], ys[3][8 * nv:]], axis=0).astype(bf16))
                    for i in range(1, 3):
                        qkvb[q3 + i] = _as_u32(jnp.concatenate([ys[i], ys[3 + i]], axis=0).astype(bf16))
                    vpu_jobs(t, ys)
                fire(n, ys[-1][8:32])
                after(n + 1)
        if which == 1:
            for i, mb in enumerate(MB):
                @pl.when(it % OG == OG - 1)
                def _():
                    b_out_start(pl.multiple_of((it - (OG - 1)) * mb, 16), OG * mb, i)
        n = 6 * NP
        step = 2 if which == 1 else SPLIT // 4
        for j in range(8):
            cs = slice(j * 128, (j + 1) * 128)
            assert len(providers) <= 7 - j and all(hd in done for hd in range(SPLIT))
            acc = None if c0 == 0 else part[0:nrow_o, cs]
            for c in range(c0, SPLIT // 4, step):
                nun = step // 2
                ties = [sum([slots.pop(2 * n + i, []) for i in range(lo, lo + nun)], []) for lo in (0, nun)]
                y = jnp.dot(_as_bf16(oc_ref[:, c * KH:(c + step) * KH]),
                            _as_bf16(tied(woa[j, c * 256:(c + step) * 256, :], zvec, *ties)),
                            preferred_element_type=f32)
                fire(n, y)
                if which == 1 and n == 6 * NP:
                    outb[S:S + 16, 0:128] = y[0:16].astype(bf16)
                acc = y if acc is None else acc + y
                for _ in range(nun):
                    n += 1
                    after(n)
            part[0:nrow_o, cs] = acc
        for merge in merges.values():
            merge()
        assert n == nend
        assert not (ps or ov or slots or bacc or pre or lrel or providers)
        o2 = _as_bf16(oc_ref[:, k1:])
        for j in range(8):
            cs = slice(j * 128, (j + 1) * 128)
            y = part[0:nrow_o, cs] + jnp.dot(o2, _as_bf16(woa[j, k1 // 2:, :]), preferred_element_type=f32)
            if which == 0:
                hb[0:8, cs] = y[0:8].astype(bf16)
                outa[pl.ds(r0, 24), cs] = y[8:32].astype(bf16)
            else:
                outa[pl.ds(r0 + 32, 32), cs] = y[0:32].astype(bf16)
                ha[40:48, cs] = y[32:40].astype(bf16)
                outa[pl.ds(r0 + 24, 8), cs] = y[40:48].astype(bf16)
                if j == 6:
                    xa[S:S + 16, 0:128] = y[32:48].astype(bf16)
                    stage_x(jnp.minimum(it + 1, NIT - 1))
                    oball[S // 2:S // 2 + 8, 0:128] = _as_u32(y[0:8])
                    stage_o(jnp.minimum(it + 1, NIT - 1))

    def a_body(it, carry):
        r0 = pl.multiple_of(it * 64, 64)
        segment(0, it, r0)

        @pl.when(it == OG - 1)
        def _():
            a_out_start(0, 64 * OG - 40)

        @pl.when(jnp.logical_and(it % OG == OG - 1, it >= OG))
        def _():
            a_out_start(r0 + 24 - 64 * OG, 64 * OG)

        segment(1, it, r0)
        return carry

    stage_x(0)
    stage_o(0)
    lax.fori_loop(0, NIT, a_body, 0)
    a_out_start(S - 40, 40)

    pltpu.make_async_copy(_rows(outb, 0, S), out_hbm.at[:, pl.ds(DM, DM)], sem_out.at[1]).wait()
    pltpu.make_async_copy(outa, out_hbm.at[:, pl.ds(0, DM)], sem_out.at[0]).wait()


@jax.jit
def pallas_concat_heads__memory_aug_recurrent_mem_tr__sliding_local_dilated__prompt_kernel(
    A_x, A_mem0, A_Wq, A_Wk, A_Wv, A_Wo, A_seg_len, B_x, B_wqkv, B_wo,
):
    del A_seg_len
    assert A_x.shape == (1, S, DM) and B_x.shape == (1, S, DM)
    vm = pltpu.VMEM
    scratch = [
        vm((S + 16, DM), bf16), vm((S, DM), bf16),
        vm((S, DM), bf16), vm((S + 16, DM), bf16),
        vm((RAWA_PAD + RG, DH), bf16),
        vm((RAWO_PAD + 32, DM), bf16),
        vm((3, DM, DM), bf16), vm((DM, DM + 128), bf16),
        vm((3 * TREG + DM // 2 + TPAD, DH), u32),
        vm((8, HA * DH // 2, 128), u32),
        vm((24, BREG + 40, 128), u32), vm((8, BREG + 40, 128), u32),
        vm((8, SB, 128), f32), vm((8, SB, 128), f32),
        vm((8, SB + HALO, 128), f32), vm((8, SB + HALO, 128), f32),
        vm((8, SB + HALO, 128), f32), vm((8, SB + HALO, 128), f32),
        vm((SB // 2, DM), u32), vm((SB // 2, DM), u32),
        vm((S // 2 + 8, DM), u32),
        vm((MB[0] // 2, DM), u32), vm((MB[1] // 2, DM), u32),
        vm((48, DM), bf16), vm((32, DM), bf16),
        vm((16, HA * DH), u32), vm((24, HA * DH), u32),
        vm((48, DM), f32),
        vm((3 * HA, 8, 128), f32), vm((HA, 8, 128), f32),
        vm((3 * HA, 8, 128), f32),
        vm((6 * NP, LA, 128), u32),
        vm((5, DM // 4, 128), u32),
        pltpu.SMEM((1,), i32),
        pltpu.SemaphoreType.DMA((NSEM,)),
        pltpu.SemaphoreType.DMA((2,)),
    ]
    out = pl.pallas_call(
        _kernel,
        out_shape=jax.ShapeDtypeStruct((S, 2 * DM), bf16),
        in_specs=[pl.BlockSpec(memory_space=pl.ANY)] * 9,
        out_specs=pl.BlockSpec(memory_space=pl.ANY),
        scratch_shapes=scratch,
        compiler_params=pltpu.CompilerParams(
            vmem_limit_bytes=120 * 1024 * 1024,
            disable_bounds_checks=True,
            disable_semaphore_checks=True,
        ),
        name="concat_heads_kernel",
    )(
        A_x.reshape(S, DM), A_mem0.reshape(MEM, DM),
        A_Wq.reshape(DM * HA, DH), A_Wk.reshape(DM * HA, DH), A_Wv.reshape(DM * HA, DH),
        A_Wo.reshape(HA * DH, DM),
        B_x.reshape(S, DM), B_wqkv, B_wo,
    )
    return out.reshape(1, S, 2 * DM)
```

```python
import functools

import jax
import jax.numpy as jnp
from jax import lax
import jax.experimental.pallas as pl
import jax.experimental.pallas.tpu as pltpu

bf16, f32, u32, i32 = jnp.bfloat16, jnp.float32, jnp.uint32, jnp.int32

S, DM = 2048, 1024
HA, DH, MEM, SEG = 32, 128, 8, 32
LA = MEM + SEG
HB, NW, DIL = 32, 8, 2
HALO = 16
NEG = -1000000000.0
LOG2E = 1.4426950408889634

SB = 128
NSTEP = S // SB
RB = 8
NRB = SB // RB
TP = 514
TREG = HA * TP
TPAD = 1032
DP = 18
BREG = HB * DP
NCH = 6
GPC = 3 * (DM // 16) // NCH
RG = 16 * HA
WOR = 640
WOREST = HA * DH - NCH * WOR
RAWA_PAD = 3 * DM * HA
RAWO_PAD = HA * DH
NIT = S // (2 * SEG)
MB = (48, 64)
NJ0 = 4
OG = 4
NP = HA // 2
SPLIT = 24
LATE = 14
NI = 2
JORD = (0, 4, 1, 5, 2, 6, 3, 7)
NSEM = 33

_NT = (((1,), (1,)), ((), ()))


def _as_bf16(x):
    return pltpu.bitcast(x, bf16)


def _as_u32(x):
    return pltpu.bitcast(x, u32)


def _sum(xs):
    return functools.reduce(lambda a, b: a + b, xs)


def _interleave(a, b, gate=None):
    mlo, mhi = jnp.uint32(0xFFFF), jnp.uint32(0xFFFF0000)
    if gate is not None:
        mlo, mhi = gate | mlo, gate | mhi
    lo = (a & mlo) | (b << 16)
    hi = (a >> 16) | (b & mhi)
    return lo, hi


def _recip(x):
    r = pl.reciprocal(x, approx=True)
    return r * (2.0 - x * r)


def _rows(ref, r0, n):
    return ref.at[pl.ds(r0, n), :]


def _kernel(xa_hbm, mem0_hbm, wq_hbm, wk_hbm, wv_hbm, wo_hbm, xb_hbm, wqkvb_hbm, wob_hbm,
            out_hbm,
            xa, xb, outa, outb, rawa, rawo, rawb, rawob, wa, woa, wt, wos,
            qb0, qb1, kb0, kb1, vb0, vb1, xs0, xs1, oball, obs0, obs1,
            ha, hb, oca, ocb, part, ex, df, sv, qkvb, wk0, zero,
            sem, sem_out):
    zero[0] = 0
    qbuf, kbuf, vbuf, xsb = (qb0, qb1), (kb0, kb1), (vb0, vb1), (xs0, xs1)

    nsem = [0]

    def cp(src, dst):
        c = pltpu.make_async_copy(src, dst, sem.at[nsem[0]])
        nsem[0] += 1
        return c

    def cp_xb(b0, nb):
        return cp(_rows(xb_hbm, b0 * SB, nb * SB), _rows(xb, b0 * SB, nb * SB))

    def cp_wb(t, k0, n):
        return cp(wqkvb_hbm.at[pl.ds(k0, n), pl.ds(t * DM, DM)], rawb.at[t, pl.ds(k0, n), :])

    cp_ch = []
    for c in range(NCH):
        w = (wq_hbm, wk_hbm, wv_hbm)[c // 2]
        cp_ch.append(cp(_rows(w, (c % 2) * GPC * RG, GPC * RG), _rows(rawa, c * GPC * RG, GPC * RG)))
        cp_ch.append(cp(_rows(wo_hbm, c * WOR, WOR), _rows(rawo, c * WOR, WOR)))
    sem_x = nsem[0]
    cp_xbs = [cp_xb(6 + 2 * c, 2) for c in range(5)]
    cp_worest = cp(_rows(wo_hbm, NCH * WOR, WOREST), _rows(rawo, NCH * WOR, WOREST))
    cp_xb0, cp_xb1, cp_xb2, cp_xb3 = cp_xb(0, 1), cp_xb(1, 1), cp_xb(2, 1), cp_xb(3, 3)
    KVQ, KQV = (1, 2, 0), (1, 0, 2)
    cp_w0 = [cp_wb(KQV[0], 0, DM // 4), cp_wb(KQV[0], DM // 4, DM // 4)]
    cp_wp = [None] + [cp_wb(KQV[h // 2], (h % 2) * (DM // 2), DM // 2) for h in range(1, 6)]
    cp_wob = [cp(wob_hbm.at[:, pl.ds(i * 512, 512)], rawob.at[:, pl.ds(i * 512, 512)]) for i in range(2)]
    cp_xa = cp(xa_hbm, _rows(xa, 0, S))
    cp_m0 = cp(mem0_hbm, _rows(ha, LA, MEM))
    assert nsem[0] == NSEM
    order = cp_w0 + [cp_xb0, cp_xb1] + cp_wp[1:5] + [cp_xb2, cp_wp[5], cp_xb3]
    for c in range(NCH):
        order += cp_ch[2 * c:2 * c + 2] + cp_xbs[c:c + 1] + ([cp_wob[c // 2]] if c in (1, 3) else [])
    order += [cp_worest, cp_m0, cp_xa]
    for c in order:
        c.start()

    def like(dst, s):
        return pltpu.make_async_copy(dst, dst, sem.at[s])

    def a_out_start(r0, n):
        r0 = pl.multiple_of(r0, 8)
        pltpu.make_async_copy(_rows(outa, r0, n), out_hbm.at[pl.ds(r0, n), pl.ds(0, DM)],
                              sem_out.at[0]).start()

    def b_out_start(r0, n, part_):
        c0, nc = (0, NJ0 * 128) if part_ == 0 else (NJ0 * 128, DM - NJ0 * 128)
        pltpu.make_async_copy(outb.at[pl.ds(r0, n), pl.ds(c0, nc)],
                              out_hbm.at[pl.ds(r0, n), pl.ds(DM + c0, nc)], sem_out.at[1]).start()

    def zeros_vec():
        return jnp.full((8, 128), zero[0], i32).astype(u32)

    def tied(w, zvec, *vals_list):
        n = w.shape[0] // len(vals_list)
        parts = []
        for i, vals in enumerate(vals_list):
            pt = w[i * n:(i + 1) * n]
            if vals:
                tie = functools.reduce(lambda a, b: a | b, [_as_u32(x) for x in vals]) & zvec
                pt = jnp.concatenate([pt[0:n - 8], pt[n - 8:] | tie], axis=0)
            parts.append(pt)
        return jnp.concatenate(parts, axis=0)

    def gate16(token):
        g = _as_u32(token[8:16]) & zeros_vec()
        return jnp.concatenate([g, g], axis=0)

    def gated(x, token):
        gate = _as_u32(token[8:16]) & zeros_vec()
        return pltpu.bitcast(_as_u32(x) | gate[None], f32)

    def run(dots, *job_lists, td=6):
        rel = {}
        for jobs, lo, hi, tr in job_lists:
            for i, job in enumerate(jobs):
                rel.setdefault(lo + i * (hi - lo) // len(jobs) - 1, []).append((job, tr))
        due = {}

        def fire(i, y):
            for job, tr in rel.get(i, []):
                vals = job(None if y is None else y[tr:tr + 16])
                if vals:
                    due.setdefault(min(i + td, len(dots) - 1), []).extend(vals)

        fire(-1, None)
        for i, th in enumerate(dots):
            fire(i, th(due.pop(i, [])))

    def prep_qkv(t, kbs):
        for kb_ in kbs:
            for ch in range(8):
                at = _as_u32(rawb[t, kb_ * 128:(kb_ + 1) * 128, ch * 128:(ch + 1) * 128].T)
                for pr in range(2):
                    lo, hi = _interleave(at[pr * 32:pr * 32 + 16], at[pr * 32 + 16:pr * 32 + 32])
                    wt[t * 8 + kb_, pl.ds(ch * 2 + pr, 16, stride=2 * DP), :] = lo
                    wt[t * 8 + kb_, pl.ds(DP + ch * 2 + pr, 16, stride=2 * DP), :] = hi

    def prep_wo_job(src_col, j, hq):
        def job(token):
            gate = gate16(token)
            dst = wos.at[j]
            for hp in range(4 * hq, 4 * hq + 4):
                src = _as_u32(rawob[hp * 64:(hp + 1) * 64, pl.ds(src_col, 128)])
                lo, hi = _interleave(src[0:16], src[16:32], gate)
                dst[pl.ds(hp, 16, stride=2 * DP), :] = lo
                dst[pl.ds(DP + hp, 16, stride=2 * DP), :] = hi
        return job

    def repack_job(src0, dst0, half):
        def job(token):
            gate = gate16(token)
            dst = _rows(wa, dst0, TREG + TPAD)
            for ii in range(half * 4, half * 4 + 4):
                src = _as_u32(_rows(rawa, src0, RG)[ii * 64:(ii + 1) * 64, :])
                lo, hi = _interleave(src[0:16], src[16:32], gate)
                dst[pl.ds(ii, 16, stride=2 * TP), :] = lo
                dst[pl.ds(ii + TP, 16, stride=2 * TP), :] = hi
        return job

    def wocopy_job(src0, dst0):
        def job(token):
            v = _as_u32(rawo[pl.ds(src0, 32), :])
            v = jnp.stack([v[:, j * 128:(j + 1) * 128] for j in range(8)])
            if token is not None:
                v = v | gate16(token)[None]
            woa[:, pl.ds(dst0, 16), :] = v
        return job

    def chunk_jobs(it):
        c = jnp.maximum(it - 1, 0)
        ja, jo, jw = [], [], []
        for i in range(GPC):
            src0 = pl.multiple_of(jnp.where(it > 0, (c * GPC + i) * RG, RAWA_PAD), RG)
            dst0 = pl.multiple_of((c // 2) * TREG + ((c % 2) * GPC + i) * 8, 8)
            ja += [repack_job(src0, dst0, 0), repack_job(src0, dst0, 1)]
        for i in range(WOR // 32):
            src0 = pl.multiple_of(jnp.where(it > 0, c * WOR + i * 32, RAWO_PAD), 32)
            jo.append(wocopy_job(src0, pl.multiple_of(c * (WOR // 2) + i * 16, 16)))
        for i in range(2):
            j = jnp.maximum(2 * (it - 3) + i, 0)
            src_col = pl.multiple_of(jnp.where(it > 2, j * 128, DM), 128)
            jw += [prep_wo_job(src_col, j, hq) for hq in range(4)]
        half = lambda js, h: js[h * len(js) // 2:(h + 1) * len(js) // 2]
        return [half(ja, h) + half(jo, h) + half(jw, h) for h in range(2)]

    def xcvt_jobs(r0, p):
        def mk(i):
            def job(token):
                xsb[p][i * 8:(i + 1) * 8, :] = _as_u32(xb[pl.ds(pl.multiple_of(r0 + i * 16, 16), 16), :])
            return job
        return [mk(i) for i in range(SB // 16)]

    def xcvt(r0, p):
        for job in xcvt_jobs(r0, p):
            job(None)

    scale_b = (DM // HB) ** -0.5

    def wt_tiles(t, c, kbs):
        wv = jnp.concatenate([wt[t * 8 + kbs[0]:t * 8 + kbs[-1] + 1, pl.ds((4 * c + dd) * DP, 16), :]
                              for dd in range(4)], axis=1)
        return [wv[i] for i in range(len(kbs))]

    def untranspose(h):
        for i, w_ in enumerate(wt_tiles(KQV[h // 2], 0, range(4 * (h % 2), 4 * (h % 2) + 4))):
            wk0[h, i * 64:(i + 1) * 64, :] = _as_u32(_as_bf16(w_).T)

    def b_proj_dots(p, ts, half=None):
        kbs = range(8) if half is None else range(4 * half, 4 * half + 4)

        def mk(t, c):
            def th(ties):
                x = _as_bf16(xsb[p][:, kbs[0] * 128:(kbs[-1] + 1) * 128])
                tiles = wt_tiles(t, c, kbs)
                if ties:
                    tiles[-1] = tied(tiles[-1], zeros_vec(), ties)
                if half is None and (p, t, c) == (0, KVQ[0], 0):
                    y = jnp.dot(x[:, :DM // 2], _as_bf16(wk0[0]), preferred_element_type=f32)
                    y = lax.dot_general(x[:, DM // 2:], _as_bf16(jnp.concatenate(tiles[4:], axis=1)), _NT,
                                        preferred_element_type=f32) + y
                elif half is not None and (p, c) == (1, 0) and 2 * KQV.index(t) + half < 5:
                    y = jnp.dot(x, _as_bf16(wk0[2 * KQV.index(t) + half]), preferred_element_type=f32)
                else:
                    y = lax.dot_general(x, _as_bf16(jnp.concatenate(tiles, axis=1)), _NT,
                                        preferred_element_type=f32)
                if t == 0:
                    qbuf[p][c] = y + qbuf[p][c] if half == 1 else y
                else:
                    g = kbuf if t == 1 else vbuf
                    if half != 0:
                        g[p][c, 0:HALO, :] = g[1 - p][c, SB:SB + HALO, :]
                    g[p][c, HALO:HALO + SB, :] = y + g[p][c, HALO:HALO + SB, :] if half == 1 else y
                return y
            return th
        return [mk(t, c) for t in ts for c in range(8)]

    def wos_all():
        return jnp.concatenate([wos[:, pl.ds(d * DP, 16), :] for d in range(HB)], axis=1)

    def b_out_dots(r0):
        w = []

        def mk(j):
            def th(ties):
                if not w:
                    w.append(wos_all())
                o = _as_bf16(oball[r0 // 2:(r0 + SB) // 2, :])
                y = jnp.dot(o, _as_bf16(w[0][j]), preferred_element_type=f32)
                outb[pl.ds(r0, SB), j * 128:(j + 1) * 128] = y.astype(bf16)
                return y
            return th
        return [mk(j) for j in range(NJ0)]

    def b_attn_qk(p, rb, first, token):
        b0 = rb * RB
        q = qbuf[p][:, b0:b0 + RB, :]
        if token is not None:
            q = gated(q, token)
        acc = [jnp.sum(q * kbuf[p][:, pl.ds(HALO + b0 - DIL * w, RB), :], axis=0) for w in range(NW)]
        a = jnp.stack(acc)
        a = a + pltpu.roll(a, 64, 2)
        a = a + pltpu.roll(a, 32, 2)
        a = a * (scale_b * LOG2E)
        if first and b0 < DIL * (NW - 1):
            row = b0 + lax.broadcasted_iota(i32, (NW, RB, 128), 1)
            a = jnp.where(row >= DIL * lax.broadcasted_iota(i32, (NW, RB, 128), 0), a, NEG * LOG2E)
        e = jnp.exp2(a - jnp.max(a, axis=0)[None])
        e = e * _recip(jnp.sum(e, axis=0))[None]
        return [e[w] for w in range(NW)]

    def b_attn_pv(p, rb, r0, ps):
        b0 = rb * RB
        dst = _rows(oball, pl.multiple_of(r0 // 2, SB // 2), SB // 2)
        g = 4
        outs = []
        for c0 in range(0, 8, g):
            o = _sum([ps[w][None] * vbuf[p][c0:c0 + g, pl.ds(HALO + b0 - DIL * w, RB), :] for w in range(NW)])
            outs += [o[c] for c in range(g)]
        dst[pl.ds(b0 // 2, RB // 2), :] = _as_u32(jnp.concatenate(outs, axis=1).astype(bf16))
        return outs

    def attn_jobs(p, r0):
        def mk(rb):
            return lambda token: b_attn_pv(p, rb, r0, b_attn_qk(p, rb, False, token))
        return [mk(rb) for rb in range(NRB)]

    z8 = pl.multiple_of(zero[0], 8)
    keep = jnp.zeros((8, 128), u32)
    qkvb[0, 0:8, :] = keep
    keep = keep | qkvb[zero[0], 0:8, :]
    for ref in (oca, ocb, obs0, obs1):
        ref[0:8, 0:128] = jnp.zeros((8, 128), u32)
        keep = keep | ref[pl.ds(z8, 8), 0:128]
    for ref in (ex, df, sv):
        ref[0] = jnp.zeros((8, 128), f32)
        keep = keep | _as_u32(ref[zero[0]])
    part[0:8, 0:128] = jnp.zeros((8, 128), f32)
    keep = keep | _as_u32(part[pl.ds(z8, 8), 0:128])
    outa[0:16, 0:128] = _as_bf16(keep)
    rawa[pl.ds(RAWA_PAD, RG), :] = jnp.zeros((RG, DH), bf16)
    rawo[pl.ds(RAWO_PAD, 32), :] = jnp.zeros((32, DM), bf16)
    rawob[:, DM:DM + 128] = jnp.zeros((DM, 128), bf16)

    def phase_b():
        for i in range(2):
            cp_w0[i].wait()
            prep_qkv(KQV[0], range(2 * i, 2 * i + 2))
        cp_xb0.wait()
        xcvt(0, 0)
        run(b_proj_dots(0, KQV[0:1], 0))
        cp_xb1.wait()
        xcvt(SB, 1)
        untranspose(0)
        NQ4 = 8
        for h in range(1, 6):
            cp_wp[h].wait()
            if h == 5:
                cp_xb2.wait()
            t0, t1 = KQV[(h - 1) // 2], KQV[h // 2]
            prep_qkv(t1, range(4 * (h % 2), 4 * (h % 2) + 4))
            if h < 5:
                untranspose(h)
            dots = b_proj_dots(1, (t0,), (h - 1) % 2) + b_proj_dots(0, (t1,), h % 2)
            if h >= 4:
                def qk_job(rb):
                    def job(token):
                        ps_ = b_attn_qk(0, rb, True, token)
                        qb0[:, rb * RB:(rb + 1) * RB, :] = jnp.stack(ps_)
                        return ps_
                    return job
                rbs = range(NQ4) if h == 4 else range(NQ4, NRB)
                run(dots, ([qk_job(rb) for rb in rbs], 4, 12, 112), td=6)
            else:
                run(dots)
            if h == 5:
                vb0[:, 0:HALO, :] = jnp.broadcast_to(vb0[:, HALO:HALO + 1, :], (8, HALO, 128))

                def pv_job(rb):
                    def job(token):
                        ps_ = qb0[:, rb * RB:(rb + 1) * RB, :]
                        if token is not None:
                            ps_ = gated(ps_, token)
                        b_attn_pv(0, rb, 0, [ps_[w] for w in range(NW)])
                    return job
                xcvt(2 * SB, 0)
                pj = [pv_job(rb) for rb in range(NRB)]
                run(b_proj_dots(1, (t1,), 1), (pj[0::2], 0, 7, 48),
                    (pj[1::2], 0, 7, 112))
        cp_xb3.wait()

        def b_step(p, r_attn, r_next, side):
            run(b_proj_dots(p, KVQ),
                (attn_jobs(1 - p, r_attn), 1, 21, 112),
                (side[0::2], 1, 24, 16), (side[1::2], 1, 24, 40),
                (xcvt_jobs(r_next, 1 - p), 0, 20, 0))

        def b_body(it, carry):
            c = jnp.maximum(it - 1, 0)
            cx = jnp.minimum(c, 4)
            waits = [(it > 0, like(_rows(rawa, pl.multiple_of(c * (GPC * RG), GPC * RG), GPC * RG), 2 * c)),
                     (it > 0, like(_rows(rawo, pl.multiple_of(c * WOR, 128), WOR), 2 * c + 1)),
                     (it - 1 == cx, like(_rows(xb, pl.multiple_of((6 + 2 * cx) * SB, 2 * SB), 2 * SB), sem_x + cx)),
                     (it == 3, cp_wob[0]), (it == 5, cp_wob[1])]
            for cond, copy in waits:
                pl.when(cond)(copy.wait)
            r0 = pl.multiple_of((2 * it + 2) * SB, 2 * SB)
            side = chunk_jobs(it)
            b_step(0, r0 - SB, r0 + SB, side[0])
            b_step(1, r0, jnp.minimum(r0 + 2 * SB, S - SB), side[1])
            return carry

        lax.fori_loop(0, NSTEP // 2 - 1, b_body, 0)
        cp_worest.wait()
        cp_m0.wait()
        cp_xa.wait()
        jo = [wocopy_job(NCH * WOR + i * 32, NCH * WOR // 2 + i * 16) for i in range(WOREST // 32)]
        dots = sum([b_out_dots(r) for r in range(NIT * MB[0], S, SB)], [])
        aj = attn_jobs(1, S - SB)
        nd = len(dots) - NJ0 - 1
        run(dots, (aj[0::2], 0, nd, 48), (aj[1::2], 0, nd, 112), (jo, 0, 0, 0))

    phase_b()
    b_out_start(NIT * MB[0], S - NIT * MB[0], 0)

    scale_a = DH ** -0.5
    qscale = scale_a * LOG2E
    k1 = SPLIT * DH
    tri = lax.broadcasted_iota(i32, (8, 8, 128), 1) >= lax.broadcasted_iota(i32, (8, 8, 128), 0)

    def masks(nv):
        qr = LA - 8 * nv
        r = lax.broadcasted_iota(i32, (2 * qr, 2 * LA), 0)
        c = lax.broadcasted_iota(i32, (2 * qr, 2 * LA), 1)
        same = (r >= qr) == (c >= LA)
        rr = jnp.where(r >= qr, r - qr, r) + 8 * nv
        cc = jnp.where(c >= LA, c - LA, c)
        valid = same & ((cc >= SEG) | (rr >= SEG) | (cc <= rr))
        return valid, jnp.where(same, NEG, -jnp.inf).astype(f32)

    def nvof(which, t):
        return 3 if which == 1 and t >= LATE else 2

    def nearly(which, t):
        return 1 if which == 1 and t >= LATE else 2

    msk = {nv: masks(nv) for nv in (2, 3)}

    def bc8(a):
        return jnp.concatenate([jnp.broadcast_to(a[j:j + 1], (8, 128)) for j in range(8)],
                               axis=0).reshape(8, 8, 128)

    def vpu_part(q, k8, v8, causal, prev):
        s_ = jnp.broadcast_to(jnp.sum(q[None] * k8, axis=-1, keepdims=True), (8, 8, 128))
        if causal:
            s_ = jnp.where(tri, s_, NEG * LOG2E)
        m = jnp.max(s_, axis=0)
        if prev is not None:
            m = jnp.maximum(m, prev[0])
        e = jnp.exp2(s_ - m[None])
        l = jnp.sum(e, axis=0)
        o = jnp.sum(e * v8, axis=0)
        if prev is not None:
            al = jnp.exp2(prev[0] - m)
            l = l + prev[1] * al
            o = o + prev[2] * al
        return m, l, o

    def stage_x(it):
        r0 = pl.multiple_of(it * 64, 64)
        ha[0:40, :] = xa[pl.ds(r0, 40), :]
        hb[8:32, :] = xa[pl.ds(r0 + 40, 24), :]

    def stage_o(it):
        for obs, mb in zip((obs0, obs1), MB):
            obs[...] = oball[pl.ds(pl.multiple_of(it * (mb // 2), 8), mb // 2), :]

    def segment(which, it, r0):
        h_ref, oc_ref = (ha, oca) if which == 0 else (hb, ocb)
        nrow_o = 32 if which == 0 else 48
        h = h_ref[...]
        zvec = zeros_vec()
        so = (18, 19)[which]
        scp = (10, 9)[which]
        pvp = (20, 20)[which]
        c0 = NI * which
        nend = 6 * NP + SPLIT - 4 * c0
        assert 2 * LATE >= SPLIT
        ov, slots, ps, bacc, pre, late, merges = {}, {}, {}, [], {}, [], {}

        LS, LU, LD = -4, 16, 6
        nlate = sum(2 * (g + 2) for t in range(NP) for g in range(nearly(which, t), nvof(which, t)))
        lrel, done = {}, set()

        def fire(n, y):
            for i, job in enumerate(lrel.pop(n, [])):
                r_ = (0, y.shape[0] - 8, 16)[i % 3]
                vals = job(_as_u32(y[r_:r_ + 8]) & zvec)
                if n + LD < nend:
                    slots.setdefault(2 * (n + LD) + i % 2, []).extend(vals)

        def wa_tile(hd, t, k0, kn):
            return wa[pl.ds(t * TREG + hd * TP + k0 // 2, kn // 2), :]

        KH = DM // 2
        if which == 1:
            wb = wos_all()
            for hd in range(2):
                for t in range(3):
                    pre[hd, t] = jnp.dot(h[:, :KH], _as_bf16(wa_tile(hd, t, 0, KH)), preferred_element_type=f32)

        def proj(hd, t, ties):
            if (hd, t) in pre:
                y = jnp.dot(h[:, KH:], _as_bf16(wa_tile(hd, t, KH, KH)), preferred_element_type=f32)
                y = y + pre.pop((hd, t))
            else:
                y = jnp.dot(h, _as_bf16(tied(wa_tile(hd, t, 0, DM), zvec, *ties)), preferred_element_type=f32)
            if which == 0:
                ex[t * HA + hd] = y[32:40]
                return jnp.concatenate([y[0:32], y[40:48]], axis=0)
            return jnp.concatenate([ex[t * HA + hd], y[8:32], y[0:8]], axis=0)

        def vpu_jobs(t, ys):
            out = []
            for e in range(2):
                hd = 2 * t + e
                q, k, v = ys[3 * e:3 * e + 3]
                ov[hd] = []
                cache = {}

                def blk(b0):
                    if b0 not in cache:
                        cache[b0] = bc8(k[b0:b0 + 8]), bc8(v[b0:b0 + 8])
                    return cache[b0]

                for g in range(nearly(which, t)):
                    q0 = q[8 * g:8 * g + 8] * qscale
                    if which == 1 and g == 0:
                        st = [sv[i * HA + hd] for i in range(3)]
                    else:
                        st = None
                        for b in range(g, -1, -1):
                            st = vpu_part(q0, *blk(8 * b), b == g, st)
                            out.append(list(st[1:]))
                    _, l, o = vpu_part(q0, *blk(SEG), False, st)
                    ov[hd].append(o * _recip(l))
                    out.append([ov[hd][-1]])
                for g in range(nearly(which, t), nvof(which, t)):
                    st = [None]
                    for b0 in [8 * b for b in range(g, -1, -1)] + [SEG]:
                        def job(tok, hd=hd, g=g, b0=b0, st=st, q=q, k=k, v=v):
                            gate = lambda x: pltpu.bitcast(_as_u32(x) | tok, f32)
                            st[0] = vpu_part(gate(q[8 * g:8 * g + 8]) * qscale, bc8(gate(k[b0:b0 + 8])),
                                             bc8(gate(v[b0:b0 + 8])), b0 == 8 * g, st[0])
                            if b0 != SEG:
                                return list(st[0][1:])
                            ov[hd].append(st[0][2] * _recip(st[0][1]))
                            return [ov[hd][-1]]
                        lrel.setdefault(6 * NP + LS + len(late) * LU // nlate, []).append(job)
                        late.append(job)
                if which == 0:
                    st = vpu_part(ex[hd] * qscale, bc8(ex[HA + hd]), bc8(ex[2 * HA + hd]), True, None)
                    for i in range(3):
                        sv[i * HA + hd] = st[i]
                    out.append(list(st[1:]))
            for i, jb in enumerate(out):
                slots.setdefault(12 * t + so + (2 * i + 1) * 6 // len(out), []).extend(jb)

        def bout_half(i):
            j, half = JORD[i // 2], i % 2
            obs, mb = (obs0, MB[0]) if j < NJ0 else (obs1, MB[1])
            o = _as_bf16(obs[:, half * KH:(half + 1) * KH])
            y = jnp.dot(o, _as_bf16(wb[j, half * 256:(half + 1) * 256]), preferred_element_type=f32)
            if half == 0:
                bacc.append(y)
            else:
                outb[pl.ds(pl.multiple_of(it * mb, 16), mb), j * 128:(j + 1) * 128] = (y + bacc.pop()).astype(bf16)

        def wo_early(hc, j):
            assert all(hd in done for hd in range(4 * hc, 4 * hc + 4))
            cs = slice(j * 128, (j + 1) * 128)
            y = jnp.dot(_as_bf16(oc_ref[:, hc * KH:(hc + 1) * KH]),
                        _as_bf16(woa[j, hc * 256:(hc + 1) * 256, :]), preferred_element_type=f32)
            part[0:nrow_o, cs] = y if hc == 0 else part[0:nrow_o, cs] + y

        providers, ppos = [], []
        if which == 1:
            providers = [functools.partial(bout_half, i) for i in range(16)]
            providers += [functools.partial(wo_early, hc, j) for hc in range(NI) for j in range(8)]
            ppos = sorted([scp + 6 * i - d for i in range(NP) for d in (0, 2)])

        def scores(p_):
            q3 = (which * NP + p_) * 3
            qr = LA - 8 * nvof(which, p_)
            valid, fill = msk[nvof(which, p_)]
            sc = lax.dot_general(_as_bf16(qkvb[q3, 0:qr, :]), _as_bf16(qkvb[q3 + 1]), _NT,
                                 preferred_element_type=f32)
            sc = jnp.where(valid, sc * scale_a, fill)
            p = jnp.exp(sc - jnp.max(sc, axis=-1, keepdims=True))
            ps[p_] = (p * _recip(jnp.sum(p, axis=-1, keepdims=True))).astype(bf16)

        def pv(p_):
            o = jnp.dot(ps.pop(p_), _as_bf16(qkvb[(which * NP + p_) * 3 + 2]), preferred_element_type=f32)
            qr = LA - 8 * nvof(which, p_)

            def merge():
                for e in range(2):
                    hd = 2 * p_ + e
                    oh = jnp.concatenate(ov.pop(hd) + [o[qr * e:qr * e + qr]], axis=0)
                    if which == 0:
                        df[hd] = oh[24:32]
                        z = jnp.concatenate([oh[32:40], oh[0:24]], axis=0)
                    else:
                        z = jnp.concatenate([oh, df[hd]], axis=0)
                    oc_ref[:, hd * DH:(hd + 1) * DH] = _as_u32(z.astype(bf16))
                    done.add(hd)
            if nvof(which, p_) > nearly(which, p_):
                merges[p_] = merge
            else:
                merge()

        def after(n):
            for pos, fn in ((pvp, pv), (scp, scores)):
                if fn is scores:
                    while ppos and ppos[0] <= n:
                        ppos.pop(0)
                        providers.pop(0)()
                if (n - pos) % 6 == 0 and 0 <= (n - pos) // 6 < NP:
                    fn((n - pos) // 6)

        for t in range(NP):
            ys = []
            for m in range(6):
                n = 6 * t + m
                ys.append(proj(2 * t + m // 3, m % 3, (slots.pop(2 * n, []), slots.pop(2 * n + 1, []))))
                if m == 5:
                    q3 = (which * NP + t) * 3
                    nv = nvof(which, t)
                    qr = LA - 8 * nv
                    qkvb[q3, 0:qr, :] = _as_u32(
                        jnp.concatenate([ys[0][8 * nv:], ys[3][8 * nv:]], axis=0).astype(bf16))
                    for i in range(1, 3):
                        qkvb[q3 + i] = _as_u32(jnp.concatenate([ys[i], ys[3 + i]], axis=0).astype(bf16))
                    vpu_jobs(t, ys)
                fire(n, ys[-1][8:32])
                after(n + 1)
        if which == 1:
            assert not bacc and len(providers) <= 8 * NI
            for i, mb in enumerate(MB):
                @pl.when(it % OG == OG - 1)
                def _():
                    b_out_start(pl.multiple_of((it - (OG - 1)) * mb, 16), OG * mb, i)
        n = 6 * NP
        step = 2 if which == 1 else SPLIT // 4
        for j in range(8):
            cs = slice(j * 128, (j + 1) * 128)
            assert len(providers) <= 7 - j and all(hd in done for hd in range(SPLIT))
            acc = None if c0 == 0 else part[0:nrow_o, cs]
            for c in range(c0, SPLIT // 4, step):
                nun = step // 2
                ties = [sum([slots.pop(2 * n + i, []) for i in range(lo, lo + nun)], []) for lo in (0, nun)]
                y = jnp.dot(_as_bf16(oc_ref[:, c * KH:(c + step) * KH]),
                            _as_bf16(tied(woa[j, c * 256:(c + step) * 256, :], zvec, *ties)),
                            preferred_element_type=f32)
                fire(n, y)
                if which == 1 and n == 6 * NP:
                    outb[S:S + 16, 0:128] = y[0:16].astype(bf16)
                acc = y if acc is None else acc + y
                for _ in range(nun):
                    n += 1
                    after(n)
            part[0:nrow_o, cs] = acc
        for merge in merges.values():
            merge()
        assert n == nend
        assert not (ps or ov or slots or bacc or pre or lrel or providers)
        o2 = _as_bf16(oc_ref[:, k1:])
        for j in range(8):
            cs = slice(j * 128, (j + 1) * 128)
            y = part[0:nrow_o, cs] + jnp.dot(o2, _as_bf16(woa[j, k1 // 2:, :]), preferred_element_type=f32)
            if which == 0:
                hb[0:8, cs] = y[0:8].astype(bf16)
                outa[pl.ds(r0, 24), cs] = y[8:32].astype(bf16)
            else:
                outa[pl.ds(r0 + 32, 32), cs] = y[0:32].astype(bf16)
                ha[40:48, cs] = y[32:40].astype(bf16)
                outa[pl.ds(r0 + 24, 8), cs] = y[40:48].astype(bf16)
                if j == 6:
                    xa[S:S + 16, 0:128] = y[32:48].astype(bf16)
                    stage_x(jnp.minimum(it + 1, NIT - 1))
                    oball[S // 2:S // 2 + 8, 0:128] = _as_u32(y[0:8])
                    stage_o(jnp.minimum(it + 1, NIT - 1))

    def a_body(it, carry):
        r0 = pl.multiple_of(it * 64, 64)
        segment(0, it, r0)

        @pl.when(it == OG - 1)
        def _():
            a_out_start(0, 64 * OG - 40)

        @pl.when(jnp.logical_and(it % OG == OG - 1, it >= OG))
        def _():
            a_out_start(r0 + 24 - 64 * OG, 64 * OG)

        segment(1, it, r0)
        return carry

    stage_x(0)
    stage_o(0)
    lax.fori_loop(0, NIT, a_body, 0)
    a_out_start(S - 40, 40)

    pltpu.make_async_copy(_rows(outb, 0, S), out_hbm.at[:, pl.ds(DM, DM)], sem_out.at[1]).wait()
    pltpu.make_async_copy(outa, out_hbm.at[:, pl.ds(0, DM)], sem_out.at[0]).wait()


@jax.jit
def pallas_concat_heads__memory_aug_recurrent_mem_tr__sliding_local_dilated__prompt_kernel(
    A_x, A_mem0, A_Wq, A_Wk, A_Wv, A_Wo, A_seg_len, B_x, B_wqkv, B_wo,
):
    del A_seg_len
    assert A_x.shape == (1, S, DM) and B_x.shape == (1, S, DM)
    vm = pltpu.VMEM
    scratch = [
        vm((S + 16, DM), bf16), vm((S, DM), bf16),
        vm((S, DM), bf16), vm((S + 16, DM), bf16),
        vm((RAWA_PAD + RG, DH), bf16),
        vm((RAWO_PAD + 32, DM), bf16),
        vm((3, DM, DM), bf16), vm((DM, DM + 128), bf16),
        vm((3 * TREG + DM // 2 + TPAD, DH), u32),
        vm((8, HA * DH // 2, 128), u32),
        vm((24, BREG + 40, 128), u32), vm((8, BREG + 40, 128), u32),
        vm((8, SB, 128), f32), vm((8, SB, 128), f32),
        vm((8, SB + HALO, 128), f32), vm((8, SB + HALO, 128), f32),
        vm((8, SB + HALO, 128), f32), vm((8, SB + HALO, 128), f32),
        vm((SB // 2, DM), u32), vm((SB // 2, DM), u32),
        vm((S // 2 + 8, DM), u32),
        vm((MB[0] // 2, DM), u32), vm((MB[1] // 2, DM), u32),
        vm((48, DM), bf16), vm((32, DM), bf16),
        vm((16, HA * DH), u32), vm((24, HA * DH), u32),
        vm((48, DM), f32),
        vm((3 * HA, 8, 128), f32), vm((HA, 8, 128), f32),
        vm((3 * HA, 8, 128), f32),
        vm((6 * NP, LA, 128), u32),
        vm((5, DM // 4, 128), u32),
        pltpu.SMEM((1,), i32),
        pltpu.SemaphoreType.DMA((NSEM,)),
        pltpu.SemaphoreType.DMA((2,)),
    ]
    out = pl.pallas_call(
        _kernel,
        out_shape=jax.ShapeDtypeStruct((S, 2 * DM), bf16),
        in_specs=[pl.BlockSpec(memory_space=pl.ANY)] * 9,
        out_specs=pl.BlockSpec(memory_space=pl.ANY),
        scratch_shapes=scratch,
        compiler_params=pltpu.CompilerParams(
            vmem_limit_bytes=120 * 1024 * 1024,
            disable_bounds_checks=True,
            disable_semaphore_checks=True,
        ),
        name="concat_heads_kernel",
    )(
        A_x.reshape(S, DM), A_mem0.reshape(MEM, DM),
        A_Wq.reshape(DM * HA, DH), A_Wk.reshape(DM * HA, DH), A_Wv.reshape(DM * HA, DH),
        A_Wo.reshape(HA * DH, DM),
        B_x.reshape(S, DM), B_wqkv, B_wo,
    )
    return out.reshape(1, S, 2 * DM)
```
